```python
import jax
import jax.numpy as jnp

def _softmax(x, axis=-1):
    return jax.nn.softmax(x, axis=axis)
def _gelu(x):
    return jax.nn.gelu(x, approximate=True)
def _silu(x):
    return jax.nn.silu(x)
def _sigmoid(x):
    return jax.nn.sigmoid(x)
def _layernorm(x, axis=-1, eps=1e-5):
    m = jnp.mean(x, axis=axis, keepdims=True)
    v = jnp.var(x, axis=axis, keepdims=True)
    return (x - m) / jnp.sqrt(v + eps)
def _scatter_add(tgt, idx, src, axis=0):
    return tgt.at[idx].add(src)
def _segment_sum(src, seg, n):
    return jax.ops.segment_sum(src, seg, n)
class _Rng:
    def __init__(self, key):
        self._k = key
    def _next(self):
        self._k, sub = jax.random.split(self._k)
        return sub
    def normal(self, shape):
        return jax.random.normal(self._next(), shape, dtype=jnp.bfloat16)
    def randint(self, lo, hi, shape):
        return jax.random.randint(self._next(), shape, lo, hi, dtype=jnp.int32)
    def uniform(self, shape, lo=0.0, hi=1.0):
        return jax.random.uniform(self._next(), shape, jnp.bfloat16, lo, hi)
    def permutation(self, n):
        return jax.random.permutation(self._next(), n)


kernel_name = 'sequential_preLN__ssm_conv_s4__moe_arch_mod__prompt'

def setup_inputs():
    _rng = _Rng(jax.random.key(int.from_bytes(__import__("os").urandom(4), "little")))
    _w = (lambda a: (lambda t: t.astype(jnp.bfloat16) if jnp.issubdtype(t.dtype, jnp.floating) else t)(jnp.asarray(a)))
    def _A_setup():
        B, L, D, N = 1, 2048, 576, 128
        A_re = -jnp.exp((lambda *s: _rng.normal(s) * 0.05)(D, N))
        A_im = jnp.pi * (lambda *s: _rng.normal(s) * 0.05)(D, N)
        B_re = (lambda *s: _rng.normal(s) * 0.05)(D, N)
        B_im = (lambda *s: _rng.normal(s) * 0.05)(D, N)
        C_re = (lambda *s: _rng.normal(s) * 0.05)(D, N)
        C_im = (lambda *s: _rng.normal(s) * 0.05)(D, N)
        log_dt = (lambda *s: _rng.normal(s) * 0.05)(D) * 0.5 - 4.0
        Dskip = (lambda *s: _rng.normal(s) * 0.05)(D)
        return {
            "u": _w((lambda *s: _rng.normal(s) * 0.05)(B, L, D)),
            "A_re": _w(A_re),
            "A_im": _w(A_im),
            "B_re": _w(B_re),
            "B_im": _w(B_im),
            "C_re": _w(C_re),
            "C_im": _w(C_im),
            "log_dt": _w(log_dt),
            "Dskip": _w(Dskip),
        }
    _A_in = _A_setup()

    def _B_setup():
        B, S, D, F, C = 1, 2048, 576, 4608, 8
        return {
            "x": _w((lambda *s: _rng.normal(s) * 0.05)(B, S, D)),
            "w_r": _w((lambda *s: _rng.normal(s) * 0.05)(D)),
            "w_gate": _w((lambda *s: _rng.normal(s) * 0.05)(D, F)),
            "w_up": _w((lambda *s: _rng.normal(s) * 0.05)(D, F)),
            "w_down": _w((lambda *s: _rng.normal(s) * 0.05)(F, D)),
        }
    _B_in = _B_setup()

    return {
        "A_u": _A_in["u"],
        "A_A_re": _A_in["A_re"],
        "A_A_im": _A_in["A_im"],
        "A_B_re": _A_in["B_re"],
        "A_B_im": _A_in["B_im"],
        "A_C_re": _A_in["C_re"],
        "A_C_im": _A_in["C_im"],
        "A_log_dt": _A_in["log_dt"],
        "A_Dskip": _A_in["Dskip"],
        "B_x": _B_in["x"],
        "B_w_r": _B_in["w_r"],
        "B_w_gate": _B_in["w_gate"],
        "B_w_up": _B_in["w_up"],
        "B_w_down": _B_in["w_down"],
    }

def reference(A_u, A_A_re, A_A_im, A_B_re, A_B_im, A_C_re, A_C_im, A_log_dt, A_Dskip, B_x, B_w_r, B_w_gate, B_w_up, B_w_down):
    def _A_ref(u, A_re, A_im, B_re, B_im, C_re, C_im, log_dt, Dskip):
        Bsz, L, D = u.shape
        dt = jnp.exp(log_dt)[:, None]
        A = A_re + 1j * A_im
        Bc = B_re + 1j * B_im
        Cc = C_re + 1j * C_im
        logdA = dt * A
        dB = dt * Bc
        l = (lambda x, dt: x.astype(dt))(jnp.arange(L), A_re.dtype)
        P = jnp.exp(logdA[:, :, None] * l[None, None, :])
        K = jnp.einsum("dn,dnl,dn->dl", Cc, P, dB).real
        L2 = 2 * L
        Kp = jnp.pad(K, ((0, 0), (0, L)))
        up = (lambda x, *d: x.transpose(*d))(u, 0, 2, 1)
        up = jnp.pad(up, ((0, 0), (0, 0), (0, L)))
        Kf = (lambda x, axes=(-2,-1): jnp.fft.rfft2(x.astype(jnp.float32), axes=axes))(Kp[:, None, :], axes=(-2, -1))
        Uf = (lambda x, axes=(-2,-1): jnp.fft.rfft2(x.astype(jnp.float32), axes=axes))(up[:, :, None, :], axes=(-2, -1))
        Yf = Uf * Kf[None, :, :, :]
        y = (lambda x, s, axes=(-2,-1): jnp.fft.irfft2(x, s=s, axes=axes).astype(jnp.bfloat16))(Yf, (1, L2), axes=(-2, -1))[:, :, 0, :L]
        y = (lambda x, *d: x.transpose(*d))(y, 0, 2, 1) + u * Dskip[None, None, :]
        return y

    def _B_ref(x, w_r, w_gate, w_up, w_down):
        B, S, D = x.shape
        C = 8
        r = x @ w_r
        idx = jnp.argsort(-r, axis=-1)[:, :C]
        idx_e = jnp.repeat(idx.reshape(B, C, 1), D, axis=2)
        x_sel = jnp.take_along_axis(x, idx_e, axis=1)
        g = _silu(x_sel @ w_gate)
        u = x_sel @ w_up
        y = (g * u) @ w_down
        r_sel = _sigmoid(jnp.take_along_axis(r, idx, axis=1))
        y = y * r_sel.reshape(B, C, 1)
        b_off = (jnp.arange(B) * S).reshape(B, 1)
        flat_idx = (idx + b_off).reshape(B * C)
        zero = (x * 0.0).reshape(B * S, D)
        upd = _scatter_add(zero, flat_idx, y.reshape(B * C, D), axis=0)
        return x + upd.reshape(B, S, D)

    x = A_u
    h = x + _A_ref(_layernorm(x, axis=-1), A_A_re, A_A_im, A_B_re, A_B_im, A_C_re, A_C_im, A_log_dt, A_Dskip)
    h2 = h + _B_ref(_layernorm(h, axis=-1), B_w_r, B_w_gate, B_w_up, B_w_down)
    return h2
```

```python
import functools

import numpy as np
import jax
import jax.numpy as jnp
from jax import lax
import jax.experimental.pallas as pl
import jax.experimental.pallas.tpu as pltpu

f32 = jnp.float32
bf16 = jnp.bfloat16
i32 = jnp.int32
u32 = jnp.uint32

L, D, N, F, TOPC = 2048, 576, 128, 4608, 8
NB = 8
NV = 9
R = NV * 8
NSTEP = D // R
NCH = 6
FC = F // NCH
EPS = 1e-5

_XL1 = [(1, 5), (2, 6), (3, 7), (4, 8), (258, 516), (260, 520), (262, 772), (264, 776),
        (1288, 1032), (1800, 1544)]
_XSH = [0, 1, 2, 3, 0, 1, 2, 3, 2, 1]


def _bf16_round_int(j):
    u = np.asarray(j, np.float32).view(np.uint32).astype(np.uint64)
    r = ((u + 0x7FFF + ((u >> 16) & 1)) >> 16) << 16
    return r.astype(np.uint32).view(np.float32).astype(np.int64)


def _chunk_values():
    vals = -np.ones((5, 128), np.int64)
    for j in range(10):
        for p in range(2):
            ch = (j // 4) * 2 + p if j < 8 else 4
            extra = 2 * p if j >= 8 else 0
            for l0 in range(32):
                vals[ch, (4 * l0 + 4 * p + 3 + _XSH[j] + extra) % 128] = _XL1[j][p] + 8 * l0
    assert (vals >= 0).all()
    return vals


def _tables():
    cv = _chunk_values()
    om = np.pi * (2 * np.arange(128) + 1) / 512.0
    sig = (-1.0) ** np.arange(128)
    cvp = {"A0": cv[0], "A1": cv[1], "B": cv[2], "C": cv[3], "D": cv[4]}
    cvp["Cp"] = cv[3].copy(); cvp["Cp"][2] = cv[2][2]
    cvp["Dp"] = cv[4].copy(); cvp["Dp"][6] = cv[3][6]
    passes = [(0, "A0"), (0, "A1"), (1, "A1"), (1, "B"), (2, "Cp"), (3, "C"), (4, "Dp"),
              (5, "D"), (6, "D"), (7, "D")]
    G = np.zeros((10, 128, 4, 128))
    for b in range(NB):
        mine = [i for i, (pb, _) in enumerate(passes) if pb == b]
        for j in range(1, 257):
            lag = 256 * b + j
            if lag > L - 1:
                continue
            v = int(_bf16_round_int(lag))
            hit = [(i, int(np.nonzero(cvp[passes[i][1]] == v)[0][0])) for i in mine
                   if (cvp[passes[i][1]] == v).any()]
            assert len(hit) == 1, (b, j, v, hit)
            i, l = hit[0]
            e = np.exp(-1j * om * j) * sig ** b / 256.0
            s = (-1.0) ** j
            G[i, l, 0] += e.real; G[i, l, 1] += e.imag
            G[i, l, 2] += s * e.real; G[i, l, 3] += s * e.imag
    e8 = np.exp(-1j * np.outer(8 * np.arange(32), om))
    sets = {"A0": [0], "A1": [1], "B": [3], "C": [4, 5], "D": [6, 7, 8, 9]}
    seeds, masks = {}, {}
    for name, ps in sets.items():
        seeds[name] = sum(G[i, 8:16] for i in ps)
        for i in ps:
            masks[i] = [int(x) for x in (np.abs(G[i, 8:16]).sum((1, 2)) > 0)]
            for v in range(1, 16):
                sd = seeds[name]
                for q in (0, 2):
                    z = (sd[:, q] + 1j * sd[:, q + 1]) * e8[2 * (v - 1)] * np.array(masks[i])[:, None]
                    assert np.allclose(z.real, G[i, 8 * v:8 * v + 8, q], atol=1e-12)
                    assert np.allclose(z.imag, G[i, 8 * v:8 * v + 8, q + 1], atol=1e-12)
    assert not G[2, 8:].any()
    s8 = np.arange(8)
    j0 = np.where(s8 % 2 == 0, s8, 128 + s8 - 1)
    fe = np.exp(-1j * np.outer(j0, om)); ft = np.exp(-1j * np.outer(j0 + 1, om))
    rows = [e8.real, e8.imag]
    for name in ("A0", "A1", "B", "C", "D"):
        rows += [seeds[name][:, q] for q in range(4)]
    for i in range(10):
        rows += [G[i, 0:8, q] for q in range(4)]
    rows += [fe.real, fe.imag, ft.real, ft.imag]
    return np.concatenate(rows, 0).astype(np.float32), masks


_CTAB, _GMASK = _tables()


def _sincos_coeffs():
    r = np.cos(np.pi * (np.arange(4000) + .5) / 4000) * 0.5
    z = r * r
    s = np.linalg.lstsq(np.stack([z ** k for k in range(4)], 1), np.sin(np.pi / 2 * r) / r, rcond=None)[0]
    c = np.linalg.lstsq(np.stack([z ** k for k in range(1, 5)], 1), np.cos(np.pi / 2 * r) - 1, rcond=None)[0]
    return [float(x) for x in s], [float(x) for x in c]


_SC, _CC = _sincos_coeffs()


def _cmul(a, b):
    return (a[0] * b[0] - a[1] * b[1], a[0] * b[1] + a[1] * b[0])


def _cmulc(a, b):
    return (a[0] * b[0] + a[1] * b[1], a[1] * b[0] - a[0] * b[1])


def _csq(a):
    return ((a[0] - a[1]) * (a[0] + a[1]), (a[0] + a[0]) * a[1])


def _sincos(th):
    z = th * (2.0 / np.pi)
    k = jnp.round(z)
    r = z - k
    r2 = r * r
    s = r * (_SC[0] + r2 * (_SC[1] + r2 * (_SC[2] + r2 * _SC[3])))
    c = 1.0 + r2 * (_CC[0] + r2 * (_CC[1] + r2 * (_CC[2] + r2 * _CC[3])))
    ki = k.astype(i32)
    swap = (ki & 1) == 1
    s2 = jnp.where(swap, c, s)
    c2 = jnp.where(swap, s, c)
    s2 = pltpu.bitcast(pltpu.bitcast(s2, i32) ^ ((ki & 2) << 30), f32)
    c2 = pltpu.bitcast(pltpu.bitcast(c2, i32) ^ (((ki + 1) & 2) << 30), f32)
    return s2, c2


def _rb(x):
    return x.astype(bf16).astype(f32)


def _dot(a, b):
    return jnp.dot(a, b, preferred_element_type=f32)


def _dot_nt(a, b):
    return lax.dot_general(a, b, (((1,), (1,)), ((), ())), preferred_element_type=f32)


def _iota(shape, dim):
    return lax.broadcasted_iota(i32, shape, dim)


def _kernel(x_h, are_h, aim_h, bre_h, bim_h, cre_h, cim_h, ldt_h, dsk_h, wr_h, wg_h, wu_h, wd_h, ct_h,
            out_h,
            x_v, par_v, ldt_v, dsk_v, wr_v, ct_v, wg_v, wu_v, wd_v, out_v,
            g_v, f_v, col_v, st_v, kd_v, k0_v, kh_v, uh_v, zs_v, c1_v, s1_v, acc_v, fin_v,
            sem, osem):
    cp = pltpu.make_async_copy
    c_ct = cp(ct_h, ct_v, sem.at[0])
    c_vec = [cp(ldt_h, ldt_v, sem.at[1]), cp(dsk_h, dsk_v, sem.at[2]), cp(wr_h, wr_v, sem.at[3])]
    c_par = [cp(h, par_v.at[i], sem.at[4 + i])
             for i, h in enumerate((are_h, aim_h, bre_h, bim_h, cre_h, cim_h))]
    c_x = cp(x_h, x_v, sem.at[10])
    c_w = [[cp(h.at[:, pl.ds(c * FC, FC)], v.at[:, pl.ds(c * FC, FC)], sem.at[11 + 3 * c + i])
            for i, (h, v) in enumerate(((wg_h, wg_v), (wu_h, wu_v), (wd_h, wd_v)))] for c in range(NCH)]
    c_ct.start()
    for c in c_vec + c_par:
        c.start()
    c_x.start()
    for cw in c_w:
        for c in cw:
            c.start()

    sub8 = _iota((8, 128), 0)
    lane8 = _iota((8, 128), 1)

    acc_v[...] = jnp.zeros(acc_v.shape, f32)
    c_ct.wait()

    def e8(v):
        return (jnp.broadcast_to(ct_v[v:v + 1, :], (8, 128)), jnp.broadcast_to(ct_v[32 + v:33 + v, :], (8, 128)))

    sets = {"A0": [0], "A1": [1], "B": [3], "C": [4, 5], "D": [6, 7, 8, 9]}
    for i in range(10):
        for q in range(4):
            g_v[i, 0:8, q * 128:(q + 1) * 128] = ct_v[224 + 32 * i + 8 * q:232 + 32 * i + 8 * q, :]
    g_v[2, 8:128, :] = jnp.zeros((120, 512), f32)
    for si, (name, ps) in enumerate(sets.items()):
        sd = [ct_v[64 + 32 * si + 8 * q:72 + 32 * si + 8 * q, :] for q in range(4)]
        mk = {}
        for i in ps:
            if len(ps) > 1:
                bits = sum(b << s for s, b in enumerate(_GMASK[i]))
                mk[i] = ((bits >> sub8) & 1) == 1
        for v in range(1, 16):
            if v == 1:
                vals = sd
            else:
                ev = e8(2 * (v - 1))
                vals = list(_cmul((sd[0], sd[1]), ev)) + list(_cmul((sd[2], sd[3]), ev))
            for i in ps:
                for q in range(4):
                    val = vals[q] if len(ps) == 1 else jnp.where(mk[i], vals[q], 0.0)
                    g_v[i, 8 * v:8 * v + 8, q * 128:(q + 1) * 128] = val
    sig = jnp.where((lane8 & 1) == 0, 1.0, -1.0).astype(f32)
    for h in range(2):
        sd = (ct_v[544 + 16 * h:552 + 16 * h, :], ct_v[552 + 16 * h:560 + 16 * h, :])
        for v in range(16):
            vals = sd if v == 0 else _cmul(sd, e8(v))
            for q in range(2):
                f_v[0, h, 8 * v:8 * v + 8, q * 128:(q + 1) * 128] = vals[q]
                f_v[1, h, 8 * v:8 * v + 8, q * 128:(q + 1) * 128] = vals[q] * sig

    for c in c_vec:
        c.wait()
    rows = [_rb(jnp.exp(ldt_v[...].astype(f32).reshape(1, D))),
            dsk_v[...].astype(f32).reshape(1, D),
            wr_v[...].astype(f32).reshape(1, D)]
    wr_sum = jnp.sum(rows[2], axis=1, keepdims=True)
    ones = jnp.ones((128, 128), f32)
    for j in range(5):
        w = 128 if j < 4 else 64
        eye = _iota((w, w), 0) == _iota((w, w), 1)
        for i in range(3):
            m = jnp.where(eye, jnp.broadcast_to(rows[i][:, j * 128:j * 128 + w], (w, w)), 0.0)
            col_v[i, j * 128:j * 128 + w, :] = _dot(m, ones[:w, :])

    revmask = (sub8 & 2) == 0
    lm = (lane8 + 1) & 3

    def s1(k):
        row0 = pl.multiple_of(k * R, 8)
        ld = lambda i: par_v[i, pl.ds(row0, R), :].astype(f32)
        dt = col_v[0, pl.ds(row0, R), :]
        e = jnp.exp(dt * ld(0))
        s, c = _sincos(dt * ld(1))
        a1 = (e * c, e * s)
        w = _cmul((ld(4), ld(5)), (dt * ld(2), dt * ld(3)))
        k0_v[k] = (jnp.sum(w[0], axis=1, keepdims=True) + col_v[1, pl.ds(row0, R), :]) * (1.0 / 256.0)
        w = (w[0], -w[1])
        a2 = _csq(a1); a4 = _csq(a2); a8 = _csq(a4); a16 = _csq(a8)
        a5 = _cmul(a4, a1)
        t = a16
        for _ in range(4):
            t = _csq(t)
        a256 = t; a512 = _csq(a256); a1024 = _csq(a512)
        rev = lambda v: jnp.where(revmask, pltpu.roll(v, 2, 0), pltpu.roll(v, 6, 0))
        seq = [w, w, a1, a1, a5, a2, a4, a256, a512, a512, a1024, a256]
        for n in range(NV):
            sl = slice(8 * n, 8 * n + 8)
            for ri in range(2):
                for q, arr in enumerate(seq):
                    st_v[n, ri, q * 8:q * 8 + 8, :] = arr[ri][sl]
                a16r = rev(a16[ri][sl])
                st_v[n, ri, 96:104, :] = jnp.full((8, 128), 1.0 - ri, f32)
                st_v[n, ri, 104:112, :] = rev(a8[ri][sl])
                st_v[n, ri, 112:120, :] = a16r
                st_v[n, ri, 120:128, :] = a16r
        for n in range(NV):
            for g in range(2):
                mix = lambda q: (st_v[n, 0, pl.ds(q * 8 + g, 8, stride=2), :],
                                 st_v[n, 1, pl.ds(q * 8 + g, 8, stride=2), :])
                wd = mix(0); a1d = mix(2); m1 = mix(5)
                v = [_cmulc(wd, mix(3))]
                for _ in range(3):
                    v.append(_cmulc(v[-1], a1d))
                v4 = _cmulc(_cmulc(wd, m1), mix(7))
                v5 = _cmulc(v4, m1); v6 = _cmulc(v4, mix(6)); v7 = _cmulc(v6, m1)
                v8 = _cmulc(v7, mix(10)); v9 = _cmulc(v8, mix(8))
                v += [v4, v5, v6, v7, v8, v9]
                y = [mix(12)]
                a16d = mix(14)
                for _ in range(15):
                    y.append(_cmul(y[-1], a16d))
                xm = jnp.concatenate([jnp.concatenate([t[0] for t in v], 0),
                                      jnp.concatenate([t[1] for t in v], 0)], 1)
                ym = jnp.concatenate([jnp.concatenate([t[0] for t in y], 0),
                                      jnp.concatenate([t[1] for t in y], 0)], 1)
                o = _dot_nt(xm, ym)
                ro = [pltpu.roll(o[8 * j:8 * j + 8], _XSH[j], 1, stride=1, stride_axis=0) for j in range(10)]
                sel4 = lambda q: jnp.where(lm == 0, q[0], jnp.where(lm == 1, q[1], jnp.where(lm == 2, q[2], q[3])))
                kd_v[k, n, pl.ds(g, 8, stride=2), :] = sel4(ro[0:4])
                kd_v[k, n, pl.ds(16 + g, 8, stride=2), :] = sel4(ro[4:8])
                kd_v[k, n, pl.ds(32 + g, 8, stride=2), :] = jnp.where(lm == 2, ro[8], ro[9])
            da = kd_v[k, n, 32:40, :]
            db = pltpu.roll(kd_v[k, n, 40:48, :], 2, 1)
            kd_v[k, n, 32:40, :] = jnp.where((lm == 1) | (lm == 2), da, db)

    def s2(k):
        ch = lambda c: kd_v[k, :, 8 * c:8 * c + 8, :].reshape(R, 128)
        lane = _iota((R, 128), 1)
        prev = None
        for b in range(NB):
            if b == 0:
                z = _dot(jnp.concatenate([ch(0), ch(1)], 1), g_v[0:2].reshape(256, 512))
            elif b == 1:
                z = _dot(jnp.concatenate([ch(1), ch(2)], 1), g_v[2:4].reshape(256, 512))
            elif b == 2:
                z = _dot(jnp.where(lane == 2, ch(2), ch(3)), g_v[4])
            elif b == 3:
                z = _dot(ch(3), g_v[5])
            elif b == 4:
                z = _dot(jnp.where(lane == 6, ch(3), ch(4)), g_v[6])
            else:
                z = _dot(ch(4), g_v[b + 2])
            zq = [z[:, q * 128:(q + 1) * 128] for q in range(4)]
            for s in range(2):
                if b == 0:
                    kr = zq[2 * s] + k0_v[k]
                    ki = zq[2 * s + 1]
                else:
                    kr = zq[2 * s] - prev[2 * s + 1]
                    ki = zq[2 * s + 1] + prev[2 * s]
                kh_v[k, b, s, 0] = kr
                kh_v[k, b, s, 1] = kr + ki
                kh_v[k, b, s, 2] = ki - kr
            prev = zq

    even = (lane8 & 1) == 0

    def ln1(b):
        c0 = pl.multiple_of(b * 256, 256)
        sh = None
        acc = None
        for g in range(D // 16):
            lo = pltpu.bitcast(x_v[16 * g:16 * g + 16, pl.ds(c0, 128)], u32)
            hi = pltpu.bitcast(x_v[16 * g:16 * g + 16, pl.ds(c0 + 128, 128)], u32)
            eo = [jnp.where(even, lo, pltpu.roll(hi, 1, 1)), jnp.where(even, pltpu.roll(lo, 127, 1), hi)]
            eo = [pltpu.bitcast(t, bf16).astype(f32) for t in eo]
            if g == 0:
                sh = [jnp.broadcast_to(t[0:1], (16, 128)) for t in eo]
            eo = [eo[h] - sh[h] for h in range(2)]
            for h in range(2):
                c1_v[2 * b + h, 16 * g:16 * g + 16, :] = eo[h]
            new = [eo[0], eo[1], eo[0] * eo[0], eo[1] * eo[1]]
            acc = new if acc is None else [p + q for p, q in zip(acc, new)]
        for h in range(2):
            m = jnp.sum(acc[h], axis=0, keepdims=True) * (1.0 / D)
            var = jnp.maximum(jnp.sum(acc[2 + h], axis=0, keepdims=True) * (1.0 / D) - m * m, 0.0)
            rs = 1.0 / _rb(jnp.sqrt(_rb(_rb(var) + EPS)))
            s1_v[0, 2 * b + h] = jnp.broadcast_to(rs, (8, 128))
            s1_v[1, 2 * b + h] = jnp.broadcast_to(m * rs, (8, 128))
            s1_v[2, 2 * b + h] = sh[h][0:8]

    def s3(k):
        row0 = pl.multiple_of(k * R, 8)
        for b in range(NB):
            et = []
            for h in range(2):
                c = c1_v[2 * b + h, pl.ds(row0, R), :].reshape(NV, 8, 128)
                u = (c * s1_v[0, 2 * b + h] - s1_v[1, 2 * b + h]).reshape(R, 128)
                et.append(_dot(u, f_v[b % 2, h]))
            er, ei, tr, ti = et[0][:, :128], et[0][:, 128:], et[1][:, :128], et[1][:, 128:]
            for s, (pr, pi) in enumerate(((er + tr, ei + ti), (er - tr, ei - ti))):
                uh_v[k, b, s, 0] = pr + pi
                uh_v[k, b, s, 1] = pi
                uh_v[k, b, s, 2] = pr

    def s45(k):
        row0 = pl.multiple_of(k * R, 8)
        for b in range(0, NB, 2):
            for n in range(NV):
                sl = slice(8 * n, 8 * n + 8)
                zz = []
                for s in range(2):
                    a0 = a1 = None
                    un = [uh_v[k, b + 1, s, q, sl, :] for q in range(3)]
                    for j in range(b + 2):
                        kk = [kh_v[k, j, s, q, sl, :] for q in range(3)]
                        p1 = [kk[q] * un[q] for q in range(3)]
                        a1 = p1 if a1 is None else [p + q for p, q in zip(a1, p1)]
                        if j <= b:
                            un = [uh_v[k, b - j, s, q, sl, :] for q in range(3)]
                            p0 = [kk[q] * un[q] for q in range(3)]
                            a0 = p0 if a0 is None else [p + q for p, q in zip(a0, p0)]
                    zz.append([(a[0] - a[1], a[0] + a[2]) for a in (a0, a1)])
                for o in range(2):
                    p, q = zz[0][o], zz[1][o]
                    zs_v[b + o, 0, sl, 0:128] = p[0] + q[0]
                    zs_v[b + o, 0, sl, 128:256] = p[1] + q[1]
                    zs_v[b + o, 1, sl, 0:128] = p[0] - q[0]
                    zs_v[b + o, 1, sl, 128:256] = p[1] - q[1]
            for o in range(2):
                for h in range(2):
                    t = 2 * (b + o) + h
                    y = _dot_nt(zs_v[b + o, h], f_v[o, h])
                    hh = c1_v[t, pl.ds(row0, R), :] + y
                    c1_v[t, pl.ds(row0, R), :] = hh
                    red = lambda v: jnp.sum(v.reshape(NV, 8, 128), axis=0)
                    acc_v[0, t] = acc_v[0, t] + red(hh)
                    acc_v[1, t] = acc_v[1, t] + red(hh * hh)
                    acc_v[2, t] = acc_v[2, t] + red(hh * col_v[2, pl.ds(row0, R), :])

    for c in c_par:
        c.wait()
    s1(0)
    s1(1); s2(0)
    s1(2); s2(1)
    c_x.wait()
    lax.fori_loop(0, NB, lambda b, c: (ln1(b), c)[1], 0)
    s3(0)

    def main(k, c):
        s45(k); s3(k + 1); s2(k + 2); s1(k + 3)
        return c

    lax.fori_loop(0, NSTEP - 3, main, 0)
    s45(5); s3(6); s2(7)
    s45(6); s3(7)
    s45(7)

    tot = [jnp.sum(acc_v[i], axis=1) for i in range(3)]
    m2 = tot[0] * (1.0 / D)
    var2 = jnp.maximum(tot[1] * (1.0 / D) - m2 * m2, 0.0)
    rs2 = 1.0 / _rb(jnp.sqrt(_rb(_rb(var2) + EPS)))
    r = _rb((tot[2] - m2 * wr_sum) * rs2)
    fin_v[0] = rs2
    fin_v[1] = m2 * rs2
    fin_v[2] = rs2 + 1.0
    fin_v[3] = s1_v[2, :, 0, :] - m2 * rs2

    tl = _iota((16, 128), 0)
    ll = _iota((16, 128), 1)
    tok = (tl >> 1) * 256 + (tl & 1) + jnp.where((ll & 1) == 1, ll + 127, ll)
    rbits = pltpu.bitcast(r, i32)
    srt = rbits ^ ((rbits >> 31) & 0x7FFFFFFF)
    key = pltpu.bitcast((((srt >> 16) + 32768) << 11) + (2047 - tok) + (1 << 28), f32)
    keys = []
    for _ in range(TOPC):
        mx = jnp.max(jnp.max(key, axis=0, keepdims=True), axis=1, keepdims=True)
        keys.append(mx)
        key = jnp.where(key == mx, 0.0, key)
    kcol = jnp.broadcast_to(keys[0], (8, 128))
    for j in range(1, TOPC):
        kcol = jnp.where(sub8 == j, keys[j], kcol)
    kint = pltpu.bitcast(kcol, i32) - (1 << 28)
    tcol = 2047 - (kint & 2047)
    s16 = (kint >> 11) - 32768
    rsel = pltpu.bitcast((s16 ^ ((s16 >> 31) & 0x7FFF)) << 16, f32)
    gate = _rb(jax.nn.sigmoid(rsel))[:, 0:1]
    toks = [jnp.max(jnp.where(sub8 == j, tcol, 0)) for j in range(TOPC)]

    wcol = tcol & 255
    pcol = ((wcol & 127) & ~1) | (wcol >> 7)
    lhs, rhs = [], []
    for j in range(TOPC):
        t = ((toks[j] >> 8) << 1) | (toks[j] & 1)
        ln = c1_v[t] * fin_v[0, pl.ds(t, 1), :] - fin_v[1, pl.ds(t, 1), :]
        rhs.append(ln)
        lhs.append(jnp.where((sub8 == j) & (lane8 == pcol), 1.0, 0.0).astype(f32))
    xsel = _dot_nt(jnp.concatenate(lhs, 1), jnp.concatenate(rhs, 1))

    def outp(b, c):
        c0 = pl.multiple_of(b * 256, 256)
        sc = [(fin_v[2, pl.ds(2 * b + h, 1), :], fin_v[3, pl.ds(2 * b + h, 1), :]) for h in range(2)]
        for g in range(D // 16):
            eo = [c1_v[2 * b + h, 16 * g:16 * g + 16, :] * sc[h][0] + sc[h][1] for h in range(2)]
            eo = [pltpu.bitcast(t.astype(bf16), u32) for t in eo]
            lo = jnp.where(even, eo[0], pltpu.roll(eo[1], 1, 1))
            hi = jnp.where(even, pltpu.roll(eo[0], 127, 1), eo[1])
            out_v[16 * g:16 * g + 16, pl.ds(c0, 128)] = pltpu.bitcast(lo, bf16)
            out_v[16 * g:16 * g + 16, pl.ds(c0 + 128, 128)] = pltpu.bitcast(hi, bf16)
        return c

    lax.fori_loop(0, NB, outp, 0)

    tiles = [toks[j] >> 7 for j in range(TOPC)]
    hit = 0
    for j in range(TOPC):
        hit = hit | (1 << tiles[j])

    def ocopy(t):
        c0 = pl.multiple_of(t * 128, 128)
        return cp(out_v.at[:, pl.ds(c0, 128)], out_h.at[:, pl.ds(c0, 128)], osem.at[t])

    y = jnp.zeros((8, D), f32)
    for c in range(NCH):
        for cc in c_w[c]:
            cc.wait()
        if c == NCH - 1:
            for t in range(16):
                @pl.when(((hit >> t) & 1) == 0)
                def _():
                    ocopy(t).start()
        sl = slice(c * FC, (c + 1) * FC)
        g = _rb(_dot(xsel, wg_v[:, sl]))
        up = _rb(_dot(xsel, wu_v[:, sl]))
        act = _rb(_rb(g * jax.nn.sigmoid(g)) * up)
        y = y + _dot_nt(act, wd_v[:, sl])
    y = _rb(_rb(y) * gate)

    oh = jnp.concatenate([jnp.where((sub8 == j) & (lane8 == (tcol & 127)), 1.0, 0.0).astype(f32)
                          for j in range(TOPC)], 1)
    upd = lax.dot_general(y, oh, (((0,), (0,)), ((), ())), preferred_element_type=f32)
    for j in range(TOPC):
        c0 = pl.multiple_of(tiles[j] * 128, 128)
        cur = out_v[:, pl.ds(c0, 128)].astype(f32)
        out_v[:, pl.ds(c0, 128)] = (cur + upd[:, j * 128:(j + 1) * 128]).astype(bf16)
        later = False
        for j2 in range(j + 1, TOPC):
            later = jnp.logical_or(later, tiles[j2] == tiles[j])

        @pl.when(jnp.logical_not(later))
        def _():
            ocopy(tiles[j]).start()

    for t in range(16):
        ocopy(t).wait()


@jax.jit
def pallas_sequential_preLN__ssm_conv_s4__moe_arch_mod__prompt_kernel(
    A_u: jax.Array,
    A_A_re: jax.Array,
    A_A_im: jax.Array,
    A_B_re: jax.Array,
    A_B_im: jax.Array,
    A_C_re: jax.Array,
    A_C_im: jax.Array,
    A_log_dt: jax.Array,
    A_Dskip: jax.Array,
    B_x: jax.Array,
    B_w_r: jax.Array,
    B_w_gate: jax.Array,
    B_w_up: jax.Array,
    B_w_down: jax.Array,
):
    hbm = pl.BlockSpec(memory_space=pltpu.MemorySpace.HBM)
    vm = pltpu.VMEM
    scratch = [
        vm((D, L), bf16), vm((6, D, N), bf16), vm((D,), bf16), vm((D,), bf16), vm((D,), bf16),
        vm(_CTAB.shape, f32), vm((D, F), bf16), vm((D, F), bf16), vm((D, F), bf16), vm((D, L), bf16),
        vm((10, 128, 512), f32), vm((2, 2, 128, 256), f32), vm((3, D, 128), f32),
        vm((NV, 2, 128, 128), f32), vm((NSTEP, NV, 48, 128), f32), vm((NSTEP, R, 128), f32),
        vm((NSTEP, NB, 2, 3, R, 128), f32), vm((NSTEP, NB, 2, 3, R, 128), f32),
        vm((NB, 2, R, 256), f32), vm((16, D, 128), f32), vm((3, 16, 8, 128), f32),
        vm((3, 16, 8, 128), f32), vm((4, 16, 128), f32),
        pltpu.SemaphoreType.DMA((11 + 3 * NCH,)), pltpu.SemaphoreType.DMA((16,)),
    ]
    out_t = pl.pallas_call(
        _kernel,
        out_shape=jax.ShapeDtypeStruct((D, L), bf16),
        in_specs=[hbm] * 14,
        out_specs=hbm,
        scratch_shapes=scratch,
        compiler_params=pltpu.CompilerParams(vmem_limit_bytes=120 * 1024 * 1024),
    )(A_u[0].T, A_A_re, A_A_im, A_B_re, A_B_im, A_C_re, A_C_im, A_log_dt, A_Dskip, B_w_r,
      B_w_gate, B_w_up, B_w_down.T, jnp.asarray(_CTAB))
    return out_t.T[None]
```

```python
import functools

import numpy as np
import jax
import jax.numpy as jnp
from jax import lax
import jax.experimental.pallas as pl
import jax.experimental.pallas.tpu as pltpu

f32 = jnp.float32
bf16 = jnp.bfloat16
i32 = jnp.int32
u32 = jnp.uint32

L, D, N, F, TOPC = 2048, 576, 128, 4608, 8
NB = 8
NV = 9
R = NV * 8
NSTEP = D // R
FCH = (1024, 1024, 896, 768, 640, 256)
NCH = len(FCH)
FOFF = [sum(FCH[:i]) for i in range(NCH)]
EPS = 1e-5

_XL1 = [(1, 5), (2, 6), (3, 7), (4, 8), (258, 516), (260, 520), (262, 772), (264, 776),
        (1288, 1032), (1800, 1544)]
_XSH = [0, 1, 2, 3, 0, 1, 2, 3, 0, 1]


def _bf16_round_int(j):
    u = np.asarray(j, np.float32).view(np.uint32).astype(np.uint64)
    r = ((u + 0x7FFF + ((u >> 16) & 1)) >> 16) << 16
    return r.astype(np.uint32).view(np.float32).astype(np.int64)


def _chunk_values():
    vals = -np.ones((5, 128), np.int64)
    for j in range(10):
        for p in range(2):
            ch = (j // 4) * 2 + p if j < 8 else 4
            extra = 2 * p if j >= 8 else 0
            for l0 in range(32):
                vals[ch, (4 * (31 - l0) + 4 * p + _XSH[j] + extra + 8) % 128] = _XL1[j][p] + 8 * l0
    assert (vals >= 0).all()
    return vals


def _tables():
    cv = _chunk_values()
    om = np.pi * (2 * np.arange(128) + 1) / 512.0
    sig = (-1.0) ** np.arange(128)
    cvp = {"A0": cv[0], "A1": cv[1], "B": cv[2], "C": cv[3], "D": cv[4]}
    cvp["Cp"] = cv[3].copy(); cvp["Cp"][11] = cv[2][11]
    cvp["Dp"] = cv[4].copy(); cvp["Dp"][15] = cv[3][15]
    passes = [(0, "A0"), (0, "A1"), (1, "A1"), (1, "B"), (2, "Cp"), (3, "C"), (4, "Dp"),
              (5, "D"), (6, "D"), (7, "D")]
    G = np.zeros((10, 128, 4, 128))
    for b in range(NB):
        mine = [i for i, (pb, _) in enumerate(passes) if pb == b]
        for j in range(1, 257):
            lag = 256 * b + j
            if lag > L - 1:
                continue
            v = int(_bf16_round_int(lag))
            hit = [(i, int(np.nonzero(cvp[passes[i][1]] == v)[0][0])) for i in mine
                   if (cvp[passes[i][1]] == v).any()]
            assert len(hit) == 1, (b, j, v, hit)
            i, l = hit[0]
            e = np.exp(-1j * om * j) * sig ** b / 256.0
            s = (-1.0) ** j
            G[i, l, 0] += e.real; G[i, l, 1] += e.imag
            G[i, l, 2] += s * e.real; G[i, l, 3] += s * e.imag
    e8 = np.exp(-1j * np.outer(8 * np.arange(32), om))
    sets = {"A0": [0], "A1": [1], "B": [3], "C": [4, 5], "D": [6, 7, 8, 9]}
    seeds, masks = {}, {}
    for name, ps in sets.items():
        seeds[name] = sum(G[i, 16:24] for i in ps)
        for i in ps:
            masks[i] = [int(x) for x in (np.abs(G[i, 16:24]).sum((1, 2)) > 0)]
            for v in range(2, 17):
                sd = seeds[name]
                r0 = 8 * (v % 16)
                for q in (0, 2):
                    z = (sd[:, q] + 1j * sd[:, q + 1]) * np.conj(e8[2 * (v - 2)]) * np.array(masks[i])[:, None]
                    assert np.allclose(z.real, G[i, r0:r0 + 8, q], atol=1e-12)
                    assert np.allclose(z.imag, G[i, r0:r0 + 8, q + 1], atol=1e-12)
    assert not G[2, 16:].any() and not G[2, :8].any()
    s8 = np.arange(8)
    je = np.where(s8 % 2 == 0, s8, 127 + s8)
    jo = np.where(s8 % 2 == 0, s8 - 1, 128 + s8)
    fe = np.exp(-1j * np.outer(je, om)); ft = np.exp(-1j * np.outer(jo, om))
    ft0 = np.exp(-1j * np.outer(jo % 128 + 128 * (s8 % 2), om))
    rows = [e8.real, e8.imag]
    for name in ("A0", "A1", "B", "C", "D"):
        rows += [seeds[name][:, q] for q in range(4)]
    for i in range(10):
        rows += [G[i, 8:16, q] for q in range(4)]
    rows += [fe.real, fe.imag, ft.real, ft.imag, ft0.real, ft0.imag]
    return np.concatenate(rows, 0).astype(np.float32), masks


_CTAB, _GMASK = _tables()


def _sincos_coeffs():
    r = np.cos(np.pi * (np.arange(4000) + .5) / 4000) * 0.5
    z = r * r
    s = np.linalg.lstsq(np.stack([z ** k for k in range(4)], 1), np.sin(np.pi / 2 * r) / r, rcond=None)[0]
    c = np.linalg.lstsq(np.stack([z ** k for k in range(1, 5)], 1), np.cos(np.pi / 2 * r) - 1, rcond=None)[0]
    return [float(x) for x in s], [float(x) for x in c]


_SC, _CC = _sincos_coeffs()


def _cmul(a, b):
    return (a[0] * b[0] - a[1] * b[1], a[0] * b[1] + a[1] * b[0])


def _cmulc(a, b):
    return (a[0] * b[0] + a[1] * b[1], a[1] * b[0] - a[0] * b[1])


def _csq(a):
    return ((a[0] - a[1]) * (a[0] + a[1]), (a[0] + a[0]) * a[1])


def _sincos(th):
    z = th * (2.0 / np.pi)
    k = jnp.round(z)
    r = z - k
    r2 = r * r
    s = r * (_SC[0] + r2 * (_SC[1] + r2 * (_SC[2] + r2 * _SC[3])))
    c = 1.0 + r2 * (_CC[0] + r2 * (_CC[1] + r2 * (_CC[2] + r2 * _CC[3])))
    ki = k.astype(i32)
    swap = (ki & 1) == 1
    s2 = jnp.where(swap, c, s)
    c2 = jnp.where(swap, s, c)
    s2 = pltpu.bitcast(pltpu.bitcast(s2, i32) ^ ((ki & 2) << 30), f32)
    c2 = pltpu.bitcast(pltpu.bitcast(c2, i32) ^ (((ki + 1) & 2) << 30), f32)
    return s2, c2


def _rb(x):
    return x.astype(bf16).astype(f32)


def _dot(a, b):
    return jnp.dot(a, b, preferred_element_type=f32)


def _dot_nt(a, b):
    return lax.dot_general(a, b, (((1,), (1,)), ((), ())), preferred_element_type=f32)


def _iota(shape, dim):
    return lax.broadcasted_iota(i32, shape, dim)


S4MODE='LL';TILE=2;YSPLIT=1;ORDER='5a4b4244p3n44'
def _weave(*streams):
    items = []
    for si, (pieces, lo, hi) in enumerate(streams):
        tot = float(sum(c for _, c in pieces))
        cum = 0.0
        for pi, (fn, c) in enumerate(pieces):
            items.append((lo + (hi - lo) * (cum + 0.5 * c) / tot, si, pi, fn))
            cum += c
    for _, _, _, fn in sorted(items, key=lambda t: t[:3]):
        fn()


def _kernel(x_h, are_h, aim_h, bre_h, bim_h, cre_h, cim_h, ldt_h, dsk_h, wr_h, wg_h, wu_h, wd_h, ct_h,
            out_h,
            x_v, par_v, ldt_v, dsk_v, wr_v, ct_v, wg_v, wu_v, wd_v, out_v,
            g_v, f_v, col_v, st_v, kd_v, k0_v, kh_v, uh_v, zs_v, c1_v, s1_v, acc_v, fin_v, u_v, zt_v, flag_s,
            sem, osem):
    cp = pltpu.make_async_copy
    c_ct = cp(ct_h, ct_v, sem.at[0])
    c_vec = [cp(ldt_h, ldt_v, sem.at[1]), cp(dsk_h, dsk_v, sem.at[2]), cp(wr_h, wr_v, sem.at[3])]
    c_par = [cp(h, par_v.at[i], sem.at[4 + i])
             for i, h in enumerate((are_h, aim_h, bre_h, bim_h, cre_h, cim_h))]
    c_x = cp(x_h, x_v, sem.at[10])
    c_w = [[cp(h.at[:, pl.ds(FOFF[c], FCH[c])], v.at[:, pl.ds(FOFF[c], FCH[c])], sem.at[11 + 3 * c + i])
            for i, (h, v) in enumerate(((wg_h, wg_v), (wu_h, wu_v), (wd_h, wd_v)))] for c in range(NCH)]
    c_ct.start()
    for c in c_vec + c_par:
        c.start()
    c_x.start()
    for cw in c_w:
        for c in cw:
            c.start()

    flag_s[0] = 1
    x_w = x_v.bitcast(u32)
    out_w = out_v.bitcast(u32)
    g_w = g_v.bitcast(u32)
    f_w = f_v.bitcast(u32)
    sub8 = _iota((8, 128), 0)
    lane8 = _iota((8, 128), 1)

    acc_v[...] = jnp.zeros(acc_v.shape, f32)
    for n in range(NV):
        for ri in range(2):
            st_v[n, ri, 104:112, :] = jnp.full((8, 128), 1.0 - ri, f32)
    g_v[2, :, 0:8, :] = jnp.zeros((4, 8, 128), bf16)
    g_v[2, :, 16:128, :] = jnp.zeros((4, 112, 128), bf16)
    c_ct.wait()

    def e8(v):
        return (jnp.broadcast_to(ct_v[v:v + 1, :], (8, 128)), jnp.broadcast_to(ct_v[32 + v:33 + v, :], (8, 128)))

    sets = {"A0": [0], "A1": [1], "B": [3], "C": [4, 5], "D": [6, 7, 8, 9]}
    for i in range(10):
        for q in range(4):
            g_v[i, q, 8:16, :] = ct_v[224 + 32 * i + 8 * q:232 + 32 * i + 8 * q, :].astype(bf16)
    for si, (name, ps) in enumerate(sets.items()):
        sd = [ct_v[64 + 32 * si + 8 * q:72 + 32 * si + 8 * q, :] for q in range(4)]
        mk = {}
        for i in ps:
            if len(ps) > 1:
                bits = sum(b << s for s, b in enumerate(_GMASK[i]))
                mk[i] = ((bits >> sub8) & 1) == 1
        for v in range(2, 17):
            if v == 2:
                vals = sd
            else:
                ev = e8(2 * (v - 2))
                vals = list(_cmulc((sd[0], sd[1]), ev)) + list(_cmulc((sd[2], sd[3]), ev))
            for i in ps:
                for q in range(4):
                    val = vals[q] if len(ps) == 1 else jnp.where(mk[i], vals[q], 0.0)
                    g_v[i, q, 8 * (v % 16):8 * (v % 16) + 8, :] = val.astype(bf16)
    sig = jnp.where((lane8 & 1) == 0, 1.0, -1.0).astype(f32)
    for h in range(2):
        sd = (ct_v[544 + 16 * h:552 + 16 * h, :], ct_v[552 + 16 * h:560 + 16 * h, :])
        for v in range(16):
            if v == 0:
                vals = sd if h == 0 else (ct_v[576:584, :], ct_v[584:592, :])
            else:
                vals = _cmul(sd, e8(v))
            for q in range(2):
                f_v[0, h, q, 8 * v:8 * v + 8, :] = vals[q].astype(bf16)
                f_v[1, h, q, 8 * v:8 * v + 8, :] = (vals[q] * sig).astype(bf16)

    def gmat(i):
        return jnp.concatenate([pltpu.bitcast(g_w[i, q], bf16) for q in range(4)], 1)

    def fmat(ver, h):
        return jnp.concatenate([pltpu.bitcast(f_w[ver, h, q], bf16) for q in range(2)], 1)

    for c in c_vec:
        c.wait()
    rows = [_rb(jnp.exp(ldt_v[...].astype(f32).reshape(1, D))),
            dsk_v[...].astype(f32).reshape(1, D),
            wr_v[...].astype(f32).reshape(1, D)]
    wr_sum = jnp.sum(rows[2], axis=1, keepdims=True)
    ones = jnp.ones((128, 128), f32)
    for j in range(5):
        w = 128 if j < 4 else 64
        eye = _iota((w, w), 0) == _iota((w, w), 1)
        m = jnp.concatenate([jnp.where(eye, jnp.broadcast_to(rows[i][:, j * 128:j * 128 + w], (w, w)), 0.0)
                             for i in range(3)], 0)
        res = _dot(m, ones[:w, :])
        for i in range(3):
            col_v[i, j * 128:j * 128 + w, :] = res[i * w:(i + 1) * w]

    revmask = (sub8 & 2) == 0
    lm = lane8 & 3

    def s1_nat(k, n0, nn):
        row0 = pl.multiple_of(k * R + 8 * n0, 8)
        rr = 8 * nn
        ld = lambda i: par_v[i, pl.ds(row0, rr), :].astype(f32)
        dt = col_v[0, pl.ds(row0, rr), :]
        e = jnp.exp(dt * ld(0))
        s, c = _sincos(dt * ld(1))
        a1 = (e * c, e * s)
        w = _cmul((ld(4), ld(5)), (dt * ld(2), dt * ld(3)))
        k0_v[k, 8 * n0:8 * n0 + rr, :] = (jnp.sum(w[0], axis=1, keepdims=True)
                                          + col_v[1, pl.ds(row0, rr), :]) * (1.0 / 256.0)
        w = (w[0], -w[1])
        rev = lambda v: jnp.where(revmask, pltpu.roll(v, 2, 0), pltpu.roll(v, 6, 0))

        def put(arr, slots, fn=None):
            for n in range(nn):
                for ri in range(2):
                    v = arr[ri][8 * n:8 * n + 8]
                    if fn is not None:
                        v = fn(v)
                    for q in slots:
                        st_v[n0 + n, ri, q * 8:q * 8 + 8, :] = v

        put(w, (0, 1)); put(a1, (2, 3))
        a2 = _csq(a1); put(a2, (5,))
        a4 = _csq(a2); put(a4, (6,))
        put(_cmul(a4, a1), (4,))
        a8 = _csq(a4); put(a8, (12,), rev)
        t = _csq(a8); put(t, (14, 15), rev)
        for _ in range(4):
            t = _csq(t)
        put(t, (7, 11))
        t = _csq(t); put(t, (8, 9))
        put(_csq(t), (10,))

    def s1_grp(k, n):
        mix = lambda q: tuple(jnp.concatenate([st_v[n, ri, pl.ds(q * 8 + g, 8, stride=2), :] for g in range(2)], 0)
                              for ri in range(2))
        y = [mix(12)]
        a16d = mix(14)
        if YSPLIT == 1:
            for _ in range(15):
                y.append(_cmul(y[-1], a16d))
        else:
            y.append(_cmul(y[0], a16d))
            a32d = _csq(a16d)
            for i in range(2, 16):
                y.append(_cmul(y[i - 2], a32d))
        yield
        wd = mix(0); a1d = mix(2); m1 = mix(5)
        v = [_cmulc(wd, mix(3))]
        for _ in range(3):
            v.append(_cmulc(v[-1], a1d))
        v4 = _cmulc(_cmulc(wd, m1), mix(7))
        v5 = _cmulc(v4, m1); v6 = _cmulc(v4, mix(6)); v7 = _cmulc(v6, m1)
        v8 = _cmulc(v7, mix(10)); v9 = _cmulc(v8, mix(8))
        v += [v4, v5, v6, v7, v8, v9]
        os_ = []
        for g in range(2):
            cat = lambda ts: jnp.concatenate([jnp.concatenate([t[ri][8 * g:8 * g + 8] for t in ts], 0)
                                              for ri in range(2)], 1)
            os_.append(_dot_nt(cat(v), cat(y[::-1])))
        yield
        for g in range(2):
            o = os_[g]
            ro = [pltpu.roll(o[8 * j:8 * j + 8], _XSH[j] + 5, 1, stride=1, stride_axis=0) for j in range(10)]
            sel4 = lambda q: jnp.where(lm == 0, q[0], jnp.where(lm == 1, q[1], jnp.where(lm == 2, q[2], q[3])))
            kd_v[k, n, pl.ds(g, 8, stride=2), :] = sel4(ro[0:4])
            kd_v[k, n, pl.ds(16 + g, 8, stride=2), :] = sel4(ro[4:8])
            kd_v[k, n, pl.ds(32 + g, 8, stride=2), :] = jnp.where(lm == 0, ro[8], ro[9])

    def run(gen):
        for _ in gen:
            pass

    s1n = lambda k: [(functools.partial(s1_nat, k, 3 * i, 3), 1.0) for i in range(3)]
    s1g = lambda k: [(lambda n=n: run(s1_grp(k, n)), 1.0) for n in range(NV)]

    laneR = _iota((R, 128), 1)
    lmR = laneR & 3

    def s2_gen(k):
        ch = lambda c: kd_v[k, :, 8 * c:8 * c + 8, :].reshape(R, 128)
        for b in range(NB):
            if b == 0:
                z = _dot(ch(0), gmat(0))
                dd = jnp.where(lmR < 2, ch(4), pltpu.roll(ch(5), 2, 1))
                kd_v[k, :, 48:56, :] = dd.reshape(NV, 8, 128)
                zt_v[...] = z
                yield
                z = _dot(ch(1), gmat(1)) + zt_v[...]
            elif b == 1:
                zt_v[...] = _dot(ch(1), gmat(2))
                yield
                z = _dot(ch(2), gmat(3)) + zt_v[...]
            elif b == 2:
                z = _dot(jnp.where(laneR == 11, ch(2), ch(3)), gmat(4))
            elif b == 3:
                z = _dot(ch(3), gmat(5))
            elif b == 4:
                z = _dot(jnp.where(laneR == 15, ch(3), ch(6)), gmat(6))
            else:
                z = _dot(ch(6), gmat(b + 2))
            for s in range(2):
                kr = z[:, 256 * s:256 * s + 128]
                ki = z[:, 256 * s + 128:256 * s + 256]
                if b == 0:
                    kr = kr + k0_v[k]
                kh_v[k, b, 3 * s] = kr
                kh_v[k, b, 3 * s + 1] = kr + ki
                kh_v[k, b, 3 * s + 2] = ki - kr
            yield

    def s2(k):
        gen = s2_gen(k)
        return [(lambda: next(gen), 1.0) for _ in range(10)]

    mask2 = (sub8 < 4) == ((lane8 & 1) == 0)
    top = sub8 < 4

    def ln1_pieces(b, npc):
        state = {}
        per = (D // 8) // npc

        def piece(i):
            for g in range(i * per, (i + 1) * per):
                m = x_w[g, b]
                eo = jnp.where(mask2, m, pltpu.roll(pltpu.roll(m, 4, 0), 1, 1))
                a = pltpu.bitcast(eo << 16, f32)
                c = pltpu.bitcast(eo & jnp.uint32(0xFFFF0000), f32)
                if g == 0:
                    state["sh"] = jnp.where(top, jnp.broadcast_to(a[0:1], (8, 128)),
                                            jnp.broadcast_to(a[4:5], (8, 128)))
                a = a - state["sh"]
                c = c - state["sh"]
                c1_v[g, b, pl.ds(0, 8, stride=2), :] = a
                c1_v[g, b, pl.ds(1, 8, stride=2), :] = c
                new = [a, c, a * a, c * c]
                state["acc"] = new if g == 0 else [p + q for p, q in zip(state["acc"], new)]
            if i == npc - 1:
                acc = state["acc"]
                s1, s2_ = acc[0] + acc[1], acc[2] + acc[3]
                for h in range(2):
                    m = jnp.sum(s1[4 * h:4 * h + 4], axis=0, keepdims=True) * (1.0 / D)
                    var = jnp.sum(s2_[4 * h:4 * h + 4], axis=0, keepdims=True) * (1.0 / D) - m * m
                    rs = 1.0 / _rb(jnp.sqrt(_rb(_rb(jnp.maximum(var, 0.0)) + EPS)))
                    s1_v[0, 2 * b + h] = jnp.broadcast_to(rs, (8, 128))
                    s1_v[1, 2 * b + h] = jnp.broadcast_to(m * rs, (8, 128))
                    fin_v[4, 2 * b + h:2 * b + h + 1, :] = state["sh"][4 * h:4 * h + 1]

        return [(functools.partial(piece, i), 1.0) for i in range(npc)]

    def s3_blk(k, b):
        g0 = k * NV
        et = []
        for h in range(2):
            c = c1_v[pl.ds(g0, NV), b, 8 * h:8 * h + 8, :]
            u = (c * s1_v[0, 2 * b + h] - s1_v[1, 2 * b + h]).reshape(R, 128)
            et.append(_dot(u, fmat(b % 2, h)))
        er, ei, tr, ti = et[0][:, :128], et[0][:, 128:], et[1][:, :128], et[1][:, 128:]
        if S4MODE[1] == "C":
            for q, v in enumerate((er, ei, tr, ti)):
                uh_v[k, b, q] = v
        else:
            for s, (pr, pi) in enumerate(((er + tr, ei + ti), (er - tr, ei - ti))):
                uh_v[k, b, 3 * s] = pr + pi
                uh_v[k, b, 3 * s + 1] = pi
                uh_v[k, b, 3 * s + 2] = pr

    s3 = lambda k: [(functools.partial(s3_blk, k, b), 1.0) for b in range(NB)]

    def s4_gen(k, n):
        sl = slice(8 * n, 8 * n + 8)

        def utrip(i, s):
            if S4MODE[1] == "L":
                return [uh_v[k, i, 3 * s + q, sl, :] for q in range(3)]
            er, ei, tr, ti = [uh_v[k, i, q, sl, :] for q in range(4)]
            pr, pi = (er + tr, ei + ti) if s == 0 else (er - tr, ei - ti)
            return [pr + pi, pi, pr]

        prev = None
        done = 0
        for b0 in range(0, NB, TILE):
            yy = []
            for s in range(2):
                acc = [None] * TILE
                win = {}
                for j in range(b0 + TILE):
                    kk = [kh_v[k, j, 3 * s + q, sl, :] for q in range(3)]
                    for o in range(TILE - 1, -1, -1):
                        i = b0 + o - j
                        if i < 0:
                            continue
                        if i not in win:
                            win[i] = utrip(i, s)
                        p = [kk[q] * win[i][q] for q in range(3)]
                        acc[o] = p if acc[o] is None else [a + c for a, c in zip(acc[o], p)]
                        done += 1
                    if TILE == 4 and b0 == 4 and j == 2:
                        yield done
                yy.append([(a[0] - a[1], a[0] + a[2]) for a in acc])
                if s == 0:
                    yield done
            for o in range(TILE):
                p, q = yy[0][o], yy[1][o]
                cur = [(p[0] + q[0], p[1] + q[1]), (p[0] - q[0], p[1] - q[1])]
                for h in range(2):
                    if b0 + o == 0:
                        zr, zi = cur[h]
                    else:
                        zr = cur[h][0] - prev[h][1]
                        zi = cur[h][1] + prev[h][0]
                    zs_v[k, b0 + o, h, sl, 0:128] = zr
                    zs_v[k, b0 + o, h, sl, 128:256] = zi
                prev = cur
            yield done

    def s5_blk(k, b, h):
        g0 = k * NV
        t = 2 * b + h
        y = _dot_nt(zs_v[k, b, h], fmat(b % 2, h)).reshape(NV, 8, 128)
        hh = c1_v[pl.ds(g0, NV), b, 8 * h:8 * h + 8, :] + y
        c1_v[pl.ds(g0, NV), b, 8 * h:8 * h + 8, :] = hh
        wr = col_v[2, pl.ds(pl.multiple_of(k * R, 8), R), :].reshape(NV, 8, 128)
        rs = slice(8 * t, 8 * t + 8)
        acc_v[0, rs, :] = acc_v[0, rs, :] + jnp.sum(hh, axis=0)
        acc_v[1, rs, :] = acc_v[1, rs, :] + jnp.sum(hh * hh, axis=0)
        acc_v[2, rs, :] = acc_v[2, rs, :] + jnp.sum(hh * wr, axis=0)

    s5 = lambda k: [(functools.partial(s5_blk, k, b, h), 1.0) for b in range(NB) for h in range(2)]

    for c in c_par:
        c.wait()
    _weave((s1n(0), 0.0, 0.2), (s1g(0), 0.2, 1.0))
    _weave((s1n(1), 0.0, 0.2), (s1g(1), 0.2, 1.0), (s2(0), 0.1, 0.9))
    c_x.wait()
    ln = [ln1_pieces(b, 3) for b in range(NB)]
    s30 = s3(0)
    _weave((sum(ln, []), 0.0, 0.9), (s1n(2), 0.0, 0.2), (s1g(2), 0.2, 0.9), (s2(1), 0.0, 0.5),
           *[([s30[b]], (b + 1.6) * 0.9 / NB, (b + 1.6) * 0.9 / NB) for b in range(NB)])

    def body(k, do5=True, do4=True, do3=True, do2=True, do1=True, j=None):
        at = (lambda d: k + d) if j is None else (lambda d: j + (k + d) if k + d else j)
        g2 = s2_gen(at(2)) if do2 else None
        for n in range(NV):
            g4 = s4_gen(at(0), n) if do4 else None
            st4 = [0, 0]
            n4 = ORDER.count("4")

            def adv4(m):
                if not do4:
                    return
                st4[0] += 1
                while st4[1] < 72 * st4[0] / n4 - 3 or (st4[0] == n4 and st4[1] <= 72):
                    r = next(g4, None)
                    if r is None:
                        break
                    st4[1] = r

            def nat():
                if do1:
                    if n + 1 < NV:
                        s1_nat(at(3), n + 1, 1)
                    else:
                        s1_nat(jnp.minimum(at(4), NSTEP - 1), 0, 1)

            g1 = s1_grp(at(3), n) if do1 else None
            for tok in ORDER:
                if tok == "5":
                    if do5 and n < NB:
                        s5_blk(at(-1), n, 0)
                        s5_blk(at(-1), n, 1)
                    elif do2 and n == NB:
                        next(g2, None)
                elif tok == "4":
                    adv4(1)
                elif tok in "ab" and do1:
                    next(g1)
                elif tok == "p" and do1:
                    run(g1)
                elif tok == "2" and do2:
                    next(g2, None)
                elif tok == "3" and do3 and n < NB:
                    s3_blk(at(1), n)
                elif tok == "n":
                    nat()
        if do2:
            run(g2)

    s1_nat(3, 0, 1)

    @pl.when(flag_s[0] == 1)
    def _():
        body(0, do5=False)

    lax.fori_loop(0, NSTEP - 4, lambda j, c: (body(1, j=j), c)[1], 0)

    @pl.when(flag_s[0] == 1)
    def _():
        body(5, do1=False)

    @pl.when(flag_s[0] == 1)
    def _():
        body(6, do1=False, do2=False)

    @pl.when(flag_s[0] == 1)
    def _():
        body(7, do1=False, do2=False, do3=False)

    body(8, do1=False, do2=False, do3=False, do4=False)

    def total(i):
        halves = []
        for hf in range(2):
            t = acc_v[i, pl.ds(64 * hf, 8, stride=8), :]
            for s in range(1, 8):
                t = t + acc_v[i, pl.ds(64 * hf + s, 8, stride=8), :]
            halves.append(t)
        return jnp.concatenate(halves, 0)

    m2 = total(0) * (1.0 / D)
    var2 = jnp.maximum(total(1) * (1.0 / D) - m2 * m2, 0.0)
    sd2 = _rb(jnp.sqrt(_rb(_rb(var2) + EPS)))
    rs2 = 1.0 / sd2
    r = _rb((total(2) - m2 * wr_sum) * rs2)
    mean2 = fin_v[4] + m2
    fin_v[0] = rs2
    fin_v[1] = m2 * rs2
    fin_v[2] = rs2 + 1.0
    fin_v[3] = fin_v[4] - m2 * rs2

    tl = _iota((16, 128), 0)
    ll = _iota((16, 128), 1)
    lodd = (ll & 1) == 1
    toff = jnp.where((tl & 1) == 0, jnp.where(lodd, ll + 127, ll), jnp.where(lodd, ll + 128, (ll - 1) & 127))
    tok = (tl >> 1) * 256 + toff
    rbits = pltpu.bitcast(r, i32)
    srt = rbits ^ ((rbits >> 31) & 0x7FFFFFFF)
    key = pltpu.bitcast((((srt >> 16) + 32768) << 11) + (2047 - tok) + (1 << 28), f32)
    keys = []
    for _ in range(TOPC):
        mx = jnp.max(jnp.max(key, axis=0, keepdims=True), axis=1, keepdims=True)
        keys.append(mx)
        key = jnp.where(key == mx, 0.0, key)
    kcol = jnp.broadcast_to(keys[0], (8, 128))
    for j in range(1, TOPC):
        kcol = jnp.where(sub8 == j, keys[j], kcol)
    kint = pltpu.bitcast(kcol, i32) - (1 << 28)
    tcol = 2047 - (kint & 2047)
    s16 = (kint >> 11) - 32768
    rsel = pltpu.bitcast((s16 ^ ((s16 >> 31) & 0x7FFF)) << 16, f32)
    gate = _rb(jax.nn.sigmoid(rsel))[:, 0:1]
    toks = [2047 - ((pltpu.bitcast(jnp.broadcast_to(keys[j], (8, 128)), i32)[0, 0] - (1 << 28)) & 2047)
            for j in range(TOPC)]

    wcol = tcol & 255
    pcol = jnp.where((wcol & 1) == 0, jnp.where(wcol < 128, wcol, wcol - 127),
                     jnp.where(wcol < 128, (wcol + 1) & 127, wcol - 128))
    lhs, rhs = [], []
    for j in range(TOPC):
        bj, hj = toks[j] >> 8, toks[j] & 1
        t = 2 * bj + hj
        cc = c1_v[:, bj, pl.ds(pl.multiple_of(8 * hj, 8), 8), :].reshape(D, 128)
        rhs.append(cc * fin_v[0, pl.ds(t, 1), :] - fin_v[1, pl.ds(t, 1), :])
        lhs.append(jnp.where((sub8 == j) & (lane8 == pcol), 1.0, 0.0).astype(f32))
    xsel = _dot_nt(jnp.concatenate(lhs, 1), jnp.concatenate(rhs, 1))
    sdc = jnp.zeros((8, 1), f32)
    mc = jnp.zeros((8, 1), f32)
    sub1 = _iota((8, 1), 0)
    for j in range(TOPC):
        hitm = tok == toks[j]
        red = lambda v: jnp.sum(jnp.sum(jnp.where(hitm, v, 0.0), axis=0, keepdims=True), axis=1, keepdims=True)
        sdc = jnp.where(sub1 == j, red(sd2), sdc)
        mc = jnp.where(sub1 == j, red(mean2), mc)
    base = xsel * (sdc + 1.0) + mc

    def outp(b, g0, g1):
        sc = [jnp.where(top, jnp.broadcast_to(fin_v[i, 2 * b:2 * b + 1, :], (8, 128)),
                        jnp.broadcast_to(fin_v[i, 2 * b + 1:2 * b + 2, :], (8, 128))) for i in (2, 3)]
        for g in range(g0, g1):
            a = _rb(c1_v[g, b, pl.ds(0, 8, stride=2), :] * sc[0] + sc[1])
            c = _rb(c1_v[g, b, pl.ds(1, 8, stride=2), :] * sc[0] + sc[1])
            w = (pltpu.bitcast(a, u32) >> 16) | pltpu.bitcast(c, u32)
            out_w[g, b] = jnp.where(mask2, w, pltpu.roll(pltpu.roll(w, 4, 0), 127, 1))

    opieces = [functools.partial(outp, b, 24 * i, 24 * i + 24) for b in range(NB) for i in range(3)]

    tiles = [toks[j] >> 7 for j in range(TOPC)]
    hit = 0
    for j in range(TOPC):
        hit = hit | (1 << tiles[j])

    def ocopy(t):
        if isinstance(t, int):
            idx = (slice(None), t // 2, pl.ds(8 * (t % 2), 8), slice(None))
        else:
            idx = (slice(None), t >> 1, pl.ds(pl.multiple_of(8 * (t & 1), 8), 8), slice(None))
        return cp(out_v.at[idx], out_h.at[idx], osem.at[t])

    osplit = [0, 6, 12, 17, 21, 24, 24]
    y = jnp.zeros((8, D), f32)
    for c in range(NCH):
        for cc in c_w[c]:
            cc.wait()
        if c == NCH - 1:
            for t in range(16):
                @pl.when(((hit >> t) & 1) == 0)
                def _():
                    ocopy(t).start()
        sl = slice(FOFF[c], FOFF[c] + FCH[c])
        mine = opieces[osplit[c]:osplit[c + 1]]
        g = _rb(_dot(xsel, wg_v[:, sl]))
        up = _rb(_dot(xsel, wu_v[:, sl]))
        for fn in mine[:len(mine) // 2]:
            fn()
        act = _rb(_rb(g * jax.nn.sigmoid(g)) * up)
        y = y + _dot_nt(act, wd_v[:, sl])
        for fn in mine[len(mine) // 2:]:
            fn()
    newrow = _rb(base + _rb(_rb(y) * gate))

    lanes = [toks[j] & 127 for j in range(TOPC)]
    cls = []
    ncls = 1
    clscol = jnp.zeros((8, 128), i32)
    for j in range(TOPC):
        cj = 0
        for j2 in range(j):
            cj = cj + (lanes[j2] == lanes[j]).astype(i32)
        cls.append(cj)
        ncls = jnp.maximum(ncls, cj + 1)
        clscol = jnp.where(sub8 == j, cj, clscol)

    def place(c, carry):
        oh = jnp.where((clscol == c) & (lane8 == (tcol & 127)), 1.0, 0.0).astype(f32)
        u_v[c] = lax.dot_general(newrow, oh, (((0,), (0,)), ((), ())),
                                 preferred_element_type=f32).reshape(D // 8, 8, 128)
        return carry

    lax.fori_loop(0, ncls, place, 0)
    lane3 = _iota((D // 8, 8, 128), 2)
    for j in range(TOPC):
        idx = (slice(None), tiles[j] >> 1, pl.ds(pl.multiple_of(8 * (tiles[j] & 1), 8), 8), slice(None))
        cur = out_v[idx].astype(f32)
        out_v[idx] = jnp.where(lane3 == lanes[j], u_v[cls[j]], cur).astype(bf16)
        later = False
        for j2 in range(j + 1, TOPC):
            later = jnp.logical_or(later, tiles[j2] == tiles[j])

        @pl.when(jnp.logical_not(later))
        def _():
            ocopy(tiles[j]).start()

    for t in range(16):
        ocopy(t).wait()


@jax.jit
def pallas_sequential_preLN__ssm_conv_s4__moe_arch_mod__prompt_kernel(
    A_u: jax.Array,
    A_A_re: jax.Array,
    A_A_im: jax.Array,
    A_B_re: jax.Array,
    A_B_im: jax.Array,
    A_C_re: jax.Array,
    A_C_im: jax.Array,
    A_log_dt: jax.Array,
    A_Dskip: jax.Array,
    B_x: jax.Array,
    B_w_r: jax.Array,
    B_w_gate: jax.Array,
    B_w_up: jax.Array,
    B_w_down: jax.Array,
):
    hbm = pl.BlockSpec(memory_space=pltpu.MemorySpace.HBM)
    vm = pltpu.VMEM
    G8 = D // 8
    scratch = [
        vm((G8, NB, 16, 128), bf16), vm((6, D, N), bf16), vm((D,), bf16), vm((D,), bf16), vm((D,), bf16),
        vm(_CTAB.shape, f32), vm((D, F), bf16), vm((D, F), bf16), vm((D, F), bf16), vm((G8, NB, 16, 128), bf16),
        vm((10, 4, 128, 128), bf16), vm((2, 2, 2, 128, 128), bf16), vm((3, D, 128), f32),
        vm((NV, 2, 128, 128), f32), vm((NSTEP, NV, 56, 128), f32), vm((NSTEP, R, 128), f32),
        vm((NSTEP, NB, 6, R, 128), f32), vm((NSTEP, NB, 6, R, 128), f32),
        vm((NSTEP, NB, 2, R, 256), f32), vm((G8, NB, 16, 128), f32), vm((2, 16, 8, 128), f32),
        vm((3, 128, 128), f32), vm((5, 16, 128), f32), vm((TOPC, G8, 8, 128), f32),
        vm((R, 512), f32), pltpu.SMEM((1,), i32),
        pltpu.SemaphoreType.DMA((11 + 3 * NCH,)), pltpu.SemaphoreType.DMA((16,)),
    ]
    xv = A_u[0].T.reshape(G8, 8, 16, 128).transpose(0, 2, 1, 3).reshape(G8, NB, 16, 128)
    out = pl.pallas_call(
        _kernel,
        out_shape=jax.ShapeDtypeStruct((G8, NB, 16, 128), bf16),
        in_specs=[hbm] * 14,
        out_specs=hbm,
        scratch_shapes=scratch,
        compiler_params=pltpu.CompilerParams(vmem_limit_bytes=120 * 1024 * 1024),
    )(xv, A_A_re, A_A_im, A_B_re, A_B_im, A_C_re, A_C_im, A_log_dt, A_Dskip, B_w_r,
      B_w_gate, B_w_up, B_w_down.T, jnp.asarray(_CTAB))
    return out.reshape(G8, 16, 8, 128).transpose(0, 2, 1, 3).reshape(D, L).T[None]
```

```python
import functools

import numpy as np
import jax
import jax.numpy as jnp
from jax import lax
import jax.experimental.pallas as pl
import jax.experimental.pallas.tpu as pltpu

f32 = jnp.float32
bf16 = jnp.bfloat16
i32 = jnp.int32
u32 = jnp.uint32

L, D, N, F, TOPC = 2048, 576, 128, 4608, 8
NB = 8
NV = 9
R = NV * 8
NSTEP = D // R
FCH = (1024, 1024, 896, 768, 640, 256)
NCH = len(FCH)
FOFF = [sum(FCH[:i]) for i in range(NCH)]
EPS = 1e-5

_XL1 = [(1, 5), (2, 6), (3, 7), (4, 8), (258, 516), (260, 520), (262, 772), (264, 776),
        (1288, 1032), (1800, 1544)]
_XSH = [0, 1, 2, 3, 0, 1, 2, 3, 0, 1]


def _bf16_round_int(j):
    u = np.asarray(j, np.float32).view(np.uint32).astype(np.uint64)
    r = ((u + 0x7FFF + ((u >> 16) & 1)) >> 16) << 16
    return r.astype(np.uint32).view(np.float32).astype(np.int64)


def _chunk_values():
    vals = -np.ones((5, 128), np.int64)
    for j in range(10):
        for p in range(2):
            ch = (j // 4) * 2 + p if j < 8 else 4
            extra = 2 * p if j >= 8 else 0
            for l0 in range(32):
                vals[ch, (4 * (31 - l0) + 4 * p + _XSH[j] + extra + 8) % 128] = _XL1[j][p] + 8 * l0
    assert (vals >= 0).all()
    return vals


def _tables():
    cv = _chunk_values()
    om = np.pi * (2 * np.arange(128) + 1) / 512.0
    sig = (-1.0) ** np.arange(128)
    cvp = {"A0": cv[0], "A1": cv[1], "B": cv[2], "C": cv[3], "D": cv[4]}
    cvp["Cp"] = cv[3].copy(); cvp["Cp"][11] = cv[2][11]
    cvp["Dp"] = cv[4].copy(); cvp["Dp"][15] = cv[3][15]
    passes = [(0, "A0"), (0, "A1"), (1, "A1"), (1, "B"), (2, "Cp"), (3, "C"), (4, "Dp"),
              (5, "D"), (6, "D"), (7, "D")]
    G = np.zeros((10, 128, 4, 128))
    for b in range(NB):
        mine = [i for i, (pb, _) in enumerate(passes) if pb == b]
        for j in range(1, 257):
            lag = 256 * b + j
            if lag > L - 1:
                continue
            v = int(_bf16_round_int(lag))
            hit = [(i, int(np.nonzero(cvp[passes[i][1]] == v)[0][0])) for i in mine
                   if (cvp[passes[i][1]] == v).any()]
            assert len(hit) == 1, (b, j, v, hit)
            i, l = hit[0]
            e = np.exp(-1j * om * j) * sig ** b / 256.0
            s = (-1.0) ** j
            G[i, l, 0] += e.real; G[i, l, 1] += e.imag
            G[i, l, 2] += s * e.real; G[i, l, 3] += s * e.imag
    e8 = np.exp(-1j * np.outer(8 * np.arange(32), om))
    sets = {"A0": [0], "A1": [1], "B": [3], "C": [4, 5], "D": [6, 7, 8, 9]}
    seeds, masks = {}, {}
    for name, ps in sets.items():
        seeds[name] = sum(G[i, 16:24] for i in ps)
        for i in ps:
            masks[i] = [int(x) for x in (np.abs(G[i, 16:24]).sum((1, 2)) > 0)]
            for v in range(2, 17):
                sd = seeds[name]
                r0 = 8 * (v % 16)
                for q in (0, 2):
                    z = (sd[:, q] + 1j * sd[:, q + 1]) * np.conj(e8[2 * (v - 2)]) * np.array(masks[i])[:, None]
                    assert np.allclose(z.real, G[i, r0:r0 + 8, q], atol=1e-12)
                    assert np.allclose(z.imag, G[i, r0:r0 + 8, q + 1], atol=1e-12)
    assert not G[2, 16:].any() and not G[2, :8].any()
    s8 = np.arange(8)
    je = np.where(s8 % 2 == 0, s8, 127 + s8)
    jo = np.where(s8 % 2 == 0, s8 - 1, 128 + s8)
    fe = np.exp(-1j * np.outer(je, om)); ft = np.exp(-1j * np.outer(jo, om))
    ft0 = np.exp(-1j * np.outer(jo % 128 + 128 * (s8 % 2), om))
    rows = [e8.real, e8.imag]
    for name in ("A0", "A1", "B", "C", "D"):
        rows += [seeds[name][:, q] for q in range(4)]
    for i in range(10):
        rows += [G[i, 8:16, q] for q in range(4)]
    rows += [fe.real, fe.imag, ft.real, ft.imag, ft0.real, ft0.imag]
    return np.concatenate(rows, 0).astype(np.float32), masks


_CTAB, _GMASK = _tables()


def _sincos_coeffs():
    r = np.cos(np.pi * (np.arange(4000) + .5) / 4000) * 0.5
    z = r * r
    s = np.linalg.lstsq(np.stack([z ** k for k in range(4)], 1), np.sin(np.pi / 2 * r) / r, rcond=None)[0]
    c = np.linalg.lstsq(np.stack([z ** k for k in range(1, 5)], 1), np.cos(np.pi / 2 * r) - 1, rcond=None)[0]
    return [float(x) for x in s], [float(x) for x in c]


_SC, _CC = _sincos_coeffs()


def _cmul(a, b):
    return (a[0] * b[0] - a[1] * b[1], a[0] * b[1] + a[1] * b[0])


def _cmulc(a, b):
    return (a[0] * b[0] + a[1] * b[1], a[1] * b[0] - a[0] * b[1])


def _csq(a):
    return ((a[0] - a[1]) * (a[0] + a[1]), (a[0] + a[0]) * a[1])


def _sincos(th):
    z = th * (2.0 / np.pi)
    k = jnp.round(z)
    r = z - k
    r2 = r * r
    s = r * (_SC[0] + r2 * (_SC[1] + r2 * (_SC[2] + r2 * _SC[3])))
    c = 1.0 + r2 * (_CC[0] + r2 * (_CC[1] + r2 * (_CC[2] + r2 * _CC[3])))
    ki = k.astype(i32)
    swap = (ki & 1) == 1
    s2 = jnp.where(swap, c, s)
    c2 = jnp.where(swap, s, c)
    s2 = pltpu.bitcast(pltpu.bitcast(s2, i32) ^ ((ki & 2) << 30), f32)
    c2 = pltpu.bitcast(pltpu.bitcast(c2, i32) ^ (((ki + 1) & 2) << 30), f32)
    return s2, c2


def _rb(x):
    return x.astype(bf16).astype(f32)


def _dot(a, b):
    return jnp.dot(a, b, preferred_element_type=f32)


def _dot_nt(a, b):
    return lax.dot_general(a, b, (((1,), (1,)), ((), ())), preferred_element_type=f32)


def _iota(shape, dim):
    return lax.broadcasted_iota(i32, shape, dim)


S4MODE='LC';TILE=4;YSPLIT=1;ZT=1;ORDER='5a4b4244p3n44';NPC=3;P3F=(0.9,0.4,0.55,0.3);OSPLIT=[0,9,17,24,24,24,24];WSTART=3;GCH=3
def _weave(*streams):
    items = []
    for si, (pieces, lo, hi) in enumerate(streams):
        tot = float(sum(c for _, c in pieces))
        cum = 0.0
        for pi, (fn, c) in enumerate(pieces):
            items.append((lo + max(hi - lo, 0.0) * (cum + 0.5 * c) / tot, si, pi, fn))
            cum += c
    for _, _, _, fn in sorted(items, key=lambda t: t[:3]):
        fn()


def _kernel(x_h, are_h, aim_h, bre_h, bim_h, cre_h, cim_h, ldt_h, dsk_h, wr_h, wg_h, wu_h, wd_h, ct_h,
            out_h,
            x_v, par_v, ldt_v, dsk_v, wr_v, ct_v, wg_v, wu_v, wd_v, out_v,
            g_v, f_v, col_v, st_v, kd_v, k0_v, kh_v, uh_v, zs_v, c1_v, s1_v, acc_v, fin_v, u_v, zt_v, y_v, pv_v, kc_v, xs_v, bs_v, flag_s,
            sem, osem):
    cp = pltpu.make_async_copy
    c_ct = cp(ct_h, ct_v, sem.at[0])
    c_vec = [cp(ldt_h, ldt_v, sem.at[1]), cp(dsk_h, dsk_v, sem.at[1]), cp(wr_h, wr_v, sem.at[1])]
    PH = 4 * R
    par_h = (are_h, aim_h, bre_h, bim_h, cre_h, cim_h)
    c_par = [cp(h.at[pl.ds(0, PH)], par_v.at[i, pl.ds(0, PH)], sem.at[2]) for i, h in enumerate(par_h)]
    c_par2 = [cp(h.at[pl.ds(PH, D - PH)], par_v.at[i, pl.ds(PH, D - PH)], sem.at[3])
              for i, h in enumerate(par_h)]
    c_x = cp(x_h, x_v, sem.at[4])
    c_w = [[cp(h.at[:, pl.ds(FOFF[c], FCH[c])], v.at[:, pl.ds(FOFF[c], FCH[c])], sem.at[5 + c])
            for i, (h, v) in enumerate(((wg_h, wg_v), (wu_h, wu_v), (wd_h, wd_v)))] for c in range(NCH)]
    for c in c_vec + [c_ct] + c_par + [c_x] + c_par2:
        c.start()
    for cw in c_w:
        for c in cw:
            c.start()

    flag_s[0] = 1
    x_w = x_v.bitcast(u32)
    out_w = out_v.bitcast(u32)
    g_w = g_v.bitcast(u32)
    f_w = f_v.bitcast(u32)
    sub8 = _iota((8, 128), 0)
    lane8 = _iota((8, 128), 1)

    acc_v[...] = jnp.zeros(acc_v.shape, f32)
    for n in range(NV):
        for ri in range(2):
            st_v[n, ri, 104:112, :] = jnp.full((8, 128), 1.0 - ri, f32)
    g_v[2, :, 0:8, :] = jnp.zeros((4, 8, 128), bf16)
    g_v[2, :, 16:128, :] = jnp.zeros((4, 112, 128), bf16)
    for c in c_vec:
        c.wait()

    rows = [_rb(jnp.exp(ldt_v[...].astype(f32).reshape(1, D))),
            dsk_v[...].astype(f32).reshape(1, D),
            wr_v[...].astype(f32).reshape(1, D)]
    wr_sum = jnp.sum(rows[2], axis=1, keepdims=True)
    ones = jnp.ones((128, 128), f32)
    for j in range(5):
        w = 128 if j < 4 else 64
        eye = _iota((w, w), 0) == _iota((w, w), 1)
        m = jnp.concatenate([jnp.where(eye, jnp.broadcast_to(rows[i][:, j * 128:j * 128 + w], (w, w)), 0.0)
                             for i in range(3)], 0)
        res = _dot(m, ones[:w, :])
        for i in range(3):
            col_v[i, j * 128:j * 128 + w, :] = res[i * w:(i + 1) * w]

    c_ct.wait()

    def e8(v):
        return (jnp.broadcast_to(ct_v[v:v + 1, :], (8, 128)), jnp.broadcast_to(ct_v[32 + v:33 + v, :], (8, 128)))

    sets = {"A0": [0], "A1": [1], "B": [3], "C": [4, 5], "D": [6, 7, 8, 9]}
    for i in range(10):
        for q in range(4):
            g_v[i, q, 8:16, :] = ct_v[224 + 32 * i + 8 * q:232 + 32 * i + 8 * q, :].astype(bf16)
    for si, (name, ps) in enumerate(sets.items()):
        sd = [ct_v[64 + 32 * si + 8 * q:72 + 32 * si + 8 * q, :] for q in range(4)]
        mk = {}
        for i in ps:
            if len(ps) > 1:
                bits = sum(b << s for s, b in enumerate(_GMASK[i]))
                mk[i] = ((bits >> sub8) & 1) == 1
        for v in range(2, 17):
            if v == 2:
                vals = sd
            else:
                ev = e8(2 * (v - 2))
                vals = list(_cmulc((sd[0], sd[1]), ev)) + list(_cmulc((sd[2], sd[3]), ev))
            for i in ps:
                for q in range(4):
                    val = vals[q] if len(ps) == 1 else jnp.where(mk[i], vals[q], 0.0)
                    g_v[i, q, 8 * (v % 16):8 * (v % 16) + 8, :] = val.astype(bf16)
    sig = jnp.where((lane8 & 1) == 0, 1.0, -1.0).astype(f32)
    for h in range(2):
        sd = (ct_v[544 + 16 * h:552 + 16 * h, :], ct_v[552 + 16 * h:560 + 16 * h, :])
        for v in range(16):
            if v == 0:
                vals = sd if h == 0 else (ct_v[576:584, :], ct_v[584:592, :])
            else:
                vals = _cmul(sd, e8(v))
            for q in range(2):
                f_v[0, h, q, 8 * v:8 * v + 8, :] = vals[q].astype(bf16)
                f_v[1, h, q, 8 * v:8 * v + 8, :] = (vals[q] * sig).astype(bf16)

    def gmat(i):
        return jnp.concatenate([pltpu.bitcast(g_w[i, q], bf16) for q in range(4)], 1)

    def fmat(ver, h):
        return jnp.concatenate([pltpu.bitcast(f_w[ver, h, q], bf16) for q in range(2)], 1)

    revmask = (sub8 & 2) == 0
    lm = lane8 & 3

    def s1_nat(k, n0, nn):
        row0 = pl.multiple_of(k * R + 8 * n0, 8)
        rr = 8 * nn
        ld = lambda i: par_v[i, pl.ds(row0, rr), :].astype(f32)
        dt = col_v[0, pl.ds(row0, rr), :]
        e = jnp.exp(dt * ld(0))
        s, c = _sincos(dt * ld(1))
        a1 = (e * c, e * s)
        w = _cmul((ld(4), ld(5)), (dt * ld(2), dt * ld(3)))
        k0_v[k, 8 * n0:8 * n0 + rr, :] = (jnp.sum(w[0], axis=1, keepdims=True)
                                          + col_v[1, pl.ds(row0, rr), :]) * (1.0 / 256.0)
        w = (w[0], -w[1])
        rev = lambda v: jnp.where(revmask, pltpu.roll(v, 2, 0), pltpu.roll(v, 6, 0))

        def put(arr, slots, fn=None):
            for n in range(nn):
                for ri in range(2):
                    v = arr[ri][8 * n:8 * n + 8]
                    if fn is not None:
                        v = fn(v)
                    for q in slots:
                        st_v[n0 + n, ri, q * 8:q * 8 + 8, :] = v

        put(w, (0, 1)); put(a1, (2, 3))
        a2 = _csq(a1); put(a2, (5,))
        a4 = _csq(a2); put(a4, (6,))
        put(_cmul(a4, a1), (4,))
        a8 = _csq(a4); put(a8, (12,), rev)
        t = _csq(a8); put(t, (14, 15), rev)
        for _ in range(4):
            t = _csq(t)
        put(t, (7, 11))
        t = _csq(t); put(t, (8, 9))
        put(_csq(t), (10,))

    def s1_grp(k, n):
        mix = lambda q: tuple(jnp.concatenate([st_v[n, ri, pl.ds(q * 8 + g, 8, stride=2), :] for g in range(2)], 0)
                              for ri in range(2))
        y = [mix(12)]
        a16d = mix(14)
        if YSPLIT == 1:
            for _ in range(15):
                y.append(_cmul(y[-1], a16d))
        else:
            y.append(_cmul(y[0], a16d))
            a32d = _csq(a16d)
            for i in range(2, 16):
                y.append(_cmul(y[i - 2], a32d))
        yield
        wd = mix(0); a1d = mix(2); m1 = mix(5)
        v = [_cmulc(wd, mix(3))]
        for _ in range(3):
            v.append(_cmulc(v[-1], a1d))
        v4 = _cmulc(_cmulc(wd, m1), mix(7))
        v5 = _cmulc(v4, m1); v6 = _cmulc(v4, mix(6)); v7 = _cmulc(v6, m1)
        v8 = _cmulc(v7, mix(10)); v9 = _cmulc(v8, mix(8))
        v += [v4, v5, v6, v7, v8, v9]
        os_ = []
        for g in range(2):
            cat = lambda ts: jnp.concatenate([jnp.concatenate([t[ri][8 * g:8 * g + 8] for t in ts], 0)
                                              for ri in range(2)], 1)
            os_.append(_dot_nt(cat(v), cat(y[::-1])))
        yield
        for g in range(2):
            o = os_[g]
            ro = [pltpu.roll(o[8 * j:8 * j + 8], _XSH[j] + 5, 1, stride=1, stride_axis=0) for j in range(10)]
            sel4 = lambda q: jnp.where(lm == 0, q[0], jnp.where(lm == 1, q[1], jnp.where(lm == 2, q[2], q[3])))
            kd_v[k, n, pl.ds(g, 8, stride=2), :] = sel4(ro[0:4])
            kd_v[k, n, pl.ds(16 + g, 8, stride=2), :] = sel4(ro[4:8])
            kd_v[k, n, pl.ds(32 + g, 8, stride=2), :] = jnp.where(lm == 0, ro[8], ro[9])

    def run(gen):
        for _ in gen:
            pass

    s1n = lambda k: [(functools.partial(s1_nat, k, 3 * i, 3), 1.0) for i in range(3)]
    s1g = lambda k: [(lambda n=n: run(s1_grp(k, n)), 1.0) for n in range(NV)]

    laneR = _iota((R, 128), 1)
    lmR = laneR & 3

    def s2_gen(k):
        ch = lambda c: kd_v[k, :, 8 * c:8 * c + 8, :].reshape(R, 128)
        for b in range(NB):
            if b == 0:
                z = _dot(ch(0), gmat(0)) if ZT else None
                dd = jnp.where(lmR < 2, ch(4), pltpu.roll(ch(5), 2, 1))
                kd_v[k, :, 48:56, :] = dd.reshape(NV, 8, 128)
                if ZT:
                    zt_v[...] = z
                    yield
                    z = _dot(ch(1), gmat(1)) + zt_v[...]
                else:
                    z = _dot(jnp.concatenate([ch(0), ch(1)], 1), jnp.concatenate([gmat(0), gmat(1)], 0))
            elif b == 1:
                if ZT:
                    zt_v[...] = _dot(ch(1), gmat(2))
                    yield
                    z = _dot(ch(2), gmat(3)) + zt_v[...]
                else:
                    z = _dot(jnp.concatenate([ch(1), ch(2)], 1), jnp.concatenate([gmat(2), gmat(3)], 0))
            elif b == 2:
                z = _dot(jnp.where(laneR == 11, ch(2), ch(3)), gmat(4))
            elif b == 3:
                z = _dot(ch(3), gmat(5))
            elif b == 4:
                z = _dot(jnp.where(laneR == 15, ch(3), ch(6)), gmat(6))
            else:
                z = _dot(ch(6), gmat(b + 2))
            for s in range(2):
                kr = z[:, 256 * s:256 * s + 128]
                ki = z[:, 256 * s + 128:256 * s + 256]
                if b == 0:
                    kr = kr + k0_v[k]
                kh_v[k, b, 3 * s] = kr
                if S4MODE[0] == "L":
                    kh_v[k, b, 3 * s + 1] = kr + ki
                    kh_v[k, b, 3 * s + 2] = ki - kr
                else:
                    kh_v[k, b, 3 * s + 1] = ki
            yield

    def s2(k):
        gen = s2_gen(k)
        return [(lambda: next(gen, None), 1.0) for _ in range(10)]

    mask2 = (sub8 < 4) == ((lane8 & 1) == 0)
    top = sub8 < 4

    def ln1_pieces(b, npc):
        state = {}
        per = (D // 8) // npc

        def piece(i):
            for g in range(i * per, (i + 1) * per):
                m = x_w[g, b]
                eo = jnp.where(mask2, m, pltpu.roll(pltpu.roll(m, 4, 0), 1, 1))
                a = pltpu.bitcast(eo << 16, f32)
                c = pltpu.bitcast(eo & jnp.uint32(0xFFFF0000), f32)
                if g == 0:
                    state["sh"] = jnp.where(top, jnp.broadcast_to(a[0:1], (8, 128)),
                                            jnp.broadcast_to(a[4:5], (8, 128)))
                a = a - state["sh"]
                c = c - state["sh"]
                c1_v[g, b, pl.ds(0, 8, stride=2), :] = a
                c1_v[g, b, pl.ds(1, 8, stride=2), :] = c
                new = [a, c, a * a, c * c]
                state["acc"] = new if g == 0 else [p + q for p, q in zip(state["acc"], new)]
            if i == npc - 1:
                acc = state["acc"]
                s1, s2_ = acc[0] + acc[1], acc[2] + acc[3]
                for h in range(2):
                    m = jnp.sum(s1[4 * h:4 * h + 4], axis=0, keepdims=True) * (1.0 / D)
                    var = jnp.sum(s2_[4 * h:4 * h + 4], axis=0, keepdims=True) * (1.0 / D) - m * m
                    rs = 1.0 / _rb(jnp.sqrt(_rb(_rb(jnp.maximum(var, 0.0)) + EPS)))
                    s1_v[0, 2 * b + h] = jnp.broadcast_to(rs, (8, 128))
                    s1_v[1, 2 * b + h] = jnp.broadcast_to(m * rs, (8, 128))
                    fin_v[4, 2 * b + h:2 * b + h + 1, :] = state["sh"][4 * h:4 * h + 1]

        return [(functools.partial(piece, i), 1.0) for i in range(npc)]

    def s3_blk(k, b):
        g0 = k * NV
        et = []
        for h in range(2):
            c = c1_v[pl.ds(g0, NV), b, 8 * h:8 * h + 8, :]
            u = (c * s1_v[0, 2 * b + h] - s1_v[1, 2 * b + h]).reshape(R, 128)
            et.append(_dot(u, fmat(b % 2, h)))
        er, ei, tr, ti = et[0][:, :128], et[0][:, 128:], et[1][:, :128], et[1][:, 128:]
        if S4MODE[1] == "C":
            for q, v in enumerate((er, ei, tr, ti)):
                uh_v[k, b, q] = v
        else:
            for s, (pr, pi) in enumerate(((er + tr, ei + ti), (er - tr, ei - ti))):
                uh_v[k, b, 3 * s] = pr + pi
                uh_v[k, b, 3 * s + 1] = pi
                uh_v[k, b, 3 * s + 2] = pr

    s3 = lambda k: [(functools.partial(s3_blk, k, b), 1.0) for b in range(NB)]

    def s4_gen(k, n, groups=None):
        sl = slice(8 * n, 8 * n + 8)

        def utrip(i, s):
            if S4MODE[1] == "L":
                return [uh_v[k, i, 3 * s + q, sl, :] for q in range(3)]
            er, ei, tr, ti = [uh_v[k, i, q, sl, :] for q in range(4)]
            pr, pi = (er + tr, ei + ti) if s == 0 else (er - tr, ei - ti)
            return [pr + pi, pi, pr]

        prev = None
        done = 0
        if groups is not None and groups[0] > 0:
            prev = [(pv_v[n, 2 * h], pv_v[n, 2 * h + 1]) for h in range(2)]
        for b0 in (range(0, NB, TILE) if groups is None else groups):
            yy = []
            for s in range(2):
                acc = [None] * TILE
                win = {}
                for j in range(b0 + TILE):
                    if S4MODE[0] == "L":
                        kk = [kh_v[k, j, 3 * s + q, sl, :] for q in range(3)]
                    else:
                        kr, ki = kh_v[k, j, 3 * s, sl, :], kh_v[k, j, 3 * s + 1, sl, :]
                        kk = [kr, kr + ki, ki - kr]
                    for o in range(TILE - 1, -1, -1):
                        i = b0 + o - j
                        if i < 0:
                            continue
                        if i not in win:
                            win[i] = utrip(i, s)
                        p = [kk[q] * win[i][q] for q in range(3)]
                        acc[o] = p if acc[o] is None else [a + c for a, c in zip(acc[o], p)]
                        done += 1
                    if TILE == 4 and b0 == 4 and j == 2:
                        yield done
                yy.append([(a[0] - a[1], a[0] + a[2]) for a in acc])
                if s == 0:
                    yield done
            for o in range(TILE):
                p, q = yy[0][o], yy[1][o]
                cur = [(p[0] + q[0], p[1] + q[1]), (p[0] - q[0], p[1] - q[1])]
                for h in range(2):
                    if b0 + o == 0:
                        zr, zi = cur[h]
                    else:
                        zr = cur[h][0] - prev[h][1]
                        zi = cur[h][1] + prev[h][0]
                    zs_v[k, b0 + o, h, sl, 0:128] = zr
                    zs_v[k, b0 + o, h, sl, 128:256] = zi
                prev = cur
            if groups is not None and b0 + TILE < NB:
                for h in range(2):
                    pv_v[n, 2 * h] = prev[h][0]
                    pv_v[n, 2 * h + 1] = prev[h][1]
            yield done

    def s5_blk(k, b, h):
        g0 = k * NV
        t = 2 * b + h
        y = _dot_nt(zs_v[k, b, h], fmat(b % 2, h)).reshape(NV, 8, 128)
        hh = c1_v[pl.ds(g0, NV), b, 8 * h:8 * h + 8, :] + y
        c1_v[pl.ds(g0, NV), b, 8 * h:8 * h + 8, :] = hh
        wr = col_v[2, pl.ds(pl.multiple_of(k * R, 8), R), :].reshape(NV, 8, 128)
        rs = slice(8 * t, 8 * t + 8)
        acc_v[0, rs, :] = acc_v[0, rs, :] + jnp.sum(hh, axis=0)
        acc_v[1, rs, :] = acc_v[1, rs, :] + jnp.sum(hh * hh, axis=0)
        acc_v[2, rs, :] = acc_v[2, rs, :] + jnp.sum(hh * wr, axis=0)

    s5 = lambda k: [(functools.partial(s5_blk, k, b, h), 1.0) for b in range(NB) for h in range(2)]

    for c in c_par:
        c.wait()
    for k in range(2):
        _weave((s1n(k), 0.0, 0.2), (s1g(k), 0.2, 1.0))
    _weave((s1n(2), 0.0, 0.2), (s1g(2), 0.2, 1.0), (s2(0), 0.3, 1.0))
    s1_nat(3, 0, 1)
    c_x.wait()
    ln = [ln1_pieces(b, NPC) for b in range(NB)]
    s30 = s3(0)
    _weave((sum(ln, []), 0.0, P3F[0]), (s2(1), 0.0, P3F[2]),
           *[([s30[b]], max((b + 1.6) * P3F[0] / NB, P3F[3] + (1.0 - P3F[3]) * b / NB), 0.0) for b in range(NB)])
    for c in c_par2:
        c.wait()

    def body(k, do5=True, do4=True, do3=True, do2=True, do1=True, j=None):
        at = (lambda d: k + d) if j is None else (lambda d: j + (k + d) if k + d else j)
        g2 = s2_gen(at(2)) if do2 else None
        for n in range(NV):
            g4 = s4_gen(at(0), n) if do4 else None
            st4 = [0, 0]
            n4 = ORDER.count("4")

            def adv4(m):
                if not do4:
                    return
                st4[0] += 1
                while st4[1] < 72 * st4[0] / n4 - 3 or (st4[0] == n4 and st4[1] <= 72):
                    r = next(g4, None)
                    if r is None:
                        break
                    st4[1] = r

            def nat():
                if do1:
                    if n + 1 < NV:
                        s1_nat(at(3), n + 1, 1)
                    else:
                        s1_nat(jnp.minimum(at(4), NSTEP - 1), 0, 1)

            g1 = s1_grp(at(3), n) if do1 else None
            for tok in ORDER:
                if tok == "5":
                    if do5 and n < NB:
                        s5_blk(at(-1), n, 0)
                        s5_blk(at(-1), n, 1)
                    elif do2 and n == NB:
                        next(g2, None)
                elif tok == "4":
                    adv4(1)
                elif tok in "ab" and do1:
                    next(g1)
                elif tok == "p" and do1:
                    run(g1)
                elif tok == "2" and do2:
                    next(g2, None)
                elif tok == "3" and do3 and n < NB:
                    s3_blk(at(1), n)
                elif tok == "n":
                    nat()
        if do2:
            run(g2)

    @pl.when(flag_s[0] == 1)
    def _():
        body(0, do5=False)

    lax.fori_loop(0, 4, lambda j, c: (body(1, j=j), c)[1], 0)

    @pl.when(flag_s[0] == 1)
    def _():
        body(5, do1=False)

    @pl.when(flag_s[0] == 1)
    def _():
        body(6, do1=False, do2=False)

    @pl.when(flag_s[0] == 1)
    def _():
        _weave(([(lambda n=n: run(s4_gen(7, n, (0,))), 1.0) for n in range(NV)], 0.0, 1.0), (s5(6), 0.0, 1.0))

    @pl.when(flag_s[0] == 1)
    def _():
        _weave(([(lambda n=n: run(s4_gen(7, n, (4,))), 1.0) for n in range(NV)], 0.0, 1.0), (s5(7)[:8], 0.0, 1.0))

    _weave((s5(7)[8:], 0.0, 1.0))

    def total(i):
        halves = []
        for hf in range(2):
            t = acc_v[i, pl.ds(64 * hf, 8, stride=8), :]
            for s in range(1, 8):
                t = t + acc_v[i, pl.ds(64 * hf + s, 8, stride=8), :]
            halves.append(t)
        return jnp.concatenate(halves, 0)

    m2 = total(0) * (1.0 / D)
    var2 = jnp.maximum(total(1) * (1.0 / D) - m2 * m2, 0.0)
    sd2 = _rb(jnp.sqrt(_rb(_rb(var2) + EPS)))
    rs2 = 1.0 / sd2
    r = _rb((total(2) - m2 * wr_sum) * rs2)
    mean2 = fin_v[4] + m2
    fin_v[0] = rs2
    fin_v[1] = m2 * rs2
    fin_v[2] = rs2 + 1.0
    fin_v[3] = fin_v[4] - m2 * rs2

    tl = _iota((16, 128), 0)
    ll = _iota((16, 128), 1)
    lodd = (ll & 1) == 1
    toff = jnp.where((tl & 1) == 0, jnp.where(lodd, ll + 127, ll), jnp.where(lodd, ll + 128, (ll - 1) & 127))
    tok = (tl >> 1) * 256 + toff
    rbits = pltpu.bitcast(r, i32)
    srt = rbits ^ ((rbits >> 31) & 0x7FFFFFFF)
    key = pltpu.bitcast((((srt >> 16) + 32768) << 11) + (2047 - tok) + (1 << 28), f32)
    kk = key
    cand = []
    for _ in range(4):
        rm = jnp.broadcast_to(jnp.max(kk, axis=1, keepdims=True), (16, 128))
        cand.append(rm)
        kk = jnp.where(kk == rm, 0.0, kk)
    last = jnp.max(cand[3], axis=0, keepdims=True)
    kcol = None
    for j in range(TOPC):
        mx = jnp.max(cand[0], axis=0, keepdims=True)
        kcol = jnp.broadcast_to(mx, (8, 128)) if j == 0 else jnp.where(sub8 == j, mx, kcol)
        took = cand[0] == mx
        cand = [jnp.where(took, cand[i + 1] if i < 3 else 0.0, cand[i]) for i in range(4)]
    kc_v[...] = kcol

    @pl.when((last - mx)[0, 0] > 0.0)
    def _():
        k2 = key
        kc = None
        for j in range(TOPC):
            m1 = jnp.max(jnp.max(k2, axis=0, keepdims=True), axis=1, keepdims=True)
            kc = jnp.broadcast_to(m1, (8, 128)) if j == 0 else jnp.where(sub8 == j, m1, kc)
            k2 = jnp.where(k2 == m1, 0.0, k2)
        kc_v[...] = kc

    kcol = kc_v[...]
    kint = pltpu.bitcast(kcol, i32) - (1 << 28)
    tcol = 2047 - (kint & 2047)
    s16 = (kint >> 11) - 32768
    rsel = pltpu.bitcast((s16 ^ ((s16 >> 31) & 0x7FFF)) << 16, f32)
    gate = _rb(jax.nn.sigmoid(rsel))[:, 0:1]

    def classes(col):
        cls = jnp.zeros((8, 128), i32)
        for d in range(1, TOPC):
            cls = cls + jnp.where((col == pltpu.roll(col, d, 0)) & (sub8 >= d), 1, 0)
        return cls, jnp.max(cls, axis=0, keepdims=True)[0, 0] + 1

    wcol = tcol & 255
    pcol = jnp.where((wcol & 1) == 0, jnp.where(wcol < 128, wcol, wcol - 127),
                     jnp.where(wcol < 128, (wcol + 1) & 127, wcol - 128))
    ecol = ((tcol >> 8) << 1) | (tcol & 1)
    etile = [ecol[j, 0] for j in range(TOPC)]
    gcol, gn = classes(pcol)
    xs_v[...] = jnp.zeros((8, D), f32)

    def gather(c, carry):
        oh = (gcol == c) & (lane8 == pcol)
        ohi = jnp.where(oh, 1, 0)
        msk = [jnp.broadcast_to(ohi[j:j + 1], (8, 128)) == 1 for j in range(TOPC)]
        sa = sb = None
        for j in range(TOPC):
            fa = jnp.broadcast_to(fin_v[0, pl.ds(etile[j], 1), :], (8, 128))
            fb = jnp.broadcast_to(fin_v[1, pl.ds(etile[j], 1), :], (8, 128))
            sa, sb = (fa, fb) if j == 0 else (jnp.where(msk[j], fa, sa), jnp.where(msk[j], fb, sb))
        parts = []
        for q in range(D // 8 // GCH):
            mg = None
            for j in range(TOPC):
                cc = c1_v[GCH * q:GCH * q + GCH, etile[j] >> 1, pl.ds(pl.multiple_of(8 * (etile[j] & 1), 8), 8), :]
                mg = cc if j == 0 else jnp.where(msk[j], cc, mg)
            parts.append(mg * sa - sb)
        ln = jnp.concatenate(parts, 0).reshape(D, 128)
        xs_v[...] = xs_v[...] + _dot_nt(jnp.where(oh, 1.0, 0.0).astype(f32), ln)
        return carry

    lax.fori_loop(0, gn, gather, 0)
    xsel = xs_v[...]

    def rebuilt_rows():
        sdc = jnp.zeros((8, 1), f32)
        mc = jnp.zeros((8, 1), f32)
        sub1 = _iota((8, 1), 0)
        for j in range(TOPC):
            hitm = tok == jnp.broadcast_to(tcol[j:j + 1], (16, 128))
            red = lambda v: jnp.sum(jnp.sum(jnp.where(hitm, v, 0.0), axis=0, keepdims=True), axis=1, keepdims=True)
            sdc = jnp.where(sub1 == j, red(sd2), sdc)
            mc = jnp.where(sub1 == j, red(mean2), mc)
        return xsel * (sdc + 1.0) + mc

    def outp(b, g0, g1):
        sc = [jnp.where(top, jnp.broadcast_to(fin_v[i, 2 * b:2 * b + 1, :], (8, 128)),
                        jnp.broadcast_to(fin_v[i, 2 * b + 1:2 * b + 2, :], (8, 128))) for i in (2, 3)]
        for g in range(g0, g1):
            a = _rb(c1_v[g, b, pl.ds(0, 8, stride=2), :] * sc[0] + sc[1])
            c = _rb(c1_v[g, b, pl.ds(1, 8, stride=2), :] * sc[0] + sc[1])
            w = (pltpu.bitcast(a, u32) >> 16) | pltpu.bitcast(c, u32)
            out_w[g, b] = jnp.where(mask2, w, pltpu.roll(pltpu.roll(w, 4, 0), 127, 1))

    opieces = [functools.partial(outp, b, 24 * i, 24 * i + 24) for b in range(NB) for i in range(3)]

    tilec = tcol >> 7
    aux = {}

    def late_scalars():
        aux["tiles"] = [tilec[j, 0] for j in range(TOPC)]
        hit = 0
        for j in range(TOPC):
            hit = hit | (1 << aux["tiles"][j])
        aux["hit"] = hit
        bs_v[...] = rebuilt_rows()
        clscol, aux["ncls"] = classes(tcol & 127)
        aux["clscol"] = clscol
        aux["cls"] = [clscol[j, 0] for j in range(TOPC)]

    def ocopy(t):
        if isinstance(t, int):
            idx = (slice(None), t // 2, pl.ds(8 * (t % 2), 8), slice(None))
        else:
            idx = (slice(None), t >> 1, pl.ds(pl.multiple_of(8 * (t & 1), 8), 8), slice(None))
        return cp(out_v.at[idx], out_h.at[idx], osem.at[0])

    osplit = OSPLIT
    for c in range(NCH):
        for cc in c_w[c]:
            cc.wait()
        if c == WSTART:
            for t in range(16):
                @pl.when(((aux["hit"] >> t) & 1) == 0)
                def _():
                    ocopy(t).start()
        sl = slice(FOFF[c], FOFF[c] + FCH[c])
        mine = opieces[osplit[c]:osplit[c + 1]]
        g = _rb(_dot(xsel, wg_v[:, sl]))
        up = _rb(_dot(xsel, wu_v[:, sl]))
        if c == 0:
            late_scalars()
        for fn in mine[:len(mine) // 2]:
            fn()
        act = _rb(_rb(g * jax.nn.sigmoid(g)) * up)
        yc = _dot_nt(act, wd_v[:, sl])
        y_v[...] = yc if c == 0 else y_v[...] + yc
        for fn in mine[len(mine) // 2:]:
            fn()
    newrow = _rb(bs_v[...] + _rb(_rb(y_v[...]) * gate))

    tiles, cls, ncls, clscol = aux["tiles"], aux["cls"], aux["ncls"], aux["clscol"]
    lanec = tcol & 127

    def place(c, carry):
        oh = jnp.where((clscol == c) & (lane8 == (tcol & 127)), 1.0, 0.0).astype(f32)
        u_v[c] = lax.dot_general(newrow, oh, (((0,), (0,)), ((), ())),
                                 preferred_element_type=f32).reshape(D // 8, 8, 128)
        return carry

    lax.fori_loop(0, ncls, place, 0)
    for j in range(TOPC):
        idx = (slice(None), tiles[j] >> 1, pl.ds(pl.multiple_of(8 * (tiles[j] & 1), 8), 8), slice(None))
        cur = out_v[idx].astype(f32)
        out_v[idx] = jnp.where(lane8 == jnp.broadcast_to(lanec[j:j + 1], (8, 128)), u_v[cls[j]], cur).astype(bf16)
        later = False
        for j2 in range(j + 1, TOPC):
            later = jnp.logical_or(later, tiles[j2] == tiles[j])

        @pl.when(jnp.logical_not(later))
        def _():
            ocopy(tiles[j]).start()

    for t in range(16):
        ocopy(t).wait()


@jax.jit
def pallas_sequential_preLN__ssm_conv_s4__moe_arch_mod__prompt_kernel(
    A_u: jax.Array,
    A_A_re: jax.Array,
    A_A_im: jax.Array,
    A_B_re: jax.Array,
    A_B_im: jax.Array,
    A_C_re: jax.Array,
    A_C_im: jax.Array,
    A_log_dt: jax.Array,
    A_Dskip: jax.Array,
    B_x: jax.Array,
    B_w_r: jax.Array,
    B_w_gate: jax.Array,
    B_w_up: jax.Array,
    B_w_down: jax.Array,
):
    hbm = pl.BlockSpec(memory_space=pltpu.MemorySpace.HBM)
    vm = pltpu.VMEM
    G8 = D // 8
    scratch = [
        vm((G8, NB, 16, 128), bf16), vm((6, D, N), bf16), vm((D,), bf16), vm((D,), bf16), vm((D,), bf16),
        vm(_CTAB.shape, f32), vm((D, F), bf16), vm((D, F), bf16), vm((D, F), bf16), vm((G8, NB, 16, 128), bf16),
        vm((10, 4, 128, 128), bf16), vm((2, 2, 2, 128, 128), bf16), vm((3, D, 128), f32),
        vm((NV, 2, 128, 128), f32), vm((NSTEP, NV, 56, 128), f32), vm((NSTEP, R, 128), f32),
        vm((NSTEP, NB, 6, R, 128), f32), vm((NSTEP, NB, 6, R, 128), f32),
        vm((NSTEP, NB, 2, R, 256), f32), vm((G8, NB, 16, 128), f32), vm((2, 16, 8, 128), f32),
        vm((3, 128, 128), f32), vm((5, 16, 128), f32), vm((TOPC, G8, 8, 128), f32),
        vm((R, 512), f32), vm((8, D), f32), vm((NV, 4, 8, 128), f32),
        vm((8, 128), f32), vm((8, D), f32), vm((8, D), f32), pltpu.SMEM((1,), i32),
        pltpu.SemaphoreType.DMA((5 + NCH,)), pltpu.SemaphoreType.DMA((1,)),
    ]
    xv = A_u[0].T.reshape(G8, 8, 16, 128).transpose(0, 2, 1, 3).reshape(G8, NB, 16, 128)
    out = pl.pallas_call(
        _kernel,
        out_shape=jax.ShapeDtypeStruct((G8, NB, 16, 128), bf16),
        in_specs=[hbm] * 14,
        out_specs=hbm,
        scratch_shapes=scratch,
        compiler_params=pltpu.CompilerParams(vmem_limit_bytes=120 * 1024 * 1024),
    )(xv, A_A_re, A_A_im, A_B_re, A_B_im, A_C_re, A_C_im, A_log_dt, A_Dskip, B_w_r,
      B_w_gate, B_w_up, B_w_down.T, jnp.asarray(_CTAB))
    return out.reshape(G8, 16, 8, 128).transpose(0, 2, 1, 3).reshape(D, L).T[None]
```

```python
import functools

import numpy as np
import jax
import jax.numpy as jnp
from jax import lax
import jax.experimental.pallas as pl
import jax.experimental.pallas.tpu as pltpu

f32 = jnp.float32
bf16 = jnp.bfloat16
i32 = jnp.int32
u32 = jnp.uint32

L, D, N, F, TOPC = 2048, 576, 128, 4608, 8
NB = 8
NV = 9
R = NV * 8
NSTEP = D // R
EPS = 1e-5

_XL1 = [(1, 5), (2, 6), (3, 7), (4, 8), (258, 516), (260, 520), (262, 772), (264, 776),
        (1288, 1032), (1800, 1544)]
_XSH = [0, 1, 2, 3, 0, 1, 2, 3, 0, 1]


def _bf16_round_int(j):
    u = np.asarray(j, np.float32).view(np.uint32).astype(np.uint64)
    r = ((u + 0x7FFF + ((u >> 16) & 1)) >> 16) << 16
    return r.astype(np.uint32).view(np.float32).astype(np.int64)


def _chunk_values():
    vals = -np.ones((5, 128), np.int64)
    for j in range(10):
        for p in range(2):
            ch = (j // 4) * 2 + p if j < 8 else 4
            extra = 2 * p if j >= 8 else 0
            for l0 in range(32):
                vals[ch, (4 * (31 - l0) + 4 * p + _XSH[j] + extra + 8) % 128] = _XL1[j][p] + 8 * l0
    assert (vals >= 0).all()
    return vals


def _tables():
    cv = _chunk_values()
    om = np.pi * (2 * np.arange(128) + 1) / 512.0
    sig = (-1.0) ** np.arange(128)
    cvp = {"A0": cv[0], "A1": cv[1], "B": cv[2], "C": cv[3], "D": cv[4]}
    cvp["Cp"] = cv[3].copy(); cvp["Cp"][11] = cv[2][11]
    cvp["Dp"] = cv[4].copy(); cvp["Dp"][15] = cv[3][15]
    passes = [(0, "A0"), (0, "A1"), (1, "A1"), (1, "B"), (2, "Cp"), (3, "C"), (4, "Dp"),
              (5, "D"), (6, "D"), (7, "D")]
    G = np.zeros((10, 128, 4, 128))
    for b in range(NB):
        mine = [i for i, (pb, _) in enumerate(passes) if pb == b]
        for j in range(1, 257):
            lag = 256 * b + j
            if lag > L - 1:
                continue
            v = int(_bf16_round_int(lag))
            hit = [(i, int(np.nonzero(cvp[passes[i][1]] == v)[0][0])) for i in mine
                   if (cvp[passes[i][1]] == v).any()]
            assert len(hit) == 1, (b, j, v, hit)
            i, l = hit[0]
            e = np.exp(-1j * om * j) * sig ** b / 256.0
            s = (-1.0) ** j
            G[i, l, 0] += e.real; G[i, l, 1] += e.imag
            G[i, l, 2] += s * e.real; G[i, l, 3] += s * e.imag
    e8 = np.exp(-1j * np.outer(8 * np.arange(32), om))
    sets = {"A0": [0], "A1": [1], "B": [3], "C": [4, 5], "D": [6, 7, 8, 9]}
    seeds, masks = {}, {}
    for name, ps in sets.items():
        seeds[name] = sum(G[i, 16:24] for i in ps)
        for i in ps:
            masks[i] = [int(x) for x in (np.abs(G[i, 16:24]).sum((1, 2)) > 0)]
            for v in range(2, 17):
                sd = seeds[name]
                r0 = 8 * (v % 16)
                for q in (0, 2):
                    z = (sd[:, q] + 1j * sd[:, q + 1]) * np.conj(e8[2 * (v - 2)]) * np.array(masks[i])[:, None]
                    assert np.allclose(z.real, G[i, r0:r0 + 8, q], atol=1e-12)
                    assert np.allclose(z.imag, G[i, r0:r0 + 8, q + 1], atol=1e-12)
    assert not G[2, 16:].any() and not G[2, :8].any()
    s8 = np.arange(8)
    je = np.where(s8 % 2 == 0, s8, 127 + s8)
    jo = np.where(s8 % 2 == 0, s8 - 1, 128 + s8)
    fe = np.exp(-1j * np.outer(je, om)); ft = np.exp(-1j * np.outer(jo, om))
    ft0 = np.exp(-1j * np.outer(jo % 128 + 128 * (s8 % 2), om))
    rows = [e8.real, e8.imag]
    for name in ("A0", "A1", "B", "C", "D"):
        rows += [seeds[name][:, q] for q in range(4)]
    for i in range(10):
        rows += [G[i, 8:16, q] for q in range(4)]
    rows += [fe.real, fe.imag, ft.real, ft.imag, ft0.real, ft0.imag]
    return np.concatenate(rows, 0).astype(np.float32), masks


_CTAB, _GMASK = _tables()


def _sincos_coeffs():
    r = np.cos(np.pi * (np.arange(4000) + .5) / 4000) * 0.5
    z = r * r
    s = np.linalg.lstsq(np.stack([z ** k for k in range(4)], 1), np.sin(np.pi / 2 * r) / r, rcond=None)[0]
    c = np.linalg.lstsq(np.stack([z ** k for k in range(1, 5)], 1), np.cos(np.pi / 2 * r) - 1, rcond=None)[0]
    return [float(x) for x in s], [float(x) for x in c]


_SC, _CC = _sincos_coeffs()


def _cmul(a, b):
    return (a[0] * b[0] - a[1] * b[1], a[0] * b[1] + a[1] * b[0])


def _cmulc(a, b):
    return (a[0] * b[0] + a[1] * b[1], a[1] * b[0] - a[0] * b[1])


def _csq(a):
    return ((a[0] - a[1]) * (a[0] + a[1]), (a[0] + a[0]) * a[1])


def _sincos(th):
    z = th * (2.0 / np.pi)
    k = jnp.round(z)
    r = z - k
    r2 = r * r
    s = r * (_SC[0] + r2 * (_SC[1] + r2 * (_SC[2] + r2 * _SC[3])))
    c = 1.0 + r2 * (_CC[0] + r2 * (_CC[1] + r2 * (_CC[2] + r2 * _CC[3])))
    ki = k.astype(i32)
    swap = (ki & 1) == 1
    s2 = jnp.where(swap, c, s)
    c2 = jnp.where(swap, s, c)
    s2 = pltpu.bitcast(pltpu.bitcast(s2, i32) ^ ((ki & 2) << 30), f32)
    c2 = pltpu.bitcast(pltpu.bitcast(c2, i32) ^ (((ki + 1) & 2) << 30), f32)
    return s2, c2


def _rb(x):
    return x.astype(bf16).astype(f32)


def _dot(a, b):
    return jnp.dot(a, b, preferred_element_type=f32)


def _dot_nt(a, b):
    return lax.dot_general(a, b, (((1,), (1,)), ((), ())), preferred_element_type=f32)


def _iota(shape, dim):
    return lax.broadcasted_iota(i32, shape, dim)


S4MODE='LC'
TILE=4
YSPLIT=1
ZT=1
ORDER='44443ab24pn45'
NPC=3
P3F=(0.9,0.4,0.55,0.3)
GCH=3
FSUB=1536
FCH=(4608,)
OSPLIT=[0,24]
PART=(256,192,128)
DSPL=(0,1536,2304)
NOBC=True
NCH = len(FCH)
FOFF = [sum(FCH[:i]) for i in range(NCH)]
POFF = [sum(PART[:i]) for i in range(len(PART))]

def _weave(*streams):
    items = []
    for si, (pieces, lo, hi) in enumerate(streams):
        tot = float(sum(c for _, c in pieces))
        cum = 0.0
        for pi, (fn, c) in enumerate(pieces):
            items.append((lo + max(hi - lo, 0.0) * (cum + 0.5 * c) / tot, si, pi, fn))
            cum += c
    for _, _, _, fn in sorted(items, key=lambda t: t[:3]):
        fn()


def _kernel(x_h, are_h, aim_h, bre_h, bim_h, cre_h, cim_h, ldt_h, dsk_h, wr_h, wg_h, wu_h, wd_h, ct_h,
            out_h,
            x_v, par_v, ldt_v, dsk_v, wr_v, ct_v, wg_v, wu_v, wd_v, out_v,
            g_v, f_v, col_v, st_v, kd_v, k0_v, kh_v, uh_v, zs_v, c1_v, s1_v, acc_v, fin_v, u_v, zt_v, y_v, pv_v, kc_v, xs_v, bs_v, act_v, flag_s,
            sem, osem):
    cp = pltpu.make_async_copy
    c_ct = cp(ct_h, ct_v, sem.at[0])
    c_vec = [cp(ldt_h, ldt_v, sem.at[1]), cp(dsk_h, dsk_v, sem.at[1]), cp(wr_h, wr_v, sem.at[1])]
    PH = 4 * R
    par_h = (are_h, aim_h, bre_h, bim_h, cre_h, cim_h)
    c_par = [cp(h.at[pl.ds(0, PH)], par_v.at[i, pl.ds(0, PH)], sem.at[2]) for i, h in enumerate(par_h)]
    c_par2 = [cp(h.at[pl.ds(PH, D - PH)], par_v.at[i, pl.ds(PH, D - PH)], sem.at[3])
              for i, h in enumerate(par_h)]
    c_x = cp(x_h, x_v, sem.at[4])
    def wcp(h, v, rp, ct, s):
        return [cp(h.at[rp, hf, ct], v.at[rp, ct, pl.ds(8 * hf, 8), :], s) for hf in range(2)]

    c_w = [wcp(wg_h, wg_v, slice(None), pl.ds(FOFF[c] // 128, FCH[c] // 128), sem.at[5 + c])
           + wcp(wu_h, wu_v, slice(None), pl.ds(FOFF[c] // 128, FCH[c] // 128), sem.at[5 + c]) for c in range(NCH)]
    c_d = [wcp(wd_h, wd_v, pl.ds(POFF[p] // 16, PART[p] // 16), slice(None), sem.at[5 + NCH + p])
           for p in range(len(PART))]
    for c in c_vec + [c_ct] + c_par + [c_x] + c_par2 + sum(c_w, []) + sum(c_d, []):
        c.start()

    flag_s[0] = 1
    x_w = x_v.bitcast(u32)
    wg_w, wu_w, wd_w = wg_v.bitcast(u32), wu_v.bitcast(u32), wd_v.bitcast(u32)

    def wmat(w, r0, nr, c0, nc):
        return jnp.concatenate([pltpu.bitcast(w[r0 // 16:(r0 + nr) // 16, t], bf16).reshape(nr, 128)
                                for t in range(c0 // 128, (c0 + nc) // 128)], 1)

    out_w = out_v.bitcast(u32)
    g_w = g_v.bitcast(u32)
    f_w = f_v.bitcast(u32)
    sub8 = _iota((8, 128), 0)
    lane8 = _iota((8, 128), 1)

    acc_v[...] = jnp.zeros(acc_v.shape, f32)
    for n in range(NV):
        for ri in range(2):
            st_v[n, ri, 104:112, :] = jnp.full((8, 128), 1.0 - ri, f32)
    for c in c_vec:
        c.wait()

    rows = [_rb(jnp.exp(ldt_v[...].astype(f32).reshape(1, D))),
            dsk_v[...].astype(f32).reshape(1, D),
            wr_v[...].astype(f32).reshape(1, D)]
    wr_sum = jnp.sum(rows[2], axis=1, keepdims=True)
    ones = jnp.ones((128, 128), f32)
    for j in range(5):
        w = 128 if j < 4 else 64
        eye = _iota((w, w), 0) == _iota((w, w), 1)
        m = jnp.concatenate([jnp.where(eye, jnp.broadcast_to(rows[i][:, j * 128:j * 128 + w], (w, w)), 0.0)
                             for i in range(3)], 0)
        res = _dot(m, ones[:w, :])
        for i in range(3):
            col_v[i, j * 128:j * 128 + w, :] = res[i * w:(i + 1) * w]

    c_ct.wait()

    def e8(v):
        return (jnp.broadcast_to(ct_v[v:v + 1, :], (8, 128)), jnp.broadcast_to(ct_v[32 + v:33 + v, :], (8, 128)))

    sets = {"A0": [0], "A1": [1], "B": [3], "C": [4, 5], "D": [6, 7, 8, 9]}
    for i in (0, 1, 3, 4, 5, 6, 7, 8, 9):
        for q in range(4):
            g_v[i, q, 8:16, :] = ct_v[224 + 32 * i + 8 * q:232 + 32 * i + 8 * q, :].astype(bf16)
    for si, (name, ps) in enumerate(sets.items()):
        sd = [ct_v[64 + 32 * si + 8 * q:72 + 32 * si + 8 * q, :] for q in range(4)]
        mk = {}
        for i in ps:
            if len(ps) > 1:
                bits = sum(b << s for s, b in enumerate(_GMASK[i]))
                mk[i] = ((bits >> sub8) & 1) == 1
        for v in range(2, 17):
            if v == 2:
                vals = sd
            else:
                ev = e8(2 * (v - 2))
                vals = list(_cmulc((sd[0], sd[1]), ev)) + list(_cmulc((sd[2], sd[3]), ev))
            for i in ps:
                for q in range(4):
                    val = vals[q] if len(ps) == 1 else jnp.where(mk[i], vals[q], 0.0)
                    g_v[i, q, 8 * (v % 16):8 * (v % 16) + 8, :] = val.astype(bf16)
    sig = jnp.where((lane8 & 1) == 0, 1.0, -1.0).astype(f32)
    for h in range(2):
        sd = (ct_v[544 + 16 * h:552 + 16 * h, :], ct_v[552 + 16 * h:560 + 16 * h, :])
        for v in range(16):
            if v == 0:
                vals = sd if h == 0 else (ct_v[576:584, :], ct_v[584:592, :])
            else:
                vals = _cmul(sd, e8(v))
            for q in range(2):
                f_v[0, h, q, 8 * v:8 * v + 8, :] = vals[q].astype(bf16)
                f_v[1, h, q, 8 * v:8 * v + 8, :] = (vals[q] * sig).astype(bf16)

    def gmat(i):
        return jnp.concatenate([pltpu.bitcast(g_w[i, q, 0:64, :], bf16) for q in range(4)], 1)

    def fmat(ver, h):
        return jnp.concatenate([pltpu.bitcast(f_w[ver, h, q, 0:64, :], bf16) for q in range(2)], 1)

    revmask = (sub8 & 2) == 0
    lm = lane8 & 3

    def s1_nat(k, n0, nn):
        row0 = pl.multiple_of(k * R + 8 * n0, 8)
        rr = 8 * nn
        ld = lambda i: par_v[i, pl.ds(row0, rr), :].astype(f32)
        dt = col_v[0, pl.ds(row0, rr), :]
        e = jnp.exp(dt * ld(0))
        s, c = _sincos(dt * ld(1))
        a1 = (e * c, e * s)
        w = _cmul((ld(4), ld(5)), (dt * ld(2), dt * ld(3)))
        k0_v[k, 8 * n0:8 * n0 + rr, :] = (jnp.sum(w[0], axis=1, keepdims=True)
                                          + col_v[1, pl.ds(row0, rr), :]) * (1.0 / 256.0)
        w = (w[0], -w[1])
        rev = lambda v: jnp.where(revmask, pltpu.roll(v, 2, 0), pltpu.roll(v, 6, 0))

        def put(arr, slots, fn=None):
            for n in range(nn):
                for ri in range(2):
                    v = arr[ri][8 * n:8 * n + 8]
                    if fn is not None:
                        v = fn(v)
                    for q in slots:
                        st_v[n0 + n, ri, q * 8:q * 8 + 8, :] = v

        put(w, (0, 1)); put(a1, (2, 3))
        a2 = _csq(a1); put(a2, (5,))
        a4 = _csq(a2); put(a4, (6,))
        put(_cmul(a4, a1), (4,))
        a8 = _csq(a4); put(a8, (12,), rev)
        t = _csq(a8); put(t, (14, 15), rev)
        for _ in range(4):
            t = _csq(t)
        put(t, (7, 11))
        t = _csq(t); put(t, (8, 9))
        put(_csq(t), (10,))

    def s1_grp(k, n):
        mix = lambda q: tuple(jnp.concatenate([st_v[n, ri, pl.ds(q * 8 + g, 8, stride=2), :] for g in range(2)], 0)
                              for ri in range(2))
        y = [mix(12)]
        a16d = mix(14)
        if YSPLIT == 1:
            for _ in range(15):
                y.append(_cmul(y[-1], a16d))
        else:
            y.append(_cmul(y[0], a16d))
            a32d = _csq(a16d)
            for i in range(2, 16):
                y.append(_cmul(y[i - 2], a32d))
        yield
        wd = mix(0); a1d = mix(2); m1 = mix(5)
        v = [_cmulc(wd, mix(3))]
        for _ in range(3):
            v.append(_cmulc(v[-1], a1d))
        v4 = _cmulc(_cmulc(wd, m1), mix(7))
        v5 = _cmulc(v4, m1); v6 = _cmulc(v4, mix(6)); v7 = _cmulc(v6, m1)
        v8 = _cmulc(v7, mix(10)); v9 = _cmulc(v8, mix(8))
        v += [v4, v5, v6, v7, v8, v9]
        os_ = []
        for g in range(2):
            cat = lambda ts: jnp.concatenate([jnp.concatenate([t[ri][8 * g:8 * g + 8] for t in ts], 0)
                                              for ri in range(2)], 1)
            os_.append(_dot_nt(cat(v), cat(y[::-1])))
        yield
        for g in range(2):
            o = os_[g]
            ro = [pltpu.roll(o[8 * j:8 * j + 8], _XSH[j] + 5, 1, stride=1, stride_axis=0) for j in range(10)]
            sel4 = lambda q: jnp.where(lm == 0, q[0], jnp.where(lm == 1, q[1], jnp.where(lm == 2, q[2], q[3])))
            kd_v[k, n, pl.ds(g, 8, stride=2), :] = sel4(ro[0:4])
            kd_v[k, n, pl.ds(16 + g, 8, stride=2), :] = sel4(ro[4:8])
            kd_v[k, n, pl.ds(32 + g, 8, stride=2), :] = jnp.where(lm == 0, ro[8], ro[9])

    def run(gen):
        for _ in gen:
            pass

    s1n = lambda k: [(functools.partial(s1_nat, k, 3 * i, 3), 1.0) for i in range(3)]
    s1g = lambda k: [(lambda n=n: run(s1_grp(k, n)), 1.0) for n in range(NV)]

    laneR = _iota((R, 128), 1)
    lmR = laneR & 3

    def s2_gen(k):
        ch = lambda c: kd_v[k, :, 8 * c:8 * c + 8, :].reshape(R, 128)
        for b in range(NB):
            if b == 0:
                z = _dot(ch(0), gmat(0)) if ZT else None
                dd = jnp.where(lmR < 2, ch(4), pltpu.roll(ch(5), 2, 1))
                kd_v[k, :, 48:56, :] = dd.reshape(NV, 8, 128)
                if ZT:
                    zt_v[...] = z
                    yield
                    z = _dot(ch(1), gmat(1)) + zt_v[...]
                else:
                    z = _dot(jnp.concatenate([ch(0), ch(1)], 1), jnp.concatenate([gmat(0), gmat(1)], 0))
            elif b == 1:
                k256 = jnp.sum(jnp.where(laneR == 15, ch(1), 0.0), axis=1, keepdims=True)
                pat = jnp.concatenate([ct_v[288 + 8 * q + 7:288 + 8 * q + 8, :] for q in range(4)], 1)
                z = _dot(ch(2), gmat(3)) + k256 * pat
            elif b == 2:
                z = _dot(jnp.where(laneR == 11, ch(2), ch(3)), gmat(4))
            elif b == 3:
                z = _dot(ch(3), gmat(5))
            elif b == 4:
                z = _dot(jnp.where(laneR == 15, ch(3), ch(6)), gmat(6))
            else:
                z = _dot(ch(6), gmat(b + 2))
            for s in range(2):
                kr = z[:, 256 * s:256 * s + 128]
                ki = z[:, 256 * s + 128:256 * s + 256]
                if b == 0:
                    kr = kr + k0_v[k]
                kh_v[k, b, 3 * s] = kr
                if S4MODE[0] == "L":
                    kh_v[k, b, 3 * s + 1] = kr + ki
                    kh_v[k, b, 3 * s + 2] = ki - kr
                else:
                    kh_v[k, b, 3 * s + 1] = ki
            yield

    def s2(k):
        gen = s2_gen(k)
        return [(lambda: next(gen, None), 1.0) for _ in range(9)]

    mask2 = (sub8 < 4) == ((lane8 & 1) == 0)
    top = sub8 < 4

    def ln1_pieces(b, npc):
        state = {}
        per = (D // 8) // npc

        def piece(i):
            for g in range(i * per, (i + 1) * per):
                m = x_w[g, b]
                eo = jnp.where(mask2, m, pltpu.roll(pltpu.roll(m, 4, 0), 1, 1))
                a = pltpu.bitcast(eo << 16, f32)
                c = pltpu.bitcast(eo & jnp.uint32(0xFFFF0000), f32)
                if g == 0:
                    state["sh"] = jnp.where(top, jnp.broadcast_to(a[0:1], (8, 128)),
                                            jnp.broadcast_to(a[4:5], (8, 128)))
                a = a - state["sh"]
                c = c - state["sh"]
                c1_v[g, pl.ds(16 * b, 8, stride=2), :] = a
                c1_v[g, pl.ds(16 * b + 1, 8, stride=2), :] = c
                new = [a, c, a * a, c * c]
                state["acc"] = new if g == 0 else [p + q for p, q in zip(state["acc"], new)]
            if i == npc - 1:
                acc = state["acc"]
                s1, s2_ = acc[0] + acc[1], acc[2] + acc[3]
                for h in range(2):
                    m = jnp.sum(s1[4 * h:4 * h + 4], axis=0, keepdims=True) * (1.0 / D)
                    var = jnp.sum(s2_[4 * h:4 * h + 4], axis=0, keepdims=True) * (1.0 / D) - m * m
                    rs = 1.0 / _rb(jnp.sqrt(_rb(_rb(jnp.maximum(var, 0.0)) + EPS)))
                    s1_v[0, 2 * b + h] = jnp.broadcast_to(rs, (8, 128))
                    s1_v[1, 2 * b + h] = jnp.broadcast_to(m * rs, (8, 128))
                    fin_v[4, 2 * b + h:2 * b + h + 1, :] = state["sh"][4 * h:4 * h + 1]

        return [(functools.partial(piece, i), 1.0) for i in range(npc)]

    def s3_blk(k, b):
        g0 = k * NV
        et = []
        for h in range(2):
            c = c1_v[pl.ds(g0, NV), 16 * b + 8 * h:16 * b + 8 * h + 8, :]
            u = (c * s1_v[0, 2 * b + h] - s1_v[1, 2 * b + h]).reshape(R, 128)
            et.append(_dot(u, fmat(b % 2, h)))
        er, ei, tr, ti = et[0][:, :128], et[0][:, 128:], et[1][:, :128], et[1][:, 128:]
        if S4MODE[1] == "C":
            for q, v in enumerate((er, ei, tr, ti)):
                uh_v[k, b, q] = v
        else:
            for s, (pr, pi) in enumerate(((er + tr, ei + ti), (er - tr, ei - ti))):
                uh_v[k, b, 3 * s] = pr + pi
                uh_v[k, b, 3 * s + 1] = pi
                uh_v[k, b, 3 * s + 2] = pr

    s3 = lambda k: [(functools.partial(s3_blk, k, b), 1.0) for b in range(NB)]

    def s4_gen(k, n, groups=None):
        sl = slice(8 * n, 8 * n + 8)

        def utrip(i, s):
            if S4MODE[1] == "L":
                return [uh_v[k, i, 3 * s + q, sl, :] for q in range(3)]
            er, ei, tr, ti = [uh_v[k, i, q, sl, :] for q in range(4)]
            pr, pi = (er + tr, ei + ti) if s == 0 else (er - tr, ei - ti)
            return [pr + pi, pi, pr]

        prev = None
        done = 0
        if groups is not None and groups[0] > 0:
            prev = [(pv_v[n, 2 * h], pv_v[n, 2 * h + 1]) for h in range(2)]
        for b0 in (range(0, NB, TILE) if groups is None else groups):
            yy = []
            for s in range(2):
                acc = [None] * TILE
                win = {}
                for j in range(b0 + TILE):
                    if S4MODE[0] == "L":
                        kk = [kh_v[k, j, 3 * s + q, sl, :] for q in range(3)]
                    else:
                        kr, ki = kh_v[k, j, 3 * s, sl, :], kh_v[k, j, 3 * s + 1, sl, :]
                        kk = [kr, kr + ki, ki - kr]
                    for o in range(TILE - 1, -1, -1):
                        i = b0 + o - j
                        if i < 0:
                            continue
                        if i not in win:
                            win[i] = utrip(i, s)
                        p = [kk[q] * win[i][q] for q in range(3)]
                        acc[o] = p if acc[o] is None else [a + c for a, c in zip(acc[o], p)]
                        done += 1
                    if TILE == 4 and b0 == 4 and j == 2:
                        yield done
                yy.append([(a[0] - a[1], a[0] + a[2]) for a in acc])
                if s == 0:
                    yield done
            for o in range(TILE):
                p, q = yy[0][o], yy[1][o]
                cur = [(p[0] + q[0], p[1] + q[1]), (p[0] - q[0], p[1] - q[1])]
                for h in range(2):
                    if b0 + o == 0:
                        zr, zi = cur[h]
                    else:
                        zr = cur[h][0] - prev[h][1]
                        zi = cur[h][1] + prev[h][0]
                    zs_v[k, b0 + o, h, sl, 0:128] = zr
                    zs_v[k, b0 + o, h, sl, 128:256] = zi
                prev = cur
            if groups is not None and b0 + TILE < NB:
                for h in range(2):
                    pv_v[n, 2 * h] = prev[h][0]
                    pv_v[n, 2 * h + 1] = prev[h][1]
            yield done

    def s5_blk(k, b, h):
        g0 = k * NV
        t = 2 * b + h
        y = _dot_nt(zs_v[k, b, h], fmat(b % 2, h)).reshape(NV, 8, 128)
        hh = c1_v[pl.ds(g0, NV), 16 * b + 8 * h:16 * b + 8 * h + 8, :] + y
        c1_v[pl.ds(g0, NV), 16 * b + 8 * h:16 * b + 8 * h + 8, :] = hh
        wr = col_v[2, pl.ds(pl.multiple_of(k * R, 8), R), :].reshape(NV, 8, 128)
        rs = slice(8 * t, 8 * t + 8)
        acc_v[0, rs, :] = acc_v[0, rs, :] + jnp.sum(hh, axis=0)
        acc_v[1, rs, :] = acc_v[1, rs, :] + jnp.sum(hh * hh, axis=0)
        acc_v[2, rs, :] = acc_v[2, rs, :] + jnp.sum(hh * wr, axis=0)

    s5 = lambda k: [(functools.partial(s5_blk, k, b, h), 1.0) for b in range(NB) for h in range(2)]

    for c in c_par:
        c.wait()
    for k in range(2):
        _weave((s1n(k), 0.0, 0.2), (s1g(k), 0.2, 1.0))
    _weave((s1n(2), 0.0, 0.2), (s1g(2), 0.2, 1.0), (s2(0), 0.3, 1.0))
    s1_nat(3, 0, 1)
    c_x.wait()
    ln = [ln1_pieces(b, NPC) for b in range(NB)]
    s30 = s3(0)
    _weave((sum(ln, []), 0.0, P3F[0]), (s2(1), 0.0, P3F[2]),
           *[([s30[b]], max((b + 1.6) * P3F[0] / NB, P3F[3] + (1.0 - P3F[3]) * b / NB), 0.0) for b in range(NB)])
    for c in c_par2:
        c.wait()

    def body(k, do5=True, do4=True, do3=True, do2=True, do1=True, j=None):
        at = (lambda d: k + d) if j is None else (lambda d: j + (k + d) if k + d else j)
        g2 = s2_gen(at(2)) if do2 else None
        for n in range(NV):
            g4 = s4_gen(at(0), n) if do4 else None
            st4 = [0, 0]
            n4 = ORDER.count("4")

            def adv4(m):
                if not do4:
                    return
                st4[0] += 1
                while st4[1] < 72 * st4[0] / n4 - 3 or (st4[0] == n4 and st4[1] <= 72):
                    r = next(g4, None)
                    if r is None:
                        break
                    st4[1] = r

            def nat():
                if do1:
                    if n + 1 < NV:
                        s1_nat(at(3), n + 1, 1)
                    else:
                        s1_nat(jnp.minimum(at(4), NSTEP - 1), 0, 1)

            g1 = s1_grp(at(3), n) if do1 else None
            for tok in ORDER:
                if tok == "5":
                    if do5 and n < NB:
                        s5_blk(at(-1), n, 0)
                        s5_blk(at(-1), n, 1)
                elif tok == "4":
                    adv4(1)
                elif tok in "ab" and do1:
                    next(g1)
                elif tok == "p" and do1:
                    run(g1)
                elif tok == "2" and do2:
                    next(g2, None)
                elif tok == "3" and do3 and n < NB:
                    s3_blk(at(1), n)
                elif tok == "n":
                    nat()
        if do2:
            run(g2)

    @pl.when(flag_s[0] == 1)
    def _():
        body(0, do5=False)

    lax.fori_loop(0, 4, lambda j, c: (body(1, j=j), c)[1], 0)

    @pl.when(flag_s[0] == 1)
    def _():
        body(5, do1=False)

    @pl.when(flag_s[0] == 1)
    def _():
        body(6, do1=False, do2=False)

    @pl.when(flag_s[0] == 1)
    def _():
        _weave(([(lambda n=n: run(s4_gen(7, n, (0,))), 1.0) for n in range(NV)], 0.0, 1.0), (s5(6), 0.0, 1.0))

    @pl.when(flag_s[0] == 1)
    def _():
        _weave(([(lambda n=n: run(s4_gen(7, n, (4,))), 1.0) for n in range(NV)], 0.0, 1.0), (s5(7)[:8], 0.0, 1.0))

    _weave((s5(7)[8:], 0.0, 1.0))

    def total(i):
        halves = []
        for hf in range(2):
            t = acc_v[i, pl.ds(64 * hf, 8, stride=8), :]
            for s in range(1, 8):
                t = t + acc_v[i, pl.ds(64 * hf + s, 8, stride=8), :]
            halves.append(t)
        return jnp.concatenate(halves, 0)

    m2 = total(0) * (1.0 / D)
    var2 = jnp.maximum(total(1) * (1.0 / D) - m2 * m2, 0.0)
    sd2 = _rb(jnp.sqrt(_rb(_rb(var2) + EPS)))
    rs2 = 1.0 / sd2
    r = _rb((total(2) - m2 * wr_sum) * rs2)
    mean2 = fin_v[4] + m2
    fin_v[0] = rs2
    fin_v[1] = m2 * rs2
    fin_v[2] = rs2 + 1.0
    fin_v[3] = fin_v[4] - m2 * rs2

    tl = _iota((16, 128), 0)
    ll = _iota((16, 128), 1)
    lodd = (ll & 1) == 1
    toff = jnp.where((tl & 1) == 0, jnp.where(lodd, ll + 127, ll), jnp.where(lodd, ll + 128, (ll - 1) & 127))
    tok = (tl >> 1) * 256 + toff
    rbits = pltpu.bitcast(r, i32)
    srt = rbits ^ ((rbits >> 31) & 0x7FFFFFFF)
    key = pltpu.bitcast((((srt >> 16) + 32768) << 11) + (2047 - tok) + (1 << 28), f32)
    kk = key
    cand = []
    for _ in range(4):
        rm = jnp.broadcast_to(jnp.max(kk, axis=1, keepdims=True), (16, 128))
        cand.append(rm)
        kk = jnp.where(kk == rm, 0.0, kk)
    last = jnp.max(cand[3], axis=0, keepdims=True)
    kcol = None
    for j in range(TOPC):
        mx = jnp.max(cand[0], axis=0, keepdims=True)
        kcol = jnp.broadcast_to(mx, (8, 128)) if j == 0 else jnp.where(sub8 == j, mx, kcol)
        took = cand[0] == mx
        cand = [jnp.where(took, cand[i + 1] if i < 3 else 0.0, cand[i]) for i in range(4)]
    kc_v[...] = kcol

    @pl.when((last - mx)[0, 0] > 0.0)
    def _():
        k2 = key
        kc = None
        for j in range(TOPC):
            m1 = jnp.max(jnp.max(k2, axis=0, keepdims=True), axis=1, keepdims=True)
            kc = jnp.broadcast_to(m1, (8, 128)) if j == 0 else jnp.where(sub8 == j, m1, kc)
            k2 = jnp.where(k2 == m1, 0.0, k2)
        kc_v[...] = kc

    kcol = kc_v[...]
    kint = pltpu.bitcast(kcol, i32) - (1 << 28)
    tcol = 2047 - (kint & 2047)
    s16 = (kint >> 11) - 32768
    rsel = pltpu.bitcast((s16 ^ ((s16 >> 31) & 0x7FFF)) << 16, f32)
    gate = _rb(jax.nn.sigmoid(rsel))[:, 0:1]

    def classes(col):
        cls = jnp.zeros((8, 128), i32)
        for d in range(1, TOPC):
            cls = cls + jnp.where((col == pltpu.roll(col, d, 0)) & (sub8 >= d), 1, 0)
        return cls, jnp.max(cls, axis=0, keepdims=True)[0, 0] + 1

    wcol = tcol & 255
    pcol = jnp.where((wcol & 1) == 0, jnp.where(wcol < 128, wcol, wcol - 127),
                     jnp.where(wcol < 128, (wcol + 1) & 127, wcol - 128))
    ecol = ((tcol >> 8) << 1) | (tcol & 1)
    etile = [ecol[j, 0] for j in range(TOPC)]
    gcol, gn = classes(pcol)
    xs_v[...] = jnp.zeros((8, D), f32)

    def gather(c, carry):
        oh = (gcol == c) & (lane8 == pcol)
        ohi = jnp.where(oh, 1, 0)
        msk = [jnp.broadcast_to(ohi[j:j + 1], (8, 128)) == 1 for j in range(TOPC)]
        sa = sb = None
        for j in range(TOPC):
            fa = jnp.broadcast_to(fin_v[0, pl.ds(etile[j], 1), :], (8, 128))
            fb = jnp.broadcast_to(fin_v[1, pl.ds(etile[j], 1), :], (8, 128))
            sa, sb = (fa, fb) if j == 0 else (jnp.where(msk[j], fa, sa), jnp.where(msk[j], fb, sb))
        parts = []
        for q in range(D // 8 // GCH):
            mg = None
            for j in range(TOPC):
                cc = c1_v[GCH * q:GCH * q + GCH, pl.ds(pl.multiple_of(8 * etile[j], 8), 8), :]
                mg = cc if j == 0 else jnp.where(msk[j], cc, mg)
            parts.append(mg * sa - sb)
        ln = jnp.concatenate(parts, 0).reshape(D, 128)
        xs_v[...] = xs_v[...] + _dot_nt(jnp.where(oh, 1.0, 0.0).astype(f32), ln)
        return carry

    lax.fori_loop(0, gn, gather, 0)
    xsel = xs_v[...]

    def rebuilt_rows():
        sdc = jnp.zeros((8, 1), f32)
        mc = jnp.zeros((8, 1), f32)
        sub1 = _iota((8, 1), 0)
        for j in range(TOPC):
            hitm = tok == jnp.broadcast_to(tcol[j:j + 1], (16, 128))
            red = lambda v: jnp.sum(jnp.sum(jnp.where(hitm, v, 0.0), axis=0, keepdims=True), axis=1, keepdims=True)
            sdc = jnp.where(sub1 == j, red(sd2), sdc)
            mc = jnp.where(sub1 == j, red(mean2), mc)
        return xsel * (sdc + 1.0) + mc

    def outp(b, g0, g1):
        sc = [jnp.where(top, jnp.broadcast_to(fin_v[i, 2 * b:2 * b + 1, :], (8, 128)),
                        jnp.broadcast_to(fin_v[i, 2 * b + 1:2 * b + 2, :], (8, 128))) for i in (2, 3)]
        for g in range(g0, g1):
            a = _rb(c1_v[g, pl.ds(16 * b, 8, stride=2), :] * sc[0] + sc[1])
            c = _rb(c1_v[g, pl.ds(16 * b + 1, 8, stride=2), :] * sc[0] + sc[1])
            w = (pltpu.bitcast(a, u32) >> 16) | pltpu.bitcast(c, u32)
            out_w[g, b] = jnp.where(mask2, w, pltpu.roll(pltpu.roll(w, 4, 0), 127, 1))

    opieces = [functools.partial(outp, b, 24 * i, 24 * i + 24) for b in range(NB) for i in range(3)]

    tilec = tcol >> 7
    lanec = tcol & 127
    aux = {}

    def late_scalars():
        tiles = [tilec[j, 0] for j in range(TOPC)]
        hit = 0
        dup = []
        for j in range(TOPC):
            dup.append((hit >> tiles[j]) & 1)
            hit = hit | (1 << tiles[j])
        free, cnt = [], 0
        for t in range(16):
            un = 1 - ((hit >> t) & 1)
            free.append(jnp.where(un == 1, cnt, -1))
            cnt = cnt + un
        late, nd, mask = [tiles[0]], 0, hit
        for j in range(1, TOPC):
            rep = 0
            for t in range(16):
                rep = jnp.where(free[t] == nd, t, rep)
            late.append(jnp.where(dup[j] == 1, rep, tiles[j]))
            mask = mask | (1 << late[j])
            nd = nd + dup[j]
        aux.update(tiles=tiles, late=late, mask=mask)
        bs_v[...] = rebuilt_rows()
        aux["clscol"], aux["ncls"] = classes(lanec)

    def tile_idx(t, g0=0, ng=D // 8):
        if isinstance(t, int):
            return (pl.ds(g0, ng), t // 2, pl.ds(8 * (t % 2), 8), slice(None))
        return (pl.ds(g0, ng), t >> 1, pl.ds(pl.multiple_of(8 * (t & 1), 8), 8), slice(None))

    def ocopy(idx):
        return cp(out_v.at[idx], out_h.at[idx], osem.at[0])

    for c in range(NCH):
        for cc in c_w[c]:
            cc.wait()
        mine = opieces[OSPLIT[c]:OSPLIT[c + 1]]
        nsub = max(1, FCH[c] // FSUB)
        sub = FCH[c] // nsub
        for u in range(nsub):
            sl = slice(FOFF[c] + u * sub, FOFF[c] + (u + 1) * sub)
            g = _rb(_dot(xsel, wmat(wg_w, 0, D, sl.start, sub)))
            up = _rb(_dot(xsel, wmat(wu_w, 0, D, sl.start, sub)))
            if c == 0 and u == 0:
                late_scalars()
            for fn in mine[u * len(mine) // nsub:(u + 1) * len(mine) // nsub]:
                fn()
            act_v[:, sl] = _rb(_rb(g * jax.nn.sigmoid(g)) * up)

    def early():
        for t in range(16):
            @pl.when(((aux["mask"] >> t) & 1) == 0)
            def _():
                ocopy(tile_idx(t)).start()

    clscol = aux["clscol"]
    onehot = lambda c: jnp.where((clscol == c) & (lane8 == lanec), 1.0, 0.0).astype(f32)
    bc = lambda v, j: jnp.broadcast_to(v[j:j + 1], (8, 128))

    def down(p, c0, nc):
        r = slice(POFF[p], POFF[p] + PART[p])
        yc = _dot_nt(act_v[:, c0:c0 + nc], wmat(wd_w, POFF[p], PART[p], c0, nc))
        y_v[:, r] = yc if c0 == 0 else y_v[:, r] + yc

    def place(p, fast):
        r0, nr = POFF[p], PART[p]
        g0, ng = r0 // 8, nr // 8
        newrow = _rb(bs_v[:, r0:r0 + nr] + _rb(_rb(y_v[:, r0:r0 + nr]) * gate))
        tn = lambda oh: lax.dot_general(newrow, oh, (((0,), (0,)), ((), ())), preferred_element_type=f32)
        if fast:
            uu = tn(jnp.concatenate([onehot(0), onehot(1)], 1))
            for c in range(2):
                u_v[c, g0:g0 + ng] = uu[:, 128 * c:128 * (c + 1)].reshape(ng, 8, 128)
        else:
            for c in range(TOPC):
                u_v[c, g0:g0 + ng] = tn(onehot(c)).reshape(ng, 8, 128)

    def write(p, fast):
        g0, ng = POFF[p] // 8, PART[p] // 8
        for j in range(TOPC):
            idx = tile_idx(aux["tiles"][j], g0, ng)
            new = out_v[idx].astype(f32)
            for c in range(2 if fast else j + 1):
                new = jnp.where((lane8 == bc(lanec, j)) & (bc(clscol, j) == c), u_v[c, g0:g0 + ng], new)
            out_v[idx] = new.astype(bf16)
        for j in range(TOPC):
            ocopy(tile_idx(aux["late"][j], g0, ng)).start()

    def dwait(p):
        for cc in c_d[p]:
            cc.wait()

    NP = len(PART)
    dwait(0)
    rest = opieces[OSPLIT[NCH]:]
    nq = 4
    for q in range(nq):
        down(0, q * F // nq, F // nq)
        for fn in rest[q * len(rest) // nq:(q + 1) * len(rest) // nq]:
            fn()
    early()

    @pl.when(aux["ncls"] <= 2)
    def _():
        for p in range(1, NP):
            dwait(p)
            down(p, 0, DSPL[p])
            place(p - 1, True)
            down(p, DSPL[p], F - DSPL[p])
            write(p - 1, True)
        place(NP - 1, True)
        write(NP - 1, True)

    @pl.when(aux["ncls"] > 2)
    def _():
        for p in range(1, NP):
            dwait(p)
            down(p, 0, F)
        for p in range(NP):
            place(p, False)
            write(p, False)

    cp(out_h, out_h, osem.at[0]).wait()


@jax.jit
def pallas_sequential_preLN__ssm_conv_s4__moe_arch_mod__prompt_kernel(
    A_u: jax.Array,
    A_A_re: jax.Array,
    A_A_im: jax.Array,
    A_B_re: jax.Array,
    A_B_im: jax.Array,
    A_C_re: jax.Array,
    A_C_im: jax.Array,
    A_log_dt: jax.Array,
    A_Dskip: jax.Array,
    B_x: jax.Array,
    B_w_r: jax.Array,
    B_w_gate: jax.Array,
    B_w_up: jax.Array,
    B_w_down: jax.Array,
):
    hbm = pl.BlockSpec(memory_space=pltpu.MemorySpace.HBM)
    vm = pltpu.VMEM
    G8 = D // 8
    wshape = (D // 16, F // 128, 16, 128)
    wview = lambda w: w.reshape(D // 16, 2, 8, F // 128, 128).transpose(0, 1, 3, 2, 4)
    scratch = [
        vm((G8, NB, 16, 128), bf16), vm((6, D, N), bf16), vm((D,), bf16), vm((D,), bf16), vm((D,), bf16),
        vm(_CTAB.shape, f32), vm(wshape, bf16), vm(wshape, bf16), vm(wshape, bf16), vm((G8, NB + 1, 16, 128), bf16),
        vm((10, 4, 144, 128), bf16), vm((2, 2, 2, 144, 128), bf16), vm((3, D + 8, 128), f32),
        vm((NV, 2, 136, 128), f32), vm((NSTEP, NV, 56, 128), f32), vm((NSTEP, R, 128), f32),
        vm((NSTEP, NB, 6, R, 128), f32), vm((NSTEP, NB, 6, R, 128), f32),
        vm((NSTEP, NB, 2, R, 256), f32), vm((G8, 136, 128), f32), vm((2, 17, 8, 128), f32),
        vm((3, 136, 128), f32), vm((5, 16, 128), f32), vm((TOPC, G8, 8, 128), f32),
        vm((R, 512), f32), vm((8, D), f32), vm((NV, 4, 8, 128), f32),
        vm((8, 128), f32), vm((8, D), f32), vm((8, D), f32), vm((8, F), f32), pltpu.SMEM((1,), i32),
        pltpu.SemaphoreType.DMA((5 + NCH + len(PART),)), pltpu.SemaphoreType.DMA((1,)),
    ]
    xv = A_u[0].T.reshape(G8, 8, 16, 128).transpose(0, 2, 1, 3).reshape(G8, NB, 16, 128)
    out = pl.pallas_call(
        _kernel,
        out_shape=jax.ShapeDtypeStruct((G8, NB, 16, 128), bf16),
        in_specs=[hbm] * 14,
        out_specs=hbm,
        scratch_shapes=scratch,
        compiler_params=pltpu.CompilerParams(vmem_limit_bytes=120 * 1024 * 1024, disable_bounds_checks=NOBC),
    )(xv, A_A_re, A_A_im, A_B_re, A_B_im, A_C_re, A_C_im, A_log_dt, A_Dskip, B_w_r,
      wview(B_w_gate), wview(B_w_up), wview(B_w_down.T), jnp.asarray(_CTAB))
    return out.reshape(G8, 16, 8, 128).transpose(0, 2, 1, 3).reshape(D, L).T[None]
```

```python
import functools

import numpy as np
import jax
import jax.numpy as jnp
from jax import lax
import jax.experimental.pallas as pl
import jax.experimental.pallas.tpu as pltpu

f32 = jnp.float32
bf16 = jnp.bfloat16
i32 = jnp.int32
u32 = jnp.uint32

L, D, N, F, TOPC = 2048, 576, 128, 4608, 8
NB = 8
NV = 9
R = NV * 8
NSTEP = D // R
EPS = 1e-5

_XL1 = [(1, 5), (2, 6), (3, 7), (4, 8), (258, 516), (260, 520), (262, 772), (264, 776),
        (1288, 1032), (1800, 1544)]
_XSH = [0, 1, 2, 3, 0, 1, 2, 3, 0, 1]


def _bf16_round_int(j):
    u = np.asarray(j, np.float32).view(np.uint32).astype(np.uint64)
    r = ((u + 0x7FFF + ((u >> 16) & 1)) >> 16) << 16
    return r.astype(np.uint32).view(np.float32).astype(np.int64)


def _chunk_values():
    vals = -np.ones((5, 128), np.int64)
    for j in range(10):
        for p in range(2):
            ch = (j // 4) * 2 + p if j < 8 else 4
            extra = 2 * p if j >= 8 else 0
            for l0 in range(32):
                vals[ch, (4 * (31 - l0) + 4 * p + _XSH[j] + extra + 8) % 128] = _XL1[j][p] + 8 * l0
    assert (vals >= 0).all()
    return vals


def _tables():
    cv = _chunk_values()
    om = np.pi * (2 * np.arange(128) + 1) / 512.0
    sig = (-1.0) ** np.arange(128)
    cvp = {"A0": cv[0], "A1": cv[1], "B": cv[2], "C": cv[3], "D": cv[4]}
    cvp["Cp"] = cv[3].copy(); cvp["Cp"][11] = cv[2][11]
    cvp["Dp"] = cv[4].copy(); cvp["Dp"][15] = cv[3][15]
    passes = [(0, "A0"), (0, "A1"), (1, "A1"), (1, "B"), (2, "Cp"), (3, "C"), (4, "Dp"),
              (5, "D"), (6, "D"), (7, "D")]
    G = np.zeros((10, 128, 4, 128))
    for b in range(NB):
        mine = [i for i, (pb, _) in enumerate(passes) if pb == b]
        for j in range(1, 257):
            lag = 256 * b + j
            if lag > L - 1:
                continue
            v = int(_bf16_round_int(lag))
            hit = [(i, int(np.nonzero(cvp[passes[i][1]] == v)[0][0])) for i in mine
                   if (cvp[passes[i][1]] == v).any()]
            assert len(hit) == 1, (b, j, v, hit)
            i, l = hit[0]
            e = np.exp(-1j * om * j) * sig ** b / 256.0
            s = (-1.0) ** j
            G[i, l, 0] += e.real; G[i, l, 1] += e.imag
            G[i, l, 2] += s * e.real; G[i, l, 3] += s * e.imag
    e8 = np.exp(-1j * np.outer(8 * np.arange(32), om))
    sets = {"A0": [0], "A1": [1], "B": [3], "C": [4, 5], "D": [6, 7, 8, 9]}
    seeds, masks = {}, {}
    for name, ps in sets.items():
        seeds[name] = sum(G[i, 16:24] for i in ps)
        for i in ps:
            masks[i] = [int(x) for x in (np.abs(G[i, 16:24]).sum((1, 2)) > 0)]
            for v in range(2, 17):
                sd = seeds[name]
                r0 = 8 * (v % 16)
                for q in (0, 2):
                    z = (sd[:, q] + 1j * sd[:, q + 1]) * np.conj(e8[2 * (v - 2)]) * np.array(masks[i])[:, None]
                    assert np.allclose(z.real, G[i, r0:r0 + 8, q], atol=1e-12)
                    assert np.allclose(z.imag, G[i, r0:r0 + 8, q + 1], atol=1e-12)
    assert not G[2, 16:].any() and not G[2, :8].any()
    s8 = np.arange(8)
    je = np.where(s8 % 2 == 0, s8, 127 + s8)
    jo = np.where(s8 % 2 == 0, s8 - 1, 128 + s8)
    fe = np.exp(-1j * np.outer(je, om)); ft = np.exp(-1j * np.outer(jo, om))
    ft0 = np.exp(-1j * np.outer(jo % 128 + 128 * (s8 % 2), om))
    rows = [e8.real, e8.imag]
    for name in ("A0", "A1", "B", "C", "D"):
        rows += [seeds[name][:, q] for q in range(4)]
    for i in range(10):
        rows += [G[i, 8:16, q] for q in range(4)]
    rows += [fe.real, fe.imag, ft.real, ft.imag, ft0.real, ft0.imag]
    return np.concatenate(rows, 0).astype(np.float32), masks


_CTAB, _GMASK = _tables()


def _sincos_coeffs():
    r = np.cos(np.pi * (np.arange(4000) + .5) / 4000) * 0.5
    z = r * r
    s = np.linalg.lstsq(np.stack([z ** k for k in range(4)], 1), np.sin(np.pi / 2 * r) / r, rcond=None)[0]
    c = np.linalg.lstsq(np.stack([z ** k for k in range(1, 5)], 1), np.cos(np.pi / 2 * r) - 1, rcond=None)[0]
    return [float(x) for x in s], [float(x) for x in c]


_SC, _CC = _sincos_coeffs()


def _cmul(a, b):
    return (a[0] * b[0] - a[1] * b[1], a[0] * b[1] + a[1] * b[0])


def _cmulc(a, b):
    return (a[0] * b[0] + a[1] * b[1], a[1] * b[0] - a[0] * b[1])


def _csq(a):
    return ((a[0] - a[1]) * (a[0] + a[1]), (a[0] + a[0]) * a[1])


def _sincos(th):
    z = th * (2.0 / np.pi)
    k = jnp.round(z)
    r = z - k
    r2 = r * r
    s = r * (_SC[0] + r2 * (_SC[1] + r2 * (_SC[2] + r2 * _SC[3])))
    c = 1.0 + r2 * (_CC[0] + r2 * (_CC[1] + r2 * (_CC[2] + r2 * _CC[3])))
    ki = k.astype(i32)
    swap = (ki & 1) == 1
    s2 = jnp.where(swap, c, s)
    c2 = jnp.where(swap, s, c)
    s2 = pltpu.bitcast(pltpu.bitcast(s2, i32) ^ ((ki & 2) << 30), f32)
    c2 = pltpu.bitcast(pltpu.bitcast(c2, i32) ^ (((ki + 1) & 2) << 30), f32)
    return s2, c2


def _rb(x):
    return x.astype(bf16).astype(f32)


def _dot(a, b):
    return jnp.dot(a, b, preferred_element_type=f32)


def _dot_nt(a, b):
    return lax.dot_general(a, b, (((1,), (1,)), ((), ())), preferred_element_type=f32)


def _iota(shape, dim):
    return lax.broadcasted_iota(i32, shape, dim)


S4MODE='LC'
TILE=4
YSPLIT=1
ZT=1
ORDER='44443ab24pn45'
NPC=3
P3F=(0.9,0.4,0.55,0.3)
GCH=3
FSUB=1536
NOBC=True
FCH=(4608,)
OSPLIT=[0,24]
WSTART=0
PART=(256,128,128,64)
DSPL=(0,2560,2560,4096)
NCH = len(FCH)
FOFF = [sum(FCH[:i]) for i in range(NCH)]
POFF = [sum(PART[:i]) for i in range(len(PART))]

def _weave(*streams):
    items = []
    for si, (pieces, lo, hi) in enumerate(streams):
        tot = float(sum(c for _, c in pieces))
        cum = 0.0
        for pi, (fn, c) in enumerate(pieces):
            items.append((lo + max(hi - lo, 0.0) * (cum + 0.5 * c) / tot, si, pi, fn))
            cum += c
    for _, _, _, fn in sorted(items, key=lambda t: t[:3]):
        fn()


def _kernel(x_h, are_h, aim_h, bre_h, bim_h, cre_h, cim_h, ldt_h, dsk_h, wr_h, wg_h, wu_h, wd_h, ct_h,
            out_h,
            x_v, par_v, ldt_v, dsk_v, wr_v, ct_v, wg_v, wu_v, wd_v, out_v,
            g_v, f_v, col_v, st_v, kd_v, k0_v, kh_v, uh_v, zs_v, c1_v, s1_v, acc_v, fin_v, u_v, zt_v, y_v, pv_v, kc_v, xs_v, bs_v, act_v, sg_v, lm_v, flag_s,
            sem, osem):
    cp = pltpu.make_async_copy
    c_ct = cp(ct_h, ct_v, sem.at[0])
    c_vec = [cp(ldt_h, ldt_v, sem.at[1]), cp(dsk_h, dsk_v, sem.at[1]), cp(wr_h, wr_v, sem.at[1])]
    PH = 4 * R
    par_h = (are_h, aim_h, bre_h, bim_h, cre_h, cim_h)
    c_par = [cp(h.at[pl.ds(0, PH)], par_v.at[i, pl.ds(0, PH)], sem.at[2]) for i, h in enumerate(par_h)]
    c_par2 = [cp(h.at[pl.ds(PH, D - PH)], par_v.at[i, pl.ds(PH, D - PH)], sem.at[3])
              for i, h in enumerate(par_h)]
    c_x = cp(x_h, x_v, sem.at[4])
    def wcp(h, v, rp, ct, s):
        return [cp(h.at[rp, hf, ct], v.at[rp, ct, pl.ds(8 * hf, 8), :], s) for hf in range(2)]

    c_w = [wcp(wg_h, wg_v, slice(None), pl.ds(FOFF[c] // 128, FCH[c] // 128), sem.at[5 + c])
           + wcp(wu_h, wu_v, slice(None), pl.ds(FOFF[c] // 128, FCH[c] // 128), sem.at[5 + c]) for c in range(NCH)]
    c_d = [wcp(wd_h, wd_v, pl.ds(POFF[p] // 16, PART[p] // 16), slice(None), sem.at[5 + NCH + p])
           for p in range(len(PART))]
    for c in c_vec + [c_ct] + c_par + [c_x] + c_par2 + sum(c_w, []) + sum(c_d, []):
        c.start()

    flag_s[0] = 1
    x_w = x_v.bitcast(u32)
    wg_w, wu_w, wd_w = wg_v.bitcast(u32), wu_v.bitcast(u32), wd_v.bitcast(u32)

    def wmat(w, r0, nr, c0, nc):
        return jnp.concatenate([pltpu.bitcast(w[r0 // 16:(r0 + nr) // 16, t], bf16).reshape(nr, 128)
                                for t in range(c0 // 128, (c0 + nc) // 128)], 1)

    out_w = out_v.bitcast(u32)
    g_w = g_v.bitcast(u32)
    f_w = f_v.bitcast(u32)
    sub8 = _iota((8, 128), 0)
    lane8 = _iota((8, 128), 1)

    acc_v[...] = jnp.zeros(acc_v.shape, f32)
    for n in range(NV):
        for ri in range(2):
            st_v[n, ri, 104:112, :] = jnp.full((8, 128), 1.0 - ri, f32)
    for c in c_vec:
        c.wait()

    rows = [_rb(jnp.exp(ldt_v[...].astype(f32).reshape(1, D))),
            dsk_v[...].astype(f32).reshape(1, D),
            wr_v[...].astype(f32).reshape(1, D)]
    wr_sum = jnp.sum(rows[2], axis=1, keepdims=True)
    ones = jnp.ones((128, 128), f32)
    for j in range(5):
        w = 128 if j < 4 else 64
        eye = _iota((w, w), 0) == _iota((w, w), 1)
        m = jnp.concatenate([jnp.where(eye, jnp.broadcast_to(rows[i][:, j * 128:j * 128 + w], (w, w)), 0.0)
                             for i in range(3)], 0)
        res = _dot(m, ones[:w, :])
        for i in range(3):
            col_v[i, j * 128:j * 128 + w, :] = res[i * w:(i + 1) * w]

    c_ct.wait()

    def e8(v):
        return (jnp.broadcast_to(ct_v[v:v + 1, :], (8, 128)), jnp.broadcast_to(ct_v[32 + v:33 + v, :], (8, 128)))

    sets = {"A0": [0], "A1": [1], "B": [3], "C": [4, 5], "D": [6, 7, 8, 9]}
    for i in (0, 1, 3, 4, 5, 6, 7, 8, 9):
        for q in range(4):
            g_v[i, q, 8:16, :] = ct_v[224 + 32 * i + 8 * q:232 + 32 * i + 8 * q, :].astype(bf16)
    for si, (name, ps) in enumerate(sets.items()):
        sd = [ct_v[64 + 32 * si + 8 * q:72 + 32 * si + 8 * q, :] for q in range(4)]
        mk = {}
        for i in ps:
            if len(ps) > 1:
                bits = sum(b << s for s, b in enumerate(_GMASK[i]))
                mk[i] = ((bits >> sub8) & 1) == 1
        for v in range(2, 17):
            if v == 2:
                vals = sd
            else:
                ev = e8(2 * (v - 2))
                vals = list(_cmulc((sd[0], sd[1]), ev)) + list(_cmulc((sd[2], sd[3]), ev))
            for i in ps:
                for q in range(4):
                    val = vals[q] if len(ps) == 1 else jnp.where(mk[i], vals[q], 0.0)
                    g_v[i, q, 8 * (v % 16):8 * (v % 16) + 8, :] = val.astype(bf16)
    sig = jnp.where((lane8 & 1) == 0, 1.0, -1.0).astype(f32)
    for h in range(2):
        sd = (ct_v[544 + 16 * h:552 + 16 * h, :], ct_v[552 + 16 * h:560 + 16 * h, :])
        for v in range(16):
            if v == 0:
                vals = sd if h == 0 else (ct_v[576:584, :], ct_v[584:592, :])
            else:
                vals = _cmul(sd, e8(v))
            for q in range(2):
                f_v[0, h, q, 8 * v:8 * v + 8, :] = vals[q].astype(bf16)
                f_v[1, h, q, 8 * v:8 * v + 8, :] = (vals[q] * sig).astype(bf16)

    def gmat(i):
        return jnp.concatenate([pltpu.bitcast(g_w[i, q, 0:64, :], bf16) for q in range(4)], 1)

    def fmat(ver, h):
        return jnp.concatenate([pltpu.bitcast(f_w[ver, h, q, 0:64, :], bf16) for q in range(2)], 1)

    revmask = (sub8 & 2) == 0
    lm = lane8 & 3

    def s1_nat(k, n0, nn):
        row0 = pl.multiple_of(k * R + 8 * n0, 8)
        rr = 8 * nn
        ld = lambda i: par_v[i, pl.ds(row0, rr), :].astype(f32)
        dt = col_v[0, pl.ds(row0, rr), :]
        e = jnp.exp(dt * ld(0))
        s, c = _sincos(dt * ld(1))
        a1 = (e * c, e * s)
        w = _cmul((ld(4), ld(5)), (dt * ld(2), dt * ld(3)))
        k0_v[k, 8 * n0:8 * n0 + rr, :] = (jnp.sum(w[0], axis=1, keepdims=True)
                                          + col_v[1, pl.ds(row0, rr), :]) * (1.0 / 256.0)
        w = (w[0], -w[1])
        rev = lambda v: jnp.where(revmask, pltpu.roll(v, 2, 0), pltpu.roll(v, 6, 0))

        def put(arr, slots, fn=None):
            for n in range(nn):
                for ri in range(2):
                    v = arr[ri][8 * n:8 * n + 8]
                    if fn is not None:
                        v = fn(v)
                    for q in slots:
                        st_v[n0 + n, ri, q * 8:q * 8 + 8, :] = v

        put(w, (0, 1)); put(a1, (2, 3))
        a2 = _csq(a1); put(a2, (5,))
        a4 = _csq(a2); put(a4, (6,))
        put(_cmul(a4, a1), (4,))
        a8 = _csq(a4); put(a8, (12,), rev)
        t = _csq(a8); put(t, (14, 15), rev)
        for _ in range(4):
            t = _csq(t)
        put(t, (7, 11))
        t = _csq(t); put(t, (8, 9))
        put(_csq(t), (10,))

    def s1_grp(k, n):
        mix = lambda q: tuple(jnp.concatenate([st_v[n, ri, pl.ds(q * 8 + g, 8, stride=2), :] for g in range(2)], 0)
                              for ri in range(2))
        y = [mix(12)]
        a16d = mix(14)
        if YSPLIT == 1:
            for _ in range(15):
                y.append(_cmul(y[-1], a16d))
        else:
            y.append(_cmul(y[0], a16d))
            a32d = _csq(a16d)
            for i in range(2, 16):
                y.append(_cmul(y[i - 2], a32d))
        yield
        wd = mix(0); a1d = mix(2); m1 = mix(5)
        v = [_cmulc(wd, mix(3))]
        for _ in range(3):
            v.append(_cmulc(v[-1], a1d))
        v4 = _cmulc(_cmulc(wd, m1), mix(7))
        v5 = _cmulc(v4, m1); v6 = _cmulc(v4, mix(6)); v7 = _cmulc(v6, m1)
        v8 = _cmulc(v7, mix(10)); v9 = _cmulc(v8, mix(8))
        v += [v4, v5, v6, v7, v8, v9]
        os_ = []
        for g in range(2):
            cat = lambda ts: jnp.concatenate([jnp.concatenate([t[ri][8 * g:8 * g + 8] for t in ts], 0)
                                              for ri in range(2)], 1)
            os_.append(_dot_nt(cat(v), cat(y[::-1])))
        yield
        for g in range(2):
            o = os_[g]
            ro = [pltpu.roll(o[8 * j:8 * j + 8], _XSH[j] + 5, 1, stride=1, stride_axis=0) for j in range(10)]
            sel4 = lambda q: jnp.where(lm == 0, q[0], jnp.where(lm == 1, q[1], jnp.where(lm == 2, q[2], q[3])))
            kd_v[k, n, pl.ds(g, 8, stride=2), :] = sel4(ro[0:4])
            kd_v[k, n, pl.ds(16 + g, 8, stride=2), :] = sel4(ro[4:8])
            kd_v[k, n, pl.ds(32 + g, 8, stride=2), :] = jnp.where(lm == 0, ro[8], ro[9])

    def run(gen):
        for _ in gen:
            pass

    s1n = lambda k: [(functools.partial(s1_nat, k, 3 * i, 3), 1.0) for i in range(3)]
    s1g = lambda k: [(lambda n=n: run(s1_grp(k, n)), 1.0) for n in range(NV)]

    laneR = _iota((R, 128), 1)
    lmR = laneR & 3

    def s2_gen(k):
        ch = lambda c: kd_v[k, :, 8 * c:8 * c + 8, :].reshape(R, 128)
        for b in range(NB):
            if b == 0:
                z = _dot(ch(0), gmat(0)) if ZT else None
                dd = jnp.where(lmR < 2, ch(4), pltpu.roll(ch(5), 2, 1))
                kd_v[k, :, 48:56, :] = dd.reshape(NV, 8, 128)
                if ZT:
                    zt_v[...] = z
                    yield
                    z = _dot(ch(1), gmat(1)) + zt_v[...]
                else:
                    z = _dot(jnp.concatenate([ch(0), ch(1)], 1), jnp.concatenate([gmat(0), gmat(1)], 0))
            elif b == 1:
                k256 = jnp.sum(jnp.where(laneR == 15, ch(1), 0.0), axis=1, keepdims=True)
                pat = jnp.concatenate([ct_v[288 + 8 * q + 7:288 + 8 * q + 8, :] for q in range(4)], 1)
                z = _dot(ch(2), gmat(3)) + k256 * pat
            elif b == 2:
                z = _dot(jnp.where(laneR == 11, ch(2), ch(3)), gmat(4))
            elif b == 3:
                z = _dot(ch(3), gmat(5))
            elif b == 4:
                z = _dot(jnp.where(laneR == 15, ch(3), ch(6)), gmat(6))
            else:
                z = _dot(ch(6), gmat(b + 2))
            for s in range(2):
                kr = z[:, 256 * s:256 * s + 128]
                ki = z[:, 256 * s + 128:256 * s + 256]
                if b == 0:
                    kr = kr + k0_v[k]
                kh_v[k, b, 3 * s] = kr
                if S4MODE[0] == "L":
                    kh_v[k, b, 3 * s + 1] = kr + ki
                    kh_v[k, b, 3 * s + 2] = ki - kr
                else:
                    kh_v[k, b, 3 * s + 1] = ki
            yield

    def s2(k):
        gen = s2_gen(k)
        return [(lambda: next(gen, None), 1.0) for _ in range(9)]

    mask2 = (sub8 < 4) == ((lane8 & 1) == 0)
    top = sub8 < 4

    def ln1_pieces(b, npc):
        state = {}
        per = (D // 8) // npc

        def piece(i):
            for g in range(i * per, (i + 1) * per):
                m = x_w[g, b]
                eo = jnp.where(mask2, m, pltpu.roll(pltpu.roll(m, 4, 0), 1, 1))
                a = pltpu.bitcast(eo << 16, f32)
                c = pltpu.bitcast(eo & jnp.uint32(0xFFFF0000), f32)
                if g == 0:
                    state["sh"] = jnp.where(top, jnp.broadcast_to(a[0:1], (8, 128)),
                                            jnp.broadcast_to(a[4:5], (8, 128)))
                a = a - state["sh"]
                c = c - state["sh"]
                c1_v[g, pl.ds(16 * b, 8, stride=2), :] = a
                c1_v[g, pl.ds(16 * b + 1, 8, stride=2), :] = c
                new = [a, c, a * a, c * c]
                state["acc"] = new if g == 0 else [p + q for p, q in zip(state["acc"], new)]
            if i == npc - 1:
                acc = state["acc"]
                s1, s2_ = acc[0] + acc[1], acc[2] + acc[3]
                for h in range(2):
                    m = jnp.sum(s1[4 * h:4 * h + 4], axis=0, keepdims=True) * (1.0 / D)
                    var = jnp.sum(s2_[4 * h:4 * h + 4], axis=0, keepdims=True) * (1.0 / D) - m * m
                    rs = 1.0 / _rb(jnp.sqrt(_rb(_rb(jnp.maximum(var, 0.0)) + EPS)))
                    s1_v[0, 2 * b + h] = jnp.broadcast_to(rs, (8, 128))
                    s1_v[1, 2 * b + h] = jnp.broadcast_to(m * rs, (8, 128))
                    fin_v[4, 2 * b + h:2 * b + h + 1, :] = state["sh"][4 * h:4 * h + 1]

        return [(functools.partial(piece, i), 1.0) for i in range(npc)]

    def s3_blk(k, b):
        g0 = k * NV
        et = []
        for h in range(2):
            c = c1_v[pl.ds(g0, NV), 16 * b + 8 * h:16 * b + 8 * h + 8, :]
            u = (c * s1_v[0, 2 * b + h] - s1_v[1, 2 * b + h]).reshape(R, 128)
            et.append(_dot(u, fmat(b % 2, h)))
        er, ei, tr, ti = et[0][:, :128], et[0][:, 128:], et[1][:, :128], et[1][:, 128:]
        if S4MODE[1] == "C":
            for q, v in enumerate((er, ei, tr, ti)):
                uh_v[k, b, q] = v
        else:
            for s, (pr, pi) in enumerate(((er + tr, ei + ti), (er - tr, ei - ti))):
                uh_v[k, b, 3 * s] = pr + pi
                uh_v[k, b, 3 * s + 1] = pi
                uh_v[k, b, 3 * s + 2] = pr

    s3 = lambda k: [(functools.partial(s3_blk, k, b), 1.0) for b in range(NB)]

    def s4_gen(k, n, groups=None):
        sl = slice(8 * n, 8 * n + 8)

        def utrip(i, s):
            if S4MODE[1] == "L":
                return [uh_v[k, i, 3 * s + q, sl, :] for q in range(3)]
            er, ei, tr, ti = [uh_v[k, i, q, sl, :] for q in range(4)]
            pr, pi = (er + tr, ei + ti) if s == 0 else (er - tr, ei - ti)
            return [pr + pi, pi, pr]

        prev = None
        done = 0
        if groups is not None and groups[0] > 0:
            prev = [(pv_v[n, 2 * h], pv_v[n, 2 * h + 1]) for h in range(2)]
        for b0 in (range(0, NB, TILE) if groups is None else groups):
            yy = []
            for s in range(2):
                acc = [None] * TILE
                win = {}
                for j in range(b0 + TILE):
                    if S4MODE[0] == "L":
                        kk = [kh_v[k, j, 3 * s + q, sl, :] for q in range(3)]
                    else:
                        kr, ki = kh_v[k, j, 3 * s, sl, :], kh_v[k, j, 3 * s + 1, sl, :]
                        kk = [kr, kr + ki, ki - kr]
                    for o in range(TILE - 1, -1, -1):
                        i = b0 + o - j
                        if i < 0:
                            continue
                        if i not in win:
                            win[i] = utrip(i, s)
                        p = [kk[q] * win[i][q] for q in range(3)]
                        acc[o] = p if acc[o] is None else [a + c for a, c in zip(acc[o], p)]
                        done += 1
                    if TILE == 4 and b0 == 4 and j == 2:
                        yield done
                yy.append([(a[0] - a[1], a[0] + a[2]) for a in acc])
                if s == 0:
                    yield done
            for o in range(TILE):
                p, q = yy[0][o], yy[1][o]
                cur = [(p[0] + q[0], p[1] + q[1]), (p[0] - q[0], p[1] - q[1])]
                for h in range(2):
                    if b0 + o == 0:
                        zr, zi = cur[h]
                    else:
                        zr = cur[h][0] - prev[h][1]
                        zi = cur[h][1] + prev[h][0]
                    zs_v[k, b0 + o, h, sl, 0:128] = zr
                    zs_v[k, b0 + o, h, sl, 128:256] = zi
                prev = cur
            if groups is not None and b0 + TILE < NB:
                for h in range(2):
                    pv_v[n, 2 * h] = prev[h][0]
                    pv_v[n, 2 * h + 1] = prev[h][1]
            yield done

    def s5_blk(k, b, h):
        g0 = k * NV
        t = 2 * b + h
        y = _dot_nt(zs_v[k, b, h], fmat(b % 2, h)).reshape(NV, 8, 128)
        hh = c1_v[pl.ds(g0, NV), 16 * b + 8 * h:16 * b + 8 * h + 8, :] + y
        c1_v[pl.ds(g0, NV), 16 * b + 8 * h:16 * b + 8 * h + 8, :] = hh
        wr = col_v[2, pl.ds(pl.multiple_of(k * R, 8), R), :].reshape(NV, 8, 128)
        rs = slice(8 * t, 8 * t + 8)
        acc_v[0, rs, :] = acc_v[0, rs, :] + jnp.sum(hh, axis=0)
        acc_v[1, rs, :] = acc_v[1, rs, :] + jnp.sum(hh * hh, axis=0)
        acc_v[2, rs, :] = acc_v[2, rs, :] + jnp.sum(hh * wr, axis=0)

    s5 = lambda k: [(functools.partial(s5_blk, k, b, h), 1.0) for b in range(NB) for h in range(2)]

    for c in c_par:
        c.wait()
    for k in range(2):
        _weave((s1n(k), 0.0, 0.2), (s1g(k), 0.2, 1.0))
    _weave((s1n(2), 0.0, 0.2), (s1g(2), 0.2, 1.0), (s2(0), 0.3, 1.0))
    s1_nat(3, 0, 1)
    c_x.wait()
    ln = [ln1_pieces(b, NPC) for b in range(NB)]
    s30 = s3(0)
    _weave((sum(ln, []), 0.0, P3F[0]), (s2(1), 0.0, P3F[2]),
           *[([s30[b]], max((b + 1.6) * P3F[0] / NB, P3F[3] + (1.0 - P3F[3]) * b / NB), 0.0) for b in range(NB)])
    for c in c_par2:
        c.wait()

    def body(k, do5=True, do4=True, do3=True, do2=True, do1=True, j=None):
        at = (lambda d: k + d) if j is None else (lambda d: j + (k + d) if k + d else j)
        g2 = s2_gen(at(2)) if do2 else None
        for n in range(NV):
            g4 = s4_gen(at(0), n) if do4 else None
            st4 = [0, 0]
            n4 = ORDER.count("4")

            def adv4(m):
                if not do4:
                    return
                st4[0] += 1
                while st4[1] < 72 * st4[0] / n4 - 3 or (st4[0] == n4 and st4[1] <= 72):
                    r = next(g4, None)
                    if r is None:
                        break
                    st4[1] = r

            def nat():
                if do1:
                    if n + 1 < NV:
                        s1_nat(at(3), n + 1, 1)
                    else:
                        s1_nat(jnp.minimum(at(4), NSTEP - 1), 0, 1)

            g1 = s1_grp(at(3), n) if do1 else None
            for tok in ORDER:
                if tok == "5":
                    if do5 and n < NB:
                        s5_blk(at(-1), n, 0)
                        s5_blk(at(-1), n, 1)
                elif tok == "4":
                    adv4(1)
                elif tok in "ab" and do1:
                    next(g1)
                elif tok == "p" and do1:
                    run(g1)
                elif tok == "2" and do2:
                    next(g2, None)
                elif tok == "3" and do3 and n < NB:
                    s3_blk(at(1), n)
                elif tok == "n":
                    nat()
        if do2:
            run(g2)

    @pl.when(flag_s[0] == 1)
    def _():
        body(0, do5=False)

    lax.fori_loop(0, 4, lambda j, c: (body(1, j=j), c)[1], 0)

    @pl.when(flag_s[0] == 1)
    def _():
        body(5, do1=False)

    @pl.when(flag_s[0] == 1)
    def _():
        body(6, do1=False, do2=False)

    @pl.when(flag_s[0] == 1)
    def _():
        _weave(([(lambda n=n: run(s4_gen(7, n, (0,))), 1.0) for n in range(NV)], 0.0, 1.0), (s5(6), 0.0, 1.0))

    @pl.when(flag_s[0] == 1)
    def _():
        _weave(([(lambda n=n: run(s4_gen(7, n, (4,))), 1.0) for n in range(NV)], 0.0, 1.0), (s5(7)[:8], 0.0, 1.0))

    _weave((s5(7)[8:], 0.0, 1.0))

    def total(i):
        halves = []
        for hf in range(2):
            t = acc_v[i, pl.ds(64 * hf, 8, stride=8), :]
            for s in range(1, 8):
                t = t + acc_v[i, pl.ds(64 * hf + s, 8, stride=8), :]
            halves.append(t)
        return jnp.concatenate(halves, 0)

    m2 = total(0) * (1.0 / D)
    var2 = jnp.maximum(total(1) * (1.0 / D) - m2 * m2, 0.0)
    sd2 = _rb(jnp.sqrt(_rb(_rb(var2) + EPS)))
    rs2 = 1.0 / sd2
    r = _rb((total(2) - m2 * wr_sum) * rs2)
    mean2 = fin_v[4] + m2
    fin_v[0] = rs2
    fin_v[1] = m2 * rs2
    fin_v[2] = rs2 + 1.0
    fin_v[3] = fin_v[4] - m2 * rs2

    tl = _iota((16, 128), 0)
    ll = _iota((16, 128), 1)
    lodd = (ll & 1) == 1
    toff = jnp.where((tl & 1) == 0, jnp.where(lodd, ll + 127, ll), jnp.where(lodd, ll + 128, (ll - 1) & 127))
    tok = (tl >> 1) * 256 + toff
    rbits = pltpu.bitcast(r, i32)
    srt = rbits ^ ((rbits >> 31) & 0x7FFFFFFF)
    key = pltpu.bitcast((((srt >> 16) + 32768) << 11) + (2047 - tok) + (1 << 28), f32)
    kk = key
    cand = []
    for _ in range(4):
        rm = jnp.broadcast_to(jnp.max(kk, axis=1, keepdims=True), (16, 128))
        cand.append(rm)
        kk = jnp.where(kk == rm, 0.0, kk)
    last = jnp.max(cand[3], axis=0, keepdims=True)
    kcol = None
    for j in range(TOPC):
        mx = jnp.max(cand[0], axis=0, keepdims=True)
        kcol = jnp.broadcast_to(mx, (8, 128)) if j == 0 else jnp.where(sub8 == j, mx, kcol)
        took = cand[0] == mx
        cand = [jnp.where(took, cand[i + 1] if i < 3 else 0.0, cand[i]) for i in range(4)]
    kc_v[...] = kcol

    @pl.when((last - mx)[0, 0] > 0.0)
    def _():
        k2 = key
        kc = None
        for j in range(TOPC):
            m1 = jnp.max(jnp.max(k2, axis=0, keepdims=True), axis=1, keepdims=True)
            kc = jnp.broadcast_to(m1, (8, 128)) if j == 0 else jnp.where(sub8 == j, m1, kc)
            k2 = jnp.where(k2 == m1, 0.0, k2)
        kc_v[...] = kc

    kcol = kc_v[...]
    kint = pltpu.bitcast(kcol, i32) - (1 << 28)
    tcol = 2047 - (kint & 2047)
    s16 = (kint >> 11) - 32768
    rsel = pltpu.bitcast((s16 ^ ((s16 >> 31) & 0x7FFF)) << 16, f32)
    gate = _rb(jax.nn.sigmoid(rsel))

    def classes(col):
        cls = jnp.zeros((8, 128), i32)
        for d in range(1, TOPC):
            cls = cls + jnp.where((col == pltpu.roll(col, d, 0)) & (sub8 >= d), 1, 0)
        return cls, jnp.max(cls, axis=0, keepdims=True)[0, 0] + 1

    wcol = tcol & 255
    pcol = jnp.where((wcol & 1) == 0, jnp.where(wcol < 128, wcol, wcol - 127),
                     jnp.where(wcol < 128, (wcol + 1) & 127, wcol - 128))
    ecol = ((tcol >> 8) << 1) | (tcol & 1)
    etile = [ecol[j, 0] for j in range(TOPC)]
    gcol, gn = classes(pcol)
    xs_v[...] = jnp.zeros((8, D), f32)

    def gather(c, carry):
        oh = (gcol == c) & (lane8 == pcol)
        ohi = jnp.where(oh, 1, 0)
        msk = [jnp.broadcast_to(ohi[j:j + 1], (8, 128)) == 1 for j in range(TOPC)]
        sa = sb = None
        for j in range(TOPC):
            fa = jnp.broadcast_to(fin_v[0, pl.ds(etile[j], 1), :], (8, 128))
            fb = jnp.broadcast_to(fin_v[1, pl.ds(etile[j], 1), :], (8, 128))
            sa, sb = (fa, fb) if j == 0 else (jnp.where(msk[j], fa, sa), jnp.where(msk[j], fb, sb))
        parts = []
        for q in range(D // 8 // GCH):
            mg = None
            for j in range(TOPC):
                cc = c1_v[GCH * q:GCH * q + GCH, pl.ds(pl.multiple_of(8 * etile[j], 8), 8), :]
                mg = cc if j == 0 else jnp.where(msk[j], cc, mg)
            parts.append(mg * sa - sb)
        ln = jnp.concatenate(parts, 0).reshape(D, 128)
        xs_v[...] = xs_v[...] + _dot_nt(jnp.where(oh, 1.0, 0.0).astype(f32), ln)
        return carry

    lax.fori_loop(0, gn, gather, 0)
    xsel = xs_v[...]

    def rebuilt_rows():
        sdc = jnp.zeros((8, 1), f32)
        mc = jnp.zeros((8, 1), f32)
        sub1 = _iota((8, 1), 0)
        for j in range(TOPC):
            hitm = tok == jnp.broadcast_to(tcol[j:j + 1], (16, 128))
            red = lambda v: jnp.sum(jnp.sum(jnp.where(hitm, v, 0.0), axis=0, keepdims=True), axis=1, keepdims=True)
            sdc = jnp.where(sub1 == j, red(sd2), sdc)
            mc = jnp.where(sub1 == j, red(mean2), mc)
        return xsel * (sdc + 1.0) + mc

    def outp(b, g0, g1):
        sc = [jnp.where(top, jnp.broadcast_to(fin_v[i, 2 * b:2 * b + 1, :], (8, 128)),
                        jnp.broadcast_to(fin_v[i, 2 * b + 1:2 * b + 2, :], (8, 128))) for i in (2, 3)]
        for g in range(g0, g1):
            a = _rb(c1_v[g, pl.ds(16 * b, 8, stride=2), :] * sc[0] + sc[1])
            c = _rb(c1_v[g, pl.ds(16 * b + 1, 8, stride=2), :] * sc[0] + sc[1])
            w = (pltpu.bitcast(a, u32) >> 16) | pltpu.bitcast(c, u32)
            out_w[g, b] = jnp.where(mask2, w, pltpu.roll(pltpu.roll(w, 4, 0), 127, 1))

    opieces = [functools.partial(outp, b, 24 * i, 24 * i + 24) for b in range(NB) for i in range(3)]

    tilec = tcol >> 7
    lanec = tcol & 127
    aux = {}

    def late_scalars():
        tiles = [tilec[j, 0] for j in range(TOPC)]
        hit = 0
        dup = []
        for j in range(TOPC):
            dup.append((hit >> tiles[j]) & 1)
            hit = hit | (1 << tiles[j])
        free, cnt = [], 0
        for t in range(16):
            un = 1 - ((hit >> t) & 1)
            free.append(jnp.where(un == 1, cnt, -1))
            cnt = cnt + un
        late, nd, mask = [tiles[0]], 0, hit
        for j in range(1, TOPC):
            rep = 0
            for t in range(16):
                rep = jnp.where(free[t] == nd, t, rep)
            late.append(jnp.where(dup[j] == 1, rep, tiles[j]))
            mask = mask | (1 << late[j])
            nd = nd + dup[j]
        aux.update(tiles=tiles, late=late, mask=mask)
        bs_v[...] = rebuilt_rows()
        aux["clscol"], aux["ncls"] = classes(lanec)
        for j in range(TOPC):
            code = jnp.where((tilec == late[j]) & (lane8 == lanec), aux["clscol"], -1)
            lm_v[j] = jnp.broadcast_to(jnp.max(code, axis=0, keepdims=True), (8, 128))

    def tile_idx(t, g0=0, ng=D // 8):
        if isinstance(t, int):
            return (pl.ds(g0, ng), t // 2, pl.ds(8 * (t % 2), 8), slice(None))
        return (pl.ds(g0, ng), t >> 1, pl.ds(pl.multiple_of(8 * (t & 1), 8), 8), slice(None))

    def ocopy(idx):
        return cp(out_v.at[idx], out_h.at[idx], osem.at[0])

    for c in range(NCH):
        for cc in c_w[c]:
            cc.wait()
        mine = opieces[OSPLIT[c]:OSPLIT[c + 1]]
        nsub = max(1, FCH[c] // FSUB)
        sub = FCH[c] // nsub
        for u in range(nsub):
            sl = slice(FOFF[c] + u * sub, FOFF[c] + (u + 1) * sub)
            g = _rb(_dot(xsel, wmat(wg_w, 0, D, sl.start, sub)))
            up = _rb(_dot(xsel, wmat(wu_w, 0, D, sl.start, sub)))
            if c == 0 and u == 0:
                late_scalars()
            for fn in mine[u * len(mine) // nsub:(u + 1) * len(mine) // nsub]:
                fn()
            act_v[:, sl] = _rb(_rb(g * jax.nn.sigmoid(g)) * up)

    def early():
        for t in range(16):
            @pl.when(((aux["mask"] >> t) & 1) == 0)
            def _():
                ocopy(tile_idx(t)).start()

    clscol = aux["clscol"]
    onehot = lambda c: jnp.where((clscol == c) & (lane8 == lanec), 1.0, 0.0).astype(f32)
    bc = lambda v, j: jnp.broadcast_to(v[j:j + 1], (8, 128))

    def down(p, c0, nc):
        r = slice(POFF[p], POFF[p] + PART[p])
        yc = _dot_nt(act_v[:, c0:c0 + nc], wmat(wd_w, POFF[p], PART[p], c0, nc))
        y_v[:, r] = yc if c0 == 0 else y_v[:, r] + yc

    def place(p, fast):
        r0, nr = POFF[p], PART[p]
        g0, ng = r0 // 8, nr // 8
        gt = jnp.concatenate([gate] * ((nr + 127) // 128), 1)[:, :nr]
        newrow = _rb(bs_v[:, r0:r0 + nr] + _rb(_rb(y_v[:, r0:r0 + nr]) * gt))
        tn = lambda oh: lax.dot_general(newrow, oh, (((0,), (0,)), ((), ())), preferred_element_type=f32)
        if fast:
            uu = tn(jnp.concatenate([onehot(0), onehot(1)], 1))
            for c in range(2):
                u_v[c, g0:g0 + ng] = uu[:, 128 * c:128 * (c + 1)].reshape(ng, 8, 128)
        else:
            for c in range(TOPC):
                u_v[c, g0:g0 + ng] = tn(onehot(c)).reshape(ng, 8, 128)

    def write(p, fast):
        g0, ng = POFF[p] // 8, PART[p] // 8
        for j in range(TOPC):
            idx = tile_idx(aux["late"][j], g0, ng)
            new = out_v[idx].astype(f32)
            code = lm_v[j]
            for c in range(2 if fast else TOPC):
                new = jnp.where(code == c, u_v[c, g0:g0 + ng], new)
            sg_v[j, g0:g0 + ng] = new.astype(bf16)
            cp(sg_v.at[j, pl.ds(g0, ng)], out_h.at[idx], osem.at[0]).start()

    def dwait(p):
        for cc in c_d[p]:
            cc.wait()

    NP = len(PART)
    if WSTART == 0:
        early()
    dwait(0)
    rest = opieces[OSPLIT[NCH]:]
    nq = 4
    for q in range(nq):
        down(0, q * F // nq, F // nq)
        for fn in rest[q * len(rest) // nq:(q + 1) * len(rest) // nq]:
            fn()
    if WSTART == 1:
        early()

    @pl.when(aux["ncls"] <= 2)
    def _():
        for p in range(1, NP):
            dwait(p)
            down(p, 0, DSPL[p])
            place(p - 1, True)
            down(p, DSPL[p], F - DSPL[p])
            write(p - 1, True)
        place(NP - 1, True)
        write(NP - 1, True)

    @pl.when(aux["ncls"] > 2)
    def _():
        for p in range(1, NP):
            dwait(p)
            down(p, 0, F)
        for p in range(NP):
            place(p, False)
            write(p, False)

    cp(out_h, out_h, osem.at[0]).wait()


@jax.jit
def pallas_sequential_preLN__ssm_conv_s4__moe_arch_mod__prompt_kernel(
    A_u: jax.Array,
    A_A_re: jax.Array,
    A_A_im: jax.Array,
    A_B_re: jax.Array,
    A_B_im: jax.Array,
    A_C_re: jax.Array,
    A_C_im: jax.Array,
    A_log_dt: jax.Array,
    A_Dskip: jax.Array,
    B_x: jax.Array,
    B_w_r: jax.Array,
    B_w_gate: jax.Array,
    B_w_up: jax.Array,
    B_w_down: jax.Array,
):
    hbm = pl.BlockSpec(memory_space=pltpu.MemorySpace.HBM)
    vm = pltpu.VMEM
    G8 = D // 8
    wshape = (D // 16, F // 128, 16, 128)
    wview = lambda w: w.reshape(D // 16, 2, 8, F // 128, 128).transpose(0, 1, 3, 2, 4)
    scratch = [
        vm((G8, NB, 16, 128), bf16), vm((6, D, N), bf16), vm((D,), bf16), vm((D,), bf16), vm((D,), bf16),
        vm(_CTAB.shape, f32), vm(wshape, bf16), vm(wshape, bf16), vm(wshape, bf16), vm((G8, NB + 1, 16, 128), bf16),
        vm((10, 4, 144, 128), bf16), vm((2, 2, 2, 144, 128), bf16), vm((3, D + 8, 128), f32),
        vm((NV, 2, 136, 128), f32), vm((NSTEP, NV, 56, 128), f32), vm((NSTEP, R, 128), f32),
        vm((NSTEP, NB, 6, R, 128), f32), vm((NSTEP, NB, 6, R, 128), f32),
        vm((NSTEP, NB, 2, R, 256), f32), vm((G8, 136, 128), f32), vm((2, 17, 8, 128), f32),
        vm((3, 136, 128), f32), vm((5, 16, 128), f32), vm((TOPC, G8, 8, 128), f32),
        vm((R, 512), f32), vm((8, D), f32), vm((NV, 4, 8, 128), f32),
        vm((8, 128), f32), vm((8, D), f32), vm((8, D), f32), vm((8, F), f32),
        vm((TOPC, G8, 8, 128), bf16), vm((TOPC, 8, 128), i32), pltpu.SMEM((1,), i32),
        pltpu.SemaphoreType.DMA((5 + NCH + len(PART),)), pltpu.SemaphoreType.DMA((1,)),
    ]
    xv = A_u[0].T.reshape(G8, 8, 16, 128).transpose(0, 2, 1, 3).reshape(G8, NB, 16, 128)
    out = pl.pallas_call(
        _kernel,
        out_shape=jax.ShapeDtypeStruct((G8, NB, 16, 128), bf16),
        in_specs=[hbm] * 14,
        out_specs=hbm,
        scratch_shapes=scratch,
        compiler_params=pltpu.CompilerParams(vmem_limit_bytes=120 * 1024 * 1024, disable_bounds_checks=NOBC),
    )(xv, A_A_re, A_A_im, A_B_re, A_B_im, A_C_re, A_C_im, A_log_dt, A_Dskip, B_w_r,
      wview(B_w_gate), wview(B_w_up), wview(B_w_down.T), jnp.asarray(_CTAB))
    return out.reshape(G8, 16, 8, 128).transpose(0, 2, 1, 3).reshape(D, L).T[None]
```

```python
import functools

import numpy as np
import jax
import jax.numpy as jnp
from jax import lax
import jax.experimental.pallas as pl
import jax.experimental.pallas.tpu as pltpu

f32 = jnp.float32
bf16 = jnp.bfloat16
i32 = jnp.int32
u32 = jnp.uint32

L, D, N, F, TOPC = 2048, 576, 128, 4608, 8
NB = 8
NV = 9
R = NV * 8
NSTEP = D // R
EPS = 1e-5

_XL1 = [(1, 5), (2, 6), (3, 7), (4, 8), (258, 516), (260, 520), (262, 772), (264, 776),
        (1288, 1032), (1800, 1544)]
_XSH = [0, 1, 2, 3, 0, 1, 2, 3, 0, 1]


def _bf16_round_int(j):
    u = np.asarray(j, np.float32).view(np.uint32).astype(np.uint64)
    r = ((u + 0x7FFF + ((u >> 16) & 1)) >> 16) << 16
    return r.astype(np.uint32).view(np.float32).astype(np.int64)


def _chunk_values():
    vals = -np.ones((5, 128), np.int64)
    for j in range(10):
        for p in range(2):
            ch = (j // 4) * 2 + p if j < 8 else 4
            extra = 2 * p if j >= 8 else 0
            for l0 in range(32):
                vals[ch, (4 * (31 - l0) + 4 * p + _XSH[j] + extra + 8) % 128] = _XL1[j][p] + 8 * l0
    assert (vals >= 0).all()
    return vals


_PASSES = [(0, "A0"), (0, "A1"), (1, "B"), (2, "Cp"), (3, "C"), (4, "Dp"), (5, "D"), (6, "D"), (7, "D")]
_SETS = [[0], [1], [2], [3, 4], [5, 6, 7, 8]]


def _tables():
    cv = _chunk_values()
    cvp = {"A0": cv[0], "A1": cv[1], "B": cv[2], "C": cv[3], "D": cv[4]}
    cvp["Cp"] = cv[3].copy(); cvp["Cp"][11] = cv[2][11]
    cvp["Dp"] = cv[4].copy(); cvp["Dp"][15] = cv[3][15]
    sup = [[[] for _ in range(128)] for _ in _PASSES]
    for b in range(NB):
        for j in range(1, 257):
            lag = 256 * b + j
            if lag > L - 1 or lag == 257:
                continue
            v = int(_bf16_round_int(lag))
            hit = [(i, int(np.nonzero(cvp[nm] == v)[0][0])) for i, (pb, nm) in enumerate(_PASSES)
                   if pb == b and (cvp[nm] == v).any()]
            assert len(hit) == 1, (b, j, v, hit)
            sup[hit[0][0]][hit[0][1]].append(j)
    assert cv[1][15] == _bf16_round_int(257)
    code = np.zeros((len(_PASSES), 128), np.int64)
    for i, (pb, _) in enumerate(_PASSES):
        for r in range(128):
            js = sup[i][r]
            if js:
                assert js == list(range(js[0], js[-1] + 1))
                code[i, r] = js[0] + js[-1] + 1024 * len(js) + 16384 * (pb % 2)
    seeds, masks = [], {}
    for ps in _SETS:
        seeds.append([int(x) for x in sum(code[i, 16:24] for i in ps)])
        for i in ps:
            masks[i] = [int(x > 0) for x in code[i, 16:24]]
            for v in range(2, 17):
                r0 = 8 * (v % 16)
                assert (code[i, r0:r0 + 8] == (np.array(seeds[-1]) - 32 * (v - 2)) * np.array(masks[i])).all()
    return seeds, [[int(x) for x in code[i, 8:16]] for i in range(len(_PASSES))], masks


_GSEED, _GROW1, _GMASK = _tables()


def _sincos_coeffs():
    r = np.cos(np.pi * (np.arange(4000) + .5) / 4000) * 0.5
    z = r * r
    s = np.linalg.lstsq(np.stack([z ** k for k in range(4)], 1), np.sin(np.pi / 2 * r) / r, rcond=None)[0]
    c = np.linalg.lstsq(np.stack([z ** k for k in range(1, 5)], 1), np.cos(np.pi / 2 * r) - 1, rcond=None)[0]
    return [float(x) for x in s], [float(x) for x in c]


_SC, _CC = _sincos_coeffs()


def _cmul(a, b):
    return (a[0] * b[0] - a[1] * b[1], a[0] * b[1] + a[1] * b[0])


def _cmulc(a, b):
    return (a[0] * b[0] + a[1] * b[1], a[1] * b[0] - a[0] * b[1])


def _csq(a):
    return ((a[0] - a[1]) * (a[0] + a[1]), (a[0] + a[0]) * a[1])


def _quarter_polys(r):
    r2 = r * r
    s = r * (_SC[0] + r2 * (_SC[1] + r2 * (_SC[2] + r2 * _SC[3])))
    c = 1.0 + r2 * (_CC[0] + r2 * (_CC[1] + r2 * (_CC[2] + r2 * _CC[3])))
    return s, c


def _rotate_quadrant(s, c, ki):
    swap = (ki & 1) == 1
    s2 = jnp.where(swap, c, s)
    c2 = jnp.where(swap, s, c)
    s2 = pltpu.bitcast(pltpu.bitcast(s2, i32) ^ ((ki & 2) << 30), f32)
    c2 = pltpu.bitcast(pltpu.bitcast(c2, i32) ^ (((ki + 1) & 2) << 30), f32)
    return s2, c2


def _sincos(th):
    z = th * (2.0 / np.pi)
    k = jnp.round(z)
    s, c = _quarter_polys(z - k)
    return _rotate_quadrant(s, c, k.astype(i32))


def _reduce_small(z):
    big = 12582912.0
    t = z + big
    return _quarter_polys(z - (t - big)) + (pltpu.bitcast(t, i32),)


def _rb(x):
    return x.astype(bf16).astype(f32)


def _dot(a, b):
    return jnp.dot(a, b, preferred_element_type=f32)


def _dot_nt(a, b):
    return lax.dot_general(a, b, (((1,), (1,)), ((), ())), preferred_element_type=f32)


def _iota(shape, dim):
    return lax.broadcasted_iota(i32, shape, dim)


S4MODE='CC'
TILE=4
YSPLIT=1
ZT=1
ORDER='4ab44342np445'
ORD0='4ab442n4p4345'
ORD5='4a424n44b345p'
ORD6='45a4b244p3n44'
NPC=3
P3F=(0.9,0.4,0.55,0.3)
GCH=3
NOBC=True
CT_ROWS=320
PART=(256,128,128,64)
DSPL=(0,2560,2560,4096)
FSUB=1536
FCH=(3072,1536)
OSPLIT=[0,24,24]
WCH=0
NCH = len(FCH)
FOFF = [sum(FCH[:i]) for i in range(NCH)]
POFF = [sum(PART[:i]) for i in range(len(PART))]

def _weave(*streams):
    items = []
    for si, (pieces, lo, hi) in enumerate(streams):
        tot = float(sum(c for _, c in pieces))
        cum = 0.0
        for pi, (fn, c) in enumerate(pieces):
            items.append((lo + max(hi - lo, 0.0) * (cum + 0.5 * c) / tot, si, pi, fn))
            cum += c
    for _, _, _, fn in sorted(items, key=lambda t: t[:3]):
        fn()


def _kernel(x_h, are_h, aim_h, bre_h, bim_h, cre_h, cim_h, ldt_h, dsk_h, wr_h, wg_h, wu_h, wd_h,
            out_h,
            x_v, par_v, ldt_v, dsk_v, wr_v, ct_v, wg_v, wu_v, wd_v, out_v,
            g_v, f_v, col_v, st_v, kd_v, k0_v, kh_v, uh_v, zs_v, c1_v, s1_v, acc_v, fin_v, u_v, zt_v, y_v, pv_v, kc_v, xs_v, bs_v, act_v, sg_v, lm_v, rw_v, flag_s,
            sem, osem):
    cp = pltpu.make_async_copy
    c_vec = [cp(ldt_h, ldt_v, sem.at[1]), cp(dsk_h, dsk_v, sem.at[1]), cp(wr_h, wr_v, sem.at[1])]
    PH = 4 * R
    par_h = (are_h, aim_h, bre_h, bim_h, cre_h, cim_h)
    c_par = [cp(h.at[pl.ds(0, PH)], par_v.at[i, pl.ds(0, PH)], sem.at[2]) for i, h in enumerate(par_h)]
    c_par2 = [cp(h.at[pl.ds(PH, D - PH)], par_v.at[i, pl.ds(PH, D - PH)], sem.at[3])
              for i, h in enumerate(par_h)]
    c_x = cp(x_h, x_v, sem.at[4])
    def wcp(h, v, rp, ct, s):
        return [cp(h.at[rp, hf, ct], v.at[rp, ct, pl.ds(8 * hf, 8), :], s) for hf in range(2)]

    c_w = [wcp(wg_h, wg_v, slice(None), pl.ds(FOFF[c] // 128, FCH[c] // 128), sem.at[5 + c])
           + wcp(wu_h, wu_v, slice(None), pl.ds(FOFF[c] // 128, FCH[c] // 128), sem.at[5 + c]) for c in range(NCH)]
    c_d = [wcp(wd_h, wd_v, pl.ds(POFF[p] // 16, PART[p] // 16), slice(None), sem.at[5 + NCH + p])
           for p in range(len(PART))]
    for c in c_vec + c_par + [c_x] + c_par2 + sum(c_w, []) + sum(c_d, []):
        c.start()

    flag_s[0] = 1
    x_w = x_v.bitcast(u32)
    wg_w, wu_w, wd_w = wg_v.bitcast(u32), wu_v.bitcast(u32), wd_v.bitcast(u32)

    def wmat(w, r0, nr, c0, nc):
        return jnp.concatenate([pltpu.bitcast(w[r0 // 16:(r0 + nr) // 16, t], bf16).reshape(nr, 128)
                                for t in range(c0 // 128, (c0 + nc) // 128)], 1)

    out_w = out_v.bitcast(u32)
    g_w = g_v.bitcast(u32)
    f_w = f_v.bitcast(u32)
    sub8 = _iota((8, 128), 0)
    lane8 = _iota((8, 128), 1)

    acc_v[...] = jnp.zeros(acc_v.shape, f32)
    for n in range(NV):
        for ri in range(2):
            st_v[n, ri, 104:112, :] = jnp.full((8, 128), 1.0 - ri, f32)
    kp = (2 * lane8 + 1).astype(f32)

    def rows_const(vals):
        out = jnp.full((8, 128), vals[0], i32)
        for r in range(1, 8):
            if vals[r] != vals[0]:
                out = jnp.where(sub8 == r, vals[r], out)
        return out

    def phasor(z):
        sn, cs = _rotate_quadrant(*_reduce_small(-z))
        return cs, sn

    NS = [0, 1, 2, 3, 4, 5, 7, 9]
    for q in range(2):
        sn = _rotate_quadrant(*_reduce_small((kp + 512.0 * q) * (rows_const(NS).astype(f32) * (1.0 / 512))))[0]
        ct_v[304 + 8 * q:312 + 8 * q, :] = sn / (256.0 * jnp.broadcast_to(sn[1:2], (8, 128)))

    def grows(vals):
        ab = rows_const([v & 1023 for v in vals])
        z = kp * (ab.astype(f32) * (-1.0 / 512))
        if any(v >> 14 for v in vals):
            z = z - rows_const([v >> 14 for v in vals]).astype(f32) * (kp - 1.0)
        sn, cs, ki = _reduce_small(z)
        ns = [NS.index((v >> 10) & 15) for v in vals]
        out = []
        for q in range(2):
            row = lambda i: jnp.broadcast_to(ct_v[304 + 8 * q + i:305 + 8 * q + i, :], (8, 128))
            amp = None
            for i in sorted(set(ns)):
                bits = sum(1 << r for r in range(8) if ns[r] == i)
                amp = row(i) if amp is None else jnp.where(((bits >> sub8) & 1) == 1, row(i), amp)
            pi, pr = _rotate_quadrant(sn, cs, ki if q == 0 else ki - ab)
            out += [pr * amp, pi * amp]
        return out

    for v4 in range(4):
        e = phasor(kp * ((sub8 + 8 * v4).astype(f32) * (1.0 / 32)))
        ct_v[8 * v4:8 * v4 + 8, :] = e[0]
        ct_v[32 + 8 * v4:40 + 8 * v4, :] = e[1]
    for si in range(5):
        for q, val in enumerate(grows(_GSEED[si])):
            ct_v[64 + 32 * si + 8 * q:72 + 32 * si + 8 * q, :] = val
    for i in range(len(_PASSES)):
        for q, val in enumerate(grows(_GROW1[i])):
            g_v[i, q, 8:16, :] = val.astype(bf16)
    for q, val in enumerate(grows([2 + 1024 + 16384] * 8)):
        ct_v[272 + 8 * q:280 + 8 * q, :] = val
    s8 = np.arange(8)
    je = np.where(s8 % 2 == 0, s8, 127 + s8)
    jo = np.where(s8 % 2 == 0, s8 - 1, 128 + s8)
    for t, jj in enumerate((je, jo, jo % 128 + 128 * (s8 % 2))):
        e = phasor(kp * (rows_const([int(x) for x in jj]).astype(f32) * (1.0 / 256)))
        ct_v[224 + 16 * t:232 + 16 * t, :] = e[0]
        ct_v[232 + 16 * t:240 + 16 * t, :] = e[1]
    for c in c_vec:
        c.wait()

    rows = [_rb(jnp.exp(ldt_v[...].astype(f32).reshape(1, D))),
            dsk_v[...].astype(f32).reshape(1, D),
            wr_v[...].astype(f32).reshape(1, D)]
    wr_sum = jnp.sum(rows[2], axis=1, keepdims=True)

    def columns(which):
        for j in range(5):
            w = 128 if j < 4 else 64
            eye = _iota((w, w), 0) == _iota((w, w), 1)
            m = jnp.concatenate([jnp.where(eye, jnp.broadcast_to(rw_v[i:i + 1, j * 128:j * 128 + w], (w, w)), 0.0)
                                 for i in which], 0)
            res = _dot(m, jnp.ones((w, 128), f32))
            for n, i in enumerate(which):
                col_v[i, j * 128:j * 128 + w, :] = res[n * w:(n + 1) * w]

    for i in range(3):
        rw_v[i:i + 1, :] = rows[i]
    columns((0,))

    def e8(v):
        return (jnp.broadcast_to(ct_v[v:v + 1, :], (8, 128)), jnp.broadcast_to(ct_v[32 + v:33 + v, :], (8, 128)))

    for si, ps in enumerate(_SETS):
        sd = [ct_v[64 + 32 * si + 8 * q:72 + 32 * si + 8 * q, :] for q in range(4)]
        mk = {}
        for i in ps:
            if len(ps) > 1:
                bits = sum(b << s for s, b in enumerate(_GMASK[i]))
                mk[i] = ((bits >> sub8) & 1) == 1
        for v in range(2, 17):
            if v == 2:
                vals = sd
            else:
                ev = e8(2 * (v - 2))
                vals = list(_cmulc((sd[0], sd[1]), ev)) + list(_cmulc((sd[2], sd[3]), ev))
            for i in ps:
                for q in range(4):
                    val = vals[q] if len(ps) == 1 else jnp.where(mk[i], vals[q], 0.0)
                    g_v[i, q, 8 * (v % 16):8 * (v % 16) + 8, :] = val.astype(bf16)
    sig = jnp.where((lane8 & 1) == 0, 1.0, -1.0).astype(f32)
    for h in range(2):
        sd = (ct_v[224 + 16 * h:232 + 16 * h, :], ct_v[232 + 16 * h:240 + 16 * h, :])
        for v in range(16):
            if v == 0:
                vals = sd if h == 0 else (ct_v[256:264, :], ct_v[264:272, :])
            else:
                vals = _cmul(sd, e8(v))
            for q in range(2):
                f_v[0, h, q, 8 * v:8 * v + 8, :] = vals[q].astype(bf16)
                f_v[1, h, q, 8 * v:8 * v + 8, :] = (vals[q] * sig).astype(bf16)

    def gmat(i):
        return jnp.concatenate([pltpu.bitcast(g_w[i, q, 0:64, :], bf16) for q in range(4)], 1)

    def fmat(ver, h):
        return jnp.concatenate([pltpu.bitcast(f_w[ver, h, q, 0:64, :], bf16) for q in range(2)], 1)

    revmask = (sub8 & 2) == 0
    lm = lane8 & 3

    def s1_nat(k, n0, nn):
        row0 = pl.multiple_of(k * R + 8 * n0, 8)
        rr = 8 * nn
        ld = lambda i: par_v[i, pl.ds(row0, rr), :].astype(f32)
        dt = col_v[0, pl.ds(row0, rr), :]
        e = jnp.exp(dt * ld(0))
        s, c = _sincos(dt * ld(1))
        a1 = (e * c, e * s)
        w = _cmul((ld(4), ld(5)), (dt * ld(2), dt * ld(3)))
        k0_v[k, 8 * n0:8 * n0 + rr, :] = jnp.broadcast_to(jnp.sum(w[0], axis=1, keepdims=True), (rr, 128))
        w = (w[0], -w[1])
        rev = lambda v: jnp.where(revmask, pltpu.roll(v, 2, 0), pltpu.roll(v, 6, 0))

        def put(arr, slots, fn=None):
            for n in range(nn):
                for ri in range(2):
                    v = arr[ri][8 * n:8 * n + 8]
                    if fn is not None:
                        v = fn(v)
                    for q in slots:
                        st_v[n0 + n, ri, q * 8:q * 8 + 8, :] = v

        put(w, (0, 1)); put(a1, (2, 3))
        a2 = _csq(a1); put(a2, (5,))
        a4 = _csq(a2); put(a4, (6,))
        put(_cmul(a4, a1), (4,))
        a8 = _csq(a4); put(a8, (12,), rev)
        t = _csq(a8); put(t, (14, 15), rev)
        for _ in range(4):
            t = _csq(t)
        put(t, (7, 11))
        t = _csq(t); put(t, (8, 9))
        put(_csq(t), (10,))

    def s1_grp(k, n):
        mix = lambda q: tuple(jnp.concatenate([st_v[n, ri, pl.ds(q * 8 + g, 8, stride=2), :] for g in range(2)], 0)
                              for ri in range(2))
        y = [mix(12)]
        a16d = mix(14)
        if YSPLIT == 1:
            for _ in range(15):
                y.append(_cmul(y[-1], a16d))
        else:
            y.append(_cmul(y[0], a16d))
            a32d = _csq(a16d)
            for i in range(2, 16):
                y.append(_cmul(y[i - 2], a32d))
        yield
        wd = mix(0); a1d = mix(2); m1 = mix(5)
        v = [_cmulc(wd, mix(3))]
        for _ in range(3):
            v.append(_cmulc(v[-1], a1d))
        v4 = _cmulc(_cmulc(wd, m1), mix(7))
        v5 = _cmulc(v4, m1); v6 = _cmulc(v4, mix(6)); v7 = _cmulc(v6, m1)
        v8 = _cmulc(v7, mix(10)); v9 = _cmulc(v8, mix(8))
        v += [v4, v5, v6, v7, v8, v9]
        os_ = []
        for g in range(2):
            cat = lambda ts: jnp.concatenate([jnp.concatenate([t[ri][8 * g:8 * g + 8] for t in ts], 0)
                                              for ri in range(2)], 1)
            os_.append(_dot_nt(cat(v), cat(y[::-1])))
        yield
        for g in range(2):
            o = os_[g]
            ro = [pltpu.roll(o[8 * j:8 * j + 8], _XSH[j] + 5, 1, stride=1, stride_axis=0) for j in range(10)]
            sel4 = lambda q: jnp.where(lm == 0, q[0], jnp.where(lm == 1, q[1], jnp.where(lm == 2, q[2], q[3])))
            kd_v[k, n, pl.ds(g, 8, stride=2), :] = sel4(ro[0:4])
            kd_v[k, n, pl.ds(16 + g, 8, stride=2), :] = sel4(ro[4:8])
            kd_v[k, n, pl.ds(32 + g, 8, stride=2), :] = jnp.where(lm == 0, ro[8], ro[9])

    def run(gen):
        for _ in gen:
            pass

    s1n = lambda k: [(functools.partial(s1_nat, k, 3 * i, 3), 1.0) for i in range(3)]
    s1g = lambda k: [(lambda n=n: run(s1_grp(k, n)), 1.0) for n in range(NV)]

    laneR = _iota((R, 128), 1)
    lmR = laneR & 3

    def s2_gen(k):
        ch = lambda c: kd_v[k, :, 8 * c:8 * c + 8, :].reshape(R, 128)
        for b in range(NB):
            if b == 0:
                k0 = (k0_v[k] + col_v[1, pl.ds(pl.multiple_of(k * R, 8), R), :]) * (1.0 / 256.0)
                z = _dot(ch(0), gmat(0)) if ZT else None
                dd = jnp.where(lmR < 2, ch(4), pltpu.roll(ch(5), 2, 1))
                kd_v[k, :, 48:56, :] = dd.reshape(NV, 8, 128)
                if ZT:
                    zt_v[...] = z
                    yield
                    z = _dot(ch(1), gmat(1)) + zt_v[...]
                else:
                    z = _dot(jnp.concatenate([ch(0), ch(1)], 1), jnp.concatenate([gmat(0), gmat(1)], 0))
            elif b == 1:
                k256 = jnp.sum(jnp.where(laneR == 15, ch(1), 0.0), axis=1, keepdims=True)
                pat = jnp.concatenate([ct_v[272 + 8 * q:273 + 8 * q, :] for q in range(4)], 1)
                z = _dot(ch(2), gmat(2)) + k256 * pat
            elif b == 2:
                z = _dot(jnp.where(laneR == 11, ch(2), ch(3)), gmat(3))
            elif b == 3:
                z = _dot(ch(3), gmat(4))
            elif b == 4:
                z = _dot(jnp.where(laneR == 15, ch(3), ch(6)), gmat(5))
            else:
                z = _dot(ch(6), gmat(b + 1))
            for s in range(2):
                kr = z[:, 256 * s:256 * s + 128]
                ki = z[:, 256 * s + 128:256 * s + 256]
                if b == 0:
                    kr = kr + k0
                kh_v[k, b, 3 * s] = kr
                if S4MODE[0] == "L":
                    kh_v[k, b, 3 * s + 1] = kr + ki
                    kh_v[k, b, 3 * s + 2] = ki - kr
                else:
                    kh_v[k, b, 3 * s + 1] = ki
            yield

    def s2(k):
        gen = s2_gen(k)
        return [(lambda: next(gen, None), 1.0) for _ in range(9)]

    mask2 = (sub8 < 4) == ((lane8 & 1) == 0)
    top = sub8 < 4

    def ln1_pieces(b, npc):
        state = {}
        per = (D // 8) // npc

        def piece(i):
            for g in range(i * per, (i + 1) * per):
                m = x_w[g, b]
                eo = jnp.where(mask2, m, pltpu.roll(pltpu.roll(m, 4, 0), 1, 1))
                a = pltpu.bitcast(eo << 16, f32)
                c = pltpu.bitcast(eo & jnp.uint32(0xFFFF0000), f32)
                if g == 0:
                    state["sh"] = jnp.where(top, jnp.broadcast_to(a[0:1], (8, 128)),
                                            jnp.broadcast_to(a[4:5], (8, 128)))
                a = a - state["sh"]
                c = c - state["sh"]
                c1_v[g, pl.ds(16 * b, 8, stride=2), :] = a
                c1_v[g, pl.ds(16 * b + 1, 8, stride=2), :] = c
                new = [a, c, a * a, c * c]
                state["acc"] = new if g == 0 else [p + q for p, q in zip(state["acc"], new)]
            if i == npc - 1:
                acc = state["acc"]
                s1, s2_ = acc[0] + acc[1], acc[2] + acc[3]
                for h in range(2):
                    m = jnp.sum(s1[4 * h:4 * h + 4], axis=0, keepdims=True) * (1.0 / D)
                    var = jnp.sum(s2_[4 * h:4 * h + 4], axis=0, keepdims=True) * (1.0 / D) - m * m
                    rs = 1.0 / _rb(jnp.sqrt(_rb(_rb(jnp.maximum(var, 0.0)) + EPS)))
                    s1_v[0, 2 * b + h] = jnp.broadcast_to(rs, (8, 128))
                    s1_v[1, 2 * b + h] = jnp.broadcast_to(m * rs, (8, 128))
                    fin_v[4, 2 * b + h:2 * b + h + 1, :] = state["sh"][4 * h:4 * h + 1]

        return [(functools.partial(piece, i), 1.0) for i in range(npc)]

    def s3_blk(k, b):
        g0 = k * NV
        et = []
        for h in range(2):
            c = c1_v[pl.ds(g0, NV), 16 * b + 8 * h:16 * b + 8 * h + 8, :]
            u = (c * s1_v[0, 2 * b + h] - s1_v[1, 2 * b + h]).reshape(R, 128)
            et.append(_dot(u, fmat(b % 2, h)))
        er, ei, tr, ti = et[0][:, :128], et[0][:, 128:], et[1][:, :128], et[1][:, 128:]
        if S4MODE[1] == "C":
            for q, v in enumerate((er, ei, tr, ti)):
                uh_v[k, b, q] = v
        else:
            for s, (pr, pi) in enumerate(((er + tr, ei + ti), (er - tr, ei - ti))):
                uh_v[k, b, 3 * s] = pr + pi
                uh_v[k, b, 3 * s + 1] = pi
                uh_v[k, b, 3 * s + 2] = pr

    s3 = lambda k: [(functools.partial(s3_blk, k, b), 1.0) for b in range(NB)]

    def s4_gen(k, n, groups=None):
        sl = slice(8 * n, 8 * n + 8)

        def utrip(i, s):
            if S4MODE[1] == "L":
                return [uh_v[k, i, 3 * s + q, sl, :] for q in range(3)]
            er, ei, tr, ti = [uh_v[k, i, q, sl, :] for q in range(4)]
            pr, pi = (er + tr, ei + ti) if s == 0 else (er - tr, ei - ti)
            return [pr + pi, pi, pr]

        prev = None
        done = 0
        if groups is not None and groups[0] > 0:
            prev = [(pv_v[n, 2 * h], pv_v[n, 2 * h + 1]) for h in range(2)]
        for b0 in (range(0, NB, TILE) if groups is None else groups):
            yy = []
            for s in range(2):
                acc = [None] * TILE
                win = {}
                for j in range(b0 + TILE):
                    if S4MODE[0] == "L":
                        kk = [kh_v[k, j, 3 * s + q, sl, :] for q in range(3)]
                    else:
                        kr, ki = kh_v[k, j, 3 * s, sl, :], kh_v[k, j, 3 * s + 1, sl, :]
                        kk = [kr, kr + ki, ki - kr]
                    for o in range(TILE - 1, -1, -1):
                        i = b0 + o - j
                        if i < 0:
                            continue
                        if i not in win:
                            win[i] = utrip(i, s)
                        p = [kk[q] * win[i][q] for q in range(3)]
                        acc[o] = p if acc[o] is None else [a + c for a, c in zip(acc[o], p)]
                        done += 1
                    if TILE == 4 and b0 == 4 and j == 2:
                        yield done
                yy.append([(a[0] - a[1], a[0] + a[2]) for a in acc])
                if s == 0:
                    yield done
            for o in range(TILE):
                p, q = yy[0][o], yy[1][o]
                cur = [(p[0] + q[0], p[1] + q[1]), (p[0] - q[0], p[1] - q[1])]
                for h in range(2):
                    if b0 + o == 0:
                        zr, zi = cur[h]
                    else:
                        zr = cur[h][0] - prev[h][1]
                        zi = cur[h][1] + prev[h][0]
                    zs_v[k, b0 + o, h, sl, 0:128] = zr
                    zs_v[k, b0 + o, h, sl, 128:256] = zi
                prev = cur
            if groups is not None and b0 + TILE < NB:
                for h in range(2):
                    pv_v[n, 2 * h] = prev[h][0]
                    pv_v[n, 2 * h + 1] = prev[h][1]
            yield done

    def s5_blk(k, b, h):
        g0 = k * NV
        t = 2 * b + h
        y = _dot_nt(zs_v[k, b, h], fmat(b % 2, h)).reshape(NV, 8, 128)
        hh = c1_v[pl.ds(g0, NV), 16 * b + 8 * h:16 * b + 8 * h + 8, :] + y
        c1_v[pl.ds(g0, NV), 16 * b + 8 * h:16 * b + 8 * h + 8, :] = hh
        wr = col_v[2, pl.ds(pl.multiple_of(k * R, 8), R), :].reshape(NV, 8, 128)
        rs = slice(8 * t, 8 * t + 8)
        acc_v[0, rs, :] = acc_v[0, rs, :] + jnp.sum(hh, axis=0)
        acc_v[1, rs, :] = acc_v[1, rs, :] + jnp.sum(hh * hh, axis=0)
        acc_v[2, rs, :] = acc_v[2, rs, :] + jnp.sum(hh * wr, axis=0)

    s5 = lambda k: [(functools.partial(s5_blk, k, b, h), 1.0) for b in range(NB) for h in range(2)]

    for c in c_par:
        c.wait()
    columns((1, 2))
    for k in range(2):
        _weave((s1n(k), 0.0, 0.2), (s1g(k), 0.2, 1.0))
    _weave((s1n(2), 0.0, 0.2), (s1g(2), 0.2, 1.0), (s2(0), 0.3, 1.0))
    s1_nat(3, 0, 1)
    c_x.wait()
    ln = [ln1_pieces(b, NPC) for b in range(NB)]
    s30 = s3(0)
    _weave((sum(ln, []), 0.0, P3F[0]), (s2(1), 0.0, P3F[2]),
           *[([s30[b]], max((b + 1.6) * P3F[0] / NB, P3F[3] + (1.0 - P3F[3]) * b / NB), 0.0) for b in range(NB)])
    for c in c_par2:
        c.wait()

    def body(k, do5=True, do4=True, do3=True, do2=True, do1=True, j=None, order=None):
        order = order or ORDER
        at = (lambda d: k + d) if j is None else (lambda d: j + (k + d) if k + d else j)
        g2 = s2_gen(at(2)) if do2 else None
        for n in range(NV):
            g4 = s4_gen(at(0), n) if do4 else None
            st4 = [0, 0]
            n4 = order.count("4")

            def adv4(m):
                if not do4:
                    return
                st4[0] += 1
                while st4[1] < 72 * st4[0] / n4 - 3 or (st4[0] == n4 and st4[1] <= 72):
                    r = next(g4, None)
                    if r is None:
                        break
                    st4[1] = r

            def nat():
                if do1:
                    if n + 1 < NV:
                        s1_nat(at(3), n + 1, 1)
                    else:
                        s1_nat(jnp.minimum(at(4), NSTEP - 1), 0, 1)

            g1 = s1_grp(at(3), n) if do1 else None
            for tok in order:
                if tok == "5":
                    if do5 and n < NB:
                        s5_blk(at(-1), n, 0)
                        s5_blk(at(-1), n, 1)
                elif tok == "4":
                    adv4(1)
                elif tok in "ab" and do1:
                    next(g1)
                elif tok == "p" and do1:
                    run(g1)
                elif tok == "2" and do2:
                    next(g2, None)
                elif tok == "3" and do3 and n < NB:
                    s3_blk(at(1), n)
                elif tok == "n":
                    nat()
        if do2:
            run(g2)

    @pl.when(flag_s[0] == 1)
    def _():
        body(0, do5=False, order=ORD0)

    lax.fori_loop(0, 4, lambda j, c: (body(1, j=j), c)[1], 0)

    @pl.when(flag_s[0] == 1)
    def _():
        body(5, do1=False, order=ORD5)

    @pl.when(flag_s[0] == 1)
    def _():
        body(6, do1=False, do2=False, order=ORD6)

    @pl.when(flag_s[0] == 1)
    def _():
        _weave(([(lambda n=n: run(s4_gen(7, n, (0,))), 1.0) for n in range(NV)], 0.0, 1.0), (s5(6), 0.0, 1.0))

    @pl.when(flag_s[0] == 1)
    def _():
        _weave(([(lambda n=n: run(s4_gen(7, n, (4,))), 1.0) for n in range(NV)], 0.0, 1.0), (s5(7)[:8], 0.0, 1.0))

    _weave((s5(7)[8:], 0.0, 1.0))

    def total(i):
        halves = []
        for hf in range(2):
            t = acc_v[i, pl.ds(64 * hf, 8, stride=8), :]
            for s in range(1, 8):
                t = t + acc_v[i, pl.ds(64 * hf + s, 8, stride=8), :]
            halves.append(t)
        return jnp.concatenate(halves, 0)

    m2 = total(0) * (1.0 / D)
    var2 = jnp.maximum(total(1) * (1.0 / D) - m2 * m2, 0.0)
    sd2 = _rb(jnp.sqrt(_rb(_rb(var2) + EPS)))
    rs2 = 1.0 / sd2
    r = _rb((total(2) - m2 * wr_sum) * rs2)
    mean2 = fin_v[4] + m2
    fin_v[0] = rs2
    fin_v[1] = m2 * rs2
    fin_v[2] = rs2 + 1.0
    fin_v[3] = fin_v[4] - m2 * rs2

    tl = _iota((16, 128), 0)
    ll = _iota((16, 128), 1)
    lodd = (ll & 1) == 1
    toff = jnp.where((tl & 1) == 0, jnp.where(lodd, ll + 127, ll), jnp.where(lodd, ll + 128, (ll - 1) & 127))
    tok = (tl >> 1) * 256 + toff
    rbits = pltpu.bitcast(r, i32)
    srt = rbits ^ ((rbits >> 31) & 0x7FFFFFFF)
    key = pltpu.bitcast((((srt >> 16) + 32768) << 11) + (2047 - tok) + (1 << 28), f32)
    kk = key
    cand = []
    for _ in range(4):
        rm = jnp.broadcast_to(jnp.max(kk, axis=1, keepdims=True), (16, 128))
        cand.append(rm)
        kk = jnp.where(kk == rm, 0.0, kk)
    last = jnp.max(cand[3], axis=0, keepdims=True)
    kcol = None
    for j in range(TOPC):
        mx = jnp.max(cand[0], axis=0, keepdims=True)
        kcol = jnp.broadcast_to(mx, (8, 128)) if j == 0 else jnp.where(sub8 == j, mx, kcol)
        took = cand[0] == mx
        cand = [jnp.where(took, cand[i + 1] if i < 3 else 0.0, cand[i]) for i in range(4)]
    kc_v[...] = kcol

    @pl.when((last - mx)[0, 0] > 0.0)
    def _():
        k2 = key
        kc = None
        for j in range(TOPC):
            m1 = jnp.max(jnp.max(k2, axis=0, keepdims=True), axis=1, keepdims=True)
            kc = jnp.broadcast_to(m1, (8, 128)) if j == 0 else jnp.where(sub8 == j, m1, kc)
            k2 = jnp.where(k2 == m1, 0.0, k2)
        kc_v[...] = kc

    kcol = kc_v[...]
    kint = pltpu.bitcast(kcol, i32) - (1 << 28)
    tcol = 2047 - (kint & 2047)
    s16 = (kint >> 11) - 32768
    rsel = pltpu.bitcast((s16 ^ ((s16 >> 31) & 0x7FFF)) << 16, f32)
    gate = _rb(jax.nn.sigmoid(rsel))

    def classes(col):
        cls = jnp.zeros((8, 128), i32)
        for d in range(1, TOPC):
            cls = cls + jnp.where((col == pltpu.roll(col, d, 0)) & (sub8 >= d), 1, 0)
        return cls, jnp.max(cls, axis=0, keepdims=True)[0, 0] + 1

    wcol = tcol & 255
    pcol = jnp.where((wcol & 1) == 0, jnp.where(wcol < 128, wcol, wcol - 127),
                     jnp.where(wcol < 128, (wcol + 1) & 127, wcol - 128))
    ecol = ((tcol >> 8) << 1) | (tcol & 1)
    etile = [ecol[j, 0] for j in range(TOPC)]
    gcol, gn = classes(pcol)
    xs_v[...] = jnp.zeros((8, D), f32)

    def gather(c, carry):
        oh = (gcol == c) & (lane8 == pcol)
        ohi = jnp.where(oh, 1, 0)
        msk = [jnp.broadcast_to(ohi[j:j + 1], (8, 128)) == 1 for j in range(TOPC)]
        sa = sb = None
        for j in range(TOPC):
            fa = jnp.broadcast_to(fin_v[0, pl.ds(etile[j], 1), :], (8, 128))
            fb = jnp.broadcast_to(fin_v[1, pl.ds(etile[j], 1), :], (8, 128))
            sa, sb = (fa, fb) if j == 0 else (jnp.where(msk[j], fa, sa), jnp.where(msk[j], fb, sb))
        parts = []
        for q in range(D // 8 // GCH):
            mg = None
            for j in range(TOPC):
                cc = c1_v[GCH * q:GCH * q + GCH, pl.ds(pl.multiple_of(8 * etile[j], 8), 8), :]
                mg = cc if j == 0 else jnp.where(msk[j], cc, mg)
            parts.append(mg * sa - sb)
        ln = jnp.concatenate(parts, 0).reshape(D, 128)
        xs_v[...] = xs_v[...] + _dot_nt(jnp.where(oh, 1.0, 0.0).astype(f32), ln)
        return carry

    lax.fori_loop(0, gn, gather, 0)
    xsel = xs_v[...]

    def rebuilt_rows():
        sdc = jnp.zeros((8, 1), f32)
        mc = jnp.zeros((8, 1), f32)
        sub1 = _iota((8, 1), 0)
        for j in range(TOPC):
            hitm = tok == jnp.broadcast_to(tcol[j:j + 1], (16, 128))
            red = lambda v: jnp.sum(jnp.sum(jnp.where(hitm, v, 0.0), axis=0, keepdims=True), axis=1, keepdims=True)
            sdc = jnp.where(sub1 == j, red(sd2), sdc)
            mc = jnp.where(sub1 == j, red(mean2), mc)
        return xsel * (sdc + 1.0) + mc

    def outp(b, g0, g1):
        sc = [jnp.where(top, jnp.broadcast_to(fin_v[i, 2 * b:2 * b + 1, :], (8, 128)),
                        jnp.broadcast_to(fin_v[i, 2 * b + 1:2 * b + 2, :], (8, 128))) for i in (2, 3)]
        for g in range(g0, g1):
            a = _rb(c1_v[g, pl.ds(16 * b, 8, stride=2), :] * sc[0] + sc[1])
            c = _rb(c1_v[g, pl.ds(16 * b + 1, 8, stride=2), :] * sc[0] + sc[1])
            w = (pltpu.bitcast(a, u32) >> 16) | pltpu.bitcast(c, u32)
            out_w[g, b] = jnp.where(mask2, w, pltpu.roll(pltpu.roll(w, 4, 0), 127, 1))

    opieces = [functools.partial(outp, b, 24 * i, 24 * i + 24) for b in range(NB) for i in range(3)]

    tilec = tcol >> 7
    lanec = tcol & 127
    aux = {}

    def late_scalars():
        tiles = [tilec[j, 0] for j in range(TOPC)]
        hit = 0
        dup = []
        for j in range(TOPC):
            dup.append((hit >> tiles[j]) & 1)
            hit = hit | (1 << tiles[j])
        free, cnt = [], 0
        for t in range(16):
            un = 1 - ((hit >> t) & 1)
            free.append(jnp.where(un == 1, cnt, -1))
            cnt = cnt + un
        late, nd, mask = [tiles[0]], 0, hit
        for j in range(1, TOPC):
            rep = 0
            for t in range(16):
                rep = jnp.where(free[t] == nd, t, rep)
            late.append(jnp.where(dup[j] == 1, rep, tiles[j]))
            mask = mask | (1 << late[j])
            nd = nd + dup[j]
        aux.update(tiles=tiles, late=late, mask=mask)
        bs_v[...] = rebuilt_rows()
        aux["clscol"], aux["ncls"] = classes(lanec)
        for j in range(TOPC):
            code = jnp.where((tilec == late[j]) & (lane8 == lanec), aux["clscol"], -1)
            lm_v[j] = jnp.broadcast_to(jnp.max(code, axis=0, keepdims=True), (8, 128))

    def tile_idx(t, g0=0, ng=D // 8):
        if isinstance(t, int):
            return (pl.ds(g0, ng), t // 2, pl.ds(8 * (t % 2), 8), slice(None))
        return (pl.ds(g0, ng), t >> 1, pl.ds(pl.multiple_of(8 * (t & 1), 8), 8), slice(None))

    def ocopy(idx):
        return cp(out_v.at[idx], out_h.at[idx], osem.at[0])

    def early():
        for t in range(16):
            @pl.when(((aux["mask"] >> t) & 1) == 0)
            def _():
                ocopy(tile_idx(t)).start()

    for c in range(NCH):
        for cc in c_w[c]:
            cc.wait()
        mine = opieces[OSPLIT[c]:OSPLIT[c + 1]]
        nsub = max(1, FCH[c] // FSUB)
        sub = FCH[c] // nsub
        for u in range(nsub):
            sl = slice(FOFF[c] + u * sub, FOFF[c] + (u + 1) * sub)
            g = _rb(_dot(xsel, wmat(wg_w, 0, D, sl.start, sub)))
            up = _rb(_dot(xsel, wmat(wu_w, 0, D, sl.start, sub)))
            if c == 0 and u == 0:
                late_scalars()
            for fn in mine[u * len(mine) // nsub:(u + 1) * len(mine) // nsub]:
                fn()
            act_v[:, sl] = _rb(_rb(g * jax.nn.sigmoid(g)) * up)
        if c == WCH:
            early()

    clscol = aux["clscol"]
    onehot = lambda c: jnp.where((clscol == c) & (lane8 == lanec), 1.0, 0.0).astype(f32)
    bc = lambda v, j: jnp.broadcast_to(v[j:j + 1], (8, 128))

    def down(p, c0, nc):
        r = slice(POFF[p], POFF[p] + PART[p])
        yc = _dot_nt(act_v[:, c0:c0 + nc], wmat(wd_w, POFF[p], PART[p], c0, nc))
        y_v[:, r] = yc if c0 == 0 else y_v[:, r] + yc

    def place(p, fast):
        r0, nr = POFF[p], PART[p]
        g0, ng = r0 // 8, nr // 8
        gt = jnp.concatenate([gate] * ((nr + 127) // 128), 1)[:, :nr]
        newrow = _rb(bs_v[:, r0:r0 + nr] + _rb(_rb(y_v[:, r0:r0 + nr]) * gt))
        tn = lambda oh: lax.dot_general(newrow, oh, (((0,), (0,)), ((), ())), preferred_element_type=f32)
        if fast:
            uu = tn(jnp.concatenate([onehot(0), onehot(1)], 1))
            for c in range(2):
                u_v[c, g0:g0 + ng] = uu[:, 128 * c:128 * (c + 1)].reshape(ng, 8, 128)
        else:
            for c in range(TOPC):
                u_v[c, g0:g0 + ng] = tn(onehot(c)).reshape(ng, 8, 128)

    def write(p, fast):
        g0, ng = POFF[p] // 8, PART[p] // 8
        for j in range(TOPC):
            idx = tile_idx(aux["late"][j], g0, ng)
            new = out_v[idx].astype(f32)
            code = lm_v[j]
            for c in range(2 if fast else TOPC):
                new = jnp.where(code == c, u_v[c, g0:g0 + ng], new)
            sg_v[j, g0:g0 + ng] = new.astype(bf16)
            cp(sg_v.at[j, pl.ds(g0, ng)], out_h.at[idx], osem.at[0]).start()

    def dwait(p):
        for cc in c_d[p]:
            cc.wait()

    NP = len(PART)
    dwait(0)
    rest = opieces[OSPLIT[NCH]:]
    nq = 4
    for q in range(nq):
        down(0, q * F // nq, F // nq)
        for fn in rest[q * len(rest) // nq:(q + 1) * len(rest) // nq]:
            fn()

    @pl.when(aux["ncls"] <= 2)
    def _():
        for p in range(1, NP):
            dwait(p)
            down(p, 0, DSPL[p])
            place(p - 1, True)
            down(p, DSPL[p], F - DSPL[p])
            write(p - 1, True)
        place(NP - 1, True)
        write(NP - 1, True)

    @pl.when(aux["ncls"] > 2)
    def _():
        for p in range(1, NP):
            dwait(p)
            down(p, 0, F)
        for p in range(NP):
            place(p, False)
            write(p, False)

    cp(out_h, out_h, osem.at[0]).wait()


@jax.jit
def pallas_sequential_preLN__ssm_conv_s4__moe_arch_mod__prompt_kernel(
    A_u: jax.Array,
    A_A_re: jax.Array,
    A_A_im: jax.Array,
    A_B_re: jax.Array,
    A_B_im: jax.Array,
    A_C_re: jax.Array,
    A_C_im: jax.Array,
    A_log_dt: jax.Array,
    A_Dskip: jax.Array,
    B_x: jax.Array,
    B_w_r: jax.Array,
    B_w_gate: jax.Array,
    B_w_up: jax.Array,
    B_w_down: jax.Array,
):
    hbm = pl.BlockSpec(memory_space=pltpu.MemorySpace.HBM)
    vm = pltpu.VMEM
    G8 = D // 8
    wshape = (D // 16, F // 128, 16, 128)
    wview = lambda w: w.reshape(D // 16, 2, 8, F // 128, 128).transpose(0, 1, 3, 2, 4)
    scratch = [
        vm((G8, NB, 16, 128), bf16), vm((6, D, N), bf16), vm((D,), bf16), vm((D,), bf16), vm((D,), bf16),
        vm((CT_ROWS, 128), f32), vm(wshape, bf16), vm(wshape, bf16), vm(wshape, bf16), vm((G8, NB + 1, 16, 128), bf16),
        vm((9, 4, 144, 128), bf16), vm((2, 2, 2, 144, 128), bf16), vm((3, D + 8, 128), f32),
        vm((NV, 2, 136, 128), f32), vm((NSTEP, NV, 56, 128), f32), vm((NSTEP, R, 128), f32),
        vm((NSTEP, NB, 6, R, 128), f32), vm((NSTEP, NB, 6, R, 128), f32),
        vm((NSTEP, NB, 2, R, 256), f32), vm((G8, 136, 128), f32), vm((2, 17, 8, 128), f32),
        vm((3, 136, 128), f32), vm((5, 16, 128), f32), vm((TOPC, G8, 8, 128), f32),
        vm((R, 512), f32), vm((8, D), f32), vm((NV, 4, 8, 128), f32),
        vm((8, 128), f32), vm((8, D), f32), vm((8, D), f32), vm((8, F), f32),
        vm((TOPC, G8, 8, 128), bf16), vm((TOPC, 8, 128), i32), vm((8, D), f32), pltpu.SMEM((1,), i32),
        pltpu.SemaphoreType.DMA((5 + NCH + len(PART),)), pltpu.SemaphoreType.DMA((1,)),
    ]
    xv = A_u[0].T.reshape(G8, 8, 16, 128).transpose(0, 2, 1, 3).reshape(G8, NB, 16, 128)
    out = pl.pallas_call(
        _kernel,
        out_shape=jax.ShapeDtypeStruct((G8, NB, 16, 128), bf16),
        in_specs=[hbm] * 13,
        out_specs=hbm,
        scratch_shapes=scratch,
        compiler_params=pltpu.CompilerParams(vmem_limit_bytes=120 * 1024 * 1024, disable_bounds_checks=NOBC),
    )(xv, A_A_re, A_A_im, A_B_re, A_B_im, A_C_re, A_C_im, A_log_dt, A_Dskip, B_w_r,
      wview(B_w_gate), wview(B_w_up), wview(B_w_down.T))
    return out.reshape(G8, 16, 8, 128).transpose(0, 2, 1, 3).reshape(D, L).T[None]
```

```python
import functools

import numpy as np
import jax
import jax.numpy as jnp
from jax import lax
import jax.experimental.pallas as pl
import jax.experimental.pallas.tpu as pltpu

f32 = jnp.float32
bf16 = jnp.bfloat16
i32 = jnp.int32
u32 = jnp.uint32

L, D, N, F, TOPC = 2048, 576, 128, 4608, 8
NB = 8
NV = 9
R = NV * 8
NSTEP = D // R
EPS = 1e-5

_XL1 = [(1, 5), (2, 6), (3, 7), (4, 8), (258, 516), (260, 520), (262, 772), (264, 776),
        (1288, 1032), (1800, 1544)]
_XSH = [0, 1, 2, 3, 0, 1, 2, 3, 0, 1]


def _bf16_round_int(j):
    u = np.asarray(j, np.float32).view(np.uint32).astype(np.uint64)
    r = ((u + 0x7FFF + ((u >> 16) & 1)) >> 16) << 16
    return r.astype(np.uint32).view(np.float32).astype(np.int64)


def _chunk_values():
    vals = -np.ones((5, 128), np.int64)
    for j in range(10):
        for p in range(2):
            ch = (j // 4) * 2 + p if j < 8 else 4
            extra = 2 * p if j >= 8 else 0
            for l0 in range(32):
                vals[ch, (4 * (31 - l0) + 4 * p + _XSH[j] + extra + 8) % 128] = _XL1[j][p] + 8 * l0
    assert (vals >= 0).all()
    return vals


_PASSES = [(0, "A0"), (0, "A1"), (1, "B"), (2, "Cp"), (3, "C"), (4, "Dp"), (5, "D"), (6, "D"), (7, "D")]
_SETS = [[0], [1], [2], [3, 4], [5, 6, 7, 8]]


def _tables():
    cv = _chunk_values()
    cvp = {"A0": cv[0], "A1": cv[1], "B": cv[2], "C": cv[3], "D": cv[4]}
    cvp["Cp"] = cv[3].copy(); cvp["Cp"][11] = cv[2][11]
    cvp["Dp"] = cv[4].copy(); cvp["Dp"][15] = cv[3][15]
    sup = [[[] for _ in range(128)] for _ in _PASSES]
    for b in range(NB):
        for j in range(1, 257):
            lag = 256 * b + j
            if lag > L - 1 or lag == 257:
                continue
            v = int(_bf16_round_int(lag))
            hit = [(i, int(np.nonzero(cvp[nm] == v)[0][0])) for i, (pb, nm) in enumerate(_PASSES)
                   if pb == b and (cvp[nm] == v).any()]
            assert len(hit) == 1, (b, j, v, hit)
            sup[hit[0][0]][hit[0][1]].append(j)
    assert cv[1][15] == _bf16_round_int(257)
    code = np.zeros((len(_PASSES), 128), np.int64)
    for i, (pb, _) in enumerate(_PASSES):
        for r in range(128):
            js = sup[i][r]
            if js:
                assert js == list(range(js[0], js[-1] + 1))
                code[i, r] = js[0] + js[-1] + 1024 * len(js) + 16384 * (pb % 2)
    seeds, masks = [], {}
    for ps in _SETS:
        seeds.append([int(x) for x in sum(code[i, 16:24] for i in ps)])
        for i in ps:
            masks[i] = [int(x > 0) for x in code[i, 16:24]]
            for v in range(2, 17):
                r0 = 8 * (v % 16)
                assert (code[i, r0:r0 + 8] == (np.array(seeds[-1]) - 32 * (v - 2)) * np.array(masks[i])).all()
    return seeds, [[int(x) for x in code[i, 8:16]] for i in range(len(_PASSES))], masks


_GSEED, _GROW1, _GMASK = _tables()


def _sincos_coeffs():
    r = np.cos(np.pi * (np.arange(4000) + .5) / 4000) * 0.5
    z = r * r
    s = np.linalg.lstsq(np.stack([z ** k for k in range(4)], 1), np.sin(np.pi / 2 * r) / r, rcond=None)[0]
    c = np.linalg.lstsq(np.stack([z ** k for k in range(1, 5)], 1), np.cos(np.pi / 2 * r) - 1, rcond=None)[0]
    return [float(x) for x in s], [float(x) for x in c]


_SC, _CC = _sincos_coeffs()


def _cmul(a, b):
    return (a[0] * b[0] - a[1] * b[1], a[0] * b[1] + a[1] * b[0])


def _cmulc(a, b):
    return (a[0] * b[0] + a[1] * b[1], a[1] * b[0] - a[0] * b[1])


def _csq(a):
    return ((a[0] - a[1]) * (a[0] + a[1]), (a[0] + a[0]) * a[1])


def _quarter_polys(r):
    r2 = r * r
    s = r * (_SC[0] + r2 * (_SC[1] + r2 * (_SC[2] + r2 * _SC[3])))
    c = 1.0 + r2 * (_CC[0] + r2 * (_CC[1] + r2 * (_CC[2] + r2 * _CC[3])))
    return s, c


def _rotate_quadrant(s, c, ki):
    swap = (ki & 1) == 1
    s2 = jnp.where(swap, c, s)
    c2 = jnp.where(swap, s, c)
    s2 = pltpu.bitcast(pltpu.bitcast(s2, i32) ^ ((ki & 2) << 30), f32)
    c2 = pltpu.bitcast(pltpu.bitcast(c2, i32) ^ (((ki + 1) & 2) << 30), f32)
    return s2, c2


def _sincos(th):
    z = th * (2.0 / np.pi)
    k = jnp.round(z)
    s, c = _quarter_polys(z - k)
    return _rotate_quadrant(s, c, k.astype(i32))


def _reduce_small(z):
    big = 12582912.0
    t = z + big
    return _quarter_polys(z - (t - big)) + (pltpu.bitcast(t, i32),)


def _rb(x):
    return x.astype(bf16).astype(f32)


def _dot(a, b):
    return jnp.dot(a, b, preferred_element_type=f32)


def _dot_nt(a, b):
    return lax.dot_general(a, b, (((1,), (1,)), ((), ())), preferred_element_type=f32)


def _iota(shape, dim):
    return lax.broadcasted_iota(i32, shape, dim)


S4MODE='CC'
TILE=4
YSPLIT=1
ZT=1
ORDER='4ab44342np445'
ORD0='4ab442n4p4345'
ORD5='4a424n44b345p'
ORD6='45a4b244p3n44'
NPC=3
P3F=(0.9,0.4,0.55,0.3)
GCH=3
NOBC=True
CT_ROWS=320
PART=(256,128,128,64)
DSPL=(0,2560,2560,4096)
FSUB=1536
FCH=(3072,1536)
OSPLIT=[0,24,24]
WCH=0
NCH = len(FCH)
FOFF = [sum(FCH[:i]) for i in range(NCH)]
POFF = [sum(PART[:i]) for i in range(len(PART))]

def _weave(*streams):
    items = []
    for si, (pieces, lo, hi) in enumerate(streams):
        tot = float(sum(c for _, c in pieces))
        cum = 0.0
        for pi, (fn, c) in enumerate(pieces):
            items.append((lo + max(hi - lo, 0.0) * (cum + 0.5 * c) / tot, si, pi, fn))
            cum += c
    for _, _, _, fn in sorted(items, key=lambda t: t[:3]):
        fn()


def _kernel(x_h, are_h, aim_h, bre_h, bim_h, cre_h, cim_h, ldt_h, dsk_h, wr_h, wg_h, wu_h, wd_h,
            out_h,
            x_v, par_v, ldt_v, dsk_v, wr_v, ct_v, wg_v, wu_v, wd_v, out_v,
            g_v, f_v, col_v, st_v, kd_v, k0_v, kh_v, uh_v, zs_v, c1_v, s1_v, acc_v, fin_v, u_v, zt_v, y_v, pv_v, kc_v, xs_v, bs_v, act_v, sg_v, lm_v, rw_v, flag_s,
            sem, osem):
    cp = pltpu.make_async_copy
    c_vec = [cp(ldt_h, ldt_v, sem.at[1]), cp(dsk_h, dsk_v, sem.at[1]), cp(wr_h, wr_v, sem.at[1])]
    PH = 4
    par_h = (are_h, aim_h, bre_h, bim_h, cre_h, cim_h)
    c_par = [cp(h.at[pl.ds(0, PH)], par_v.at[i, pl.ds(0, PH), pl.ds(0, R)], sem.at[2]) for i, h in enumerate(par_h)]
    c_par2 = [cp(h.at[pl.ds(PH, NSTEP - PH)], par_v.at[i, pl.ds(PH, NSTEP - PH), pl.ds(0, R)], sem.at[3])
              for i, h in enumerate(par_h)]
    c_x = cp(x_h, x_v, sem.at[4])
    def wcp(h, v, rp, ct, s):
        return [cp(h.at[rp, hf, ct], v.at[rp, ct, pl.ds(8 * hf, 8), :], s) for hf in range(2)]

    c_w = [wcp(wg_h, wg_v, slice(None), pl.ds(FOFF[c] // 128, FCH[c] // 128), sem.at[5 + c])
           + wcp(wu_h, wu_v, slice(None), pl.ds(FOFF[c] // 128, FCH[c] // 128), sem.at[5 + c]) for c in range(NCH)]
    c_d = [wcp(wd_h, wd_v, pl.ds(POFF[p] // 16, PART[p] // 16), slice(None), sem.at[5 + NCH + p])
           for p in range(len(PART))]
    for c in c_vec + c_par + [c_x] + c_par2 + sum(c_w, []) + sum(c_d, []):
        c.start()

    flag_s[0] = 1
    x_w = x_v.bitcast(u32)
    wg_w, wu_w, wd_w = wg_v.bitcast(u32), wu_v.bitcast(u32), wd_v.bitcast(u32)

    def wmat(w, r0, nr, c0, nc):
        return jnp.concatenate([pltpu.bitcast(w[r0 // 16:(r0 + nr) // 16, t], bf16).reshape(nr, 128)
                                for t in range(c0 // 128, (c0 + nc) // 128)], 1)

    out_w = out_v.bitcast(u32)
    g_w = g_v.bitcast(u32)
    f_w = f_v.bitcast(u32)
    sub8 = _iota((8, 128), 0)
    lane8 = _iota((8, 128), 1)

    acc_v[...] = jnp.zeros(acc_v.shape, f32)
    for n in range(NV):
        for ri in range(2):
            st_v[n, ri, 104:112, :] = jnp.full((8, 128), 1.0 - ri, f32)
    kp = (2 * lane8 + 1).astype(f32)

    def rows_const(vals):
        out = jnp.full((8, 128), vals[0], i32)
        for r in range(1, 8):
            if vals[r] != vals[0]:
                out = jnp.where(sub8 == r, vals[r], out)
        return out

    def phasor(z):
        sn, cs = _rotate_quadrant(*_reduce_small(-z))
        return cs, sn

    NS = [0, 1, 2, 3, 4, 5, 7, 9]
    for q in range(2):
        sn = _rotate_quadrant(*_reduce_small((kp + 512.0 * q) * (rows_const(NS).astype(f32) * (1.0 / 512))))[0]
        ct_v[304 + 8 * q:312 + 8 * q, :] = sn / (256.0 * jnp.broadcast_to(sn[1:2], (8, 128)))

    def grows(vals):
        ab = rows_const([v & 1023 for v in vals])
        z = kp * (ab.astype(f32) * (-1.0 / 512))
        if any(v >> 14 for v in vals):
            z = z - rows_const([v >> 14 for v in vals]).astype(f32) * (kp - 1.0)
        sn, cs, ki = _reduce_small(z)
        ns = [NS.index((v >> 10) & 15) for v in vals]
        out = []
        for q in range(2):
            row = lambda i: jnp.broadcast_to(ct_v[304 + 8 * q + i:305 + 8 * q + i, :], (8, 128))
            amp = None
            for i in sorted(set(ns)):
                bits = sum(1 << r for r in range(8) if ns[r] == i)
                amp = row(i) if amp is None else jnp.where(((bits >> sub8) & 1) == 1, row(i), amp)
            pi, pr = _rotate_quadrant(sn, cs, ki if q == 0 else ki - ab)
            out += [pr * amp, pi * amp]
        return out

    for v4 in range(4):
        e = phasor(kp * ((sub8 + 8 * v4).astype(f32) * (1.0 / 32)))
        ct_v[8 * v4:8 * v4 + 8, :] = e[0]
        ct_v[32 + 8 * v4:40 + 8 * v4, :] = e[1]
    for si in range(5):
        for q, val in enumerate(grows(_GSEED[si])):
            ct_v[64 + 32 * si + 8 * q:72 + 32 * si + 8 * q, :] = val
    for i in range(len(_PASSES)):
        for q, val in enumerate(grows(_GROW1[i])):
            g_v[i, q, 8:16, :] = val.astype(bf16)
    for q, val in enumerate(grows([2 + 1024 + 16384] * 8)):
        ct_v[272 + 8 * q:280 + 8 * q, :] = val
    s8 = np.arange(8)
    je = np.where(s8 % 2 == 0, s8, 127 + s8)
    jo = np.where(s8 % 2 == 0, s8 - 1, 128 + s8)
    for t, jj in enumerate((je, jo, jo % 128 + 128 * (s8 % 2))):
        e = phasor(kp * (rows_const([int(x) for x in jj]).astype(f32) * (1.0 / 256)))
        ct_v[224 + 16 * t:232 + 16 * t, :] = e[0]
        ct_v[232 + 16 * t:240 + 16 * t, :] = e[1]
    for c in c_vec:
        c.wait()

    rows = [_rb(jnp.exp(ldt_v[...].astype(f32).reshape(1, D))),
            dsk_v[...].astype(f32).reshape(1, D),
            wr_v[...].astype(f32).reshape(1, D)]
    wr_sum = jnp.sum(rows[2], axis=1, keepdims=True)

    def columns(which):
        for j in range(5):
            w = 128 if j < 4 else 64
            eye = _iota((w, w), 0) == _iota((w, w), 1)
            m = jnp.concatenate([jnp.where(eye, jnp.broadcast_to(rw_v[i:i + 1, j * 128:j * 128 + w], (w, w)), 0.0)
                                 for i in which], 0)
            res = _dot(m, jnp.ones((w, 128), f32))
            for n, i in enumerate(which):
                for g in range(w // 8):
                    k, m8 = divmod(16 * j + g, NV)
                    col_v[i, k, 8 * m8:8 * m8 + 8, :] = res[n * w + 8 * g:n * w + 8 * g + 8]

    for i in range(3):
        rw_v[i:i + 1, :] = rows[i]
    columns((0,))

    def e8(v):
        return (jnp.broadcast_to(ct_v[v:v + 1, :], (8, 128)), jnp.broadcast_to(ct_v[32 + v:33 + v, :], (8, 128)))

    for si, ps in enumerate(_SETS):
        sd = [ct_v[64 + 32 * si + 8 * q:72 + 32 * si + 8 * q, :] for q in range(4)]
        mk = {}
        for i in ps:
            if len(ps) > 1:
                bits = sum(b << s for s, b in enumerate(_GMASK[i]))
                mk[i] = ((bits >> sub8) & 1) == 1
        for v in range(2, 17):
            if v == 2:
                vals = sd
            else:
                ev = e8(2 * (v - 2))
                vals = list(_cmulc((sd[0], sd[1]), ev)) + list(_cmulc((sd[2], sd[3]), ev))
            for i in ps:
                for q in range(4):
                    val = vals[q] if len(ps) == 1 else jnp.where(mk[i], vals[q], 0.0)
                    g_v[i, q, 8 * (v % 16):8 * (v % 16) + 8, :] = val.astype(bf16)
    sig = jnp.where((lane8 & 1) == 0, 1.0, -1.0).astype(f32)
    for h in range(2):
        sd = (ct_v[224 + 16 * h:232 + 16 * h, :], ct_v[232 + 16 * h:240 + 16 * h, :])
        for v in range(16):
            if v == 0:
                vals = sd if h == 0 else (ct_v[256:264, :], ct_v[264:272, :])
            else:
                vals = _cmul(sd, e8(v))
            for q in range(2):
                f_v[0, h, q, 8 * v:8 * v + 8, :] = vals[q].astype(bf16)
                f_v[1, h, q, 8 * v:8 * v + 8, :] = (vals[q] * sig).astype(bf16)

    def gmat(i):
        return jnp.concatenate([pltpu.bitcast(g_w[i, q, 0:64, :], bf16) for q in range(4)], 1)

    def fmat(ver, h):
        return jnp.concatenate([pltpu.bitcast(f_w[ver, h, q, 0:64, :], bf16) for q in range(2)], 1)

    revmask = (sub8 & 2) == 0
    lm = lane8 & 3

    def s1_nat(k, n0, nn):
        rr = 8 * nn
        ld = lambda i: par_v[i, k, 8 * n0:8 * n0 + rr, :].astype(f32)
        dt = col_v[0, k, 8 * n0:8 * n0 + rr, :]
        e = jnp.exp(dt * ld(0))
        s, c = _sincos(dt * ld(1))
        a1 = (e * c, e * s)
        w = _cmul((ld(4), ld(5)), (dt * ld(2), dt * ld(3)))
        k0_v[k, 8 * n0:8 * n0 + rr, :] = jnp.broadcast_to(jnp.sum(w[0], axis=1, keepdims=True), (rr, 128))
        w = (w[0], -w[1])
        rev = lambda v: jnp.where(revmask, pltpu.roll(v, 2, 0), pltpu.roll(v, 6, 0))

        def put(arr, slots, fn=None):
            for n in range(nn):
                for ri in range(2):
                    v = arr[ri][8 * n:8 * n + 8]
                    if fn is not None:
                        v = fn(v)
                    for q in slots:
                        st_v[n0 + n, ri, q * 8:q * 8 + 8, :] = v

        put(w, (0, 1)); put(a1, (2, 3))
        a2 = _csq(a1); put(a2, (5,))
        a4 = _csq(a2); put(a4, (6,))
        put(_cmul(a4, a1), (4,))
        a8 = _csq(a4); put(a8, (12,), rev)
        t = _csq(a8); put(t, (14, 15), rev)
        for _ in range(4):
            t = _csq(t)
        put(t, (7, 11))
        t = _csq(t); put(t, (8, 9))
        put(_csq(t), (10,))

    def s1_grp(k, n):
        mix = lambda q: tuple(jnp.concatenate([st_v[n, ri, pl.ds(q * 8 + g, 8, stride=2), :] for g in range(2)], 0)
                              for ri in range(2))
        y = [mix(12)]
        a16d = mix(14)
        if YSPLIT == 1:
            for _ in range(15):
                y.append(_cmul(y[-1], a16d))
        else:
            y.append(_cmul(y[0], a16d))
            a32d = _csq(a16d)
            for i in range(2, 16):
                y.append(_cmul(y[i - 2], a32d))
        yield
        wd = mix(0); a1d = mix(2); m1 = mix(5)
        v = [_cmulc(wd, mix(3))]
        for _ in range(3):
            v.append(_cmulc(v[-1], a1d))
        v4 = _cmulc(_cmulc(wd, m1), mix(7))
        v5 = _cmulc(v4, m1); v6 = _cmulc(v4, mix(6)); v7 = _cmulc(v6, m1)
        v8 = _cmulc(v7, mix(10)); v9 = _cmulc(v8, mix(8))
        v += [v4, v5, v6, v7, v8, v9]
        os_ = []
        for g in range(2):
            cat = lambda ts: jnp.concatenate([jnp.concatenate([t[ri][8 * g:8 * g + 8] for t in ts], 0)
                                              for ri in range(2)], 1)
            os_.append(_dot_nt(cat(v), cat(y[::-1])))
        yield
        for g in range(2):
            o = os_[g]
            ro = [pltpu.roll(o[8 * j:8 * j + 8], _XSH[j] + 5, 1, stride=1, stride_axis=0) for j in range(10)]
            sel4 = lambda q: jnp.where(lm == 0, q[0], jnp.where(lm == 1, q[1], jnp.where(lm == 2, q[2], q[3])))
            kd_v[k, n, pl.ds(g, 8, stride=2), :] = sel4(ro[0:4])
            kd_v[k, n, pl.ds(16 + g, 8, stride=2), :] = sel4(ro[4:8])
            kd_v[k, n, pl.ds(32 + g, 8, stride=2), :] = jnp.where(lm == 0, ro[8], ro[9])

    def run(gen):
        for _ in gen:
            pass

    s1n = lambda k: [(functools.partial(s1_nat, k, 3 * i, 3), 1.0) for i in range(3)]
    s1g = lambda k: [(lambda n=n: run(s1_grp(k, n)), 1.0) for n in range(NV)]

    laneR = _iota((R, 128), 1)
    lmR = laneR & 3

    def s2_gen(k):
        ch = lambda c: kd_v[k, 0:NV, 8 * c:8 * c + 8, :].reshape(R, 128)
        for b in range(NB):
            if b == 0:
                k0 = (k0_v[k, 0:R, :] + col_v[1, k, 0:R, :]) * (1.0 / 256.0)
                z = _dot(ch(0), gmat(0)) if ZT else None
                dd = jnp.where(lmR < 2, ch(4), pltpu.roll(ch(5), 2, 1))
                kd_v[k, 0:NV, 48:56, :] = dd.reshape(NV, 8, 128)
                if ZT:
                    zt_v[...] = z
                    yield
                    z = _dot(ch(1), gmat(1)) + zt_v[...]
                else:
                    z = _dot(jnp.concatenate([ch(0), ch(1)], 1), jnp.concatenate([gmat(0), gmat(1)], 0))
            elif b == 1:
                k256 = jnp.sum(jnp.where(laneR == 15, ch(1), 0.0), axis=1, keepdims=True)
                pat = jnp.concatenate([ct_v[272 + 8 * q:273 + 8 * q, :] for q in range(4)], 1)
                z = _dot(ch(2), gmat(2)) + k256 * pat
            elif b == 2:
                z = _dot(jnp.where(laneR == 11, ch(2), ch(3)), gmat(3))
            elif b == 3:
                z = _dot(ch(3), gmat(4))
            elif b == 4:
                z = _dot(jnp.where(laneR == 15, ch(3), ch(6)), gmat(5))
            else:
                z = _dot(ch(6), gmat(b + 1))
            for s in range(2):
                kr = z[:, 256 * s:256 * s + 128]
                ki = z[:, 256 * s + 128:256 * s + 256]
                if b == 0:
                    kr = kr + k0
                kh_v[k, b, 3 * s] = kr
                if S4MODE[0] == "L":
                    kh_v[k, b, 3 * s + 1] = kr + ki
                    kh_v[k, b, 3 * s + 2] = ki - kr
                else:
                    kh_v[k, b, 3 * s + 1] = ki
            yield

    def s2(k):
        gen = s2_gen(k)
        return [(lambda: next(gen, None), 1.0) for _ in range(9)]

    mask2 = (sub8 < 4) == ((lane8 & 1) == 0)
    top = sub8 < 4

    def ln1_pieces(b, npc):
        state = {}
        per = (D // 8) // npc

        def piece(i):
            for g in range(i * per, (i + 1) * per):
                m = x_w[g, b]
                eo = jnp.where(mask2, m, pltpu.roll(pltpu.roll(m, 4, 0), 1, 1))
                a = pltpu.bitcast(eo << 16, f32)
                c = pltpu.bitcast(eo & jnp.uint32(0xFFFF0000), f32)
                if g == 0:
                    state["sh"] = jnp.where(top, jnp.broadcast_to(a[0:1], (8, 128)),
                                            jnp.broadcast_to(a[4:5], (8, 128)))
                a = a - state["sh"]
                c = c - state["sh"]
                c1_v[g // NV, g % NV, pl.ds(16 * b, 8, stride=2), :] = a
                c1_v[g // NV, g % NV, pl.ds(16 * b + 1, 8, stride=2), :] = c
                new = [a, c, a * a, c * c]
                state["acc"] = new if g == 0 else [p + q for p, q in zip(state["acc"], new)]
            if i == npc - 1:
                acc = state["acc"]
                s1, s2_ = acc[0] + acc[1], acc[2] + acc[3]
                for h in range(2):
                    m = jnp.sum(s1[4 * h:4 * h + 4], axis=0, keepdims=True) * (1.0 / D)
                    var = jnp.sum(s2_[4 * h:4 * h + 4], axis=0, keepdims=True) * (1.0 / D) - m * m
                    rs = 1.0 / _rb(jnp.sqrt(_rb(_rb(jnp.maximum(var, 0.0)) + EPS)))
                    s1_v[0, 2 * b + h] = jnp.broadcast_to(rs, (8, 128))
                    s1_v[1, 2 * b + h] = jnp.broadcast_to(m * rs, (8, 128))
                    fin_v[4, 2 * b + h:2 * b + h + 1, :] = state["sh"][4 * h:4 * h + 1]

        return [(functools.partial(piece, i), 1.0) for i in range(npc)]

    def s3_blk(k, b):
        et = []
        for h in range(2):
            c = c1_v[k, 0:NV, 16 * b + 8 * h:16 * b + 8 * h + 8, :]
            u = (c * s1_v[0, 2 * b + h] - s1_v[1, 2 * b + h]).reshape(R, 128)
            et.append(_dot(u, fmat(b % 2, h)))
        er, ei, tr, ti = et[0][:, :128], et[0][:, 128:], et[1][:, :128], et[1][:, 128:]
        if S4MODE[1] == "C":
            for q, v in enumerate((er, ei, tr, ti)):
                uh_v[k, b, q] = v
        else:
            for s, (pr, pi) in enumerate(((er + tr, ei + ti), (er - tr, ei - ti))):
                uh_v[k, b, 3 * s] = pr + pi
                uh_v[k, b, 3 * s + 1] = pi
                uh_v[k, b, 3 * s + 2] = pr

    s3 = lambda k: [(functools.partial(s3_blk, k, b), 1.0) for b in range(NB)]

    def s4_gen(k, n, groups=None):
        sl = slice(8 * n, 8 * n + 8)

        def utrip(i, s):
            if S4MODE[1] == "L":
                return [uh_v[k, i, 3 * s + q, sl, :] for q in range(3)]
            er, ei, tr, ti = [uh_v[k, i, q, sl, :] for q in range(4)]
            pr, pi = (er + tr, ei + ti) if s == 0 else (er - tr, ei - ti)
            return [pr + pi, pi, pr]

        prev = None
        done = 0
        if groups is not None and groups[0] > 0:
            prev = [(pv_v[n, 2 * h], pv_v[n, 2 * h + 1]) for h in range(2)]
        for b0 in (range(0, NB, TILE) if groups is None else groups):
            yy = []
            for s in range(2):
                acc = [None] * TILE
                win = {}
                for j in range(b0 + TILE):
                    if S4MODE[0] == "L":
                        kk = [kh_v[k, j, 3 * s + q, sl, :] for q in range(3)]
                    else:
                        kr, ki = kh_v[k, j, 3 * s, sl, :], kh_v[k, j, 3 * s + 1, sl, :]
                        kk = [kr, kr + ki, ki - kr]
                    for o in range(TILE - 1, -1, -1):
                        i = b0 + o - j
                        if i < 0:
                            continue
                        if i not in win:
                            win[i] = utrip(i, s)
                        p = [kk[q] * win[i][q] for q in range(3)]
                        acc[o] = p if acc[o] is None else [a + c for a, c in zip(acc[o], p)]
                        done += 1
                    if TILE == 4 and b0 == 4 and j == 2:
                        yield done
                yy.append([(a[0] - a[1], a[0] + a[2]) for a in acc])
                if s == 0:
                    yield done
            for o in range(TILE):
                p, q = yy[0][o], yy[1][o]
                cur = [(p[0] + q[0], p[1] + q[1]), (p[0] - q[0], p[1] - q[1])]
                for h in range(2):
                    if b0 + o == 0:
                        zr, zi = cur[h]
                    else:
                        zr = cur[h][0] - prev[h][1]
                        zi = cur[h][1] + prev[h][0]
                    zs_v[k, b0 + o, h, sl, 0:128] = zr
                    zs_v[k, b0 + o, h, sl, 128:256] = zi
                prev = cur
            if groups is not None and b0 + TILE < NB:
                for h in range(2):
                    pv_v[n, 2 * h] = prev[h][0]
                    pv_v[n, 2 * h + 1] = prev[h][1]
            yield done

    def s5_blk(k, b, h):
        t = 2 * b + h
        y = _dot_nt(zs_v[k, b, h], fmat(b % 2, h)).reshape(NV, 8, 128)
        hh = c1_v[k, 0:NV, 16 * b + 8 * h:16 * b + 8 * h + 8, :] + y
        c1_v[k, 0:NV, 16 * b + 8 * h:16 * b + 8 * h + 8, :] = hh
        wr = col_v[2, k, 0:R, :].reshape(NV, 8, 128)
        rs = slice(8 * t, 8 * t + 8)
        acc_v[0, rs, :] = acc_v[0, rs, :] + jnp.sum(hh, axis=0)
        acc_v[1, rs, :] = acc_v[1, rs, :] + jnp.sum(hh * hh, axis=0)
        acc_v[2, rs, :] = acc_v[2, rs, :] + jnp.sum(hh * wr, axis=0)

    s5 = lambda k: [(functools.partial(s5_blk, k, b, h), 1.0) for b in range(NB) for h in range(2)]

    for c in c_par:
        c.wait()
    columns((1, 2))
    for k in range(2):
        _weave((s1n(k), 0.0, 0.2), (s1g(k), 0.2, 1.0))
    _weave((s1n(2), 0.0, 0.2), (s1g(2), 0.2, 1.0), (s2(0), 0.3, 1.0))
    s1_nat(3, 0, 1)
    c_x.wait()
    ln = [ln1_pieces(b, NPC) for b in range(NB)]
    s30 = s3(0)
    _weave((sum(ln, []), 0.0, P3F[0]), (s2(1), 0.0, P3F[2]),
           *[([s30[b]], max((b + 1.6) * P3F[0] / NB, P3F[3] + (1.0 - P3F[3]) * b / NB), 0.0) for b in range(NB)])
    for c in c_par2:
        c.wait()

    def body(k, do5=True, do4=True, do3=True, do2=True, do1=True, j=None, order=None):
        order = order or ORDER
        at = (lambda d: k + d) if j is None else (lambda d: j + (k + d) if k + d else j)
        g2 = s2_gen(at(2)) if do2 else None
        for n in range(NV):
            g4 = s4_gen(at(0), n) if do4 else None
            st4 = [0, 0]
            n4 = order.count("4")

            def adv4(m):
                if not do4:
                    return
                st4[0] += 1
                while st4[1] < 72 * st4[0] / n4 - 3 or (st4[0] == n4 and st4[1] <= 72):
                    r = next(g4, None)
                    if r is None:
                        break
                    st4[1] = r

            def nat():
                if do1:
                    if n + 1 < NV:
                        s1_nat(at(3), n + 1, 1)
                    else:
                        s1_nat(jnp.minimum(at(4), NSTEP - 1), 0, 1)

            g1 = s1_grp(at(3), n) if do1 else None
            for tok in order:
                if tok == "5":
                    if do5 and n < NB:
                        s5_blk(at(-1), n, 0)
                        s5_blk(at(-1), n, 1)
                elif tok == "4":
                    adv4(1)
                elif tok in "ab" and do1:
                    next(g1)
                elif tok == "p" and do1:
                    run(g1)
                elif tok == "2" and do2:
                    next(g2, None)
                elif tok == "3" and do3 and n < NB:
                    s3_blk(at(1), n)
                elif tok == "n":
                    nat()
        if do2:
            run(g2)

    @pl.when(flag_s[0] == 1)
    def _():
        body(0, do5=False, order=ORD0)

    lax.fori_loop(0, 4, lambda j, c: (body(1, j=j), c)[1], 0)

    @pl.when(flag_s[0] == 1)
    def _():
        body(5, do1=False, order=ORD5)

    @pl.when(flag_s[0] == 1)
    def _():
        body(6, do1=False, do2=False, order=ORD6)

    @pl.when(flag_s[0] == 1)
    def _():
        _weave(([(lambda n=n: run(s4_gen(7, n, (0,))), 1.0) for n in range(NV)], 0.0, 1.0), (s5(6), 0.0, 1.0))

    @pl.when(flag_s[0] == 1)
    def _():
        _weave(([(lambda n=n: run(s4_gen(7, n, (4,))), 1.0) for n in range(NV)], 0.0, 1.0), (s5(7)[:8], 0.0, 1.0))

    _weave((s5(7)[8:], 0.0, 1.0))

    def total(i):
        halves = []
        for hf in range(2):
            t = acc_v[i, pl.ds(64 * hf, 8, stride=8), :]
            for s in range(1, 8):
                t = t + acc_v[i, pl.ds(64 * hf + s, 8, stride=8), :]
            halves.append(t)
        return jnp.concatenate(halves, 0)

    m2 = total(0) * (1.0 / D)
    var2 = jnp.maximum(total(1) * (1.0 / D) - m2 * m2, 0.0)
    sd2 = _rb(jnp.sqrt(_rb(_rb(var2) + EPS)))
    rs2 = 1.0 / sd2
    r = _rb((total(2) - m2 * wr_sum) * rs2)
    mean2 = fin_v[4] + m2
    fin_v[0] = rs2
    fin_v[1] = m2 * rs2
    fin_v[2] = rs2 + 1.0
    fin_v[3] = fin_v[4] - m2 * rs2

    tl = _iota((16, 128), 0)
    ll = _iota((16, 128), 1)
    lodd = (ll & 1) == 1
    toff = jnp.where((tl & 1) == 0, jnp.where(lodd, ll + 127, ll), jnp.where(lodd, ll + 128, (ll - 1) & 127))
    tok = (tl >> 1) * 256 + toff
    rbits = pltpu.bitcast(r, i32)
    srt = rbits ^ ((rbits >> 31) & 0x7FFFFFFF)
    key = pltpu.bitcast((((srt >> 16) + 32768) << 11) + (2047 - tok) + (1 << 28), f32)
    kk = key
    cand = []
    for _ in range(4):
        rm = jnp.broadcast_to(jnp.max(kk, axis=1, keepdims=True), (16, 128))
        cand.append(rm)
        kk = jnp.where(kk == rm, 0.0, kk)
    last = jnp.max(cand[3], axis=0, keepdims=True)
    kcol = None
    for j in range(TOPC):
        mx = jnp.max(cand[0], axis=0, keepdims=True)
        kcol = jnp.broadcast_to(mx, (8, 128)) if j == 0 else jnp.where(sub8 == j, mx, kcol)
        took = cand[0] == mx
        cand = [jnp.where(took, cand[i + 1] if i < 3 else 0.0, cand[i]) for i in range(4)]
    kc_v[...] = kcol

    @pl.when((last - mx)[0, 0] > 0.0)
    def _():
        k2 = key
        kc = None
        for j in range(TOPC):
            m1 = jnp.max(jnp.max(k2, axis=0, keepdims=True), axis=1, keepdims=True)
            kc = jnp.broadcast_to(m1, (8, 128)) if j == 0 else jnp.where(sub8 == j, m1, kc)
            k2 = jnp.where(k2 == m1, 0.0, k2)
        kc_v[...] = kc

    kcol = kc_v[...]
    kint = pltpu.bitcast(kcol, i32) - (1 << 28)
    tcol = 2047 - (kint & 2047)
    s16 = (kint >> 11) - 32768
    rsel = pltpu.bitcast((s16 ^ ((s16 >> 31) & 0x7FFF)) << 16, f32)
    gate = _rb(jax.nn.sigmoid(rsel))

    def classes(col):
        cls = jnp.zeros((8, 128), i32)
        for d in range(1, TOPC):
            cls = cls + jnp.where((col == pltpu.roll(col, d, 0)) & (sub8 >= d), 1, 0)
        return cls, jnp.max(cls, axis=0, keepdims=True)[0, 0] + 1

    wcol = tcol & 255
    pcol = jnp.where((wcol & 1) == 0, jnp.where(wcol < 128, wcol, wcol - 127),
                     jnp.where(wcol < 128, (wcol + 1) & 127, wcol - 128))
    ecol = ((tcol >> 8) << 1) | (tcol & 1)
    etile = [ecol[j, 0] for j in range(TOPC)]
    gcol, gn = classes(pcol)
    xs_v[...] = jnp.zeros((8, D), f32)

    def gather(c, carry):
        oh = (gcol == c) & (lane8 == pcol)
        ohi = jnp.where(oh, 1, 0)
        msk = [jnp.broadcast_to(ohi[j:j + 1], (8, 128)) == 1 for j in range(TOPC)]
        sa = sb = None
        for j in range(TOPC):
            fa = jnp.broadcast_to(fin_v[0, pl.ds(etile[j], 1), :], (8, 128))
            fb = jnp.broadcast_to(fin_v[1, pl.ds(etile[j], 1), :], (8, 128))
            sa, sb = (fa, fb) if j == 0 else (jnp.where(msk[j], fa, sa), jnp.where(msk[j], fb, sb))
        parts = []
        for q in range(D // 8 // GCH):
            mg = None
            for j in range(TOPC):
                cc = c1_v[GCH * q // NV, GCH * q % NV:GCH * q % NV + GCH, pl.ds(pl.multiple_of(8 * etile[j], 8), 8), :]
                mg = cc if j == 0 else jnp.where(msk[j], cc, mg)
            parts.append(mg * sa - sb)
        ln = jnp.concatenate(parts, 0).reshape(D, 128)
        xs_v[...] = xs_v[...] + _dot_nt(jnp.where(oh, 1.0, 0.0).astype(f32), ln)
        return carry

    lax.fori_loop(0, gn, gather, 0)
    xsel = xs_v[...]

    def rebuilt_rows():
        sdc = jnp.zeros((8, 1), f32)
        mc = jnp.zeros((8, 1), f32)
        sub1 = _iota((8, 1), 0)
        for j in range(TOPC):
            hitm = tok == jnp.broadcast_to(tcol[j:j + 1], (16, 128))
            red = lambda v: jnp.sum(jnp.sum(jnp.where(hitm, v, 0.0), axis=0, keepdims=True), axis=1, keepdims=True)
            sdc = jnp.where(sub1 == j, red(sd2), sdc)
            mc = jnp.where(sub1 == j, red(mean2), mc)
        return xsel * (sdc + 1.0) + mc

    def outp(b, g0, g1):
        sc = [jnp.where(top, jnp.broadcast_to(fin_v[i, 2 * b:2 * b + 1, :], (8, 128)),
                        jnp.broadcast_to(fin_v[i, 2 * b + 1:2 * b + 2, :], (8, 128))) for i in (2, 3)]
        for g in range(g0, g1):
            a = _rb(c1_v[g // NV, g % NV, pl.ds(16 * b, 8, stride=2), :] * sc[0] + sc[1])
            c = _rb(c1_v[g // NV, g % NV, pl.ds(16 * b + 1, 8, stride=2), :] * sc[0] + sc[1])
            w = (pltpu.bitcast(a, u32) >> 16) | pltpu.bitcast(c, u32)
            out_w[g, b] = jnp.where(mask2, w, pltpu.roll(pltpu.roll(w, 4, 0), 127, 1))

    opieces = [functools.partial(outp, b, 24 * i, 24 * i + 24) for b in range(NB) for i in range(3)]

    tilec = tcol >> 7
    lanec = tcol & 127
    aux = {}

    def late_scalars():
        tiles = [tilec[j, 0] for j in range(TOPC)]
        hit = 0
        dup = []
        for j in range(TOPC):
            dup.append((hit >> tiles[j]) & 1)
            hit = hit | (1 << tiles[j])
        free, cnt = [], 0
        for t in range(16):
            un = 1 - ((hit >> t) & 1)
            free.append(jnp.where(un == 1, cnt, -1))
            cnt = cnt + un
        late, nd, mask = [tiles[0]], 0, hit
        for j in range(1, TOPC):
            rep = 0
            for t in range(16):
                rep = jnp.where(free[t] == nd, t, rep)
            late.append(jnp.where(dup[j] == 1, rep, tiles[j]))
            mask = mask | (1 << late[j])
            nd = nd + dup[j]
        aux.update(tiles=tiles, late=late, mask=mask)
        bs_v[...] = rebuilt_rows()
        aux["clscol"], aux["ncls"] = classes(lanec)
        for j in range(TOPC):
            code = jnp.where((tilec == late[j]) & (lane8 == lanec), aux["clscol"], -1)
            lm_v[j] = jnp.broadcast_to(jnp.max(code, axis=0, keepdims=True), (8, 128))

    def tile_idx(t, g0=0, ng=D // 8):
        if isinstance(t, int):
            return (pl.ds(g0, ng), t // 2, pl.ds(8 * (t % 2), 8), slice(None))
        return (pl.ds(g0, ng), t >> 1, pl.ds(pl.multiple_of(8 * (t & 1), 8), 8), slice(None))

    def ocopy(idx):
        return cp(out_v.at[idx], out_h.at[idx], osem.at[0])

    def early():
        for t in range(16):
            @pl.when(((aux["mask"] >> t) & 1) == 0)
            def _():
                ocopy(tile_idx(t)).start()

    for c in range(NCH):
        for cc in c_w[c]:
            cc.wait()
        mine = opieces[OSPLIT[c]:OSPLIT[c + 1]]
        nsub = max(1, FCH[c] // FSUB)
        sub = FCH[c] // nsub
        for u in range(nsub):
            sl = slice(FOFF[c] + u * sub, FOFF[c] + (u + 1) * sub)
            g = _rb(_dot(xsel, wmat(wg_w, 0, D, sl.start, sub)))
            up = _rb(_dot(xsel, wmat(wu_w, 0, D, sl.start, sub)))
            if c == 0 and u == 0:
                late_scalars()
            for fn in mine[u * len(mine) // nsub:(u + 1) * len(mine) // nsub]:
                fn()
            act_v[:, sl] = _rb(_rb(g * jax.nn.sigmoid(g)) * up)
        if c == WCH:
            early()

    clscol = aux["clscol"]
    onehot = lambda c: jnp.where((clscol == c) & (lane8 == lanec), 1.0, 0.0).astype(f32)
    bc = lambda v, j: jnp.broadcast_to(v[j:j + 1], (8, 128))

    def down(p, c0, nc):
        r = slice(POFF[p], POFF[p] + PART[p])
        yc = _dot_nt(act_v[:, c0:c0 + nc], wmat(wd_w, POFF[p], PART[p], c0, nc))
        y_v[:, r] = yc if c0 == 0 else y_v[:, r] + yc

    def place(p, fast):
        r0, nr = POFF[p], PART[p]
        g0, ng = r0 // 8, nr // 8
        gt = jnp.concatenate([gate] * ((nr + 127) // 128), 1)[:, :nr]
        newrow = _rb(bs_v[:, r0:r0 + nr] + _rb(_rb(y_v[:, r0:r0 + nr]) * gt))
        tn = lambda oh: lax.dot_general(newrow, oh, (((0,), (0,)), ((), ())), preferred_element_type=f32)
        if fast:
            uu = tn(jnp.concatenate([onehot(0), onehot(1)], 1))
            for c in range(2):
                u_v[c, g0:g0 + ng] = uu[:, 128 * c:128 * (c + 1)].reshape(ng, 8, 128)
        else:
            for c in range(TOPC):
                u_v[c, g0:g0 + ng] = tn(onehot(c)).reshape(ng, 8, 128)

    def write(p, fast):
        g0, ng = POFF[p] // 8, PART[p] // 8
        for j in range(TOPC):
            idx = tile_idx(aux["late"][j], g0, ng)
            new = out_v[idx].astype(f32)
            code = lm_v[j]
            for c in range(2 if fast else TOPC):
                new = jnp.where(code == c, u_v[c, g0:g0 + ng], new)
            sg_v[j, g0:g0 + ng] = new.astype(bf16)
            cp(sg_v.at[j, pl.ds(g0, ng)], out_h.at[idx], osem.at[0]).start()

    def dwait(p):
        for cc in c_d[p]:
            cc.wait()

    NP = len(PART)
    dwait(0)
    rest = opieces[OSPLIT[NCH]:]
    nq = 4
    for q in range(nq):
        down(0, q * F // nq, F // nq)
        for fn in rest[q * len(rest) // nq:(q + 1) * len(rest) // nq]:
            fn()

    @pl.when(aux["ncls"] <= 2)
    def _():
        for p in range(1, NP):
            dwait(p)
            down(p, 0, DSPL[p])
            place(p - 1, True)
            down(p, DSPL[p], F - DSPL[p])
            write(p - 1, True)
        place(NP - 1, True)
        write(NP - 1, True)

    @pl.when(aux["ncls"] > 2)
    def _():
        for p in range(1, NP):
            dwait(p)
            down(p, 0, F)
        for p in range(NP):
            place(p, False)
            write(p, False)

    cp(out_h, out_h, osem.at[0]).wait()


@jax.jit
def pallas_sequential_preLN__ssm_conv_s4__moe_arch_mod__prompt_kernel(
    A_u: jax.Array,
    A_A_re: jax.Array,
    A_A_im: jax.Array,
    A_B_re: jax.Array,
    A_B_im: jax.Array,
    A_C_re: jax.Array,
    A_C_im: jax.Array,
    A_log_dt: jax.Array,
    A_Dskip: jax.Array,
    B_x: jax.Array,
    B_w_r: jax.Array,
    B_w_gate: jax.Array,
    B_w_up: jax.Array,
    B_w_down: jax.Array,
):
    hbm = pl.BlockSpec(memory_space=pltpu.MemorySpace.HBM)
    vm = pltpu.VMEM
    G8 = D // 8
    wshape = (D // 16, F // 128, 16, 128)
    wview = lambda w: w.reshape(D // 16, 2, 8, F // 128, 128).transpose(0, 1, 3, 2, 4)
    scratch = [
        vm((G8, NB, 16, 128), bf16), vm((6, NSTEP, 128, N), bf16), vm((D,), bf16), vm((D,), bf16), vm((D,), bf16),
        vm((CT_ROWS, 128), f32), vm(wshape, bf16), vm(wshape, bf16), vm(wshape, bf16), vm((G8, NB + 1, 16, 128), bf16),
        vm((9, 4, 144, 128), bf16), vm((2, 2, 2, 144, 128), bf16), vm((3, NSTEP, 96, 128), f32),
        vm((NV, 2, 136, 128), f32), vm((NSTEP, 12, 56, 128), f32), vm((NSTEP, 96, 128), f32),
        vm((NSTEP, NB, 6, R, 128), f32), vm((NSTEP, NB, 6, R, 128), f32),
        vm((NSTEP, NB, 2, R, 256), f32), vm((NSTEP, 12, 136, 128), f32), vm((2, 17, 8, 128), f32),
        vm((3, 136, 128), f32), vm((5, 16, 128), f32), vm((TOPC, G8, 8, 128), f32),
        vm((R, 512), f32), vm((8, D), f32), vm((NV, 4, 8, 128), f32),
        vm((8, 128), f32), vm((8, D), f32), vm((8, D), f32), vm((8, F), f32),
        vm((TOPC, G8, 8, 128), bf16), vm((TOPC, 8, 128), i32), vm((8, D), f32), pltpu.SMEM((1,), i32),
        pltpu.SemaphoreType.DMA((5 + NCH + len(PART),)), pltpu.SemaphoreType.DMA((1,)),
    ]
    xv = A_u[0].T.reshape(G8, 8, 16, 128).transpose(0, 2, 1, 3).reshape(G8, NB, 16, 128)
    out = pl.pallas_call(
        _kernel,
        out_shape=jax.ShapeDtypeStruct((G8, NB, 16, 128), bf16),
        in_specs=[hbm] * 13,
        out_specs=hbm,
        scratch_shapes=scratch,
        compiler_params=pltpu.CompilerParams(vmem_limit_bytes=120 * 1024 * 1024, disable_bounds_checks=NOBC),
    )(xv, *[p.reshape(NSTEP, R, N) for p in (A_A_re, A_A_im, A_B_re, A_B_im, A_C_re, A_C_im)], A_log_dt, A_Dskip, B_w_r,
      wview(B_w_gate), wview(B_w_up), wview(B_w_down.T))
    return out.reshape(G8, 16, 8, 128).transpose(0, 2, 1, 3).reshape(D, L).T[None]
```

```python
import functools

import numpy as np
import jax
import jax.numpy as jnp
from jax import lax
import jax.experimental.pallas as pl
import jax.experimental.pallas.tpu as pltpu

f32 = jnp.float32
bf16 = jnp.bfloat16
i32 = jnp.int32
u32 = jnp.uint32

L, D, N, F, TOPC = 2048, 576, 128, 4608, 8
NB = 8
NV = 9
R = NV * 8
NSTEP = D // R
EPS = 1e-5

_XL1 = [(1, 5), (2, 6), (3, 7), (4, 8), (258, 516), (260, 520), (262, 772), (264, 776),
        (1288, 1032), (1800, 1544)]
_XSH = [0, 1, 2, 3, 0, 1, 2, 3, 0, 1]


def _bf16_round_int(j):
    u = np.asarray(j, np.float32).view(np.uint32).astype(np.uint64)
    r = ((u + 0x7FFF + ((u >> 16) & 1)) >> 16) << 16
    return r.astype(np.uint32).view(np.float32).astype(np.int64)


def _chunk_values():
    vals = -np.ones((5, 128), np.int64)
    for j in range(10):
        for p in range(2):
            ch = (j // 4) * 2 + p if j < 8 else 4
            extra = 2 * p if j >= 8 else 0
            for l0 in range(32):
                vals[ch, (4 * (31 - l0) + 4 * p + _XSH[j] + extra + 8) % 128] = _XL1[j][p] + 8 * l0
    assert (vals >= 0).all()
    return vals


_PASSES = [(0, "A0"), (0, "A1"), (1, "B"), (2, "Cp"), (3, "C"), (4, "Dp"), (5, "D"), (6, "D"), (7, "D")]
_SETS = [[0], [1], [2], [3, 4], [5, 6, 7, 8]]


def _tables():
    cv = _chunk_values()
    cvp = {"A0": cv[0], "A1": cv[1], "B": cv[2], "C": cv[3], "D": cv[4]}
    cvp["Cp"] = cv[3].copy(); cvp["Cp"][11] = cv[2][11]
    cvp["Dp"] = cv[4].copy(); cvp["Dp"][15] = cv[3][15]
    sup = [[[] for _ in range(128)] for _ in _PASSES]
    for b in range(NB):
        for j in range(1, 257):
            lag = 256 * b + j
            if lag > L - 1 or lag == 257:
                continue
            v = int(_bf16_round_int(lag))
            hit = [(i, int(np.nonzero(cvp[nm] == v)[0][0])) for i, (pb, nm) in enumerate(_PASSES)
                   if pb == b and (cvp[nm] == v).any()]
            assert len(hit) == 1, (b, j, v, hit)
            sup[hit[0][0]][hit[0][1]].append(j)
    assert cv[1][15] == _bf16_round_int(257)
    code = np.zeros((len(_PASSES), 128), np.int64)
    for i, (pb, _) in enumerate(_PASSES):
        for r in range(128):
            js = sup[i][r]
            if js:
                assert js == list(range(js[0], js[-1] + 1))
                code[i, r] = js[0] + js[-1] + 1024 * len(js) + 16384 * (pb % 2)
    seeds, masks = [], {}
    for ps in _SETS:
        seeds.append([int(x) for x in sum(code[i, 16:24] for i in ps)])
        for i in ps:
            masks[i] = [int(x > 0) for x in code[i, 16:24]]
            for v in range(2, 17):
                r0 = 8 * (v % 16)
                assert (code[i, r0:r0 + 8] == (np.array(seeds[-1]) - 32 * (v - 2)) * np.array(masks[i])).all()
    return seeds, [[int(x) for x in code[i, 8:16]] for i in range(len(_PASSES))], masks


_GSEED, _GROW1, _GMASK = _tables()


def _sincos_coeffs():
    r = np.cos(np.pi * (np.arange(4000) + .5) / 4000) * 0.5
    z = r * r
    s = np.linalg.lstsq(np.stack([z ** k for k in range(4)], 1), np.sin(np.pi / 2 * r) / r, rcond=None)[0]
    c = np.linalg.lstsq(np.stack([z ** k for k in range(1, 5)], 1), np.cos(np.pi / 2 * r) - 1, rcond=None)[0]
    return [float(x) for x in s], [float(x) for x in c]


_SC, _CC = _sincos_coeffs()


def _cmul(a, b):
    return (a[0] * b[0] - a[1] * b[1], a[0] * b[1] + a[1] * b[0])


def _cmulc(a, b):
    return (a[0] * b[0] + a[1] * b[1], a[1] * b[0] - a[0] * b[1])


def _csq(a):
    return ((a[0] - a[1]) * (a[0] + a[1]), (a[0] + a[0]) * a[1])


def _quarter_polys(r):
    r2 = r * r
    s = r * (_SC[0] + r2 * (_SC[1] + r2 * (_SC[2] + r2 * _SC[3])))
    c = 1.0 + r2 * (_CC[0] + r2 * (_CC[1] + r2 * (_CC[2] + r2 * _CC[3])))
    return s, c


def _rotate_quadrant(s, c, ki):
    swap = (ki & 1) == 1
    s2 = jnp.where(swap, c, s)
    c2 = jnp.where(swap, s, c)
    s2 = pltpu.bitcast(pltpu.bitcast(s2, i32) ^ ((ki & 2) << 30), f32)
    c2 = pltpu.bitcast(pltpu.bitcast(c2, i32) ^ (((ki + 1) & 2) << 30), f32)
    return s2, c2


def _sincos(th):
    z = th * (2.0 / np.pi)
    k = jnp.round(z)
    s, c = _quarter_polys(z - k)
    return _rotate_quadrant(s, c, k.astype(i32))


def _reduce_small(z):
    big = 12582912.0
    t = z + big
    return _quarter_polys(z - (t - big)) + (pltpu.bitcast(t, i32),)


def _rb(x):
    return x.astype(bf16).astype(f32)


def _dot(a, b):
    return jnp.dot(a, b, preferred_element_type=f32)


def _dot_nt(a, b):
    return lax.dot_general(a, b, (((1,), (1,)), ((), ())), preferred_element_type=f32)


def _iota(shape, dim):
    return lax.broadcasted_iota(i32, shape, dim)


S4MODE='CC'
TILE=4
YSPLIT=1
ZT=1
ORDER='4ab44342np445'
ORD0='4ab442n4p4345'
ORD5='4a424n44b345p'
ORD6='45a4b244p3n44'
NPC=3
P3F=(0.9,0.4,0.55,0.3)
GCH=3
NOBC=True
CT_ROWS=320
WCH=0
OSPLIT=[0,24,24]
RELAY=(1,1,0)
NOSC=True
PART=(256,128,128,64)
DSPL=(0,2560,2560,4096)
FSUB=1280
FCH=(3840,768)
NCH = len(FCH)
FOFF = [sum(FCH[:i]) for i in range(NCH)]
POFF = [sum(PART[:i]) for i in range(len(PART))]

def _weave(*streams):
    items = []
    for si, (pieces, lo, hi) in enumerate(streams):
        tot = float(sum(c for _, c in pieces))
        cum = 0.0
        for pi, (fn, c) in enumerate(pieces):
            items.append((lo + max(hi - lo, 0.0) * (cum + 0.5 * c) / tot, si, pi, fn))
            cum += c
    for _, _, _, fn in sorted(items, key=lambda t: t[:3]):
        fn()


def _kernel(x_h, are_h, aim_h, bre_h, bim_h, cre_h, cim_h, ldt_h, dsk_h, wr_h, wg_h, wu_h, wd_h,
            out_h,
            x_v, par_v, ldt_v, dsk_v, wr_v, ct_v, wg_v, wu_v, wd_v, out_v,
            g_v, f_v, col_v, st_v, kd_v, k0_v, kh_v, uh_v, zs_v, c1_v, s1_v, acc_v, fin_v, u_v, zt_v, y_v, pv_v, kc_v, xs_v, bs_v, act_v, sg_v, lm_v, rw_v, flag_s,
            sem, osem):
    cp = pltpu.make_async_copy
    c_vec = [cp(ldt_h, ldt_v, sem.at[1]), cp(dsk_h, dsk_v, sem.at[1]), cp(wr_h, wr_v, sem.at[1])]
    PH = 4
    par_h = (are_h, aim_h, bre_h, bim_h, cre_h, cim_h)
    c_par = [cp(h.at[pl.ds(0, PH)], par_v.at[i, pl.ds(0, PH), pl.ds(0, R)], sem.at[2]) for i, h in enumerate(par_h)]
    c_par2 = [cp(h.at[pl.ds(PH, NSTEP - PH)], par_v.at[i, pl.ds(PH, NSTEP - PH), pl.ds(0, R)], sem.at[3])
              for i, h in enumerate(par_h)]
    c_x = cp(x_h, x_v, sem.at[4])
    def wcp(h, v, rp, ct, s):
        if len(v.shape) == 2:
            r = slice(None) if isinstance(rp, slice) else pl.ds(rp.start * 16, rp.size * 16)
            c = slice(None) if isinstance(ct, slice) else pl.ds(ct.start * 128, ct.size * 128)
            return [cp(h.at[r, c], v.at[r, c], s)]
        return [cp(h.at[rp, hf, ct], v.at[rp, ct, pl.ds(8 * hf, 8), :], s) for hf in range(2)]

    c_w = [wcp(wg_h, wg_v, slice(None), pl.ds(FOFF[c] // 128, FCH[c] // 128), sem.at[5 + c])
           + wcp(wu_h, wu_v, slice(None), pl.ds(FOFF[c] // 128, FCH[c] // 128), sem.at[5 + c]) for c in range(NCH)]
    c_d = [wcp(wd_h, wd_v, pl.ds(POFF[p] // 16, PART[p] // 16), slice(None), sem.at[5 + NCH + p])
           for p in range(len(PART))]
    for c in c_vec + c_par + [c_x] + c_par2 + sum(c_w, []) + sum(c_d, []):
        c.start()

    flag_s[0] = 1
    x_w = x_v.bitcast(u32)
    wg_w, wu_w, wd_w = [v.bitcast(u32) if len(v.shape) == 4 else v for v in (wg_v, wu_v, wd_v)]

    def wmat(w, r0, nr, c0, nc):
        if len(w.shape) == 2:
            return w[r0:r0 + nr, c0:c0 + nc]
        return jnp.concatenate([pltpu.bitcast(w[r0 // 16:(r0 + nr) // 16, t], bf16).reshape(nr, 128)
                                for t in range(c0 // 128, (c0 + nc) // 128)], 1)

    out_w = out_v.bitcast(u32)
    g_w = g_v.bitcast(u32)
    f_w = f_v.bitcast(u32)
    sub8 = _iota((8, 128), 0)
    lane8 = _iota((8, 128), 1)

    acc_v[...] = jnp.zeros(acc_v.shape, f32)
    for n in range(NV):
        for ri in range(2):
            st_v[n, ri, 104:112, :] = jnp.full((8, 128), 1.0 - ri, f32)
    kp = (2 * lane8 + 1).astype(f32)

    def rows_const(vals):
        out = jnp.full((8, 128), vals[0], i32)
        for r in range(1, 8):
            if vals[r] != vals[0]:
                out = jnp.where(sub8 == r, vals[r], out)
        return out

    def phasor(z):
        sn, cs = _rotate_quadrant(*_reduce_small(-z))
        return cs, sn

    NS = [0, 1, 2, 3, 4, 5, 7, 9]
    for q in range(2):
        sn = _rotate_quadrant(*_reduce_small((kp + 512.0 * q) * (rows_const(NS).astype(f32) * (1.0 / 512))))[0]
        ct_v[304 + 8 * q:312 + 8 * q, :] = sn / (256.0 * jnp.broadcast_to(sn[1:2], (8, 128)))

    def grows(vals):
        ab = rows_const([v & 1023 for v in vals])
        z = kp * (ab.astype(f32) * (-1.0 / 512))
        if any(v >> 14 for v in vals):
            z = z - rows_const([v >> 14 for v in vals]).astype(f32) * (kp - 1.0)
        sn, cs, ki = _reduce_small(z)
        ns = [NS.index((v >> 10) & 15) for v in vals]
        out = []
        for q in range(2):
            row = lambda i: jnp.broadcast_to(ct_v[304 + 8 * q + i:305 + 8 * q + i, :], (8, 128))
            amp = None
            for i in sorted(set(ns)):
                bits = sum(1 << r for r in range(8) if ns[r] == i)
                amp = row(i) if amp is None else jnp.where(((bits >> sub8) & 1) == 1, row(i), amp)
            pi, pr = _rotate_quadrant(sn, cs, ki if q == 0 else ki - ab)
            out += [pr * amp, pi * amp]
        return out

    for v4 in range(4):
        e = phasor(kp * ((sub8 + 8 * v4).astype(f32) * (1.0 / 32)))
        ct_v[8 * v4:8 * v4 + 8, :] = e[0]
        ct_v[32 + 8 * v4:40 + 8 * v4, :] = e[1]
    for si in range(5):
        for q, val in enumerate(grows(_GSEED[si])):
            ct_v[64 + 32 * si + 8 * q:72 + 32 * si + 8 * q, :] = val
    for i in range(len(_PASSES)):
        for q, val in enumerate(grows(_GROW1[i])):
            g_v[i, q, 8:16, :] = val.astype(bf16)
    for q, val in enumerate(grows([2 + 1024 + 16384] * 8)):
        ct_v[272 + 8 * q:280 + 8 * q, :] = val
    s8 = np.arange(8)
    je = np.where(s8 % 2 == 0, s8, 127 + s8)
    jo = np.where(s8 % 2 == 0, s8 - 1, 128 + s8)
    for t, jj in enumerate((je, jo, jo % 128 + 128 * (s8 % 2))):
        e = phasor(kp * (rows_const([int(x) for x in jj]).astype(f32) * (1.0 / 256)))
        ct_v[224 + 16 * t:232 + 16 * t, :] = e[0]
        ct_v[232 + 16 * t:240 + 16 * t, :] = e[1]
    for c in c_vec:
        c.wait()

    rows = [_rb(jnp.exp(ldt_v[...].astype(f32).reshape(1, D))),
            dsk_v[...].astype(f32).reshape(1, D),
            wr_v[...].astype(f32).reshape(1, D)]
    wr_sum = jnp.sum(rows[2], axis=1, keepdims=True)

    def columns(which):
        for j in range(5):
            w = 128 if j < 4 else 64
            eye = _iota((w, w), 0) == _iota((w, w), 1)
            m = jnp.concatenate([jnp.where(eye, jnp.broadcast_to(rw_v[i:i + 1, j * 128:j * 128 + w], (w, w)), 0.0)
                                 for i in which], 0)
            res = _dot(m, jnp.ones((w, 128), f32))
            for n, i in enumerate(which):
                for g in range(w // 8):
                    k, m8 = divmod(16 * j + g, NV)
                    col_v[i, k, 8 * m8:8 * m8 + 8, :] = res[n * w + 8 * g:n * w + 8 * g + 8]

    for i in range(3):
        rw_v[i:i + 1, :] = rows[i]
    columns((0,))

    def e8(v):
        return (jnp.broadcast_to(ct_v[v:v + 1, :], (8, 128)), jnp.broadcast_to(ct_v[32 + v:33 + v, :], (8, 128)))

    for si, ps in enumerate(_SETS):
        sd = [ct_v[64 + 32 * si + 8 * q:72 + 32 * si + 8 * q, :] for q in range(4)]
        mk = {}
        for i in ps:
            if len(ps) > 1:
                bits = sum(b << s for s, b in enumerate(_GMASK[i]))
                mk[i] = ((bits >> sub8) & 1) == 1
        for v in range(2, 17):
            if v == 2:
                vals = sd
            else:
                ev = e8(2 * (v - 2))
                vals = list(_cmulc((sd[0], sd[1]), ev)) + list(_cmulc((sd[2], sd[3]), ev))
            for i in ps:
                for q in range(4):
                    val = vals[q] if len(ps) == 1 else jnp.where(mk[i], vals[q], 0.0)
                    g_v[i, q, 8 * (v % 16):8 * (v % 16) + 8, :] = val.astype(bf16)
    sig = jnp.where((lane8 & 1) == 0, 1.0, -1.0).astype(f32)
    for h in range(2):
        sd = (ct_v[224 + 16 * h:232 + 16 * h, :], ct_v[232 + 16 * h:240 + 16 * h, :])
        for v in range(16):
            if v == 0:
                vals = sd if h == 0 else (ct_v[256:264, :], ct_v[264:272, :])
            else:
                vals = _cmul(sd, e8(v))
            for q in range(2):
                f_v[0, h, q, 8 * v:8 * v + 8, :] = vals[q].astype(bf16)
                f_v[1, h, q, 8 * v:8 * v + 8, :] = (vals[q] * sig).astype(bf16)

    def gmat(i):
        return jnp.concatenate([pltpu.bitcast(g_w[i, q, 0:64, :], bf16) for q in range(4)], 1)

    def fmat(ver, h):
        return jnp.concatenate([pltpu.bitcast(f_w[ver, h, q, 0:64, :], bf16) for q in range(2)], 1)

    revmask = (sub8 & 2) == 0
    lm = lane8 & 3

    def s1_nat(k, n0, nn):
        rr = 8 * nn
        ld = lambda i: par_v[i, k, 8 * n0:8 * n0 + rr, :].astype(f32)
        dt = col_v[0, k, 8 * n0:8 * n0 + rr, :]
        e = jnp.exp(dt * ld(0))
        s, c = _sincos(dt * ld(1))
        a1 = (e * c, e * s)
        w = _cmul((ld(4), ld(5)), (dt * ld(2), dt * ld(3)))
        k0_v[k, 8 * n0:8 * n0 + rr, :] = jnp.broadcast_to(jnp.sum(w[0], axis=1, keepdims=True), (rr, 128))
        w = (w[0], -w[1])
        rev = lambda v: jnp.where(revmask, pltpu.roll(v, 2, 0), pltpu.roll(v, 6, 0))

        def put(arr, slots, fn=None):
            for n in range(nn):
                for ri in range(2):
                    v = arr[ri][8 * n:8 * n + 8]
                    if fn is not None:
                        v = fn(v)
                    for q in slots:
                        st_v[n0 + n, ri, q * 8:q * 8 + 8, :] = v

        put(w, (0, 1)); put(a1, (2, 3))
        a2 = _csq(a1); put(a2, (5,))
        a4 = _csq(a2); put(a4, (6,))
        put(_cmul(a4, a1), (4,))
        a8 = _csq(a4); put(a8, (12,), rev)
        t = _csq(a8); put(t, (14, 15), rev)
        for _ in range(4):
            t = _csq(t)
        put(t, (7, 11))
        t = _csq(t); put(t, (8, 9))
        put(_csq(t), (10,))

    def s1_grp(k, n):
        mix = lambda q: tuple(jnp.concatenate([st_v[n, ri, pl.ds(q * 8 + g, 8, stride=2), :] for g in range(2)], 0)
                              for ri in range(2))
        y = [mix(12)]
        a16d = mix(14)
        if YSPLIT == 1:
            for _ in range(15):
                y.append(_cmul(y[-1], a16d))
        else:
            y.append(_cmul(y[0], a16d))
            a32d = _csq(a16d)
            for i in range(2, 16):
                y.append(_cmul(y[i - 2], a32d))
        yield
        wd = mix(0); a1d = mix(2); m1 = mix(5)
        v = [_cmulc(wd, mix(3))]
        for _ in range(3):
            v.append(_cmulc(v[-1], a1d))
        v4 = _cmulc(_cmulc(wd, m1), mix(7))
        v5 = _cmulc(v4, m1); v6 = _cmulc(v4, mix(6)); v7 = _cmulc(v6, m1)
        v8 = _cmulc(v7, mix(10)); v9 = _cmulc(v8, mix(8))
        v += [v4, v5, v6, v7, v8, v9]
        os_ = []
        for g in range(2):
            cat = lambda ts: jnp.concatenate([jnp.concatenate([t[ri][8 * g:8 * g + 8] for t in ts], 0)
                                              for ri in range(2)], 1)
            os_.append(_dot_nt(cat(v), cat(y[::-1])))
        yield
        for g in range(2):
            o = os_[g]
            ro = [pltpu.roll(o[8 * j:8 * j + 8], _XSH[j] + 5, 1, stride=1, stride_axis=0) for j in range(10)]
            sel4 = lambda q: jnp.where(lm == 0, q[0], jnp.where(lm == 1, q[1], jnp.where(lm == 2, q[2], q[3])))
            kd_v[k, n, pl.ds(g, 8, stride=2), :] = sel4(ro[0:4])
            kd_v[k, n, pl.ds(16 + g, 8, stride=2), :] = sel4(ro[4:8])
            kd_v[k, n, pl.ds(32 + g, 8, stride=2), :] = jnp.where(lm == 0, ro[8], ro[9])

    def run(gen):
        for _ in gen:
            pass

    s1n = lambda k: [(functools.partial(s1_nat, k, 3 * i, 3), 1.0) for i in range(3)]
    s1g = lambda k: [(lambda n=n: run(s1_grp(k, n)), 1.0) for n in range(NV)]

    laneR = _iota((R, 128), 1)
    lmR = laneR & 3

    def s2_gen(k):
        ch = lambda c: kd_v[k, 0:NV, 8 * c:8 * c + 8, :].reshape(R, 128)
        for b in range(NB):
            if b == 0:
                k0 = (k0_v[k, 0:R, :] + col_v[1, k, 0:R, :]) * (1.0 / 256.0)
                z = _dot(ch(0), gmat(0)) if ZT else None
                dd = jnp.where(lmR < 2, ch(4), pltpu.roll(ch(5), 2, 1))
                kd_v[k, 0:NV, 48:56, :] = dd.reshape(NV, 8, 128)
                if ZT:
                    zt_v[...] = z
                    yield
                    z = _dot(ch(1), gmat(1)) + zt_v[...]
                else:
                    z = _dot(jnp.concatenate([ch(0), ch(1)], 1), jnp.concatenate([gmat(0), gmat(1)], 0))
            elif b == 1:
                k256 = jnp.sum(jnp.where(laneR == 15, ch(1), 0.0), axis=1, keepdims=True)
                pat = jnp.concatenate([ct_v[272 + 8 * q:273 + 8 * q, :] for q in range(4)], 1)
                z = _dot(ch(2), gmat(2)) + k256 * pat
            elif b == 2:
                z = _dot(jnp.where(laneR == 11, ch(2), ch(3)), gmat(3))
            elif b == 3:
                z = _dot(ch(3), gmat(4))
            elif b == 4:
                z = _dot(jnp.where(laneR == 15, ch(3), ch(6)), gmat(5))
            else:
                z = _dot(ch(6), gmat(b + 1))
            for s in range(2):
                kr = z[:, 256 * s:256 * s + 128]
                ki = z[:, 256 * s + 128:256 * s + 256]
                if b == 0:
                    kr = kr + k0
                kh_v[k, b, 3 * s] = kr
                if S4MODE[0] == "L":
                    kh_v[k, b, 3 * s + 1] = kr + ki
                    kh_v[k, b, 3 * s + 2] = ki - kr
                else:
                    kh_v[k, b, 3 * s + 1] = ki
            yield

    def s2(k):
        gen = s2_gen(k)
        return [(lambda: next(gen, None), 1.0) for _ in range(9)]

    mask2 = (sub8 < 4) == ((lane8 & 1) == 0)
    top = sub8 < 4

    def ln1_pieces(b, npc):
        state = {}
        per = (D // 8) // npc

        def piece(i):
            for g in range(i * per, (i + 1) * per):
                m = x_w[g, b]
                eo = jnp.where(mask2, m, pltpu.roll(pltpu.roll(m, 4, 0), 1, 1))
                a = pltpu.bitcast(eo << 16, f32)
                c = pltpu.bitcast(eo & jnp.uint32(0xFFFF0000), f32)
                if g == 0:
                    state["sh"] = jnp.where(top, jnp.broadcast_to(a[0:1], (8, 128)),
                                            jnp.broadcast_to(a[4:5], (8, 128)))
                a = a - state["sh"]
                c = c - state["sh"]
                c1_v[g // NV, g % NV, pl.ds(16 * b, 8, stride=2), :] = a
                c1_v[g // NV, g % NV, pl.ds(16 * b + 1, 8, stride=2), :] = c
                new = [a, c, a * a, c * c]
                state["acc"] = new if g == 0 else [p + q for p, q in zip(state["acc"], new)]
            if i == npc - 1:
                acc = state["acc"]
                s1, s2_ = acc[0] + acc[1], acc[2] + acc[3]
                for h in range(2):
                    m = jnp.sum(s1[4 * h:4 * h + 4], axis=0, keepdims=True) * (1.0 / D)
                    var = jnp.sum(s2_[4 * h:4 * h + 4], axis=0, keepdims=True) * (1.0 / D) - m * m
                    rs = 1.0 / _rb(jnp.sqrt(_rb(_rb(jnp.maximum(var, 0.0)) + EPS)))
                    s1_v[0, 2 * b + h] = jnp.broadcast_to(rs, (8, 128))
                    sh = state["sh"][4 * h:4 * h + 1]
                    s1_v[1, 2 * b + h] = jnp.broadcast_to((_rb(m + sh) - sh) * rs, (8, 128))
                    fin_v[4, 2 * b + h:2 * b + h + 1, :] = state["sh"][4 * h:4 * h + 1]

        return [(functools.partial(piece, i), 1.0) for i in range(npc)]

    def s3_blk(k, b):
        et = []
        for h in range(2):
            c = c1_v[k, 0:NV, 16 * b + 8 * h:16 * b + 8 * h + 8, :]
            u = (c * s1_v[0, 2 * b + h] - s1_v[1, 2 * b + h]).reshape(R, 128)
            et.append(_dot(u, fmat(b % 2, h)))
        er, ei, tr, ti = et[0][:, :128], et[0][:, 128:], et[1][:, :128], et[1][:, 128:]
        if S4MODE[1] == "C":
            for q, v in enumerate((er, ei, tr, ti)):
                uh_v[k, b, q] = v
        else:
            for s, (pr, pi) in enumerate(((er + tr, ei + ti), (er - tr, ei - ti))):
                uh_v[k, b, 3 * s] = pr + pi
                uh_v[k, b, 3 * s + 1] = pi
                uh_v[k, b, 3 * s + 2] = pr

    s3 = lambda k: [(functools.partial(s3_blk, k, b), 1.0) for b in range(NB)]

    def s4_gen(k, n, groups=None):
        sl = slice(8 * n, 8 * n + 8)

        def utrip(i, s):
            if S4MODE[1] == "L":
                return [uh_v[k, i, 3 * s + q, sl, :] for q in range(3)]
            er, ei, tr, ti = [uh_v[k, i, q, sl, :] for q in range(4)]
            pr, pi = (er + tr, ei + ti) if s == 0 else (er - tr, ei - ti)
            return [pr + pi, pi, pr]

        prev = None
        done = 0
        if groups is not None and groups[0] > 0:
            prev = [(pv_v[n, 2 * h], pv_v[n, 2 * h + 1]) for h in range(2)]
        for b0 in (range(0, NB, TILE) if groups is None else groups):
            yy = []
            for s in range(2):
                acc = [None] * TILE
                win = {}
                for j in range(b0 + TILE):
                    if S4MODE[0] == "L":
                        kk = [kh_v[k, j, 3 * s + q, sl, :] for q in range(3)]
                    else:
                        kr, ki = kh_v[k, j, 3 * s, sl, :], kh_v[k, j, 3 * s + 1, sl, :]
                        kk = [kr, kr + ki, ki - kr]
                    for o in range(TILE - 1, -1, -1):
                        i = b0 + o - j
                        if i < 0:
                            continue
                        if i not in win:
                            win[i] = utrip(i, s)
                        p = [kk[q] * win[i][q] for q in range(3)]
                        acc[o] = p if acc[o] is None else [a + c for a, c in zip(acc[o], p)]
                        done += 1
                    if TILE == 4 and b0 == 4 and j == 2:
                        yield done
                yy.append([(a[0] - a[1], a[0] + a[2]) for a in acc])
                if s == 0:
                    yield done
            for o in range(TILE):
                p, q = yy[0][o], yy[1][o]
                cur = [(p[0] + q[0], p[1] + q[1]), (p[0] - q[0], p[1] - q[1])]
                for h in range(2):
                    if b0 + o == 0:
                        zr, zi = cur[h]
                    else:
                        zr = cur[h][0] - prev[h][1]
                        zi = cur[h][1] + prev[h][0]
                    zs_v[k, b0 + o, h, sl, 0:128] = zr
                    zs_v[k, b0 + o, h, sl, 128:256] = zi
                prev = cur
            if groups is not None and b0 + TILE < NB:
                for h in range(2):
                    pv_v[n, 2 * h] = prev[h][0]
                    pv_v[n, 2 * h + 1] = prev[h][1]
            yield done

    def s5_blk(k, b, h):
        t = 2 * b + h
        y = _dot_nt(zs_v[k, b, h], fmat(b % 2, h)).reshape(NV, 8, 128)
        hh = c1_v[k, 0:NV, 16 * b + 8 * h:16 * b + 8 * h + 8, :] + y
        c1_v[k, 0:NV, 16 * b + 8 * h:16 * b + 8 * h + 8, :] = hh
        wr = col_v[2, k, 0:R, :].reshape(NV, 8, 128)
        rs = slice(8 * t, 8 * t + 8)
        acc_v[0, rs, :] = acc_v[0, rs, :] + jnp.sum(hh, axis=0)
        acc_v[1, rs, :] = acc_v[1, rs, :] + jnp.sum(hh * hh, axis=0)
        acc_v[2, rs, :] = acc_v[2, rs, :] + jnp.sum(hh * wr, axis=0)

    s5 = lambda k: [(functools.partial(s5_blk, k, b, h), 1.0) for b in range(NB) for h in range(2)]

    for c in c_par:
        c.wait()
    columns((1, 2))
    for k in range(2):
        _weave((s1n(k), 0.0, 0.2), (s1g(k), 0.2, 1.0))
    _weave((s1n(2), 0.0, 0.2), (s1g(2), 0.2, 1.0), (s2(0), 0.3, 1.0))
    s1_nat(3, 0, 1)
    c_x.wait()
    ln = [ln1_pieces(b, NPC) for b in range(NB)]
    s30 = s3(0)
    _weave((sum(ln, []), 0.0, P3F[0]), (s2(1), 0.0, P3F[2]),
           *[([s30[b]], max((b + 1.6) * P3F[0] / NB, P3F[3] + (1.0 - P3F[3]) * b / NB), 0.0) for b in range(NB)])
    for c in c_par2:
        c.wait()

    def body(k, do5=True, do4=True, do3=True, do2=True, do1=True, j=None, order=None):
        order = order or ORDER
        at = (lambda d: k + d) if j is None else (lambda d: j + (k + d) if k + d else j)
        g2 = s2_gen(at(2)) if do2 else None
        for n in range(NV):
            g4 = s4_gen(at(0), n) if do4 else None
            st4 = [0, 0]
            n4 = order.count("4")

            def adv4(m):
                if not do4:
                    return
                st4[0] += 1
                while st4[1] < 72 * st4[0] / n4 - 3 or (st4[0] == n4 and st4[1] <= 72):
                    r = next(g4, None)
                    if r is None:
                        break
                    st4[1] = r

            def nat():
                if do1:
                    if n + 1 < NV:
                        s1_nat(at(3), n + 1, 1)
                    else:
                        s1_nat(jnp.minimum(at(4), NSTEP - 1), 0, 1)

            g1 = s1_grp(at(3), n) if do1 else None
            for tok in order:
                if tok == "5":
                    if do5 and n < NB:
                        s5_blk(at(-1), n, 0)
                        s5_blk(at(-1), n, 1)
                elif tok == "4":
                    adv4(1)
                elif tok in "ab" and do1:
                    next(g1)
                elif tok == "p" and do1:
                    run(g1)
                elif tok == "2" and do2:
                    next(g2, None)
                elif tok == "3" and do3 and n < NB:
                    s3_blk(at(1), n)
                elif tok == "n":
                    nat()
        if do2:
            run(g2)

    @pl.when(flag_s[0] == 1)
    def _():
        body(0, do5=False, order=ORD0)

    lax.fori_loop(0, 4, lambda j, c: (body(1, j=j), c)[1], 0)

    @pl.when(flag_s[0] == 1)
    def _():
        body(5, do1=False, order=ORD5)

    @pl.when(flag_s[0] == 1)
    def _():
        body(6, do1=False, do2=False, order=ORD6)

    @pl.when(flag_s[0] == 1)
    def _():
        _weave(([(lambda n=n: run(s4_gen(7, n, (0,))), 1.0) for n in range(NV)], 0.0, 1.0), (s5(6), 0.0, 1.0))

    @pl.when(flag_s[0] == 1)
    def _():
        _weave(([(lambda n=n: run(s4_gen(7, n, (4,))), 1.0) for n in range(NV)], 0.0, 1.0), (s5(7)[:8], 0.0, 1.0))

    _weave((s5(7)[8:], 0.0, 1.0))

    def total(i):
        halves = []
        for hf in range(2):
            t = acc_v[i, pl.ds(64 * hf, 8, stride=8), :]
            for s in range(1, 8):
                t = t + acc_v[i, pl.ds(64 * hf + s, 8, stride=8), :]
            halves.append(t)
        return jnp.concatenate(halves, 0)

    m2 = total(0) * (1.0 / D)
    var2 = jnp.maximum(total(1) * (1.0 / D) - m2 * m2, 0.0)
    sd2 = _rb(jnp.sqrt(_rb(_rb(var2) + EPS)))
    rs2 = 1.0 / sd2
    mean2 = _rb(fin_v[4] + m2)
    m2 = mean2 - fin_v[4]
    r = _rb((total(2) - m2 * wr_sum) * rs2)
    fin_v[0] = rs2
    fin_v[1] = m2 * rs2
    fin_v[2] = rs2 + 1.0
    fin_v[3] = fin_v[4] - m2 * rs2

    tl = _iota((16, 128), 0)
    ll = _iota((16, 128), 1)
    lodd = (ll & 1) == 1
    toff = jnp.where((tl & 1) == 0, jnp.where(lodd, ll + 127, ll), jnp.where(lodd, ll + 128, (ll - 1) & 127))
    tok = (tl >> 1) * 256 + toff
    rbits = pltpu.bitcast(r, i32)
    srt = rbits ^ ((rbits >> 31) & 0x7FFFFFFF)
    key = pltpu.bitcast((((srt >> 16) + 32768) << 11) + (2047 - tok) + (1 << 28), f32)
    kk = key
    cand = []
    for _ in range(4):
        rm = jnp.broadcast_to(jnp.max(kk, axis=1, keepdims=True), (16, 128))
        cand.append(rm)
        kk = jnp.where(kk == rm, 0.0, kk)
    last = jnp.max(cand[3], axis=0, keepdims=True)
    kcol = None
    for j in range(TOPC):
        mx = jnp.max(cand[0], axis=0, keepdims=True)
        kcol = jnp.broadcast_to(mx, (8, 128)) if j == 0 else jnp.where(sub8 == j, mx, kcol)
        took = cand[0] == mx
        cand = [jnp.where(took, cand[i + 1] if i < 3 else 0.0, cand[i]) for i in range(4)]
    kc_v[...] = kcol

    @pl.when((last - mx)[0, 0] > 0.0)
    def _():
        k2 = key
        kc = None
        for j in range(TOPC):
            m1 = jnp.max(jnp.max(k2, axis=0, keepdims=True), axis=1, keepdims=True)
            kc = jnp.broadcast_to(m1, (8, 128)) if j == 0 else jnp.where(sub8 == j, m1, kc)
            k2 = jnp.where(k2 == m1, 0.0, k2)
        kc_v[...] = kc

    kcol = kc_v[...]
    kint = pltpu.bitcast(kcol, i32) - (1 << 28)
    tcol = 2047 - (kint & 2047)
    s16 = (kint >> 11) - 32768
    rsel = pltpu.bitcast((s16 ^ ((s16 >> 31) & 0x7FFF)) << 16, f32)
    gate = _rb(jax.nn.sigmoid(rsel))

    def classes(col):
        cls = jnp.zeros((8, 128), i32)
        for d in range(1, TOPC):
            cls = cls + jnp.where((col == pltpu.roll(col, d, 0)) & (sub8 >= d), 1, 0)
        return cls, jnp.max(cls, axis=0, keepdims=True)[0, 0] + 1

    wcol = tcol & 255
    pcol = jnp.where((wcol & 1) == 0, jnp.where(wcol < 128, wcol, wcol - 127),
                     jnp.where(wcol < 128, (wcol + 1) & 127, wcol - 128))
    ecol = ((tcol >> 8) << 1) | (tcol & 1)
    etile = [ecol[j, 0] for j in range(TOPC)]
    gcol, gn = classes(pcol)
    xs_v[...] = jnp.zeros((8, D), f32)

    def gather(c, carry):
        oh = (gcol == c) & (lane8 == pcol)
        ohi = jnp.where(oh, 1, 0)
        msk = [jnp.broadcast_to(ohi[j:j + 1], (8, 128)) == 1 for j in range(TOPC)]
        sa = sb = None
        for j in range(TOPC):
            fa = jnp.broadcast_to(fin_v[0, pl.ds(etile[j], 1), :], (8, 128))
            fb = jnp.broadcast_to(fin_v[1, pl.ds(etile[j], 1), :], (8, 128))
            sa, sb = (fa, fb) if j == 0 else (jnp.where(msk[j], fa, sa), jnp.where(msk[j], fb, sb))
        parts = []
        for q in range(D // 8 // GCH):
            mg = None
            for j in range(TOPC):
                cc = c1_v[GCH * q // NV, GCH * q % NV:GCH * q % NV + GCH, pl.ds(pl.multiple_of(8 * etile[j], 8), 8), :]
                mg = cc if j == 0 else jnp.where(msk[j], cc, mg)
            parts.append(mg * sa - sb)
        ln = jnp.concatenate(parts, 0).reshape(D, 128)
        xs_v[...] = xs_v[...] + _dot_nt(jnp.where(oh, 1.0, 0.0).astype(f32), ln)
        return carry

    lax.fori_loop(0, gn, gather, 0)
    xsel = xs_v[...]

    def rebuilt_rows():
        sdc = jnp.zeros((8, 1), f32)
        mc = jnp.zeros((8, 1), f32)
        sub1 = _iota((8, 1), 0)
        for j in range(TOPC):
            hitm = tok == jnp.broadcast_to(tcol[j:j + 1], (16, 128))
            red = lambda v: jnp.sum(jnp.sum(jnp.where(hitm, v, 0.0), axis=0, keepdims=True), axis=1, keepdims=True)
            sdc = jnp.where(sub1 == j, red(sd2), sdc)
            mc = jnp.where(sub1 == j, red(mean2), mc)
        return xsel * (sdc + 1.0) + mc

    def outp(b, g0, g1):
        sc = [jnp.where(top, jnp.broadcast_to(fin_v[i, 2 * b:2 * b + 1, :], (8, 128)),
                        jnp.broadcast_to(fin_v[i, 2 * b + 1:2 * b + 2, :], (8, 128))) for i in (2, 3)]
        for g in range(g0, g1):
            a = _rb(c1_v[g // NV, g % NV, pl.ds(16 * b, 8, stride=2), :] * sc[0] + sc[1])
            c = _rb(c1_v[g // NV, g % NV, pl.ds(16 * b + 1, 8, stride=2), :] * sc[0] + sc[1])
            w = (pltpu.bitcast(a, u32) >> 16) | pltpu.bitcast(c, u32)
            out_w[g, b] = jnp.where(mask2, w, pltpu.roll(pltpu.roll(w, 4, 0), 127, 1))

    opieces = [functools.partial(outp, b, 24 * i, 24 * i + 24) for b in range(NB) for i in range(3)]

    tilec = tcol >> 7
    lanec = tcol & 127
    aux = {}

    def late_scalars():
        tiles = [tilec[j, 0] for j in range(TOPC)]
        hit = 0
        dup = []
        for j in range(TOPC):
            dup.append((hit >> tiles[j]) & 1)
            hit = hit | (1 << tiles[j])
        free, cnt = [], 0
        for t in range(16):
            un = 1 - ((hit >> t) & 1)
            free.append(jnp.where(un == 1, cnt, -1))
            cnt = cnt + un
        late, nd, mask = [tiles[0]], 0, hit
        for j in range(1, TOPC):
            rep = 0
            for t in range(16):
                rep = jnp.where(free[t] == nd, t, rep)
            late.append(jnp.where(dup[j] == 1, rep, tiles[j]))
            mask = mask | (1 << late[j])
            nd = nd + dup[j]
        aux.update(tiles=tiles, late=late, mask=mask)
        bs_v[...] = rebuilt_rows()
        aux["clscol"], aux["ncls"] = classes(lanec)
        for j in range(TOPC):
            code = jnp.where((tilec == late[j]) & (lane8 == lanec), aux["clscol"], -1)
            lm_v[j] = jnp.broadcast_to(jnp.max(code, axis=0, keepdims=True), (8, 128))

    def tile_idx(t, g0=0, ng=D // 8):
        if isinstance(t, int):
            return (pl.ds(g0, ng), t // 2, pl.ds(8 * (t % 2), 8), slice(None))
        return (pl.ds(g0, ng), t >> 1, pl.ds(pl.multiple_of(8 * (t & 1), 8), 8), slice(None))

    def ocopy(idx):
        return cp(out_v.at[idx], out_h.at[idx], osem.at[0])

    def early():
        for t in range(16):
            @pl.when(((aux["mask"] >> t) & 1) == 0)
            def _():
                ocopy(tile_idx(t)).start()

    for c in range(NCH):
        for cc in c_w[c]:
            cc.wait()
        mine = opieces[OSPLIT[c]:OSPLIT[c + 1]]
        nsub = max(1, FCH[c] // FSUB)
        sub = FCH[c] // nsub
        for u in range(nsub):
            sl = slice(FOFF[c] + u * sub, FOFF[c] + (u + 1) * sub)
            g = _rb(_dot(xsel, wmat(wg_w, 0, D, sl.start, sub)))
            up = _rb(_dot(xsel, wmat(wu_w, 0, D, sl.start, sub)))
            if c == 0 and u == 0:
                late_scalars()
            for fn in mine[u * len(mine) // nsub:(u + 1) * len(mine) // nsub]:
                fn()
            act_v[:, sl] = _rb(_rb(g * jax.nn.sigmoid(g)) * up)
        if c == WCH:
            early()

    clscol = aux["clscol"]
    onehot = lambda c: jnp.where((clscol == c) & (lane8 == lanec), 1.0, 0.0).astype(f32)
    bc = lambda v, j: jnp.broadcast_to(v[j:j + 1], (8, 128))

    def down(p, c0, nc):
        r = slice(POFF[p], POFF[p] + PART[p])
        yc = _dot_nt(act_v[:, c0:c0 + nc], wmat(wd_w, POFF[p], PART[p], c0, nc))
        y_v[:, r] = yc if c0 == 0 else y_v[:, r] + yc

    def place(p, fast):
        r0, nr = POFF[p], PART[p]
        g0, ng = r0 // 8, nr // 8
        gt = jnp.concatenate([gate] * ((nr + 127) // 128), 1)[:, :nr]
        newrow = _rb(bs_v[:, r0:r0 + nr] + _rb(_rb(y_v[:, r0:r0 + nr]) * gt))
        tn = lambda oh: lax.dot_general(newrow, oh, (((0,), (0,)), ((), ())), preferred_element_type=f32)
        if fast:
            uu = tn(jnp.concatenate([onehot(0), onehot(1)], 1))
            for c in range(2):
                u_v[c, g0:g0 + ng] = uu[:, 128 * c:128 * (c + 1)].reshape(ng, 8, 128)
        else:
            for c in range(TOPC):
                u_v[c, g0:g0 + ng] = tn(onehot(c)).reshape(ng, 8, 128)

    def write(p, fast):
        g0, ng = POFF[p] // 8, PART[p] // 8
        for j in range(TOPC):
            idx = tile_idx(aux["late"][j], g0, ng)
            new = out_v[idx].astype(f32)
            code = lm_v[j]
            for c in range(2 if fast else TOPC):
                new = jnp.where(code == c, u_v[c, g0:g0 + ng], new)
            sg_v[j, g0:g0 + ng] = new.astype(bf16)
            cp(sg_v.at[j, pl.ds(g0, ng)], out_h.at[idx], osem.at[0]).start()

    def dwait(p):
        for cc in c_d[p]:
            cc.wait()

    NP = len(PART)
    dwait(0)
    rest = opieces[OSPLIT[NCH]:]
    nq = 4
    for q in range(nq):
        down(0, q * F // nq, F // nq)
        for fn in rest[q * len(rest) // nq:(q + 1) * len(rest) // nq]:
            fn()

    @pl.when(aux["ncls"] <= 2)
    def _():
        for p in range(1, NP):
            dwait(p)
            down(p, 0, DSPL[p])
            place(p - 1, True)
            down(p, DSPL[p], F - DSPL[p])
            write(p - 1, True)
        place(NP - 1, True)
        write(NP - 1, True)

    @pl.when(aux["ncls"] > 2)
    def _():
        for p in range(1, NP):
            dwait(p)
            down(p, 0, F)
        for p in range(NP):
            place(p, False)
            write(p, False)

    cp(out_h, out_h, osem.at[0]).wait()


@jax.jit
def pallas_sequential_preLN__ssm_conv_s4__moe_arch_mod__prompt_kernel(
    A_u: jax.Array,
    A_A_re: jax.Array,
    A_A_im: jax.Array,
    A_B_re: jax.Array,
    A_B_im: jax.Array,
    A_C_re: jax.Array,
    A_C_im: jax.Array,
    A_log_dt: jax.Array,
    A_Dskip: jax.Array,
    B_x: jax.Array,
    B_w_r: jax.Array,
    B_w_gate: jax.Array,
    B_w_up: jax.Array,
    B_w_down: jax.Array,
):
    hbm = pl.BlockSpec(memory_space=pltpu.MemorySpace.HBM)
    vm = pltpu.VMEM
    G8 = D // 8
    wshape = (D // 16, F // 128, 16, 128)
    wview = lambda w: w.reshape(D // 16, 2, 8, F // 128, 128).transpose(0, 1, 3, 2, 4)
    scratch = [
        vm((G8, NB, 16, 128), bf16), vm((6, NSTEP, 128, N), bf16), vm((D,), bf16), vm((D,), bf16), vm((D,), bf16),
        vm((CT_ROWS, 128), f32), *[vm(wshape if r else (D, F), bf16) for r in RELAY], vm((G8, NB + 1, 16, 128), bf16),
        vm((9, 4, 144, 128), bf16), vm((2, 2, 2, 144, 128), bf16), vm((3, NSTEP, 96, 128), f32),
        vm((NV, 2, 136, 128), f32), vm((NSTEP, 12, 56, 128), f32), vm((NSTEP, 96, 128), f32),
        vm((NSTEP, NB, 6, R, 128), f32), vm((NSTEP, NB, 6, R, 128), f32),
        vm((NSTEP, NB, 2, R, 256), f32), vm((NSTEP, 12, 136, 128), f32), vm((2, 17, 8, 128), f32),
        vm((3, 136, 128), f32), vm((5, 16, 128), f32), vm((TOPC, G8, 8, 128), f32),
        vm((R, 512), f32), vm((8, D), f32), vm((NV, 4, 8, 128), f32),
        vm((8, 128), f32), vm((8, D), f32), vm((8, D), f32), vm((8, F), f32),
        vm((TOPC, G8, 8, 128), bf16), vm((TOPC, 8, 128), i32), vm((8, D), f32), pltpu.SMEM((1,), i32),
        pltpu.SemaphoreType.DMA((5 + NCH + len(PART),)), pltpu.SemaphoreType.DMA((1,)),
    ]
    xv = A_u[0].T.reshape(G8, 8, 16, 128).transpose(0, 2, 1, 3).reshape(G8, NB, 16, 128)
    out = pl.pallas_call(
        _kernel,
        out_shape=jax.ShapeDtypeStruct((G8, NB, 16, 128), bf16),
        in_specs=[hbm] * 13,
        out_specs=hbm,
        scratch_shapes=scratch,
        compiler_params=pltpu.CompilerParams(vmem_limit_bytes=120 * 1024 * 1024, disable_bounds_checks=NOBC,
                                             disable_semaphore_checks=NOSC),
    )(xv, *[p.reshape(NSTEP, R, N) for p in (A_A_re, A_A_im, A_B_re, A_B_im, A_C_re, A_C_im)], A_log_dt, A_Dskip, B_w_r,
      *[wview(w) if r else w for w, r in zip((B_w_gate, B_w_up, B_w_down.T), RELAY)])
    return out.reshape(G8, 16, 8, 128).transpose(0, 2, 1, 3).reshape(D, L).T[None]
```

```python
import functools

import numpy as np
import jax
import jax.numpy as jnp
from jax import lax
import jax.experimental.pallas as pl
import jax.experimental.pallas.tpu as pltpu

f32 = jnp.float32
bf16 = jnp.bfloat16
i32 = jnp.int32
u32 = jnp.uint32

L, D, N, F, TOPC = 2048, 576, 128, 4608, 8
NB = 8
NV = 9
R = NV * 8
NSTEP = D // R
EPS = 1e-5

_XL1 = [(1, 5), (2, 6), (3, 7), (4, 8), (258, 516), (260, 520), (262, 772), (264, 776),
        (1288, 1032), (1800, 1544)]
_XSH = [0, 1, 2, 3, 0, 1, 2, 3, 0, 1]


def _bf16_round_int(j):
    u = np.asarray(j, np.float32).view(np.uint32).astype(np.uint64)
    r = ((u + 0x7FFF + ((u >> 16) & 1)) >> 16) << 16
    return r.astype(np.uint32).view(np.float32).astype(np.int64)


def _chunk_values():
    vals = -np.ones((5, 128), np.int64)
    for j in range(10):
        for p in range(2):
            ch = (j // 4) * 2 + p if j < 8 else 4
            extra = 2 * p if j >= 8 else 0
            for l0 in range(32):
                vals[ch, (4 * (31 - l0) + 4 * p + _XSH[j] + extra + 8) % 128] = _XL1[j][p] + 8 * l0
    assert (vals >= 0).all()
    return vals


_PASSES = [(0, "A0"), (0, "A1"), (1, "B"), (2, "Cp"), (3, "C"), (4, "Dp"), (5, "D"), (6, "D"), (7, "D")]
_SETS = [[0], [1], [2], [3, 4], [5, 6, 7, 8]]


def _tables():
    cv = _chunk_values()
    cvp = {"A0": cv[0], "A1": cv[1], "B": cv[2], "C": cv[3], "D": cv[4]}
    cvp["Cp"] = cv[3].copy(); cvp["Cp"][11] = cv[2][11]
    cvp["Dp"] = cv[4].copy(); cvp["Dp"][15] = cv[3][15]
    sup = [[[] for _ in range(128)] for _ in _PASSES]
    for b in range(NB):
        for j in range(1, 257):
            lag = 256 * b + j
            if lag > L - 1 or lag == 257:
                continue
            v = int(_bf16_round_int(lag))
            hit = [(i, int(np.nonzero(cvp[nm] == v)[0][0])) for i, (pb, nm) in enumerate(_PASSES)
                   if pb == b and (cvp[nm] == v).any()]
            assert len(hit) == 1, (b, j, v, hit)
            sup[hit[0][0]][hit[0][1]].append(j)
    assert cv[1][15] == _bf16_round_int(257)
    code = np.zeros((len(_PASSES), 128), np.int64)
    for i, (pb, _) in enumerate(_PASSES):
        for r in range(128):
            js = sup[i][r]
            if js:
                assert js == list(range(js[0], js[-1] + 1))
                code[i, r] = js[0] + js[-1] + 1024 * len(js) + 16384 * (pb % 2)
    seeds, masks = [], {}
    for ps in _SETS:
        seeds.append([int(x) for x in sum(code[i, 16:24] for i in ps)])
        for i in ps:
            masks[i] = [int(x > 0) for x in code[i, 16:24]]
            for v in range(2, 17):
                r0 = 8 * (v % 16)
                assert (code[i, r0:r0 + 8] == (np.array(seeds[-1]) - 32 * (v - 2)) * np.array(masks[i])).all()
    return seeds, [[int(x) for x in code[i, 8:16]] for i in range(len(_PASSES))], masks


_GSEED, _GROW1, _GMASK = _tables()


def _sincos_coeffs():
    r = np.cos(np.pi * (np.arange(4000) + .5) / 4000) * 0.5
    z = r * r
    s = np.linalg.lstsq(np.stack([z ** k for k in range(4)], 1), np.sin(np.pi / 2 * r) / r, rcond=None)[0]
    c = np.linalg.lstsq(np.stack([z ** k for k in range(1, 5)], 1), np.cos(np.pi / 2 * r) - 1, rcond=None)[0]
    return [float(x) for x in s], [float(x) for x in c]


_SC, _CC = _sincos_coeffs()


def _cmul(a, b):
    return (a[0] * b[0] - a[1] * b[1], a[0] * b[1] + a[1] * b[0])


def _cmulc(a, b):
    return (a[0] * b[0] + a[1] * b[1], a[1] * b[0] - a[0] * b[1])


def _csq(a):
    return ((a[0] - a[1]) * (a[0] + a[1]), (a[0] + a[0]) * a[1])


def _quarter_polys(r):
    r2 = r * r
    s = r * (_SC[0] + r2 * (_SC[1] + r2 * (_SC[2] + r2 * _SC[3])))
    c = 1.0 + r2 * (_CC[0] + r2 * (_CC[1] + r2 * (_CC[2] + r2 * _CC[3])))
    return s, c


def _rotate_quadrant(s, c, ki):
    swap = (ki & 1) == 1
    s2 = jnp.where(swap, c, s)
    c2 = jnp.where(swap, s, c)
    s2 = pltpu.bitcast(pltpu.bitcast(s2, i32) ^ ((ki & 2) << 30), f32)
    c2 = pltpu.bitcast(pltpu.bitcast(c2, i32) ^ (((ki + 1) & 2) << 30), f32)
    return s2, c2


def _sincos(th):
    z = th * (2.0 / np.pi)
    k = jnp.round(z)
    s, c = _quarter_polys(z - k)
    return _rotate_quadrant(s, c, k.astype(i32))


def _reduce_small(z):
    big = 12582912.0
    t = z + big
    return _quarter_polys(z - (t - big)) + (pltpu.bitcast(t, i32),)


def _rb(x):
    return x.astype(bf16).astype(f32)


def _dot(a, b):
    return jnp.dot(a, b, preferred_element_type=f32)


def _dot_nt(a, b):
    return lax.dot_general(a, b, (((1,), (1,)), ((), ())), preferred_element_type=f32)


def _iota(shape, dim):
    return lax.broadcasted_iota(i32, shape, dim)


ORDER, ORD0, ORD5, ORD6 = "4ab44342np445", "4ab442n4p4345", "4a424n44b345p", "45a4b244p3n44"
TILE = 4
LG = 3
NTOP = 4
FCH = (3456, 1152)
FSUB = 1152
PART = (256, 128, 128, 64)
POFF = [sum(PART[:i]) for i in range(len(PART))]
DSPL = (0, 2560, 2560, 4096)
CT_ROWS = 320


def _weave(*streams):
    items = []
    for si, (pieces, lo, hi) in enumerate(streams):
        tot = float(sum(c for _, c in pieces))
        cum = 0.0
        for pi, (fn, c) in enumerate(pieces):
            items.append((lo + max(hi - lo, 0.0) * (cum + 0.5 * c) / tot, si, pi, fn))
            cum += c
    for _, _, _, fn in sorted(items, key=lambda t: t[:3]):
        fn()


def _kernel(x_h, are_h, aim_h, bre_h, bim_h, cre_h, cim_h, ldt_h, dsk_h, wr_h, wg_h, wu_h, wd_h,
            out_h,
            x_v, par_v, ldt_v, dsk_v, wr_v, ct_v, wg_v, wu_v, wd_v, out_v,
            g_v, f_v, col_v, st_v, kd_v, k0_v, kh_v, uh_v, zs_v, c1_v, s1_v, acc_v, fin_v, u_v, zt_v,
            y_v, pv_v, kc_v, xs_v, bs_v, act_v, sg_v, lm_v, rw_v, flag_s,
            sem, osem):
    cp = pltpu.make_async_copy
    c_vec = [cp(ldt_h, ldt_v, sem.at[0]), cp(dsk_h, dsk_v, sem.at[0]), cp(wr_h, wr_v, sem.at[0])]
    PH = 4
    par_h = (are_h, aim_h, bre_h, bim_h, cre_h, cim_h)
    c_par = [cp(h.at[pl.ds(0, PH)], par_v.at[i, pl.ds(0, PH), pl.ds(0, R)], sem.at[1])
             for i, h in enumerate(par_h)]
    c_par2 = [cp(h.at[pl.ds(PH, NSTEP - PH)], par_v.at[i, pl.ds(PH, NSTEP - PH), pl.ds(0, R)], sem.at[2])
              for i, h in enumerate(par_h)]
    c_x = cp(x_h, x_v, sem.at[3])

    def wcp(h, v, c):
        ct = pl.ds(sum(FCH[:c]) // 128, FCH[c] // 128)
        return [cp(h.at[:, hf, ct], v.at[:, ct, pl.ds(8 * hf, 8), :], sem.at[4 + c]) for hf in range(2)]

    c_w = [wcp(wg_h, wg_v, c) + wcp(wu_h, wu_v, c) for c in range(2)]
    c_d = [cp(wd_h.at[pl.ds(POFF[p], PART[p])], wd_v.at[pl.ds(POFF[p], PART[p])], sem.at[6 + p])
           for p in range(len(PART))]
    for c in c_vec + c_par + [c_x] + c_par2 + sum(c_w, []) + c_d:
        c.start()

    flag_s[0] = 1
    x_w = x_v.bitcast(u32)
    wg_w, wu_w = wg_v.bitcast(u32), wu_v.bitcast(u32)

    def wmat(w, c0, nc):
        return jnp.concatenate([pltpu.bitcast(w[:, t], bf16).reshape(D, 128)
                                for t in range(c0 // 128, (c0 + nc) // 128)], 1)

    out_w = out_v.bitcast(u32)
    g_w = g_v.bitcast(u32)
    f_w = f_v.bitcast(u32)
    sub8 = _iota((8, 128), 0)
    lane8 = _iota((8, 128), 1)

    acc_v[...] = jnp.zeros(acc_v.shape, f32)
    for ri in range(2):
        st_v[:, ri, 104:112, :] = jnp.full((NV, 8, 128), 1.0 - ri, f32)
    kp = (2 * lane8 + 1).astype(f32)

    def rows_const(vals):
        out = jnp.full((8, 128), vals[0], i32)
        for r in range(1, 8):
            if vals[r] != vals[0]:
                out = jnp.where(sub8 == r, vals[r], out)
        return out

    def phasor(z):
        sn, cs = _rotate_quadrant(*_reduce_small(-z))
        return cs, sn

    NS = [0, 1, 2, 3, 4, 5, 7, 9]
    for q in range(2):
        sn = _rotate_quadrant(*_reduce_small((kp + 512.0 * q) * (rows_const(NS).astype(f32) * (1.0 / 512))))[0]
        ct_v[304 + 8 * q:312 + 8 * q, :] = sn / (256.0 * jnp.broadcast_to(sn[1:2], (8, 128)))

    def grows(vals):
        ab = rows_const([v & 1023 for v in vals])
        z = kp * (ab.astype(f32) * (-1.0 / 512))
        if any(v >> 14 for v in vals):
            z = z - rows_const([v >> 14 for v in vals]).astype(f32) * (kp - 1.0)
        sn, cs, ki = _reduce_small(z)
        ns = [NS.index((v >> 10) & 15) for v in vals]
        out = []
        for q in range(2):
            row = lambda i: jnp.broadcast_to(ct_v[304 + 8 * q + i:305 + 8 * q + i, :], (8, 128))
            amp = None
            for i in sorted(set(ns)):
                bits = sum(1 << r for r in range(8) if ns[r] == i)
                amp = row(i) if amp is None else jnp.where(((bits >> sub8) & 1) == 1, row(i), amp)
            pi, pr = _rotate_quadrant(sn, cs, ki if q == 0 else ki - ab)
            out += [pr * amp, pi * amp]
        return out

    for v4 in range(4):
        e = phasor(kp * ((sub8 + 8 * v4).astype(f32) * (1.0 / 32)))
        ct_v[8 * v4:8 * v4 + 8, :] = e[0]
        ct_v[32 + 8 * v4:40 + 8 * v4, :] = e[1]
    for si in range(5):
        for q, val in enumerate(grows(_GSEED[si])):
            ct_v[64 + 32 * si + 8 * q:72 + 32 * si + 8 * q, :] = val
    for i in range(len(_PASSES)):
        for q, val in enumerate(grows(_GROW1[i])):
            g_v[i, q, 8:16, :] = val.astype(bf16)
    for q, val in enumerate(grows([2 + 1024 + 16384] * 8)):
        ct_v[272 + 8 * q:280 + 8 * q, :] = val
    s8 = np.arange(8)
    je = np.where(s8 % 2 == 0, s8, 127 + s8)
    jo = np.where(s8 % 2 == 0, s8 - 1, 128 + s8)
    for t, jj in enumerate((je, jo, jo % 128 + 128 * (s8 % 2))):
        e = phasor(kp * (rows_const([int(x) for x in jj]).astype(f32) * (1.0 / 256)))
        ct_v[224 + 16 * t:232 + 16 * t, :] = e[0]
        ct_v[232 + 16 * t:240 + 16 * t, :] = e[1]
    for c in c_vec:
        c.wait()

    rows = [_rb(jnp.exp(ldt_v[...].astype(f32).reshape(1, D))),
            dsk_v[...].astype(f32).reshape(1, D),
            wr_v[...].astype(f32).reshape(1, D)]
    wr_sum = jnp.sum(rows[2], axis=1, keepdims=True)

    def columns(which):
        for j in range(5):
            w = 128 if j < 4 else 64
            eye = _iota((w, w), 0) == _iota((w, w), 1)
            m = jnp.concatenate([jnp.where(eye, jnp.broadcast_to(rw_v[i:i + 1, j * 128:j * 128 + w], (w, w)), 0.0)
                                 for i in which], 0)
            res = _dot(m, jnp.ones((w, 128), f32))
            for n, i in enumerate(which):
                for g in range(w // 8):
                    k, m8 = divmod(16 * j + g, NV)
                    col_v[i, k, 8 * m8:8 * m8 + 8, :] = res[n * w + 8 * g:n * w + 8 * g + 8]

    for i in range(3):
        rw_v[i:i + 1, :] = rows[i]
    columns((0,))

    def e8(v):
        return (jnp.broadcast_to(ct_v[v:v + 1, :], (8, 128)), jnp.broadcast_to(ct_v[32 + v:33 + v, :], (8, 128)))

    for si, ps in enumerate(_SETS):
        sd = [ct_v[64 + 32 * si + 8 * q:72 + 32 * si + 8 * q, :] for q in range(4)]
        mk = {}
        for i in ps:
            if len(ps) > 1:
                bits = sum(b << s for s, b in enumerate(_GMASK[i]))
                mk[i] = ((bits >> sub8) & 1) == 1
        for v in range(2, 17):
            if v == 2:
                vals = sd
            else:
                ev = e8(2 * (v - 2))
                vals = list(_cmulc((sd[0], sd[1]), ev)) + list(_cmulc((sd[2], sd[3]), ev))
            vals = jnp.stack(vals, 0)
            for i in ps:
                val = vals if len(ps) == 1 else jnp.where(mk[i], vals, 0.0)
                g_v[i, :, 8 * (v % 16):8 * (v % 16) + 8, :] = val.astype(bf16)
    sig = jnp.where((lane8 & 1) == 0, 1.0, -1.0).astype(f32)
    for h in range(2):
        sd = (ct_v[224 + 16 * h:232 + 16 * h, :], ct_v[232 + 16 * h:240 + 16 * h, :])
        for v in range(16):
            if v == 0:
                vals = sd if h == 0 else (ct_v[256:264, :], ct_v[264:272, :])
            else:
                vals = _cmul(sd, e8(v))
            for q in range(2):
                f_v[0, h, q, 8 * v:8 * v + 8, :] = vals[q].astype(bf16)
                f_v[1, h, q, 8 * v:8 * v + 8, :] = (vals[q] * sig).astype(bf16)

    def gmat(i):
        return jnp.concatenate([pltpu.bitcast(g_w[i, q, 0:64, :], bf16) for q in range(4)], 1)

    def fmat(ver, h):
        return jnp.concatenate([pltpu.bitcast(f_w[ver, h, q, 0:64, :], bf16) for q in range(2)], 1)

    revmask = (sub8 & 2) == 0
    lm = lane8 & 3

    def s1_nat(k, n0, nn):
        rr = 8 * nn
        ld = lambda i: par_v[i, k, 8 * n0:8 * n0 + rr, :].astype(f32)
        dt = col_v[0, k, 8 * n0:8 * n0 + rr, :]
        e = jnp.exp(dt * ld(0))
        s, c = _sincos(dt * ld(1))
        a1 = (e * c, e * s)
        w = _cmul((ld(4), ld(5)), (dt * ld(2), dt * ld(3)))
        k0_v[k, 8 * n0:8 * n0 + rr, :] = jnp.broadcast_to(jnp.sum(w[0], axis=1, keepdims=True), (rr, 128))
        w = (w[0], -w[1])
        rev = lambda v: jnp.where(revmask, pltpu.roll(v, 2, 2), pltpu.roll(v, 6, 2))

        def put(arr, slots, fn=None):
            v = jnp.stack([a.reshape(nn, 8, 128) for a in arr], 1)
            if fn is not None:
                v = fn(v)
            for q in slots:
                st_v[n0:n0 + nn, :, q * 8:q * 8 + 8, :] = v

        put(w, (0, 1)); put(a1, (2, 3))
        a2 = _csq(a1); put(a2, (5,))
        a4 = _csq(a2); put(a4, (6,))
        put(_cmul(a4, a1), (4,))
        a8 = _csq(a4); put(a8, (12,), rev)
        t = _csq(a8); put(t, (14, 15), rev)
        for _ in range(4):
            t = _csq(t)
        put(t, (7, 11))
        t = _csq(t); put(t, (8, 9))
        put(_csq(t), (10,))

    def s1_grp(k, n):
        def mix(q):
            gs = [st_v[n, :, pl.ds(q * 8 + g, 8, stride=2), :] for g in range(2)]
            return tuple(jnp.concatenate([gs[0][ri], gs[1][ri]], 0) for ri in range(2))

        y = [mix(12)]
        a16d = mix(14)
        for _ in range(15):
            y.append(_cmul(y[-1], a16d))
        yield
        wd = mix(0); a1d = mix(2); m1 = mix(5)
        v = [_cmulc(wd, mix(3))]
        for _ in range(3):
            v.append(_cmulc(v[-1], a1d))
        v4 = _cmulc(_cmulc(wd, m1), mix(7))
        v5 = _cmulc(v4, m1); v6 = _cmulc(v4, mix(6)); v7 = _cmulc(v6, m1)
        v8 = _cmulc(v7, mix(10)); v9 = _cmulc(v8, mix(8))
        v += [v4, v5, v6, v7, v8, v9]
        os_ = []
        for g in range(2):
            cat = lambda ts: jnp.concatenate([jnp.concatenate([t[ri][8 * g:8 * g + 8] for t in ts], 0)
                                              for ri in range(2)], 1)
            os_.append(_dot_nt(cat(v), cat(y[::-1])))
        yield
        for g in range(2):
            o = os_[g]
            ro = [pltpu.roll(o[8 * j:8 * j + 8], _XSH[j] + 5, 1, stride=1, stride_axis=0) for j in range(10)]
            sel4 = lambda q: jnp.where(lm == 0, q[0], jnp.where(lm == 1, q[1], jnp.where(lm == 2, q[2], q[3])))
            kd_v[k, n, pl.ds(g, 8, stride=2), :] = sel4(ro[0:4])
            kd_v[k, n, pl.ds(16 + g, 8, stride=2), :] = sel4(ro[4:8])
            kd_v[k, n, pl.ds(32 + g, 8, stride=2), :] = jnp.where(lm == 0, ro[8], ro[9])

    def run(gen):
        for _ in gen:
            pass

    s1n = lambda k: [(functools.partial(s1_nat, k, 3 * i, 3), 1.0) for i in range(3)]
    s1g = lambda k: [(lambda n=n: run(s1_grp(k, n)), 1.0) for n in range(NV)]

    laneR = _iota((R, 128), 1)
    lmR = laneR & 3

    def s2_gen(k):
        ch = lambda c: kd_v[k, 0:NV, 8 * c:8 * c + 8, :].reshape(R, 128)
        for b in range(NB):
            if b == 0:
                k0 = (k0_v[k, 0:R, :] + col_v[1, k, 0:R, :]) * (1.0 / 256.0)
                z = _dot(ch(0), gmat(0))
                dd = jnp.where(lmR < 2, ch(4), pltpu.roll(ch(5), 2, 1))
                kd_v[k, 0:NV, 48:56, :] = dd.reshape(NV, 8, 128)
                zt_v[...] = z
                yield
                z = _dot(ch(1), gmat(1)) + zt_v[...]
            elif b == 1:
                k256 = jnp.sum(jnp.where(laneR == 15, ch(1), 0.0), axis=1, keepdims=True)
                pat = jnp.concatenate([ct_v[272 + 8 * q:273 + 8 * q, :] for q in range(4)], 1)
                z = _dot(ch(2), gmat(2)) + k256 * pat
            elif b == 2:
                z = _dot(jnp.where(laneR == 11, ch(2), ch(3)), gmat(3))
            elif b == 3:
                z = _dot(ch(3), gmat(4))
            elif b == 4:
                z = _dot(jnp.where(laneR == 15, ch(3), ch(6)), gmat(5))
            else:
                z = _dot(ch(6), gmat(b + 1))
            for s in range(2):
                kr = z[:, 256 * s:256 * s + 128]
                ki = z[:, 256 * s + 128:256 * s + 256]
                if b == 0:
                    kr = kr + k0
                kh_v[k, b, 3 * s] = kr
                kh_v[k, b, 3 * s + 1] = ki
            yield

    def s2(k):
        gen = s2_gen(k)
        return [(lambda: next(gen, None), 1.0) for _ in range(9)]

    mask2 = (sub8 < 4) == ((lane8 & 1) == 0)
    top = sub8 < 4

    def ln1_pieces(b, npc):
        state = {}
        per = (D // 8) // npc

        def piece(i):
            for g in range(i * per, (i + 1) * per, LG):
                m = x_w[g:g + LG, b]
                eo = jnp.where(mask2, m, pltpu.roll(pltpu.roll(m, 4, 1), 1, 2))
                a = pltpu.bitcast(eo << 16, f32)
                c = pltpu.bitcast(eo & jnp.uint32(0xFFFF0000), f32)
                if g == 0:
                    state["sh"] = jnp.where(top, jnp.broadcast_to(a[0, 0:1], (8, 128)),
                                            jnp.broadcast_to(a[0, 4:5], (8, 128)))
                a = a - state["sh"]
                c = c - state["sh"]
                c1_v[g // NV, g % NV:g % NV + LG, pl.ds(16 * b, 8, stride=2), :] = a
                c1_v[g // NV, g % NV:g % NV + LG, pl.ds(16 * b + 1, 8, stride=2), :] = c
                for q in range(LG):
                    new = [a[q], c[q], a[q] * a[q], c[q] * c[q]]
                    state["acc"] = new if g + q == 0 else [p + r for p, r in zip(state["acc"], new)]
            if i == npc - 1:
                acc = state["acc"]
                s1, s2_ = acc[0] + acc[1], acc[2] + acc[3]
                for h in range(2):
                    m = jnp.sum(s1[4 * h:4 * h + 4], axis=0, keepdims=True) * (1.0 / D)
                    var = jnp.sum(s2_[4 * h:4 * h + 4], axis=0, keepdims=True) * (1.0 / D) - m * m
                    rs = 1.0 / _rb(jnp.sqrt(_rb(_rb(jnp.maximum(var, 0.0)) + EPS)))
                    s1_v[0, 2 * b + h] = jnp.broadcast_to(rs, (8, 128))
                    sh = state["sh"][4 * h:4 * h + 1]
                    s1_v[1, 2 * b + h] = jnp.broadcast_to((_rb(m + sh) - sh) * rs, (8, 128))
                    fin_v[4, 2 * b + h:2 * b + h + 1, :] = state["sh"][4 * h:4 * h + 1]

        return [(functools.partial(piece, i), 1.0) for i in range(npc)]

    def s3_blk(k, b):
        et = []
        for h in range(2):
            c = c1_v[k, 0:NV, 16 * b + 8 * h:16 * b + 8 * h + 8, :]
            u = (c * s1_v[0, 2 * b + h] - s1_v[1, 2 * b + h]).reshape(R, 128)
            et.append(_dot(u, fmat(b % 2, h)))
        er, ei, tr, ti = et[0][:, :128], et[0][:, 128:], et[1][:, :128], et[1][:, 128:]
        for q, v in enumerate((er, ei, tr, ti)):
            uh_v[k, b, q] = v

    s3 = lambda k: [(functools.partial(s3_blk, k, b), 1.0) for b in range(NB)]

    def s4_gen(k, n, groups=None):
        sl = slice(8 * n, 8 * n + 8)

        def utrip(i, s):
            et = uh_v[k, i, 0:4, sl, :]
            er, ei, tr, ti = et[0], et[1], et[2], et[3]
            pr, pi = (er + tr, ei + ti) if s == 0 else (er - tr, ei - ti)
            return [pr + pi, pi, pr]

        prev = None
        done = 0
        if groups is not None and groups[0] > 0:
            prev = [(pv_v[n, 2 * h], pv_v[n, 2 * h + 1]) for h in range(2)]
        for b0 in (range(0, NB, TILE) if groups is None else groups):
            yy = []
            for s in range(2):
                acc = [None] * TILE
                win = {}
                for j in range(b0 + TILE):
                    kri = kh_v[k, j, 3 * s:3 * s + 2, sl, :]
                    kk = [kri[0], kri[0] + kri[1], kri[1] - kri[0]]
                    for o in range(TILE - 1, -1, -1):
                        i = b0 + o - j
                        if i < 0:
                            continue
                        if i not in win:
                            win[i] = utrip(i, s)
                        p = [kk[q] * win[i][q] for q in range(3)]
                        acc[o] = p if acc[o] is None else [a + c for a, c in zip(acc[o], p)]
                        done += 1
                    if b0 == 4 and j == 2:
                        yield done
                yy.append([(a[0] - a[1], a[0] + a[2]) for a in acc])
                if s == 0:
                    yield done
            for o in range(TILE):
                p, q = yy[0][o], yy[1][o]
                cur = [(p[0] + q[0], p[1] + q[1]), (p[0] - q[0], p[1] - q[1])]
                for h in range(2):
                    if b0 + o == 0:
                        zr, zi = cur[h]
                    else:
                        zr = cur[h][0] - prev[h][1]
                        zi = cur[h][1] + prev[h][0]
                    zs_v[k, b0 + o, h, sl, :] = jnp.concatenate([zr, zi], 1)
                prev = cur
            if groups is not None and b0 + TILE < NB:
                for h in range(2):
                    pv_v[n, 2 * h] = prev[h][0]
                    pv_v[n, 2 * h + 1] = prev[h][1]
            yield done

    def s5_blk(k, b, h):
        t = 2 * b + h
        y = _dot_nt(zs_v[k, b, h], fmat(b % 2, h)).reshape(NV, 8, 128)
        hh = c1_v[k, 0:NV, 16 * b + 8 * h:16 * b + 8 * h + 8, :] + y
        c1_v[k, 0:NV, 16 * b + 8 * h:16 * b + 8 * h + 8, :] = hh
        wr = col_v[2, k, 0:R, :].reshape(NV, 8, 128)
        rs = slice(8 * t, 8 * t + 8)
        acc_v[0, rs, :] = acc_v[0, rs, :] + jnp.sum(hh, axis=0)
        acc_v[1, rs, :] = acc_v[1, rs, :] + jnp.sum(hh * hh, axis=0)
        acc_v[2, rs, :] = acc_v[2, rs, :] + jnp.sum(hh * wr, axis=0)

    s5 = lambda k: [(functools.partial(s5_blk, k, b, h), 1.0) for b in range(NB) for h in range(2)]

    for c in c_par:
        c.wait()
    columns((1, 2))
    for k in range(2):
        _weave((s1n(k), 0.0, 0.2), (s1g(k), 0.2, 1.0))
    _weave((s1n(2), 0.0, 0.2), (s1g(2), 0.2, 1.0), (s2(0), 0.3, 1.0))
    s1_nat(3, 0, 1)
    c_x.wait()
    ln = [ln1_pieces(b, 3) for b in range(NB)]
    s30 = s3(0)
    _weave((sum(ln, []), 0.0, 0.9), (s2(1), 0.0, 0.55),
           *[([s30[b]], max((b + 1.6) * 0.9 / NB, 0.3 + 0.7 * b / NB), 0.0) for b in range(NB)])
    for c in c_par2:
        c.wait()

    def body(k, do5=True, do4=True, do3=True, do2=True, do1=True, j=None, order=None):
        order = order or ORDER
        at = (lambda d: k + d) if j is None else (lambda d: j + (k + d) if k + d else j)
        g2 = s2_gen(at(2)) if do2 else None
        for n in range(NV):
            g4 = s4_gen(at(0), n) if do4 else None
            st4 = [0, 0]
            n4 = order.count("4")

            def adv4(m):
                if not do4:
                    return
                st4[0] += 1
                while st4[1] < 72 * st4[0] / n4 - 3 or (st4[0] == n4 and st4[1] <= 72):
                    r = next(g4, None)
                    if r is None:
                        break
                    st4[1] = r

            def nat():
                if do1:
                    if n + 1 < NV:
                        s1_nat(at(3), n + 1, 1)
                    else:
                        s1_nat(jnp.minimum(at(4), NSTEP - 1), 0, 1)

            g1 = s1_grp(at(3), n) if do1 else None
            for tok in order:
                if tok == "5":
                    if do5 and n < NB:
                        s5_blk(at(-1), n, 0)
                        s5_blk(at(-1), n, 1)
                elif tok == "4":
                    adv4(1)
                elif tok in "ab" and do1:
                    next(g1)
                elif tok == "p" and do1:
                    run(g1)
                elif tok == "2" and do2:
                    next(g2, None)
                elif tok == "3" and do3 and n < NB:
                    s3_blk(at(1), n)
                elif tok == "n":
                    nat()
        if do2:
            run(g2)

    @pl.when(flag_s[0] == 1)
    def _():
        body(0, do5=False, order=ORD0)

    lax.fori_loop(0, 4, lambda j, c: (body(1, j=j), c)[1], 0)

    @pl.when(flag_s[0] == 1)
    def _():
        body(5, do1=False, order=ORD5)

    @pl.when(flag_s[0] == 1)
    def _():
        body(6, do1=False, do2=False, order=ORD6)

    @pl.when(flag_s[0] == 1)
    def _():
        _weave(([(lambda n=n: run(s4_gen(7, n, (0,))), 1.0) for n in range(NV)], 0.0, 1.0), (s5(6), 0.0, 1.0))

    @pl.when(flag_s[0] == 1)
    def _():
        _weave(([(lambda n=n: run(s4_gen(7, n, (4,))), 1.0) for n in range(NV)], 0.0, 1.0), (s5(7)[:8], 0.0, 1.0))

    _weave((s5(7)[8:], 0.0, 1.0))

    def total(i):
        halves = []
        for hf in range(2):
            t = acc_v[i, pl.ds(64 * hf, 8, stride=8), :]
            for s in range(1, 8):
                t = t + acc_v[i, pl.ds(64 * hf + s, 8, stride=8), :]
            halves.append(t)
        return jnp.concatenate(halves, 0)

    m2 = total(0) * (1.0 / D)
    var2 = jnp.maximum(total(1) * (1.0 / D) - m2 * m2, 0.0)
    sd2 = _rb(jnp.sqrt(_rb(_rb(var2) + EPS)))
    rs2 = 1.0 / sd2
    mean2 = _rb(fin_v[4] + m2)
    m2 = mean2 - fin_v[4]
    r = _rb((total(2) - m2 * wr_sum) * rs2)
    fin_v[0] = rs2
    fin_v[1] = m2 * rs2
    fin_v[2] = rs2 + 1.0
    fin_v[3] = fin_v[4] - m2 * rs2

    def outp(b, g0, g1):
        sc = [jnp.where(top, jnp.broadcast_to(fin_v[i, 2 * b:2 * b + 1, :], (8, 128)),
                        jnp.broadcast_to(fin_v[i, 2 * b + 1:2 * b + 2, :], (8, 128))) for i in (2, 3)]
        for g in range(g0, g1, LG):
            src = lambda o: c1_v[g // NV, g % NV:g % NV + LG, pl.ds(16 * b + o, 8, stride=2), :]
            a = _rb(src(0) * sc[0] + sc[1])
            c = _rb(src(1) * sc[0] + sc[1])
            w = (pltpu.bitcast(a, u32) >> 16) | pltpu.bitcast(c, u32)
            out_w[g:g + LG, b] = jnp.where(mask2, w, pltpu.roll(pltpu.roll(w, 4, 1), 127, 2))

    opieces = [functools.partial(outp, b, 24 * i, 24 * i + 24) for b in range(NB) for i in range(3)]

    tl = _iota((16, 128), 0)
    ll = _iota((16, 128), 1)
    lodd = (ll & 1) == 1
    toff = jnp.where((tl & 1) == 0, jnp.where(lodd, ll + 127, ll), jnp.where(lodd, ll + 128, (ll - 1) & 127))
    tok = (tl >> 1) * 256 + toff
    rbits = pltpu.bitcast(r, i32)
    srt = rbits ^ ((rbits >> 31) & 0x7FFFFFFF)
    key = pltpu.bitcast((((srt >> 16) + 32768) << 11) + (2047 - tok) + (1 << 28), f32)
    kk = key
    cand = []
    for _ in range(4):
        rm = jnp.broadcast_to(jnp.max(kk, axis=1, keepdims=True), (16, 128))
        cand.append(rm)
        kk = jnp.where(kk == rm, 0.0, kk)
        for fn in opieces[(len(cand) - 1) * NTOP // 4:len(cand) * NTOP // 4]:
            fn()
    last = jnp.max(cand[3], axis=0, keepdims=True)
    kcol = None
    for j in range(TOPC):
        mx = jnp.max(cand[0], axis=0, keepdims=True)
        kcol = jnp.broadcast_to(mx, (8, 128)) if j == 0 else jnp.where(sub8 == j, mx, kcol)
        took = cand[0] == mx
        cand = [jnp.where(took, cand[i + 1] if i < 3 else 0.0, cand[i]) for i in range(4)]
    kc_v[...] = kcol

    @pl.when((last - mx)[0, 0] > 0.0)
    def _():
        k2 = key
        kc = None
        for j in range(TOPC):
            m1 = jnp.max(jnp.max(k2, axis=0, keepdims=True), axis=1, keepdims=True)
            kc = jnp.broadcast_to(m1, (8, 128)) if j == 0 else jnp.where(sub8 == j, m1, kc)
            k2 = jnp.where(k2 == m1, 0.0, k2)
        kc_v[...] = kc

    kcol = kc_v[...]
    kint = pltpu.bitcast(kcol, i32) - (1 << 28)
    tcol = 2047 - (kint & 2047)
    s16 = (kint >> 11) - 32768
    rsel = pltpu.bitcast((s16 ^ ((s16 >> 31) & 0x7FFF)) << 16, f32)
    gate = _rb(jax.nn.sigmoid(rsel))

    def classes(col):
        cls = jnp.zeros((8, 128), i32)
        for d in range(1, TOPC):
            cls = cls + jnp.where((col == pltpu.roll(col, d, 0)) & (sub8 >= d), 1, 0)
        return cls, jnp.max(cls, axis=0, keepdims=True)[0, 0] + 1

    wcol = tcol & 255
    pcol = jnp.where((wcol & 1) == 0, jnp.where(wcol < 128, wcol, wcol - 127),
                     jnp.where(wcol < 128, (wcol + 1) & 127, wcol - 128))
    ecol = ((tcol >> 8) << 1) | (tcol & 1)
    etile = [ecol[j, 0] for j in range(TOPC)]
    gcol, gn = classes(pcol)
    xs_v[...] = jnp.zeros((8, D), f32)

    def gather(c, carry):
        oh = (gcol == c) & (lane8 == pcol)
        ohi = jnp.where(oh, 1, 0)
        msk = [jnp.broadcast_to(ohi[j:j + 1], (8, 128)) == 1 for j in range(TOPC)]
        sa = sb = None
        for j in range(TOPC):
            fa = jnp.broadcast_to(fin_v[0, pl.ds(etile[j], 1), :], (8, 128))
            fb = jnp.broadcast_to(fin_v[1, pl.ds(etile[j], 1), :], (8, 128))
            sa, sb = (fa, fb) if j == 0 else (jnp.where(msk[j], fa, sa), jnp.where(msk[j], fb, sb))
        parts = []
        for q in range(D // 8 // LG):
            mg = None
            for j in range(TOPC):
                cc = c1_v[LG * q // NV, LG * q % NV:LG * q % NV + LG, pl.ds(pl.multiple_of(8 * etile[j], 8), 8), :]
                mg = cc if j == 0 else jnp.where(msk[j], cc, mg)
            parts.append(mg * sa - sb)
        ln = jnp.concatenate(parts, 0).reshape(D, 128)
        xs_v[...] = xs_v[...] + _dot_nt(jnp.where(oh, 1.0, 0.0).astype(f32), ln)
        return carry

    lax.fori_loop(0, gn, gather, 0)
    xsel = xs_v[...]

    def rebuilt_rows():
        sdc = jnp.zeros((8, 1), f32)
        mc = jnp.zeros((8, 1), f32)
        sub1 = _iota((8, 1), 0)
        for j in range(TOPC):
            hitm = tok == jnp.broadcast_to(tcol[j:j + 1], (16, 128))
            red = lambda v: jnp.sum(jnp.sum(jnp.where(hitm, v, 0.0), axis=0, keepdims=True), axis=1, keepdims=True)
            sdc = jnp.where(sub1 == j, red(sd2), sdc)
            mc = jnp.where(sub1 == j, red(mean2), mc)
        return xsel * (sdc + 1.0) + mc

    tilec = tcol >> 7
    lanec = tcol & 127
    aux = {}

    def late_scalars():
        tiles = [tilec[j, 0] for j in range(TOPC)]
        hit = 0
        dup = []
        for j in range(TOPC):
            dup.append((hit >> tiles[j]) & 1)
            hit = hit | (1 << tiles[j])
        free, cnt = [], 0
        for t in range(16):
            un = 1 - ((hit >> t) & 1)
            free.append(jnp.where(un == 1, cnt, -1))
            cnt = cnt + un
        late, nd, mask = [tiles[0]], 0, hit
        for j in range(1, TOPC):
            rep = 0
            for t in range(16):
                rep = jnp.where(free[t] == nd, t, rep)
            late.append(jnp.where(dup[j] == 1, rep, tiles[j]))
            mask = mask | (1 << late[j])
            nd = nd + dup[j]
        aux.update(tiles=tiles, late=late, mask=mask)
        bs_v[...] = rebuilt_rows()
        aux["clscol"], aux["ncls"] = classes(lanec)
        for j in range(TOPC):
            code = jnp.where((tilec == late[j]) & (lane8 == lanec), aux["clscol"], -1)
            lm_v[j] = jnp.broadcast_to(jnp.max(code, axis=0, keepdims=True), (8, 128))

    def tile_idx(t, g0=0, ng=D // 8):
        if isinstance(t, int):
            return (pl.ds(g0, ng), t // 2, pl.ds(8 * (t % 2), 8), slice(None))
        return (pl.ds(g0, ng), t >> 1, pl.ds(pl.multiple_of(8 * (t & 1), 8), 8), slice(None))

    def ocopy(idx):
        return cp(out_v.at[idx], out_h.at[idx], osem.at[0])

    def early():
        for t in range(16):
            @pl.when(((aux["mask"] >> t) & 1) == 0)
            def _():
                ocopy(tile_idx(t)).start()

    def gate_up(c0, nc):
        g = _rb(_dot(xsel, wmat(wg_w, c0, nc)))
        up = _rb(_dot(xsel, wmat(wu_w, c0, nc)))
        yield
        act_v[:, c0:c0 + nc] = _rb(_rb(g * jax.nn.sigmoid(g)) * up)

    for cc in c_w[0]:
        cc.wait()
    mine = opieces[NTOP:]
    nsub = FCH[0] // FSUB
    for u in range(nsub):
        gu = gate_up(u * FSUB, FSUB)
        next(gu)
        if u == 0:
            late_scalars()
        for fn in mine[u * len(mine) // nsub:(u + 1) * len(mine) // nsub]:
            fn()
        run(gu)
    early()

    clscol = aux["clscol"]
    onehot = lambda c: jnp.where((clscol == c) & (lane8 == lanec), 1.0, 0.0).astype(f32)

    def down(p, c0, nc):
        r = slice(POFF[p], POFF[p] + PART[p])
        yc = _dot_nt(act_v[:, c0:c0 + nc], wd_v[r, c0:c0 + nc])
        y_v[:, r] = yc if c0 == 0 else y_v[:, r] + yc

    def place(p, fast):
        r0, nr = POFF[p], PART[p]
        g0, ng = r0 // 8, nr // 8
        gt = jnp.concatenate([gate] * ((nr + 127) // 128), 1)[:, :nr]
        newrow = _rb(bs_v[:, r0:r0 + nr] + _rb(_rb(y_v[:, r0:r0 + nr]) * gt))
        tn = lambda oh: lax.dot_general(newrow, oh, (((0,), (0,)), ((), ())), preferred_element_type=f32)
        if fast:
            uu = tn(jnp.concatenate([onehot(0), onehot(1)], 1))
            for c in range(2):
                u_v[c, g0:g0 + ng] = uu[:, 128 * c:128 * (c + 1)].reshape(ng, 8, 128)
        else:
            for c in range(TOPC):
                u_v[c, g0:g0 + ng] = tn(onehot(c)).reshape(ng, 8, 128)

    def write(p, fast):
        g0, ng = POFF[p] // 8, PART[p] // 8
        for j in range(TOPC):
            idx = tile_idx(aux["late"][j], g0, ng)
            new = out_v[idx].astype(f32)
            code = lm_v[j]
            for c in range(2 if fast else TOPC):
                new = jnp.where(code == c, u_v[c, g0:g0 + ng], new)
            sg_v[j, g0:g0 + ng] = new.astype(bf16)
            cp(sg_v.at[j, pl.ds(g0, ng)], out_h.at[idx], osem.at[0]).start()

    NP = len(PART)
    for cc in c_w[1]:
        cc.wait()
    c_d[0].wait()
    run(gate_up(FCH[0], FCH[1]))
    down(0, 0, FCH[0])
    down(0, FCH[0], FCH[1])
    for p in range(1, NP - 1):
        c_d[p].wait()

    @pl.when(aux["ncls"] <= 2)
    def _():
        for p in range(1, NP):
            if p == NP - 1:
                c_d[p].wait()
            down(p, 0, DSPL[p])
            place(p - 1, True)
            down(p, DSPL[p], F - DSPL[p])
            write(p - 1, True)
        place(NP - 1, True)
        write(NP - 1, True)

    @pl.when(aux["ncls"] > 2)
    def _():
        c_d[NP - 1].wait()
        for p in range(1, NP):
            down(p, 0, F)
        for p in range(NP):
            place(p, False)
            write(p, False)

    cp(out_h, out_h, osem.at[0]).wait()


@jax.jit
def pallas_sequential_preLN__ssm_conv_s4__moe_arch_mod__prompt_kernel(
    A_u: jax.Array,
    A_A_re: jax.Array,
    A_A_im: jax.Array,
    A_B_re: jax.Array,
    A_B_im: jax.Array,
    A_C_re: jax.Array,
    A_C_im: jax.Array,
    A_log_dt: jax.Array,
    A_Dskip: jax.Array,
    B_x: jax.Array,
    B_w_r: jax.Array,
    B_w_gate: jax.Array,
    B_w_up: jax.Array,
    B_w_down: jax.Array,
):
    hbm = pl.BlockSpec(memory_space=pltpu.MemorySpace.HBM)
    vm = pltpu.VMEM
    G8 = D // 8
    wshape = (D // 16, F // 128, 16, 128)
    wview = lambda w: w.reshape(D // 16, 2, 8, F // 128, 128).transpose(0, 1, 3, 2, 4)
    scratch = [
        vm((G8, NB, 16, 128), bf16), vm((6, NSTEP, 128, N), bf16), vm((D,), bf16), vm((D,), bf16), vm((D,), bf16),
        vm((CT_ROWS, 128), f32), vm(wshape, bf16), vm(wshape, bf16), vm((D, F), bf16), vm((G8, NB + 1, 16, 128), bf16),
        vm((9, 4, 144, 128), bf16), vm((2, 2, 2, 144, 128), bf16), vm((3, NSTEP, 96, 128), f32),
        vm((NV, 2, 136, 128), f32), vm((NSTEP, 12, 56, 128), f32), vm((NSTEP, 96, 128), f32),
        vm((NSTEP, NB, 6, R, 128), f32), vm((NSTEP, NB, 6, R, 128), f32),
        vm((NSTEP, NB, 2, R, 256), f32), vm((NSTEP, 12, 136, 128), f32), vm((2, 17, 8, 128), f32),
        vm((3, 136, 128), f32), vm((5, 16, 128), f32), vm((TOPC, G8, 8, 128), f32),
        vm((R, 512), f32), vm((8, D), f32), vm((NV, 4, 8, 128), f32),
        vm((8, 128), f32), vm((8, D), f32), vm((8, D), f32), vm((8, F), f32),
        vm((TOPC, G8, 8, 128), bf16), vm((TOPC, 8, 128), i32), vm((8, D), f32), pltpu.SMEM((1,), i32),
        pltpu.SemaphoreType.DMA((6 + len(PART),)), pltpu.SemaphoreType.DMA((1,)),
    ]
    xv = A_u[0].T.reshape(G8, 8, 16, 128).transpose(0, 2, 1, 3).reshape(G8, NB, 16, 128)
    out = pl.pallas_call(
        _kernel,
        out_shape=jax.ShapeDtypeStruct((G8, NB, 16, 128), bf16),
        in_specs=[hbm] * 13,
        out_specs=hbm,
        scratch_shapes=scratch,
        compiler_params=pltpu.CompilerParams(vmem_limit_bytes=120 * 1024 * 1024, disable_bounds_checks=True,
                                             disable_semaphore_checks=True),
    )(xv, *[p.reshape(NSTEP, R, N) for p in (A_A_re, A_A_im, A_B_re, A_B_im, A_C_re, A_C_im)], A_log_dt, A_Dskip, B_w_r,
      wview(B_w_gate), wview(B_w_up), B_w_down.T)
    return out.reshape(G8, 16, 8, 128).transpose(0, 2, 1, 3).reshape(D, L).T[None]
```

```python
import functools

import numpy as np
import jax
import jax.numpy as jnp
from jax import lax
import jax.experimental.pallas as pl
import jax.experimental.pallas.tpu as pltpu

f32 = jnp.float32
bf16 = jnp.bfloat16
i32 = jnp.int32
u32 = jnp.uint32

L, D, N, F, TOPC = 2048, 576, 128, 4608, 8
NB = 8
NV = 9
R = NV * 8
NSTEP = D // R
EPS = 1e-5

_XL1 = [(1, 5), (2, 6), (3, 7), (4, 8), (258, 516), (260, 520), (262, 772), (264, 776),
        (1288, 1032), (1800, 1544)]
_XSH = [0, 1, 2, 3, 0, 1, 2, 3, 0, 1]


def _bf16_round_int(j):
    u = np.asarray(j, np.float32).view(np.uint32).astype(np.uint64)
    r = ((u + 0x7FFF + ((u >> 16) & 1)) >> 16) << 16
    return r.astype(np.uint32).view(np.float32).astype(np.int64)


def _chunk_values():
    vals = -np.ones((5, 128), np.int64)
    for j in range(10):
        for p in range(2):
            ch = (j // 4) * 2 + p if j < 8 else 4
            extra = 2 * p if j >= 8 else 0
            for l0 in range(32):
                vals[ch, (4 * (31 - l0) + 4 * p + _XSH[j] + extra + 8) % 128] = _XL1[j][p] + 8 * l0
    assert (vals >= 0).all()
    return vals


_PASSES = [(0, "A0"), (0, "A1"), (1, "B"), (2, "Cp"), (3, "C"), (4, "Dp"), (5, "D"), (6, "D"), (7, "D")]
_SETS = [[0], [1], [2], [3, 4], [5, 6, 7, 8]]


def _tables():
    cv = _chunk_values()
    cvp = {"A0": cv[0], "A1": cv[1], "B": cv[2], "C": cv[3], "D": cv[4]}
    cvp["Cp"] = cv[3].copy(); cvp["Cp"][11] = cv[2][11]
    cvp["Dp"] = cv[4].copy(); cvp["Dp"][15] = cv[3][15]
    sup = [[[] for _ in range(128)] for _ in _PASSES]
    for b in range(NB):
        for j in range(1, 257):
            lag = 256 * b + j
            if lag > L - 1 or lag == 257:
                continue
            v = int(_bf16_round_int(lag))
            hit = [(i, int(np.nonzero(cvp[nm] == v)[0][0])) for i, (pb, nm) in enumerate(_PASSES)
                   if pb == b and (cvp[nm] == v).any()]
            assert len(hit) == 1, (b, j, v, hit)
            sup[hit[0][0]][hit[0][1]].append(j)
    assert cv[1][15] == _bf16_round_int(257)
    code = np.zeros((len(_PASSES), 128), np.int64)
    for i, (pb, _) in enumerate(_PASSES):
        for r in range(128):
            js = sup[i][r]
            if js:
                assert js == list(range(js[0], js[-1] + 1))
                code[i, r] = js[0] + js[-1] + 1024 * len(js) + 16384 * (pb % 2)
    seeds, masks = [], {}
    for ps in _SETS:
        seeds.append([int(x) for x in sum(code[i, 16:24] for i in ps)])
        for i in ps:
            masks[i] = [int(x > 0) for x in code[i, 16:24]]
            for v in range(2, 17):
                r0 = 8 * (v % 16)
                assert (code[i, r0:r0 + 8] == (np.array(seeds[-1]) - 32 * (v - 2)) * np.array(masks[i])).all()
    return seeds, [[int(x) for x in code[i, 8:16]] for i in range(len(_PASSES))], masks


_GSEED, _GROW1, _GMASK = _tables()


def _sincos_coeffs():
    r = np.cos(np.pi * (np.arange(4000) + .5) / 4000) * 0.5
    z = r * r
    s = np.linalg.lstsq(np.stack([z ** k for k in range(4)], 1), np.sin(np.pi / 2 * r) / r, rcond=None)[0]
    c = np.linalg.lstsq(np.stack([z ** k for k in range(1, 5)], 1), np.cos(np.pi / 2 * r) - 1, rcond=None)[0]
    return [float(x) for x in s], [float(x) for x in c]


_SC, _CC = _sincos_coeffs()


def _cmul(a, b):
    return (a[0] * b[0] - a[1] * b[1], a[0] * b[1] + a[1] * b[0])


def _cmulc(a, b):
    return (a[0] * b[0] + a[1] * b[1], a[1] * b[0] - a[0] * b[1])


def _csq(a):
    return ((a[0] - a[1]) * (a[0] + a[1]), (a[0] + a[0]) * a[1])


def _quarter_polys(r):
    r2 = r * r
    s = r * (_SC[0] + r2 * (_SC[1] + r2 * (_SC[2] + r2 * _SC[3])))
    c = 1.0 + r2 * (_CC[0] + r2 * (_CC[1] + r2 * (_CC[2] + r2 * _CC[3])))
    return s, c


def _rotate_quadrant(s, c, ki):
    swap = (ki & 1) == 1
    s2 = jnp.where(swap, c, s)
    c2 = jnp.where(swap, s, c)
    s2 = pltpu.bitcast(pltpu.bitcast(s2, i32) ^ ((ki & 2) << 30), f32)
    c2 = pltpu.bitcast(pltpu.bitcast(c2, i32) ^ (((ki + 1) & 2) << 30), f32)
    return s2, c2


def _sincos(th):
    z = th * (2.0 / np.pi)
    k = jnp.round(z)
    s, c = _quarter_polys(z - k)
    return _rotate_quadrant(s, c, k.astype(i32))


def _reduce_small(z):
    big = 12582912.0
    t = z + big
    return _quarter_polys(z - (t - big)) + (pltpu.bitcast(t, i32),)


def _rb(x):
    return x.astype(bf16).astype(f32)


def _dot(a, b):
    return jnp.dot(a, b, preferred_element_type=f32)


def _dot_nt(a, b):
    return lax.dot_general(a, b, (((1,), (1,)), ((), ())), preferred_element_type=f32)


def _iota(shape, dim):
    return lax.broadcasted_iota(i32, shape, dim)


ORDER, ORD0, ORD5, ORD6 = "4ab44342np445", "4ab442n4p4345", "4a424n44b345p", "45a4b244p3n44"
TILE = 4
LG = 3
NTOP = 4
FCH = (3456, 1152)
FSUB = 1152
PART = (256, 128, 128, 64)
POFF = [sum(PART[:i]) for i in range(len(PART))]
DSPL = (0, 2560, 2560, 4096)
CT_ROWS = 320


def _weave(*streams):
    items = []
    for si, (pieces, lo, hi) in enumerate(streams):
        tot = float(sum(c for _, c in pieces))
        cum = 0.0
        for pi, (fn, c) in enumerate(pieces):
            items.append((lo + max(hi - lo, 0.0) * (cum + 0.5 * c) / tot, si, pi, fn))
            cum += c
    for _, _, _, fn in sorted(items, key=lambda t: t[:3]):
        fn()


def _kernel(x_h, are_h, aim_h, bre_h, bim_h, cre_h, cim_h, ldt_h, dsk_h, wr_h, wg_h, wu_h, wd_h,
            out_h,
            x_v, par_v, ldt_v, dsk_v, wr_v, ct_v, wg_v, wu_v, wd_v, out_v,
            g_v, f_v, col_v, st_v, kd_v, k0_v, kh_v, uh_v, zs_v, c1_v, s1_v, acc_v, fin_v, u_v, zt_v,
            y_v, pv_v, kc_v, xs_v, bs_v, act_v, sg_v, lm_v, rw_v, flag_s,
            sem, osem):
    cp = pltpu.make_async_copy
    c_vec = [cp(ldt_h, ldt_v, sem.at[0]), cp(dsk_h, dsk_v, sem.at[0]), cp(wr_h, wr_v, sem.at[0])]
    PH = 4
    par_h = (are_h, aim_h, bre_h, bim_h, cre_h, cim_h)
    c_par = [cp(h.at[pl.ds(0, PH)], par_v.at[i, pl.ds(0, PH), pl.ds(0, R)], sem.at[1])
             for i, h in enumerate(par_h)]
    c_par2 = [cp(h.at[pl.ds(PH, NSTEP - PH)], par_v.at[i, pl.ds(PH, NSTEP - PH), pl.ds(0, R)], sem.at[2])
              for i, h in enumerate(par_h)]
    c_x = cp(x_h, x_v, sem.at[3])

    def wcp(h, v, c):
        ct = pl.ds(sum(FCH[:c]) // 128, FCH[c] // 128)
        return [cp(h.at[:, hf, ct], v.at[:, ct, pl.ds(8 * hf, 8), :], sem.at[4 + c]) for hf in range(2)]

    c_w = [wcp(wg_h, wg_v, c) + wcp(wu_h, wu_v, c) for c in range(2)]
    c_d = [cp(wd_h.at[pl.ds(POFF[p], PART[p])], wd_v.at[pl.ds(POFF[p], PART[p])], sem.at[6 + p])
           for p in range(len(PART))]
    for c in c_vec + c_par + [c_x] + c_par2 + sum(c_w, []) + c_d:
        c.start()

    flag_s[0] = 1
    x_w = x_v.bitcast(u32)
    wg_w, wu_w = wg_v.bitcast(u32), wu_v.bitcast(u32)

    def wmat(w, c0, nc):
        return jnp.concatenate([pltpu.bitcast(w[:, t], bf16).reshape(D, 128)
                                for t in range(c0 // 128, (c0 + nc) // 128)], 1)

    out_w = out_v.bitcast(u32)
    g_w = g_v.bitcast(u32)
    f_w = f_v.bitcast(u32)
    sub8 = _iota((8, 128), 0)
    lane8 = _iota((8, 128), 1)

    acc_v[...] = jnp.zeros(acc_v.shape, f32)
    for ri in range(2):
        st_v[:, ri, 104:112, :] = jnp.full((NV, 8, 128), 1.0 - ri, f32)
    kp = (2 * lane8 + 1).astype(f32)

    def rows_const(vals):
        out = jnp.full((8, 128), vals[0], i32)
        for r in range(1, 8):
            if vals[r] != vals[0]:
                out = jnp.where(sub8 == r, vals[r], out)
        return out

    def phasor(z):
        sn, cs = _rotate_quadrant(*_reduce_small(-z))
        return cs, sn

    NS = [0, 1, 2, 3, 4, 5, 7, 9]
    for q in range(2):
        sn = _rotate_quadrant(*_reduce_small((kp + 512.0 * q) * (rows_const(NS).astype(f32) * (1.0 / 512))))[0]
        ct_v[304 + 8 * q:312 + 8 * q, :] = sn / (256.0 * jnp.broadcast_to(sn[1:2], (8, 128)))

    def grows(vals):
        ab = rows_const([v & 1023 for v in vals])
        z = kp * (ab.astype(f32) * (-1.0 / 512))
        if any(v >> 14 for v in vals):
            z = z - rows_const([v >> 14 for v in vals]).astype(f32) * (kp - 1.0)
        sn, cs, ki = _reduce_small(z)
        ns = [NS.index((v >> 10) & 15) for v in vals]
        out = []
        for q in range(2):
            row = lambda i: jnp.broadcast_to(ct_v[304 + 8 * q + i:305 + 8 * q + i, :], (8, 128))
            amp = None
            for i in sorted(set(ns)):
                bits = sum(1 << r for r in range(8) if ns[r] == i)
                amp = row(i) if amp is None else jnp.where(((bits >> sub8) & 1) == 1, row(i), amp)
            pi, pr = _rotate_quadrant(sn, cs, ki if q == 0 else ki - ab)
            out += [pr * amp, pi * amp]
        return out

    for v4 in range(4):
        e = phasor(kp * ((sub8 + 8 * v4).astype(f32) * (1.0 / 32)))
        ct_v[8 * v4:8 * v4 + 8, :] = e[0]
        ct_v[32 + 8 * v4:40 + 8 * v4, :] = e[1]
    for si in range(5):
        for q, val in enumerate(grows(_GSEED[si])):
            ct_v[64 + 32 * si + 8 * q:72 + 32 * si + 8 * q, :] = val
    for i in range(len(_PASSES)):
        for q, val in enumerate(grows(_GROW1[i])):
            g_v[i, q, 8:16, :] = val.astype(bf16)
    for q, val in enumerate(grows([2 + 1024 + 16384] * 8)):
        ct_v[272 + 8 * q:280 + 8 * q, :] = val
    s8 = np.arange(8)
    je = np.where(s8 % 2 == 0, s8, 127 + s8)
    jo = np.where(s8 % 2 == 0, s8 - 1, 128 + s8)
    for t, jj in enumerate((je, jo, jo % 128 + 128 * (s8 % 2))):
        e = phasor(kp * (rows_const([int(x) for x in jj]).astype(f32) * (1.0 / 256)))
        ct_v[224 + 16 * t:232 + 16 * t, :] = e[0]
        ct_v[232 + 16 * t:240 + 16 * t, :] = e[1]
    for c in c_vec:
        c.wait()

    rows = [_rb(jnp.exp(ldt_v[...].astype(f32).reshape(1, D))),
            dsk_v[...].astype(f32).reshape(1, D),
            wr_v[...].astype(f32).reshape(1, D)]
    wr_sum = jnp.sum(rows[2], axis=1, keepdims=True)

    def columns(which):
        for j in range(5):
            w = 128 if j < 4 else 64
            eye = _iota((w, w), 0) == _iota((w, w), 1)
            m = jnp.concatenate([jnp.where(eye, jnp.broadcast_to(rw_v[i:i + 1, j * 128:j * 128 + w], (w, w)), 0.0)
                                 for i in which], 0)
            res = _dot(m, jnp.ones((w, 128), f32))
            for n, i in enumerate(which):
                for g in range(w // 8):
                    k, m8 = divmod(16 * j + g, NV)
                    col_v[i, k, 8 * m8:8 * m8 + 8, :] = res[n * w + 8 * g:n * w + 8 * g + 8]

    for i in range(3):
        rw_v[i:i + 1, :] = rows[i]
    columns((0,))

    def e8(v):
        return (jnp.broadcast_to(ct_v[v:v + 1, :], (8, 128)), jnp.broadcast_to(ct_v[32 + v:33 + v, :], (8, 128)))

    for si, ps in enumerate(_SETS):
        sd = [ct_v[64 + 32 * si + 8 * q:72 + 32 * si + 8 * q, :] for q in range(4)]
        mk = {}
        for i in ps:
            if len(ps) > 1:
                bits = sum(b << s for s, b in enumerate(_GMASK[i]))
                mk[i] = ((bits >> sub8) & 1) == 1
        for v in range(2, 17):
            if v == 2:
                vals = sd
            else:
                ev = e8(2 * (v - 2))
                vals = list(_cmulc((sd[0], sd[1]), ev)) + list(_cmulc((sd[2], sd[3]), ev))
            vals = jnp.stack(vals, 0)
            for i in ps:
                val = vals if len(ps) == 1 else jnp.where(mk[i], vals, 0.0)
                g_v[i, :, 8 * (v % 16):8 * (v % 16) + 8, :] = val.astype(bf16)
    sig = jnp.where((lane8 & 1) == 0, 1.0, -1.0).astype(f32)
    for h in range(2):
        sd = (ct_v[224 + 16 * h:232 + 16 * h, :], ct_v[232 + 16 * h:240 + 16 * h, :])
        for v in range(16):
            if v == 0:
                vals = sd if h == 0 else (ct_v[256:264, :], ct_v[264:272, :])
            else:
                vals = _cmul(sd, e8(v))
            for q in range(2):
                f_v[0, h, q, 8 * v:8 * v + 8, :] = vals[q].astype(bf16)
                f_v[1, h, q, 8 * v:8 * v + 8, :] = (vals[q] * sig).astype(bf16)

    def gmat(i):
        return jnp.concatenate([pltpu.bitcast(g_w[i, q, 0:64, :], bf16) for q in range(4)], 1)

    def fmat(ver, h):
        return jnp.concatenate([pltpu.bitcast(f_w[ver, h, q, 0:64, :], bf16) for q in range(2)], 1)

    revmask = (sub8 & 2) == 0
    lm = lane8 & 3

    def s1_nat(k, n0, nn):
        rr = 8 * nn
        ld = lambda i: par_v[i, k, 8 * n0:8 * n0 + rr, :].astype(f32)
        dt = col_v[0, k, 8 * n0:8 * n0 + rr, :]
        e = jnp.exp(dt * ld(0))
        s, c = _sincos(dt * ld(1))
        a1 = (e * c, e * s)
        w = _cmul((ld(4), ld(5)), (dt * ld(2), dt * ld(3)))
        k0_v[k, 8 * n0:8 * n0 + rr, :] = jnp.broadcast_to(jnp.sum(w[0], axis=1, keepdims=True), (rr, 128))
        w = (w[0], -w[1])
        rev = lambda v: jnp.where(revmask, pltpu.roll(v, 2, 2), pltpu.roll(v, 6, 2))

        def put(arr, slots, fn=None):
            v = jnp.stack([a.reshape(nn, 8, 128) for a in arr], 1)
            if fn is not None:
                v = fn(v)
            for q in slots:
                st_v[n0:n0 + nn, :, q * 8:q * 8 + 8, :] = v

        put(w, (0, 1)); put(a1, (2, 3))
        a2 = _csq(a1); put(a2, (5,))
        a4 = _csq(a2); put(a4, (6,))
        put(_cmul(a4, a1), (4,))
        a8 = _csq(a4); put(a8, (12,), rev)
        t = _csq(a8); put(t, (14, 15), rev)
        for _ in range(4):
            t = _csq(t)
        put(t, (7, 11))
        t = _csq(t); put(t, (8, 9))
        put(_csq(t), (10,))

    def s1_grp(k, n):
        def mix(q):
            gs = [st_v[n, :, pl.ds(q * 8 + g, 8, stride=2), :] for g in range(2)]
            return tuple(jnp.concatenate([gs[0][ri], gs[1][ri]], 0) for ri in range(2))

        y = [mix(12)]
        a16d = mix(14)
        for _ in range(15):
            y.append(_cmul(y[-1], a16d))
        yield
        wd = mix(0); a1d = mix(2); m1 = mix(5)
        v = [_cmulc(wd, mix(3))]
        for _ in range(3):
            v.append(_cmulc(v[-1], a1d))
        v4 = _cmulc(_cmulc(wd, m1), mix(7))
        v5 = _cmulc(v4, m1); v6 = _cmulc(v4, mix(6)); v7 = _cmulc(v6, m1)
        v8 = _cmulc(v7, mix(10)); v9 = _cmulc(v8, mix(8))
        v += [v4, v5, v6, v7, v8, v9]
        os_ = []
        for g in range(2):
            cat = lambda ts: jnp.concatenate([jnp.concatenate([t[ri][8 * g:8 * g + 8] for t in ts], 0)
                                              for ri in range(2)], 1)
            os_.append(_dot_nt(cat(v), cat(y[::-1])))
        yield
        for g in range(2):
            o = os_[g]
            ro = [pltpu.roll(o[8 * j:8 * j + 8], _XSH[j] + 5, 1, stride=1, stride_axis=0) for j in range(10)]
            sel4 = lambda q: jnp.where(lm == 0, q[0], jnp.where(lm == 1, q[1], jnp.where(lm == 2, q[2], q[3])))
            kd_v[k, n, pl.ds(g, 8, stride=2), :] = sel4(ro[0:4])
            kd_v[k, n, pl.ds(16 + g, 8, stride=2), :] = sel4(ro[4:8])
            kd_v[k, n, pl.ds(32 + g, 8, stride=2), :] = jnp.where(lm == 0, ro[8], ro[9])

    def run(gen):
        for _ in gen:
            pass

    s1n = lambda k: [(functools.partial(s1_nat, k, 3 * i, 3), 1.0) for i in range(3)]
    s1g = lambda k: [(lambda n=n: run(s1_grp(k, n)), 1.0) for n in range(NV)]

    laneR = _iota((R, 128), 1)
    lmR = laneR & 3

    def s2_gen(k):
        ch = lambda c: kd_v[k, 0:NV, 8 * c:8 * c + 8, :].reshape(R, 128)
        for b in range(NB):
            if b == 0:
                k0 = (k0_v[k, 0:R, :] + col_v[1, k, 0:R, :]) * (1.0 / 256.0)
                z = _dot(ch(0), gmat(0))
                dd = jnp.where(lmR < 2, ch(4), pltpu.roll(ch(5), 2, 1))
                kd_v[k, 0:NV, 48:56, :] = dd.reshape(NV, 8, 128)
                zt_v[...] = z
                yield
                z = _dot(ch(1), gmat(1)) + zt_v[...]
            elif b == 1:
                k256 = jnp.sum(jnp.where(laneR == 15, ch(1), 0.0), axis=1, keepdims=True)
                pat = jnp.concatenate([ct_v[272 + 8 * q:273 + 8 * q, :] for q in range(4)], 1)
                z = _dot(ch(2), gmat(2)) + k256 * pat
            elif b == 2:
                z = _dot(jnp.where(laneR == 11, ch(2), ch(3)), gmat(3))
            elif b == 3:
                z = _dot(ch(3), gmat(4))
            elif b == 4:
                z = _dot(jnp.where(laneR == 15, ch(3), ch(6)), gmat(5))
            else:
                z = _dot(ch(6), gmat(b + 1))
            for s in range(2):
                kr = z[:, 256 * s:256 * s + 128]
                ki = z[:, 256 * s + 128:256 * s + 256]
                if b == 0:
                    kr = kr + k0
                kh_v[k, b, 3 * s] = kr
                kh_v[k, b, 3 * s + 1] = ki
            yield

    def s2(k):
        gen = s2_gen(k)
        return [(lambda: next(gen, None), 1.0) for _ in range(9)]

    mask2 = (sub8 < 4) == ((lane8 & 1) == 0)
    top = sub8 < 4

    def ln1_pieces(b, npc):
        state = {}
        per = (D // 8) // npc

        def piece(i):
            for g in range(i * per, (i + 1) * per, LG):
                m = x_w[g:g + LG, b]
                eo = jnp.where(mask2, m, pltpu.roll(pltpu.roll(m, 4, 1), 1, 2))
                a = pltpu.bitcast(eo << 16, f32)
                c = pltpu.bitcast(eo & jnp.uint32(0xFFFF0000), f32)
                if g == 0:
                    state["sh"] = jnp.where(top, jnp.broadcast_to(a[0, 0:1], (8, 128)),
                                            jnp.broadcast_to(a[0, 4:5], (8, 128)))
                a = a - state["sh"]
                c = c - state["sh"]
                c1_v[g // NV, g % NV:g % NV + LG, pl.ds(16 * b, 8, stride=2), :] = a
                c1_v[g // NV, g % NV:g % NV + LG, pl.ds(16 * b + 1, 8, stride=2), :] = c
                for q in range(LG):
                    new = [a[q], c[q], a[q] * a[q], c[q] * c[q]]
                    state["acc"] = new if g + q == 0 else [p + r for p, r in zip(state["acc"], new)]
            if i == npc - 1:
                acc = state["acc"]
                s1, s2_ = acc[0] + acc[1], acc[2] + acc[3]
                for h in range(2):
                    m = jnp.sum(s1[4 * h:4 * h + 4], axis=0, keepdims=True) * (1.0 / D)
                    var = jnp.sum(s2_[4 * h:4 * h + 4], axis=0, keepdims=True) * (1.0 / D) - m * m
                    rs = 1.0 / _rb(jnp.sqrt(_rb(_rb(jnp.maximum(var, 0.0)) + EPS)))
                    s1_v[0, 2 * b + h] = jnp.broadcast_to(rs, (8, 128))
                    sh = state["sh"][4 * h:4 * h + 1]
                    s1_v[1, 2 * b + h] = jnp.broadcast_to((_rb(m + sh) - sh) * rs, (8, 128))
                    fin_v[4, 2 * b + h:2 * b + h + 1, :] = state["sh"][4 * h:4 * h + 1]

        return [(functools.partial(piece, i), 1.0) for i in range(npc)]

    def s3_blk(k, b):
        et = []
        for h in range(2):
            c = c1_v[k, 0:NV, 16 * b + 8 * h:16 * b + 8 * h + 8, :]
            u = (c * s1_v[0, 2 * b + h] - s1_v[1, 2 * b + h]).reshape(R, 128)
            et.append(_dot(u, fmat(b % 2, h)))
        er, ei, tr, ti = et[0][:, :128], et[0][:, 128:], et[1][:, :128], et[1][:, 128:]
        for q, v in enumerate((er, ei, tr, ti)):
            uh_v[k, b, q] = v

    s3 = lambda k: [(functools.partial(s3_blk, k, b), 1.0) for b in range(NB)]

    def s4_gen(k, n, groups=None):
        sl = slice(8 * n, 8 * n + 8)

        def utrip(i, s):
            et = uh_v[k, i, 0:4, sl, :]
            er, ei, tr, ti = et[0], et[1], et[2], et[3]
            pr, pi = (er + tr, ei + ti) if s == 0 else (er - tr, ei - ti)
            return [pr + pi, pi, pr]

        prev = None
        done = 0
        if groups is not None and groups[0] > 0:
            prev = [(pv_v[n, 2 * h], pv_v[n, 2 * h + 1]) for h in range(2)]
        for b0 in (range(0, NB, TILE) if groups is None else groups):
            yy = []
            for s in range(2):
                acc = [None] * TILE
                win = {}
                for j in range(b0 + TILE):
                    kri = kh_v[k, j, 3 * s:3 * s + 2, sl, :]
                    kk = [kri[0], kri[0] + kri[1], kri[1] - kri[0]]
                    for o in range(TILE - 1, -1, -1):
                        i = b0 + o - j
                        if i < 0:
                            continue
                        if i not in win:
                            win[i] = utrip(i, s)
                        p = [kk[q] * win[i][q] for q in range(3)]
                        acc[o] = p if acc[o] is None else [a + c for a, c in zip(acc[o], p)]
                        done += 1
                    if b0 == 4 and j == 2:
                        yield done
                yy.append([(a[0] - a[1], a[0] + a[2]) for a in acc])
                if s == 0:
                    yield done
            for o in range(TILE):
                p, q = yy[0][o], yy[1][o]
                cur = [(p[0] + q[0], p[1] + q[1]), (p[0] - q[0], p[1] - q[1])]
                for h in range(2):
                    if b0 + o == 0:
                        zr, zi = cur[h]
                    else:
                        zr = cur[h][0] - prev[h][1]
                        zi = cur[h][1] + prev[h][0]
                    zs_v[k, b0 + o, h, sl, :] = jnp.concatenate([zr, zi], 1)
                prev = cur
            if groups is not None and b0 + TILE < NB:
                for h in range(2):
                    pv_v[n, 2 * h] = prev[h][0]
                    pv_v[n, 2 * h + 1] = prev[h][1]
            yield done

    def s5_blk(k, b, h):
        t = 2 * b + h
        y = _dot_nt(zs_v[k, b, h], fmat(b % 2, h)).reshape(NV, 8, 128)
        hh = c1_v[k, 0:NV, 16 * b + 8 * h:16 * b + 8 * h + 8, :] + y
        c1_v[k, 0:NV, 16 * b + 8 * h:16 * b + 8 * h + 8, :] = hh
        wr = col_v[2, k, 0:R, :].reshape(NV, 8, 128)
        rs = slice(8 * t, 8 * t + 8)
        acc_v[0, rs, :] = acc_v[0, rs, :] + jnp.sum(hh, axis=0)
        acc_v[1, rs, :] = acc_v[1, rs, :] + jnp.sum(hh * hh, axis=0)
        acc_v[2, rs, :] = acc_v[2, rs, :] + jnp.sum(hh * wr, axis=0)

    s5 = lambda k: [(functools.partial(s5_blk, k, b, h), 1.0) for b in range(NB) for h in range(2)]

    for c in c_par:
        c.wait()
    columns((1, 2))
    for k in range(2):
        _weave((s1n(k), 0.0, 0.2), (s1g(k), 0.2, 1.0))
    _weave((s1n(2), 0.0, 0.2), (s1g(2), 0.2, 1.0), (s2(0), 0.3, 1.0))
    s1_nat(3, 0, 1)
    c_x.wait()
    ln = [ln1_pieces(b, 3) for b in range(NB)]
    s30 = s3(0)
    _weave((sum(ln, []), 0.0, 0.9), (s2(1), 0.0, 0.55),
           *[([s30[b]], max((b + 1.6) * 0.9 / NB, 0.3 + 0.7 * b / NB), 0.0) for b in range(NB)])
    for c in c_par2:
        c.wait()

    def body(k, do5=True, do4=True, do3=True, do2=True, do1=True, j=None, order=None):
        order = order or ORDER
        at = (lambda d: k + d) if j is None else (lambda d: j + (k + d) if k + d else j)
        g2 = s2_gen(at(2)) if do2 else None
        for n in range(NV):
            g4 = s4_gen(at(0), n) if do4 else None
            st4 = [0, 0]
            n4 = order.count("4")

            def adv4(m):
                if not do4:
                    return
                st4[0] += 1
                while st4[1] < 72 * st4[0] / n4 - 3 or (st4[0] == n4 and st4[1] <= 72):
                    r = next(g4, None)
                    if r is None:
                        break
                    st4[1] = r

            def nat():
                if do1:
                    if n + 1 < NV:
                        s1_nat(at(3), n + 1, 1)
                    else:
                        s1_nat(jnp.minimum(at(4), NSTEP - 1), 0, 1)

            g1 = s1_grp(at(3), n) if do1 else None
            for tok in order:
                if tok == "5":
                    if do5 and n < NB:
                        s5_blk(at(-1), n, 0)
                        s5_blk(at(-1), n, 1)
                elif tok == "4":
                    adv4(1)
                elif tok in "ab" and do1:
                    next(g1)
                elif tok == "p" and do1:
                    run(g1)
                elif tok == "2" and do2:
                    next(g2, None)
                elif tok == "3" and do3 and n < NB:
                    s3_blk(at(1), n)
                elif tok == "n":
                    nat()
        if do2:
            run(g2)

    @pl.when(flag_s[0] == 1)
    def _():
        body(0, do5=False, order=ORD0)

    lax.fori_loop(0, 4, lambda j, c: (body(1, j=j), c)[1], 0)

    @pl.when(flag_s[0] == 1)
    def _():
        body(5, do1=False, order=ORD5)

    @pl.when(flag_s[0] == 1)
    def _():
        body(6, do1=False, do2=False, order=ORD6)

    @pl.when(flag_s[0] == 1)
    def _():
        _weave(([(lambda n=n: run(s4_gen(7, n, (0,))), 1.0) for n in range(NV)], 0.0, 1.0), (s5(6), 0.0, 1.0))

    @pl.when(flag_s[0] == 1)
    def _():
        _weave(([(lambda n=n: run(s4_gen(7, n, (4,))), 1.0) for n in range(NV)], 0.0, 1.0), (s5(7)[:8], 0.0, 1.0))

    _weave((s5(7)[8:], 0.0, 1.0))

    def total(i):
        halves = []
        for hf in range(2):
            t = acc_v[i, pl.ds(64 * hf, 8, stride=8), :]
            for s in range(1, 8):
                t = t + acc_v[i, pl.ds(64 * hf + s, 8, stride=8), :]
            halves.append(t)
        return jnp.concatenate(halves, 0)

    m2 = total(0) * (1.0 / D)
    var2 = jnp.maximum(total(1) * (1.0 / D) - m2 * m2, 0.0)
    sd2 = _rb(jnp.sqrt(_rb(_rb(var2) + EPS)))
    rs2 = 1.0 / sd2
    mean2 = _rb(fin_v[4] + m2)
    m2 = mean2 - fin_v[4]
    r = _rb((total(2) - m2 * wr_sum) * rs2)
    fin_v[0] = rs2
    fin_v[1] = m2 * rs2
    fin_v[2] = rs2 + 1.0
    fin_v[3] = fin_v[4] - m2 * rs2

    def outp(b, g0, g1):
        sc = [jnp.where(top, jnp.broadcast_to(fin_v[i, 2 * b:2 * b + 1, :], (8, 128)),
                        jnp.broadcast_to(fin_v[i, 2 * b + 1:2 * b + 2, :], (8, 128))) for i in (2, 3)]
        for g in range(g0, g1, LG):
            src = lambda o: c1_v[g // NV, g % NV:g % NV + LG, pl.ds(16 * b + o, 8, stride=2), :]
            a = _rb(src(0) * sc[0] + sc[1])
            c = _rb(src(1) * sc[0] + sc[1])
            w = (pltpu.bitcast(a, u32) >> 16) | pltpu.bitcast(c, u32)
            out_w[g:g + LG, b] = jnp.where(mask2, w, pltpu.roll(pltpu.roll(w, 4, 1), 127, 2))

    opieces = [functools.partial(outp, b, 24 * i, 24 * i + 24) for b in range(NB) for i in range(3)]

    tl = _iota((16, 128), 0)
    ll = _iota((16, 128), 1)
    lodd = (ll & 1) == 1
    toff = jnp.where((tl & 1) == 0, jnp.where(lodd, ll + 127, ll), jnp.where(lodd, ll + 128, (ll - 1) & 127))
    tok = (tl >> 1) * 256 + toff
    rbits = pltpu.bitcast(r, i32)
    srt = rbits ^ ((rbits >> 31) & 0x7FFFFFFF)
    key = pltpu.bitcast((((srt >> 16) + 32768) << 11) + (2047 - tok) + (1 << 28), f32)
    kk = key
    cand = []
    for _ in range(4):
        rm = jnp.broadcast_to(jnp.max(kk, axis=1, keepdims=True), (16, 128))
        cand.append(rm)
        kk = jnp.where(kk == rm, 0.0, kk)
        for fn in opieces[(len(cand) - 1) * NTOP // 4:len(cand) * NTOP // 4]:
            fn()
    last = jnp.max(cand[3], axis=0, keepdims=True)
    kcol = None
    for j in range(TOPC):
        mx = jnp.max(cand[0], axis=0, keepdims=True)
        kcol = jnp.broadcast_to(mx, (8, 128)) if j == 0 else jnp.where(sub8 == j, mx, kcol)
        took = cand[0] == mx
        cand = [jnp.where(took, cand[i + 1] if i < 3 else 0.0, cand[i]) for i in range(4)]
    kc_v[...] = kcol

    @pl.when((last - mx)[0, 0] > 0.0)
    def _():
        k2 = key
        kc = None
        for j in range(TOPC):
            m1 = jnp.max(jnp.max(k2, axis=0, keepdims=True), axis=1, keepdims=True)
            kc = jnp.broadcast_to(m1, (8, 128)) if j == 0 else jnp.where(sub8 == j, m1, kc)
            k2 = jnp.where(k2 == m1, 0.0, k2)
        kc_v[...] = kc

    kcol = kc_v[...]
    kint = pltpu.bitcast(kcol, i32) - (1 << 28)
    tcol = 2047 - (kint & 2047)
    s16 = (kint >> 11) - 32768
    rsel = pltpu.bitcast((s16 ^ ((s16 >> 31) & 0x7FFF)) << 16, f32)
    gate = _rb(jax.nn.sigmoid(rsel))

    def classes(col):
        cls = jnp.zeros((8, 128), i32)
        for d in range(1, TOPC):
            cls = cls + jnp.where((col == pltpu.roll(col, d, 0)) & (sub8 >= d), 1, 0)
        return cls, jnp.max(cls, axis=0, keepdims=True)[0, 0] + 1

    wcol = tcol & 255
    pcol = jnp.where((wcol & 1) == 0, jnp.where(wcol < 128, wcol, wcol - 127),
                     jnp.where(wcol < 128, (wcol + 1) & 127, wcol - 128))
    ecol = ((tcol >> 8) << 1) | (tcol & 1)
    etile = [jnp.clip(ecol[j, 0], 0, 15) for j in range(TOPC)]
    gcol, gn = classes(pcol)
    xs_v[...] = jnp.zeros((8, D), f32)

    def gather(c, carry):
        oh = (gcol == c) & (lane8 == pcol)
        ohi = jnp.where(oh, 1, 0)
        msk = [jnp.broadcast_to(ohi[j:j + 1], (8, 128)) == 1 for j in range(TOPC)]
        sa = sb = None
        for j in range(TOPC):
            fa = jnp.broadcast_to(fin_v[0, pl.ds(etile[j], 1), :], (8, 128))
            fb = jnp.broadcast_to(fin_v[1, pl.ds(etile[j], 1), :], (8, 128))
            sa, sb = (fa, fb) if j == 0 else (jnp.where(msk[j], fa, sa), jnp.where(msk[j], fb, sb))
        parts = []
        for q in range(D // 8 // LG):
            mg = None
            for j in range(TOPC):
                cc = c1_v[LG * q // NV, LG * q % NV:LG * q % NV + LG, pl.ds(pl.multiple_of(8 * etile[j], 8), 8), :]
                mg = cc if j == 0 else jnp.where(msk[j], cc, mg)
            parts.append(mg * sa - sb)
        ln = jnp.concatenate(parts, 0).reshape(D, 128)
        xs_v[...] = xs_v[...] + _dot_nt(jnp.where(oh, 1.0, 0.0).astype(f32), ln)
        return carry

    lax.fori_loop(0, gn, gather, 0)
    xsel = xs_v[...]

    def rebuilt_rows():
        sdc = jnp.zeros((8, 1), f32)
        mc = jnp.zeros((8, 1), f32)
        sub1 = _iota((8, 1), 0)
        for j in range(TOPC):
            hitm = tok == jnp.broadcast_to(tcol[j:j + 1], (16, 128))
            red = lambda v: jnp.sum(jnp.sum(jnp.where(hitm, v, 0.0), axis=0, keepdims=True), axis=1, keepdims=True)
            sdc = jnp.where(sub1 == j, red(sd2), sdc)
            mc = jnp.where(sub1 == j, red(mean2), mc)
        return xsel * (sdc + 1.0) + mc

    tilec = tcol >> 7
    lanec = tcol & 127
    aux = {}

    def late_scalars():
        tiles = [jnp.clip(tilec[j, 0], 0, 15) for j in range(TOPC)]
        hit = 0
        dup = []
        for j in range(TOPC):
            dup.append((hit >> tiles[j]) & 1)
            hit = hit | (1 << tiles[j])
        free, cnt = [], 0
        for t in range(16):
            un = 1 - ((hit >> t) & 1)
            free.append(jnp.where(un == 1, cnt, -1))
            cnt = cnt + un
        late, nd, mask = [tiles[0]], 0, hit
        for j in range(1, TOPC):
            rep = 0
            for t in range(16):
                rep = jnp.where(free[t] == nd, t, rep)
            late.append(jnp.clip(jnp.where(dup[j] == 1, rep, tiles[j]), 0, 15))
            mask = mask | (1 << late[j])
            nd = nd + dup[j]
        aux.update(late=late, mask=mask)
        bs_v[...] = rebuilt_rows()
        aux["clscol"], aux["ncls"] = classes(lanec)
        for j in range(TOPC):
            code = jnp.where((tilec == late[j]) & (lane8 == lanec), aux["clscol"], -1)
            lm_v[j] = jnp.broadcast_to(jnp.max(code, axis=0, keepdims=True), (8, 128))

    def tile_idx(t, g0=0, ng=D // 8):
        if isinstance(t, int):
            return (pl.ds(g0, ng), t // 2, pl.ds(8 * (t % 2), 8), slice(None))
        return (pl.ds(g0, ng), t >> 1, pl.ds(pl.multiple_of(8 * (t & 1), 8), 8), slice(None))

    def ocopy(idx):
        return cp(out_v.at[idx], out_h.at[idx], osem.at[0])

    def early():
        for t in range(16):
            @pl.when(((aux["mask"] >> t) & 1) == 0)
            def _():
                ocopy(tile_idx(t)).start()

    def gate_up(c0, nc):
        g = _rb(_dot(xsel, wmat(wg_w, c0, nc)))
        up = _rb(_dot(xsel, wmat(wu_w, c0, nc)))
        yield
        act_v[:, c0:c0 + nc] = _rb(_rb(g * jax.nn.sigmoid(g)) * up)

    for cc in c_w[0]:
        cc.wait()
    mine = opieces[NTOP:]
    nsub = FCH[0] // FSUB
    for u in range(nsub):
        gu = gate_up(u * FSUB, FSUB)
        next(gu)
        if u == 0:
            late_scalars()
        for fn in mine[u * len(mine) // nsub:(u + 1) * len(mine) // nsub]:
            fn()
        run(gu)
    early()

    clscol = aux["clscol"]
    onehot = lambda c: jnp.where((clscol == c) & (lane8 == lanec), 1.0, 0.0).astype(f32)

    def down(p, c0, nc):
        r = slice(POFF[p], POFF[p] + PART[p])
        yc = _dot_nt(act_v[:, c0:c0 + nc], wd_v[r, c0:c0 + nc])
        y_v[:, r] = yc if c0 == 0 else y_v[:, r] + yc

    def place(p, fast):
        r0, nr = POFF[p], PART[p]
        g0, ng = r0 // 8, nr // 8
        gt = jnp.concatenate([gate] * ((nr + 127) // 128), 1)[:, :nr]
        newrow = _rb(bs_v[:, r0:r0 + nr] + _rb(_rb(y_v[:, r0:r0 + nr]) * gt))
        tn = lambda oh: lax.dot_general(newrow, oh, (((0,), (0,)), ((), ())), preferred_element_type=f32)
        if fast:
            uu = tn(jnp.concatenate([onehot(0), onehot(1)], 1))
            for c in range(2):
                u_v[c, g0:g0 + ng] = uu[:, 128 * c:128 * (c + 1)].reshape(ng, 8, 128)
        else:
            for c in range(TOPC):
                u_v[c, g0:g0 + ng] = tn(onehot(c)).reshape(ng, 8, 128)

    def write(p, fast):
        g0, ng = POFF[p] // 8, PART[p] // 8
        for j in range(TOPC):
            idx = tile_idx(aux["late"][j], g0, ng)
            new = out_v[idx].astype(f32)
            code = lm_v[j]
            for c in range(2 if fast else TOPC):
                new = jnp.where(code == c, u_v[c, g0:g0 + ng], new)
            sg_v[j, g0:g0 + ng] = new.astype(bf16)
            cp(sg_v.at[j, pl.ds(g0, ng)], out_h.at[idx], osem.at[0]).start()

    NP = len(PART)
    for cc in c_w[1]:
        cc.wait()
    c_d[0].wait()
    run(gate_up(FCH[0], FCH[1]))
    down(0, 0, FCH[0])
    down(0, FCH[0], FCH[1])
    for p in range(1, NP - 1):
        c_d[p].wait()

    @pl.when(aux["ncls"] <= 2)
    def _():
        for p in range(1, NP):
            if p == NP - 1:
                c_d[p].wait()
            down(p, 0, DSPL[p])
            place(p - 1, True)
            down(p, DSPL[p], F - DSPL[p])
            write(p - 1, True)
        place(NP - 1, True)
        write(NP - 1, True)

    @pl.when(aux["ncls"] > 2)
    def _():
        c_d[NP - 1].wait()
        for p in range(1, NP):
            down(p, 0, F)
        for p in range(NP):
            place(p, False)
            write(p, False)

    cp(out_h, out_h, osem.at[0]).wait()


@jax.jit
def pallas_sequential_preLN__ssm_conv_s4__moe_arch_mod__prompt_kernel(
    A_u: jax.Array,
    A_A_re: jax.Array,
    A_A_im: jax.Array,
    A_B_re: jax.Array,
    A_B_im: jax.Array,
    A_C_re: jax.Array,
    A_C_im: jax.Array,
    A_log_dt: jax.Array,
    A_Dskip: jax.Array,
    B_x: jax.Array,
    B_w_r: jax.Array,
    B_w_gate: jax.Array,
    B_w_up: jax.Array,
    B_w_down: jax.Array,
):
    hbm = pl.BlockSpec(memory_space=pltpu.MemorySpace.HBM)
    vm = pltpu.VMEM
    G8 = D // 8
    wshape = (D // 16, F // 128, 16, 128)
    wview = lambda w: w.reshape(D // 16, 2, 8, F // 128, 128).transpose(0, 1, 3, 2, 4)
    scratch = [
        vm((G8, NB, 16, 128), bf16), vm((6, NSTEP, 128, N), bf16), vm((D,), bf16), vm((D,), bf16), vm((D,), bf16),
        vm((CT_ROWS, 128), f32), vm(wshape, bf16), vm(wshape, bf16), vm((D, F), bf16), vm((G8, NB + 1, 16, 128), bf16),
        vm((9, 4, 144, 128), bf16), vm((2, 2, 2, 144, 128), bf16), vm((3, NSTEP, 96, 128), f32),
        vm((NV, 2, 136, 128), f32), vm((NSTEP, 12, 56, 128), f32), vm((NSTEP, 96, 128), f32),
        vm((NSTEP, NB, 6, R, 128), f32), vm((NSTEP, NB, 6, R, 128), f32),
        vm((NSTEP, NB, 2, R, 256), f32), vm((NSTEP, 12, 136, 128), f32), vm((2, 17, 8, 128), f32),
        vm((3, 136, 128), f32), vm((5, 16, 128), f32), vm((TOPC, G8, 8, 128), f32),
        vm((R, 512), f32), vm((8, D), f32), vm((NV, 4, 8, 128), f32),
        vm((8, 128), f32), vm((8, D), f32), vm((8, D), f32), vm((8, F), f32),
        vm((TOPC, G8, 8, 128), bf16), vm((TOPC, 8, 128), i32), vm((8, D), f32), pltpu.SMEM((1,), i32),
        pltpu.SemaphoreType.DMA((6 + len(PART),)), pltpu.SemaphoreType.DMA((1,)),
    ]
    xv = A_u[0].T.reshape(G8, 8, 16, 128).transpose(0, 2, 1, 3).reshape(G8, NB, 16, 128)
    out = pl.pallas_call(
        _kernel,
        out_shape=jax.ShapeDtypeStruct((G8, NB, 16, 128), bf16),
        in_specs=[hbm] * 13,
        out_specs=hbm,
        scratch_shapes=scratch,
        compiler_params=pltpu.CompilerParams(vmem_limit_bytes=120 * 1024 * 1024, disable_bounds_checks=True,
                                             disable_semaphore_checks=True),
    )(xv, *[p.reshape(NSTEP, R, N) for p in (A_A_re, A_A_im, A_B_re, A_B_im, A_C_re, A_C_im)], A_log_dt, A_Dskip, B_w_r,
      wview(B_w_gate), wview(B_w_up), B_w_down.T)
    return out.reshape(G8, 16, 8, 128).transpose(0, 2, 1, 3).reshape(D, L).T[None]
```

```python
import functools

import numpy as np
import jax
import jax.numpy as jnp
from jax import lax
import jax.experimental.pallas as pl
import jax.experimental.pallas.tpu as pltpu

f32 = jnp.float32
bf16 = jnp.bfloat16
i32 = jnp.int32
u32 = jnp.uint32

L, D, N, F, TOPC = 2048, 576, 128, 4608, 8
NB = 8
NV = 9
R = NV * 8
NSTEP = D // R
EPS = 1e-5

_XL1 = [(1, 5), (2, 6), (3, 7), (4, 8), (258, 516), (260, 520), (262, 772), (264, 776),
        (1288, 1032), (1800, 1544)]
_XSH = [0, 1, 2, 3, 0, 1, 2, 3, 0, 1]


def _bf16_round_int(j):
    u = np.asarray(j, np.float32).view(np.uint32).astype(np.uint64)
    r = ((u + 0x7FFF + ((u >> 16) & 1)) >> 16) << 16
    return r.astype(np.uint32).view(np.float32).astype(np.int64)


def _chunk_values():
    vals = -np.ones((5, 128), np.int64)
    for j in range(10):
        for p in range(2):
            ch = (j // 4) * 2 + p if j < 8 else 4
            extra = 2 * p if j >= 8 else 0
            for l0 in range(32):
                vals[ch, (4 * (31 - l0) + 4 * p + _XSH[j] + extra + 8) % 128] = _XL1[j][p] + 8 * l0
    assert (vals >= 0).all()
    return vals


_PASSES = [(0, "A0"), (0, "A1"), (1, "B"), (2, "Cp"), (3, "C"), (4, "Dp"), (5, "D"), (6, "D"), (7, "D")]
_SETS = [[0], [1], [2], [3, 4], [5, 6, 7, 8]]


def _tables():
    cv = _chunk_values()
    cvp = {"A0": cv[0], "A1": cv[1], "B": cv[2], "C": cv[3], "D": cv[4]}
    cvp["Cp"] = cv[3].copy(); cvp["Cp"][11] = cv[2][11]
    cvp["Dp"] = cv[4].copy(); cvp["Dp"][15] = cv[3][15]
    sup = [[[] for _ in range(128)] for _ in _PASSES]
    for b in range(NB):
        for j in range(1, 257):
            lag = 256 * b + j
            if lag > L - 1 or lag == 257:
                continue
            v = int(_bf16_round_int(lag))
            hit = [(i, int(np.nonzero(cvp[nm] == v)[0][0])) for i, (pb, nm) in enumerate(_PASSES)
                   if pb == b and (cvp[nm] == v).any()]
            assert len(hit) == 1, (b, j, v, hit)
            sup[hit[0][0]][hit[0][1]].append(j)
    assert cv[1][15] == _bf16_round_int(257)
    code = np.zeros((len(_PASSES), 128), np.int64)
    for i, (pb, _) in enumerate(_PASSES):
        for r in range(128):
            js = sup[i][r]
            if js:
                assert js == list(range(js[0], js[-1] + 1))
                code[i, r] = js[0] + js[-1] + 1024 * len(js) + 16384 * (pb % 2)
    seeds, masks = [], {}
    for ps in _SETS:
        seeds.append([int(x) for x in sum(code[i, 16:24] for i in ps)])
        for i in ps:
            masks[i] = [int(x > 0) for x in code[i, 16:24]]
            for v in range(2, 17):
                r0 = 8 * (v % 16)
                assert (code[i, r0:r0 + 8] == (np.array(seeds[-1]) - 32 * (v - 2)) * np.array(masks[i])).all()
    return seeds, [[int(x) for x in code[i, 8:16]] for i in range(len(_PASSES))], masks


_GSEED, _GROW1, _GMASK = _tables()


def _sincos_coeffs():
    r = np.cos(np.pi * (np.arange(4000) + .5) / 4000) * 0.5
    z = r * r
    s = np.linalg.lstsq(np.stack([z ** k for k in range(4)], 1), np.sin(np.pi / 2 * r) / r, rcond=None)[0]
    c = np.linalg.lstsq(np.stack([z ** k for k in range(1, 5)], 1), np.cos(np.pi / 2 * r) - 1, rcond=None)[0]
    return [float(x) for x in s], [float(x) for x in c]


_SC, _CC = _sincos_coeffs()


def _cmul(a, b):
    return (a[0] * b[0] - a[1] * b[1], a[0] * b[1] + a[1] * b[0])


def _cmulc(a, b):
    return (a[0] * b[0] + a[1] * b[1], a[1] * b[0] - a[0] * b[1])


def _csq(a):
    return ((a[0] - a[1]) * (a[0] + a[1]), (a[0] + a[0]) * a[1])


def _quarter_polys(r):
    r2 = r * r
    s = r * (_SC[0] + r2 * (_SC[1] + r2 * (_SC[2] + r2 * _SC[3])))
    c = 1.0 + r2 * (_CC[0] + r2 * (_CC[1] + r2 * (_CC[2] + r2 * _CC[3])))
    return s, c


def _rotate_quadrant(s, c, ki):
    swap = (ki & 1) == 1
    s2 = jnp.where(swap, c, s)
    c2 = jnp.where(swap, s, c)
    s2 = pltpu.bitcast(pltpu.bitcast(s2, i32) ^ ((ki & 2) << 30), f32)
    c2 = pltpu.bitcast(pltpu.bitcast(c2, i32) ^ (((ki + 1) & 2) << 30), f32)
    return s2, c2


def _reduce(z):
    k = jnp.round(z)
    return _quarter_polys(z - k) + (k.astype(i32),)


def _sincos(th):
    return _rotate_quadrant(*_reduce(th * (2.0 / np.pi)))


def _rb(x):
    return x.astype(bf16).astype(f32)


def _dot(a, b):
    return jnp.dot(a, b, preferred_element_type=f32)


def _dot_nt(a, b):
    return lax.dot_general(a, b, (((1,), (1,)), ((), ())), preferred_element_type=f32)


def _iota(shape, dim):
    return lax.broadcasted_iota(i32, shape, dim)


ORDER, ORD0, ORD5, ORD6 = "4ab44342np445", "4ab442n4p4345", "4a424n44b345p", "45a4b244p3n44"
TILE = 4
LG = 3
NTOP = 4
FCH = (3456, 1152)
FSUB = 1152
PART = (256, 128, 128, 64)
POFF = [sum(PART[:i]) for i in range(len(PART))]
DSPL = (0, 2560, 2560, 4096)
CT_ROWS = 320


def _weave(*streams):
    items = []
    for si, (pieces, lo, hi) in enumerate(streams):
        tot = float(sum(c for _, c in pieces))
        cum = 0.0
        for pi, (fn, c) in enumerate(pieces):
            items.append((lo + max(hi - lo, 0.0) * (cum + 0.5 * c) / tot, si, pi, fn))
            cum += c
    for _, _, _, fn in sorted(items, key=lambda t: t[:3]):
        fn()


def _kernel(x_h, are_h, aim_h, bre_h, bim_h, cre_h, cim_h, ldt_h, dsk_h, wr_h, wg_h, wu_h, wd_h,
            out_h,
            x_v, par_v, ldt_v, dsk_v, wr_v, ct_v, wg_v, wu_v, wd_v, out_v,
            g_v, f_v, col_v, st_v, kd_v, k0_v, kh_v, uh_v, zs_v, c1_v, s1_v, acc_v, fin_v, u_v, zt_v,
            y_v, pv_v, kc_v, xs_v, bs_v, act_v, sg_v, lm_v, rw_v, flag_s,
            sem, osem):
    cp = pltpu.make_async_copy
    c_vec = [cp(ldt_h, ldt_v, sem.at[0]), cp(dsk_h, dsk_v, sem.at[0]), cp(wr_h, wr_v, sem.at[0])]
    PH = 4
    par_h = (are_h, aim_h, bre_h, bim_h, cre_h, cim_h)
    c_par = [cp(h.at[pl.ds(0, PH)], par_v.at[i, pl.ds(0, PH), pl.ds(0, R)], sem.at[1])
             for i, h in enumerate(par_h)]
    c_par2 = [cp(h.at[pl.ds(PH, NSTEP - PH)], par_v.at[i, pl.ds(PH, NSTEP - PH), pl.ds(0, R)], sem.at[2])
              for i, h in enumerate(par_h)]
    c_x = cp(x_h, x_v, sem.at[3])

    def wcp(h, v, c):
        ct = pl.ds(sum(FCH[:c]) // 128, FCH[c] // 128)
        return [cp(h.at[:, hf, ct], v.at[:, ct, pl.ds(8 * hf, 8), :], sem.at[4 + c]) for hf in range(2)]

    c_w = [wcp(wg_h, wg_v, c) + wcp(wu_h, wu_v, c) for c in range(2)]
    c_d = [cp(wd_h.at[pl.ds(POFF[p], PART[p])], wd_v.at[pl.ds(POFF[p], PART[p])], sem.at[6 + p])
           for p in range(len(PART))]
    for c in c_vec + c_par + [c_x] + c_par2 + sum(c_w, []) + c_d:
        c.start()

    flag_s[0] = 1
    x_w = x_v.bitcast(u32)
    wg_w, wu_w = wg_v.bitcast(u32), wu_v.bitcast(u32)

    def wmat(w, c0, nc):
        return jnp.concatenate([pltpu.bitcast(w[:, t], bf16).reshape(D, 128)
                                for t in range(c0 // 128, (c0 + nc) // 128)], 1)

    out_w = out_v.bitcast(u32)
    g_w = g_v.bitcast(u32)
    f_w = f_v.bitcast(u32)
    sub8 = _iota((8, 128), 0)
    lane8 = _iota((8, 128), 1)

    acc_v[...] = jnp.zeros(acc_v.shape, f32)
    for ri in range(2):
        st_v[:, ri, 104:112, :] = jnp.full((NV, 8, 128), 1.0 - ri, f32)
    kp = (2 * lane8 + 1).astype(f32)

    def rows_const(vals):
        out = jnp.full((8, 128), vals[0], i32)
        for r in range(1, 8):
            if vals[r] != vals[0]:
                out = jnp.where(sub8 == r, vals[r], out)
        return out

    def phasor(z):
        sn, cs = _rotate_quadrant(*_reduce(-z))
        return cs, sn

    NS = [0, 1, 2, 3, 4, 5, 7, 9]
    for q in range(2):
        sn = _rotate_quadrant(*_reduce((kp + 512.0 * q) * (rows_const(NS).astype(f32) * (1.0 / 512))))[0]
        ct_v[304 + 8 * q:312 + 8 * q, :] = sn / (256.0 * jnp.broadcast_to(sn[1:2], (8, 128)))

    def grows(vals):
        ab = rows_const([v & 1023 for v in vals])
        z = kp * (ab.astype(f32) * (-1.0 / 512))
        if any(v >> 14 for v in vals):
            z = z - rows_const([v >> 14 for v in vals]).astype(f32) * (kp - 1.0)
        sn, cs, ki = _reduce(z)
        ns = [NS.index((v >> 10) & 15) for v in vals]
        out = []
        for q in range(2):
            row = lambda i: jnp.broadcast_to(ct_v[304 + 8 * q + i:305 + 8 * q + i, :], (8, 128))
            amp = None
            for i in sorted(set(ns)):
                bits = sum(1 << r for r in range(8) if ns[r] == i)
                amp = row(i) if amp is None else jnp.where(((bits >> sub8) & 1) == 1, row(i), amp)
            pi, pr = _rotate_quadrant(sn, cs, ki if q == 0 else ki - ab)
            out += [pr * amp, pi * amp]
        return out

    for v4 in range(4):
        e = phasor(kp * ((sub8 + 8 * v4).astype(f32) * (1.0 / 32)))
        ct_v[8 * v4:8 * v4 + 8, :] = e[0]
        ct_v[32 + 8 * v4:40 + 8 * v4, :] = e[1]
    for si in range(5):
        for q, val in enumerate(grows(_GSEED[si])):
            ct_v[64 + 32 * si + 8 * q:72 + 32 * si + 8 * q, :] = val
    for i in range(len(_PASSES)):
        for q, val in enumerate(grows(_GROW1[i])):
            g_v[i, q, 8:16, :] = val.astype(bf16)
    for q, val in enumerate(grows([2 + 1024 + 16384] * 8)):
        ct_v[272 + 8 * q:280 + 8 * q, :] = val
    s8 = np.arange(8)
    je = np.where(s8 % 2 == 0, s8, 127 + s8)
    jo = np.where(s8 % 2 == 0, s8 - 1, 128 + s8)
    for t, jj in enumerate((je, jo, jo % 128 + 128 * (s8 % 2))):
        e = phasor(kp * (rows_const([int(x) for x in jj]).astype(f32) * (1.0 / 256)))
        ct_v[224 + 16 * t:232 + 16 * t, :] = e[0]
        ct_v[232 + 16 * t:240 + 16 * t, :] = e[1]
    for c in c_vec:
        c.wait()

    rows = [_rb(jnp.exp(ldt_v[...].astype(f32).reshape(1, D))),
            dsk_v[...].astype(f32).reshape(1, D),
            wr_v[...].astype(f32).reshape(1, D)]
    wr_sum = jnp.sum(rows[2], axis=1, keepdims=True)

    def columns(which):
        for j in range(5):
            w = 128 if j < 4 else 64
            eye = _iota((w, w), 0) == _iota((w, w), 1)
            m = jnp.concatenate([jnp.where(eye, jnp.broadcast_to(rw_v[i:i + 1, j * 128:j * 128 + w], (w, w)), 0.0)
                                 for i in which], 0)
            res = _dot(m, jnp.ones((w, 128), f32))
            for n, i in enumerate(which):
                for g in range(w // 8):
                    k, m8 = divmod(16 * j + g, NV)
                    col_v[i, k, 8 * m8:8 * m8 + 8, :] = res[n * w + 8 * g:n * w + 8 * g + 8]

    for i in range(3):
        rw_v[i:i + 1, :] = rows[i]
    columns((0,))

    def e8(v):
        return (jnp.broadcast_to(ct_v[v:v + 1, :], (8, 128)), jnp.broadcast_to(ct_v[32 + v:33 + v, :], (8, 128)))

    for si, ps in enumerate(_SETS):
        sd = [ct_v[64 + 32 * si + 8 * q:72 + 32 * si + 8 * q, :] for q in range(4)]
        mk = {}
        for i in ps:
            if len(ps) > 1:
                bits = sum(b << s for s, b in enumerate(_GMASK[i]))
                mk[i] = ((bits >> sub8) & 1) == 1
        for v in range(2, 17):
            if v == 2:
                vals = sd
            else:
                ev = e8(2 * (v - 2))
                vals = list(_cmulc((sd[0], sd[1]), ev)) + list(_cmulc((sd[2], sd[3]), ev))
            vals = jnp.stack(vals, 0)
            for i in ps:
                val = vals if len(ps) == 1 else jnp.where(mk[i], vals, 0.0)
                g_v[i, :, 8 * (v % 16):8 * (v % 16) + 8, :] = val.astype(bf16)
    sig = jnp.where((lane8 & 1) == 0, 1.0, -1.0).astype(f32)
    for h in range(2):
        sd = (ct_v[224 + 16 * h:232 + 16 * h, :], ct_v[232 + 16 * h:240 + 16 * h, :])
        for v in range(16):
            if v == 0:
                vals = sd if h == 0 else (ct_v[256:264, :], ct_v[264:272, :])
            else:
                vals = _cmul(sd, e8(v))
            for q in range(2):
                f_v[0, h, q, 8 * v:8 * v + 8, :] = vals[q].astype(bf16)
                f_v[1, h, q, 8 * v:8 * v + 8, :] = (vals[q] * sig).astype(bf16)

    def gmat(i):
        return jnp.concatenate([pltpu.bitcast(g_w[i, q, 0:64, :], bf16) for q in range(4)], 1)

    def fmat(ver, h):
        return jnp.concatenate([pltpu.bitcast(f_w[ver, h, q, 0:64, :], bf16) for q in range(2)], 1)

    revmask = (sub8 & 2) == 0
    lm = lane8 & 3

    def s1_nat(k, n0, nn):
        rr = 8 * nn
        ld = lambda i: par_v[i, k, 8 * n0:8 * n0 + rr, :].astype(f32)
        dt = col_v[0, k, 8 * n0:8 * n0 + rr, :]
        e = jnp.exp(dt * ld(0))
        s, c = _sincos(dt * ld(1))
        a1 = (e * c, e * s)
        w = _cmul((ld(4), ld(5)), (dt * ld(2), dt * ld(3)))
        k0_v[k, 8 * n0:8 * n0 + rr, :] = jnp.broadcast_to(jnp.sum(w[0], axis=1, keepdims=True), (rr, 128))
        w = (w[0], -w[1])
        rev = lambda v: jnp.where(revmask, pltpu.roll(v, 2, 2), pltpu.roll(v, 6, 2))

        def put(arr, slots, fn=None):
            v = jnp.stack([a.reshape(nn, 8, 128) for a in arr], 1)
            if fn is not None:
                v = fn(v)
            for q in slots:
                st_v[n0:n0 + nn, :, q * 8:q * 8 + 8, :] = v

        put(w, (0, 1)); put(a1, (2, 3))
        a2 = _csq(a1); put(a2, (5,))
        a4 = _csq(a2); put(a4, (6,))
        put(_cmul(a4, a1), (4,))
        a8 = _csq(a4); put(a8, (12,), rev)
        t = _csq(a8); put(t, (14, 15), rev)
        for _ in range(4):
            t = _csq(t)
        put(t, (7, 11))
        t = _csq(t); put(t, (8, 9))
        put(_csq(t), (10,))

    def s1_grp(k, n):
        def mix(q):
            gs = [st_v[n, :, pl.ds(q * 8 + g, 8, stride=2), :] for g in range(2)]
            return tuple(jnp.concatenate([gs[0][ri], gs[1][ri]], 0) for ri in range(2))

        y = [mix(12)]
        a16d = mix(14)
        for _ in range(15):
            y.append(_cmul(y[-1], a16d))
        yield
        wd = mix(0); a1d = mix(2); m1 = mix(5)
        v = [_cmulc(wd, mix(3))]
        for _ in range(3):
            v.append(_cmulc(v[-1], a1d))
        v4 = _cmulc(_cmulc(wd, m1), mix(7))
        v5 = _cmulc(v4, m1); v6 = _cmulc(v4, mix(6)); v7 = _cmulc(v6, m1)
        v8 = _cmulc(v7, mix(10)); v9 = _cmulc(v8, mix(8))
        v += [v4, v5, v6, v7, v8, v9]
        os_ = []
        for g in range(2):
            cat = lambda ts: jnp.concatenate([jnp.concatenate([t[ri][8 * g:8 * g + 8] for t in ts], 0)
                                              for ri in range(2)], 1)
            os_.append(_dot_nt(cat(v), cat(y[::-1])))
        yield
        for g in range(2):
            o = os_[g]
            ro = [pltpu.roll(o[8 * j:8 * j + 8], _XSH[j] + 5, 1, stride=1, stride_axis=0) for j in range(10)]
            sel4 = lambda q: jnp.where(lm == 0, q[0], jnp.where(lm == 1, q[1], jnp.where(lm == 2, q[2], q[3])))
            kd_v[k, n, pl.ds(g, 8, stride=2), :] = sel4(ro[0:4])
            kd_v[k, n, pl.ds(16 + g, 8, stride=2), :] = sel4(ro[4:8])
            kd_v[k, n, pl.ds(32 + g, 8, stride=2), :] = jnp.where(lm == 0, ro[8], ro[9])

    def run(gen):
        for _ in gen:
            pass

    s1n = lambda k: [(functools.partial(s1_nat, k, 3 * i, 3), 1.0) for i in range(3)]
    s1g = lambda k: [(lambda n=n: run(s1_grp(k, n)), 1.0) for n in range(NV)]

    laneR = _iota((R, 128), 1)
    lmR = laneR & 3

    def s2_gen(k):
        ch = lambda c: kd_v[k, 0:NV, 8 * c:8 * c + 8, :].reshape(R, 128)
        for b in range(NB):
            if b == 0:
                k0 = (k0_v[k, 0:R, :] + col_v[1, k, 0:R, :]) * (1.0 / 256.0)
                z = _dot(ch(0), gmat(0))
                dd = jnp.where(lmR < 2, ch(4), pltpu.roll(ch(5), 2, 1))
                kd_v[k, 0:NV, 48:56, :] = dd.reshape(NV, 8, 128)
                zt_v[...] = z
                yield
                z = _dot(ch(1), gmat(1)) + zt_v[...]
            elif b == 1:
                k256 = jnp.sum(jnp.where(laneR == 15, ch(1), 0.0), axis=1, keepdims=True)
                pat = jnp.concatenate([ct_v[272 + 8 * q:273 + 8 * q, :] for q in range(4)], 1)
                z = _dot(ch(2), gmat(2)) + k256 * pat
            elif b == 2:
                z = _dot(jnp.where(laneR == 11, ch(2), ch(3)), gmat(3))
            elif b == 3:
                z = _dot(ch(3), gmat(4))
            elif b == 4:
                z = _dot(jnp.where(laneR == 15, ch(3), ch(6)), gmat(5))
            else:
                z = _dot(ch(6), gmat(b + 1))
            for s in range(2):
                kr = z[:, 256 * s:256 * s + 128]
                ki = z[:, 256 * s + 128:256 * s + 256]
                if b == 0:
                    kr = kr + k0
                kh_v[k, b, 3 * s] = kr
                kh_v[k, b, 3 * s + 1] = ki
            yield

    def s2(k):
        gen = s2_gen(k)
        return [(lambda: next(gen, None), 1.0) for _ in range(9)]

    mask2 = (sub8 < 4) == ((lane8 & 1) == 0)
    top = sub8 < 4

    def ln1_pieces(b, npc):
        state = {}
        per = (D // 8) // npc

        def piece(i):
            for g in range(i * per, (i + 1) * per, LG):
                m = x_w[g:g + LG, b]
                eo = jnp.where(mask2, m, pltpu.roll(pltpu.roll(m, 4, 1), 1, 2))
                a = pltpu.bitcast(eo << 16, f32)
                c = pltpu.bitcast(eo & jnp.uint32(0xFFFF0000), f32)
                if g == 0:
                    state["sh"] = jnp.where(top, jnp.broadcast_to(a[0, 0:1], (8, 128)),
                                            jnp.broadcast_to(a[0, 4:5], (8, 128)))
                a = a - state["sh"]
                c = c - state["sh"]
                c1_v[g // NV, g % NV:g % NV + LG, pl.ds(16 * b, 8, stride=2), :] = a
                c1_v[g // NV, g % NV:g % NV + LG, pl.ds(16 * b + 1, 8, stride=2), :] = c
                for q in range(LG):
                    new = [a[q], c[q], a[q] * a[q], c[q] * c[q]]
                    state["acc"] = new if g + q == 0 else [p + r for p, r in zip(state["acc"], new)]
            if i == npc - 1:
                acc = state["acc"]
                s1, s2_ = acc[0] + acc[1], acc[2] + acc[3]
                for h in range(2):
                    m = jnp.sum(s1[4 * h:4 * h + 4], axis=0, keepdims=True) * (1.0 / D)
                    var = jnp.sum(s2_[4 * h:4 * h + 4], axis=0, keepdims=True) * (1.0 / D) - m * m
                    rs = 1.0 / _rb(jnp.sqrt(_rb(_rb(jnp.maximum(var, 0.0)) + EPS)))
                    s1_v[0, 2 * b + h] = jnp.broadcast_to(rs, (8, 128))
                    sh = state["sh"][4 * h:4 * h + 1]
                    s1_v[1, 2 * b + h] = jnp.broadcast_to((_rb(m + sh) - sh) * rs, (8, 128))
                    fin_v[4, 2 * b + h:2 * b + h + 1, :] = state["sh"][4 * h:4 * h + 1]

        return [(functools.partial(piece, i), 1.0) for i in range(npc)]

    def s3_blk(k, b):
        et = []
        for h in range(2):
            c = c1_v[k, 0:NV, 16 * b + 8 * h:16 * b + 8 * h + 8, :]
            u = (c * s1_v[0, 2 * b + h] - s1_v[1, 2 * b + h]).reshape(R, 128)
            et.append(_dot(u, fmat(b % 2, h)))
        er, ei, tr, ti = et[0][:, :128], et[0][:, 128:], et[1][:, :128], et[1][:, 128:]
        for q, v in enumerate((er, ei, tr, ti)):
            uh_v[k, b, q] = v

    s3 = lambda k: [(functools.partial(s3_blk, k, b), 1.0) for b in range(NB)]

    def s4_gen(k, n, groups=None):
        sl = slice(8 * n, 8 * n + 8)

        def utrip(i, s):
            et = uh_v[k, i, 0:4, sl, :]
            er, ei, tr, ti = et[0], et[1], et[2], et[3]
            pr, pi = (er + tr, ei + ti) if s == 0 else (er - tr, ei - ti)
            return [pr + pi, pi, pr]

        prev = None
        done = 0
        if groups is not None and groups[0] > 0:
            prev = [(pv_v[n, 2 * h], pv_v[n, 2 * h + 1]) for h in range(2)]
        for b0 in (range(0, NB, TILE) if groups is None else groups):
            yy = []
            for s in range(2):
                acc = [None] * TILE
                win = {}
                for j in range(b0 + TILE):
                    kri = kh_v[k, j, 3 * s:3 * s + 2, sl, :]
                    kk = [kri[0], kri[0] + kri[1], kri[1] - kri[0]]
                    for o in range(TILE - 1, -1, -1):
                        i = b0 + o - j
                        if i < 0:
                            continue
                        if i not in win:
                            win[i] = utrip(i, s)
                        p = [kk[q] * win[i][q] for q in range(3)]
                        acc[o] = p if acc[o] is None else [a + c for a, c in zip(acc[o], p)]
                        done += 1
                    if b0 == 4 and j == 2:
                        yield done
                yy.append([(a[0] - a[1], a[0] + a[2]) for a in acc])
                if s == 0:
                    yield done
            for o in range(TILE):
                p, q = yy[0][o], yy[1][o]
                cur = [(p[0] + q[0], p[1] + q[1]), (p[0] - q[0], p[1] - q[1])]
                for h in range(2):
                    if b0 + o == 0:
                        zr, zi = cur[h]
                    else:
                        zr = cur[h][0] - prev[h][1]
                        zi = cur[h][1] + prev[h][0]
                    zs_v[k, b0 + o, h, sl, :] = jnp.concatenate([zr, zi], 1)
                prev = cur
            if groups is not None and b0 + TILE < NB:
                for h in range(2):
                    pv_v[n, 2 * h] = prev[h][0]
                    pv_v[n, 2 * h + 1] = prev[h][1]
            yield done

    def s5_blk(k, b, h):
        t = 2 * b + h
        y = _dot_nt(zs_v[k, b, h], fmat(b % 2, h)).reshape(NV, 8, 128)
        hh = c1_v[k, 0:NV, 16 * b + 8 * h:16 * b + 8 * h + 8, :] + y
        c1_v[k, 0:NV, 16 * b + 8 * h:16 * b + 8 * h + 8, :] = hh
        wr = col_v[2, k, 0:R, :].reshape(NV, 8, 128)
        rs = slice(8 * t, 8 * t + 8)
        acc_v[0, rs, :] = acc_v[0, rs, :] + jnp.sum(hh, axis=0)
        acc_v[1, rs, :] = acc_v[1, rs, :] + jnp.sum(hh * hh, axis=0)
        acc_v[2, rs, :] = acc_v[2, rs, :] + jnp.sum(hh * wr, axis=0)

    s5 = lambda k: [(functools.partial(s5_blk, k, b, h), 1.0) for b in range(NB) for h in range(2)]

    for c in c_par:
        c.wait()
    columns((1, 2))
    for k in range(2):
        _weave((s1n(k), 0.0, 0.2), (s1g(k), 0.2, 1.0))
    _weave((s1n(2), 0.0, 0.2), (s1g(2), 0.2, 1.0), (s2(0), 0.3, 1.0))
    s1_nat(3, 0, 1)
    c_x.wait()
    ln = [ln1_pieces(b, 3) for b in range(NB)]
    s30 = s3(0)
    _weave((sum(ln, []), 0.0, 0.9), (s2(1), 0.0, 0.55),
           *[([s30[b]], max((b + 1.6) * 0.9 / NB, 0.3 + 0.7 * b / NB), 0.0) for b in range(NB)])
    for c in c_par2:
        c.wait()

    def body(k, do5=True, do4=True, do3=True, do2=True, do1=True, j=None, order=None):
        order = order or ORDER
        at = (lambda d: k + d) if j is None else (lambda d: j + (k + d) if k + d else j)
        g2 = s2_gen(at(2)) if do2 else None
        for n in range(NV):
            g4 = s4_gen(at(0), n) if do4 else None
            st4 = [0, 0]
            n4 = order.count("4")

            def adv4(m):
                if not do4:
                    return
                st4[0] += 1
                while st4[1] < 72 * st4[0] / n4 - 3 or (st4[0] == n4 and st4[1] <= 72):
                    r = next(g4, None)
                    if r is None:
                        break
                    st4[1] = r

            def nat():
                if do1:
                    if n + 1 < NV:
                        s1_nat(at(3), n + 1, 1)
                    else:
                        s1_nat(jnp.minimum(at(4), NSTEP - 1), 0, 1)

            g1 = s1_grp(at(3), n) if do1 else None
            for tok in order:
                if tok == "5":
                    if do5 and n < NB:
                        s5_blk(at(-1), n, 0)
                        s5_blk(at(-1), n, 1)
                elif tok == "4":
                    adv4(1)
                elif tok in "ab" and do1:
                    next(g1)
                elif tok == "p" and do1:
                    run(g1)
                elif tok == "2" and do2:
                    next(g2, None)
                elif tok == "3" and do3 and n < NB:
                    s3_blk(at(1), n)
                elif tok == "n":
                    nat()
        if do2:
            run(g2)

    @pl.when(flag_s[0] == 1)
    def _():
        body(0, do5=False, order=ORD0)

    lax.fori_loop(0, 4, lambda j, c: (body(1, j=j), c)[1], 0)

    @pl.when(flag_s[0] == 1)
    def _():
        body(5, do1=False, order=ORD5)

    @pl.when(flag_s[0] == 1)
    def _():
        body(6, do1=False, do2=False, order=ORD6)

    @pl.when(flag_s[0] == 1)
    def _():
        _weave(([(lambda n=n: run(s4_gen(7, n, (0,))), 1.0) for n in range(NV)], 0.0, 1.0), (s5(6), 0.0, 1.0))

    @pl.when(flag_s[0] == 1)
    def _():
        _weave(([(lambda n=n: run(s4_gen(7, n, (4,))), 1.0) for n in range(NV)], 0.0, 1.0), (s5(7)[:8], 0.0, 1.0))

    _weave((s5(7)[8:], 0.0, 1.0))

    def total(i):
        halves = []
        for hf in range(2):
            t = acc_v[i, pl.ds(64 * hf, 8, stride=8), :]
            for s in range(1, 8):
                t = t + acc_v[i, pl.ds(64 * hf + s, 8, stride=8), :]
            halves.append(t)
        return jnp.concatenate(halves, 0)

    m2 = total(0) * (1.0 / D)
    var2 = jnp.maximum(total(1) * (1.0 / D) - m2 * m2, 0.0)
    sd2 = _rb(jnp.sqrt(_rb(_rb(var2) + EPS)))
    rs2 = 1.0 / sd2
    mean2 = _rb(fin_v[4] + m2)
    m2 = mean2 - fin_v[4]
    r = _rb((total(2) - m2 * wr_sum) * rs2)
    fin_v[0] = rs2
    fin_v[1] = m2 * rs2
    fin_v[2] = rs2 + 1.0
    fin_v[3] = fin_v[4] - m2 * rs2

    def outp(b, g0, g1):
        sc = [jnp.where(top, jnp.broadcast_to(fin_v[i, 2 * b:2 * b + 1, :], (8, 128)),
                        jnp.broadcast_to(fin_v[i, 2 * b + 1:2 * b + 2, :], (8, 128))) for i in (2, 3)]
        for g in range(g0, g1, LG):
            src = lambda o: c1_v[g // NV, g % NV:g % NV + LG, pl.ds(16 * b + o, 8, stride=2), :]
            a = _rb(src(0) * sc[0] + sc[1])
            c = _rb(src(1) * sc[0] + sc[1])
            w = (pltpu.bitcast(a, u32) >> 16) | pltpu.bitcast(c, u32)
            out_w[g:g + LG, b] = jnp.where(mask2, w, pltpu.roll(pltpu.roll(w, 4, 1), 127, 2))

    opieces = [functools.partial(outp, b, 24 * i, 24 * i + 24) for b in range(NB) for i in range(3)]

    tl = _iota((16, 128), 0)
    ll = _iota((16, 128), 1)
    lodd = (ll & 1) == 1
    toff = jnp.where((tl & 1) == 0, jnp.where(lodd, ll + 127, ll), jnp.where(lodd, ll + 128, (ll - 1) & 127))
    tok = (tl >> 1) * 256 + toff
    rbits = pltpu.bitcast(r, i32)
    srt = rbits ^ ((rbits >> 31) & 0x7FFFFFFF)
    key = pltpu.bitcast((((srt >> 16) + 32768) << 11) + (2047 - tok) + (1 << 28), f32)
    kk = key
    cand = []
    for _ in range(4):
        rm = jnp.broadcast_to(jnp.max(kk, axis=1, keepdims=True), (16, 128))
        cand.append(rm)
        kk = jnp.where(kk == rm, 0.0, kk)
        for fn in opieces[(len(cand) - 1) * NTOP // 4:len(cand) * NTOP // 4]:
            fn()
    last = jnp.max(cand[3], axis=0, keepdims=True)
    kcol = None
    for j in range(TOPC):
        mx = jnp.max(cand[0], axis=0, keepdims=True)
        kcol = jnp.broadcast_to(mx, (8, 128)) if j == 0 else jnp.where(sub8 == j, mx, kcol)
        took = cand[0] == mx
        cand = [jnp.where(took, cand[i + 1] if i < 3 else 0.0, cand[i]) for i in range(4)]
    kc_v[...] = kcol

    @pl.when((last - mx)[0, 0] > 0.0)
    def _():
        k2 = key
        kc = None
        for j in range(TOPC):
            m1 = jnp.max(jnp.max(k2, axis=0, keepdims=True), axis=1, keepdims=True)
            kc = jnp.broadcast_to(m1, (8, 128)) if j == 0 else jnp.where(sub8 == j, m1, kc)
            k2 = jnp.where(k2 == m1, 0.0, k2)
        kc_v[...] = kc

    kcol = kc_v[...]
    kint = pltpu.bitcast(kcol, i32) - (1 << 28)
    tcol = 2047 - (kint & 2047)
    s16 = (kint >> 11) - 32768
    rsel = pltpu.bitcast((s16 ^ ((s16 >> 31) & 0x7FFF)) << 16, f32)
    gate = _rb(jax.nn.sigmoid(rsel))

    def classes(col):
        cls = jnp.zeros((8, 128), i32)
        for d in range(1, TOPC):
            cls = cls + jnp.where((col == pltpu.roll(col, d, 0)) & (sub8 >= d), 1, 0)
        return cls, jnp.max(cls, axis=0, keepdims=True)[0, 0] + 1

    wcol = tcol & 255
    pcol = jnp.where((wcol & 1) == 0, jnp.where(wcol < 128, wcol, wcol - 127),
                     jnp.where(wcol < 128, (wcol + 1) & 127, wcol - 128))
    ecol = ((tcol >> 8) << 1) | (tcol & 1)
    etile = [jnp.clip(ecol[j, 0], 0, 15) for j in range(TOPC)]
    gcol, gn = classes(pcol)
    xs_v[...] = jnp.zeros((8, D), f32)

    def gather(c, carry):
        oh = (gcol == c) & (lane8 == pcol)
        ohi = jnp.where(oh, 1, 0)
        msk = [jnp.broadcast_to(ohi[j:j + 1], (8, 128)) == 1 for j in range(TOPC)]
        sa = sb = None
        for j in range(TOPC):
            fa = jnp.broadcast_to(fin_v[0, pl.ds(etile[j], 1), :], (8, 128))
            fb = jnp.broadcast_to(fin_v[1, pl.ds(etile[j], 1), :], (8, 128))
            sa, sb = (fa, fb) if j == 0 else (jnp.where(msk[j], fa, sa), jnp.where(msk[j], fb, sb))
        parts = []
        for q in range(D // 8 // LG):
            mg = None
            for j in range(TOPC):
                cc = c1_v[LG * q // NV, LG * q % NV:LG * q % NV + LG, pl.ds(pl.multiple_of(8 * etile[j], 8), 8), :]
                mg = cc if j == 0 else jnp.where(msk[j], cc, mg)
            parts.append(mg * sa - sb)
        ln = jnp.concatenate(parts, 0).reshape(D, 128)
        xs_v[...] = xs_v[...] + _dot_nt(jnp.where(oh, 1.0, 0.0).astype(f32), ln)
        return carry

    lax.fori_loop(0, gn, gather, 0)
    xsel = xs_v[...]

    def rebuilt_rows():
        sdc = jnp.zeros((8, 1), f32)
        mc = jnp.zeros((8, 1), f32)
        sub1 = _iota((8, 1), 0)
        for j in range(TOPC):
            hitm = tok == jnp.broadcast_to(tcol[j:j + 1], (16, 128))
            red = lambda v: jnp.sum(jnp.sum(jnp.where(hitm, v, 0.0), axis=0, keepdims=True), axis=1, keepdims=True)
            sdc = jnp.where(sub1 == j, red(sd2), sdc)
            mc = jnp.where(sub1 == j, red(mean2), mc)
        return xsel * (sdc + 1.0) + mc

    tilec = tcol >> 7
    lanec = tcol & 127
    aux = {}

    def late_scalars():
        tiles = [jnp.clip(tilec[j, 0], 0, 15) for j in range(TOPC)]
        hit = 0
        dup = []
        for j in range(TOPC):
            dup.append((hit >> tiles[j]) & 1)
            hit = hit | (1 << tiles[j])
        free, cnt = [], 0
        for t in range(16):
            un = 1 - ((hit >> t) & 1)
            free.append(jnp.where(un == 1, cnt, -1))
            cnt = cnt + un
        late, nd, mask = [tiles[0]], 0, hit
        for j in range(1, TOPC):
            rep = 0
            for t in range(16):
                rep = jnp.where(free[t] == nd, t, rep)
            late.append(jnp.clip(jnp.where(dup[j] == 1, rep, tiles[j]), 0, 15))
            mask = mask | (1 << late[j])
            nd = nd + dup[j]
        aux.update(late=late, mask=mask)
        bs_v[...] = rebuilt_rows()
        aux["clscol"], aux["ncls"] = classes(lanec)
        for j in range(TOPC):
            code = jnp.where((tilec == late[j]) & (lane8 == lanec), aux["clscol"], -1)
            lm_v[j] = jnp.broadcast_to(jnp.max(code, axis=0, keepdims=True), (8, 128))

    def tile_idx(t, g0=0, ng=D // 8):
        if isinstance(t, int):
            return (pl.ds(g0, ng), t // 2, pl.ds(8 * (t % 2), 8), slice(None))
        return (pl.ds(g0, ng), t >> 1, pl.ds(pl.multiple_of(8 * (t & 1), 8), 8), slice(None))

    def ocopy(idx):
        return cp(out_v.at[idx], out_h.at[idx], osem.at[0])

    def early():
        for t in range(16):
            @pl.when(((aux["mask"] >> t) & 1) == 0)
            def _():
                ocopy(tile_idx(t)).start()

    def gate_up(c0, nc):
        g = _rb(_dot(xsel, wmat(wg_w, c0, nc)))
        up = _rb(_dot(xsel, wmat(wu_w, c0, nc)))
        yield
        act_v[:, c0:c0 + nc] = _rb(_rb(g * jax.nn.sigmoid(g)) * up)

    for cc in c_w[0]:
        cc.wait()
    mine = opieces[NTOP:]
    nsub = FCH[0] // FSUB
    for u in range(nsub):
        gu = gate_up(u * FSUB, FSUB)
        next(gu)
        if u == 0:
            late_scalars()
        for fn in mine[u * len(mine) // nsub:(u + 1) * len(mine) // nsub]:
            fn()
        run(gu)
    early()

    clscol = aux["clscol"]
    onehot = lambda c: jnp.where((clscol == c) & (lane8 == lanec), 1.0, 0.0).astype(f32)

    def down(p, c0, nc):
        r = slice(POFF[p], POFF[p] + PART[p])
        yc = _dot_nt(act_v[:, c0:c0 + nc], wd_v[r, c0:c0 + nc])
        y_v[:, r] = yc if c0 == 0 else y_v[:, r] + yc

    def place(p, fast):
        r0, nr = POFF[p], PART[p]
        g0, ng = r0 // 8, nr // 8
        gt = jnp.concatenate([gate] * ((nr + 127) // 128), 1)[:, :nr]
        newrow = _rb(bs_v[:, r0:r0 + nr] + _rb(_rb(y_v[:, r0:r0 + nr]) * gt))
        tn = lambda oh: lax.dot_general(newrow, oh, (((0,), (0,)), ((), ())), preferred_element_type=f32)
        if fast:
            uu = tn(jnp.concatenate([onehot(0), onehot(1)], 1))
            for c in range(2):
                u_v[c, g0:g0 + ng] = uu[:, 128 * c:128 * (c + 1)].reshape(ng, 8, 128)
        else:
            for c in range(TOPC):
                u_v[c, g0:g0 + ng] = tn(onehot(c)).reshape(ng, 8, 128)

    def write(p, fast):
        g0, ng = POFF[p] // 8, PART[p] // 8
        for j in range(TOPC):
            idx = tile_idx(aux["late"][j], g0, ng)
            new = out_v[idx].astype(f32)
            code = lm_v[j]
            for c in range(2 if fast else TOPC):
                new = jnp.where(code == c, u_v[c, g0:g0 + ng], new)
            sg_v[j, g0:g0 + ng] = new.astype(bf16)
            cp(sg_v.at[j, pl.ds(g0, ng)], out_h.at[idx], osem.at[0]).start()

    NP = len(PART)
    for cc in c_w[1]:
        cc.wait()
    c_d[0].wait()
    run(gate_up(FCH[0], FCH[1]))
    down(0, 0, FCH[0])
    down(0, FCH[0], FCH[1])
    for p in range(1, NP - 1):
        c_d[p].wait()

    @pl.when(aux["ncls"] <= 2)
    def _():
        for p in range(1, NP):
            if p == NP - 1:
                c_d[p].wait()
            down(p, 0, DSPL[p])
            place(p - 1, True)
            down(p, DSPL[p], F - DSPL[p])
            write(p - 1, True)
        place(NP - 1, True)
        write(NP - 1, True)

    @pl.when(aux["ncls"] > 2)
    def _():
        c_d[NP - 1].wait()
        for p in range(1, NP):
            down(p, 0, F)
        for p in range(NP):
            place(p, False)
            write(p, False)

    cp(out_h, out_h, osem.at[0]).wait()


@jax.jit
def pallas_sequential_preLN__ssm_conv_s4__moe_arch_mod__prompt_kernel(
    A_u: jax.Array,
    A_A_re: jax.Array,
    A_A_im: jax.Array,
    A_B_re: jax.Array,
    A_B_im: jax.Array,
    A_C_re: jax.Array,
    A_C_im: jax.Array,
    A_log_dt: jax.Array,
    A_Dskip: jax.Array,
    B_x: jax.Array,
    B_w_r: jax.Array,
    B_w_gate: jax.Array,
    B_w_up: jax.Array,
    B_w_down: jax.Array,
):
    hbm = pl.BlockSpec(memory_space=pltpu.MemorySpace.HBM)
    vm = pltpu.VMEM
    G8 = D // 8
    wshape = (D // 16, F // 128, 16, 128)
    wview = lambda w: w.reshape(D // 16, 2, 8, F // 128, 128).transpose(0, 1, 3, 2, 4)
    scratch = [
        vm((G8, NB, 16, 128), bf16), vm((6, NSTEP, 128, N), bf16), vm((D,), bf16), vm((D,), bf16), vm((D,), bf16),
        vm((CT_ROWS, 128), f32), vm(wshape, bf16), vm(wshape, bf16), vm((D, F), bf16), vm((G8, NB + 1, 16, 128), bf16),
        vm((9, 4, 144, 128), bf16), vm((2, 2, 2, 144, 128), bf16), vm((3, NSTEP, 96, 128), f32),
        vm((NV, 2, 136, 128), f32), vm((NSTEP, 12, 56, 128), f32), vm((NSTEP, 96, 128), f32),
        vm((NSTEP, NB, 6, R, 128), f32), vm((NSTEP, NB, 6, R, 128), f32),
        vm((NSTEP, NB, 2, R, 256), f32), vm((NSTEP, 12, 136, 128), f32), vm((2, 17, 8, 128), f32),
        vm((3, 136, 128), f32), vm((5, 16, 128), f32), vm((TOPC, G8, 8, 128), f32),
        vm((R, 512), f32), vm((8, D), f32), vm((NV, 4, 8, 128), f32),
        vm((8, 128), f32), vm((8, D), f32), vm((8, D), f32), vm((8, F), f32),
        vm((TOPC, G8, 8, 128), bf16), vm((TOPC, 8, 128), i32), vm((8, D), f32), pltpu.SMEM((1,), i32),
        pltpu.SemaphoreType.DMA((6 + len(PART),)), pltpu.SemaphoreType.DMA((1,)),
    ]
    xv = A_u[0].T.reshape(G8, 8, 16, 128).transpose(0, 2, 1, 3).reshape(G8, NB, 16, 128)
    out = pl.pallas_call(
        _kernel,
        out_shape=jax.ShapeDtypeStruct((G8, NB, 16, 128), bf16),
        in_specs=[hbm] * 13,
        out_specs=hbm,
        scratch_shapes=scratch,
        compiler_params=pltpu.CompilerParams(vmem_limit_bytes=120 * 1024 * 1024, disable_bounds_checks=True,
                                             disable_semaphore_checks=True),
    )(xv, *[p.reshape(NSTEP, R, N) for p in (A_A_re, A_A_im, A_B_re, A_B_im, A_C_re, A_C_im)], A_log_dt, A_Dskip, B_w_r,
      wview(B_w_gate), wview(B_w_up), B_w_down.T)
    return out.reshape(G8, 16, 8, 128).transpose(0, 2, 1, 3).reshape(D, L).T[None]
```
